```python
import jax
import jax.numpy as jnp

def _softmax(x, axis=-1):
    return jax.nn.softmax(x, axis=axis)

def _gelu(x):
    return jax.nn.gelu(x, approximate=True)

def _silu(x):
    return jax.nn.silu(x)

def _sigmoid(x):
    return jax.nn.sigmoid(x)

def _layernorm(x, axis=-1, eps=1e-05):
    m = jnp.mean(x, axis=axis, keepdims=True)
    v = jnp.var(x, axis=axis, keepdims=True)
    return (x - m) / jnp.sqrt(v + eps)

def _scatter_add(tgt, idx, src, axis=0):
    return tgt.at[idx].add(src)

def _segment_sum(src, seg, n):
    return jax.ops.segment_sum(src, seg, n)

class _Rng:

    def __init__(self, key):
        self._k = key

    def _next(self):
        self._k, sub = jax.random.split(self._k)
        return sub

    def normal(self, shape):
        return jax.random.normal(self._next(), shape, dtype=jnp.bfloat16)

    def randint(self, lo, hi, shape):
        return jax.random.randint(self._next(), shape, lo, hi, dtype=jnp.int32)

    def uniform(self, shape, lo=0.0, hi=1.0):
        return jax.random.uniform(self._next(), shape, jnp.bfloat16, lo, hi)

    def permutation(self, n):
        return jax.random.permutation(self._next(), n)
kernel_name = 'adaLN_cond__memory_aug_recurrent_mem_tr__moe_arch_mod__prompt'

def setup_inputs():
    _rng = _Rng(jax.random.key(int.from_bytes(__import__("os").urandom(4), "little")))
    _w = lambda a: (lambda t: t.astype(jnp.bfloat16) if jnp.issubdtype(t.dtype, jnp.floating) else t)(jnp.asarray(a))

    def _A_setup():
        B, S, Dm = (1, 2048, 1024)
        H, Dh = (32, 128)
        M, seg = (8, 32)
        seg = min(seg, S)
        S = S // seg * seg
        return {'x': _w((lambda *s: _rng.normal(s) * 0.05)(B, S, Dm)), 'mem0': _w((lambda *s: _rng.normal(s) * 0.05)(B, M, Dm)), 'Wq': _w((lambda *s: _rng.normal(s) * 0.05)(Dm, H, Dh) * Dm ** (-0.5)), 'Wk': _w((lambda *s: _rng.normal(s) * 0.05)(Dm, H, Dh) * Dm ** (-0.5)), 'Wv': _w((lambda *s: _rng.normal(s) * 0.05)(Dm, H, Dh) * Dm ** (-0.5)), 'Wo': _w((lambda *s: _rng.normal(s) * 0.05)(H, Dh, Dm) * (H * Dh) ** (-0.5)), 'seg_len': seg}
    _A_in = _A_setup()

    def _B_setup():
        B, S, D, F, C = (1, 2048, 1024, 3584, 2)
        return {'x': _w((lambda *s: _rng.normal(s) * 0.05)(B, S, D)), 'w_r': _w((lambda *s: _rng.normal(s) * 0.05)(D)), 'w_gate': _w((lambda *s: _rng.normal(s) * 0.05)(D, F)), 'w_up': _w((lambda *s: _rng.normal(s) * 0.05)(D, F)), 'w_down': _w((lambda *s: _rng.normal(s) * 0.05)(F, D))}
    _B_in = _B_setup()
    return {'A_x': _A_in['x'], 'A_mem0': _A_in['mem0'], 'A_Wq': _A_in['Wq'], 'A_Wk': _A_in['Wk'], 'A_Wv': _A_in['Wv'], 'A_Wo': _A_in['Wo'], 'A_seg_len': _A_in['seg_len'], 'B_x': _B_in['x'], 'B_w_r': _B_in['w_r'], 'B_w_gate': _B_in['w_gate'], 'B_w_up': _B_in['w_up'], 'B_w_down': _B_in['w_down'], 'c': _w((lambda *s: _rng.normal(s) * 0.05)(1, 1024)), 'w_mod': _w((lambda *s: _rng.normal(s) * 0.05)(1024, 6 * 1024) * 1024 ** (-0.5))}

def reference(A_x, A_mem0, A_Wq, A_Wk, A_Wv, A_Wo, A_seg_len, B_x, B_w_r, B_w_gate, B_w_up, B_w_down, c, w_mod):

    def _A_ref(x, mem0, Wq, Wk, Wv, Wo, seg_len):
        B, S, Dm = x.shape
        H, Dh = (Wq.shape[1], Wq.shape[2])
        M = mem0.shape[1]
        scale = Dh ** (-0.5)
        n_seg = S // seg_len
        L = M + seg_len
        idx = jnp.arange(L)
        mask = (idx[:, None] < M) | (idx[:, None] >= idx[None, :])
        mem = mem0
        outs = []
        for s in range(n_seg):
            xs = x[:, s * seg_len:(s + 1) * seg_len, :].copy()
            h = jnp.concatenate([mem, xs], axis=1)
            q = jnp.einsum('btd,dhe->bhte', h, Wq)
            k = jnp.einsum('btd,dhe->bhte', h, Wk)
            v = jnp.einsum('btd,dhe->bhte', h, Wv)
            scores = jnp.einsum('bhqe,bhke->bhqk', q, k) * scale
            scores = jnp.where(mask[None, None], scores, -1000000000.0)
            p = _softmax(scores, axis=-1)
            o = jnp.einsum('bhqk,bhke->bhqe', p, v)
            o = jnp.einsum('bhte,hed->btd', o, Wo)
            mem = o[:, :M, :].copy()
            outs.append(o[:, M:, :])
        return jnp.concatenate(outs, axis=1)

    def _B_ref(x, w_r, w_gate, w_up, w_down):
        B, S, D = x.shape
        C = 2
        r = x @ w_r
        idx = jnp.argsort(-r, axis=-1)[:, :C]
        idx_e = jnp.repeat(idx.reshape(B, C, 1), D, axis=2)
        x_sel = jnp.take_along_axis(x, idx_e, axis=1)
        g = _silu(x_sel @ w_gate)
        u = x_sel @ w_up
        y = g * u @ w_down
        r_sel = _sigmoid(jnp.take_along_axis(r, idx, axis=1))
        y = y * r_sel.reshape(B, C, 1)
        b_off = (jnp.arange(B) * S).reshape(B, 1)
        flat_idx = (idx + b_off).reshape(B * C)
        zero = (x * 0.0).reshape(B * S, D)
        upd = _scatter_add(zero, flat_idx, y.reshape(B * C, D), axis=0)
        return x + upd.reshape(B, S, D)
    x = A_x
    mod = (_silu(c) @ w_mod).reshape(c.shape[0], 6, 1, -1)
    sa, ca, ga, sb, cb, gb = (mod[:, 0].copy(), mod[:, 1].copy(), mod[:, 2].copy(), mod[:, 3].copy(), mod[:, 4].copy(), mod[:, 5].copy())
    h = _layernorm(x, axis=-1) * (1 + ca) + sa
    x = x + ga * _A_ref(h, A_mem0, A_Wq, A_Wk, A_Wv, A_Wo, A_seg_len)
    h = _layernorm(x, axis=-1) * (1 + cb) + sb
    x = x + gb * _B_ref(h, B_w_r, B_w_gate, B_w_up, B_w_down)
    return x
```

```python
import jax
import jax.numpy as jnp
from jax import lax
import jax.experimental.pallas as pl
import jax.experimental.pallas.tpu as pltpu

BF = jnp.bfloat16
F32 = jnp.float32
U32 = jnp.uint32

S = 2048
D = 1024
H = 32
DH = 128
M = 8
SEG = 32
NSEG = S // SEG
F = 3584
NP = H // 2
RIDE = 24
PRE = S - NSEG * RIDE
NSLOT = 17
NOSLOT = 17
NB = 4
KS = 3072
LAG_S = 1
LAG_P = 3
EPS = 1e-5
SCALE = DH ** -0.5
NSTAGE = 3


def _rb(v):
    return v.astype(BF).astype(F32)


def _layernorm(x):
    mu = jnp.sum(x, axis=-1, keepdims=True) * (1.0 / D)
    xc = x - mu
    var = jnp.sum(xc * xc, axis=-1, keepdims=True) * (1.0 / D)
    sd = _rb(jnp.sqrt(_rb(_rb(var) + EPS)))
    return _rb(_rb(x - _rb(mu)) / sd)


def _kernel(x_hbm, mem0_hbm, wq_hbm, wk_hbm, wv_hbm, wo_hbm, wr_hbm, wg_hbm, wu_hbm,
            wd_hbm, c_hbm, wmod_hbm, out_hbm,
            xbuf, h0buf, hbuf, outbuf, rbuf, abuf, modb, cbuf, wrbuf,
            wq_v, wk_v, wv_v, wo_v, wmod_v, wg_v, wu_v, wd_v, stage, tmp,
            obuf1, obuf2, qkv0, qkv1, qkv2, qkv3, sems, wsems):
    qkvbufs = (qkv0, qkv1, qkv2, qkv3)
    w_hbms = (wq_hbm, wk_hbm, wv_hbm)
    w_vs = (wq_v, wk_v, wv_v)

    def cp(src, dst, i):
        return pltpu.make_async_copy(src, dst, sems.at[i])

    cp_c = cp(c_hbm, cbuf, 0)
    cp_mem = cp(mem0_hbm.at[0], hbuf.at[0:M], 1)
    cp_wr = cp(wr_hbm, wrbuf, 2)
    cp_x0 = cp(x_hbm.at[0, 0:PRE], xbuf.at[0:PRE], 3)
    cp_x1 = cp(x_hbm.at[0, PRE:S], xbuf.at[PRE:S], 4)
    cp_moda = [cp(wmod_hbm.at[:, n * 128:(n + 1) * 128], wmod_v.at[n], 5) for n in range(16)]
    cp_modb = [cp(wmod_hbm.at[:, n * 128:(n + 1) * 128], wmod_v.at[n], 6) for n in range(16, 48)]
    cp_wo = [cp(wo_hbm.at[:, :, n * 128:(n + 1) * 128], wo_v.at[n], 7) for n in range(8)]
    cp_ffn = ([cp(wg_hbm.at[:, n * 128:(n + 1) * 128], wg_v.at[n], 8) for n in range(F // 128)]
              + [cp(wu_hbm.at[:, n * 128:(n + 1) * 128], wu_v.at[n], 8) for n in range(F // 128)]
              + [cp(wd_hbm.at[:, n * 128:(n + 1) * 128], wd_v.at[n], 8) for n in range(8)])

    def w_copy(t, g):
        return pltpu.make_async_copy(
            w_hbms[t].at[:, pl.ds(pl.multiple_of(g * 8, 8), 8), :], stage.at[t], wsems.at[t])

    cp_c.start()
    cp_x0.start()
    for c_ in cp_moda:
        c_.start()
    w_copy(0, 0).start()
    w_copy(1, 0).start()
    cp_mem.start()
    cp_wr.start()
    cp_x1.start()

    def mod_part(sc16, lo, hi):
        w = jnp.concatenate([wmod_v[n] for n in range(lo, hi)], axis=1)
        return _rb(jnp.dot(sc16, w, preferred_element_type=F32))[0:8]

    def relayout(t, g):
        for b in range(16):
            v = stage[t, b * 64:(b + 1) * 64].reshape(512, 128)
            tmp[b * 256:(b + 1) * 256, :] = pltpu.bitcast(v, U32)
        for i in range(4):
            for b in range(8):
                a = tmp[pl.ds(b * 512 + i, 64, stride=8), :]
                c2 = tmp[pl.ds(b * 512 + 4 + i, 64, stride=8), :]
                w_vs[t][g * 8 + 2 * i, b * 64:(b + 1) * 64, :] = (a & U32(0xFFFF)) | (c2 << 16)
                w_vs[t][g * 8 + 2 * i + 1, b * 64:(b + 1) * 64, :] = (
                    (a >> 16) | (c2 & U32(0xFFFF0000)))

    def ln1_rows(src_row, dst, dst_row):
        xv = xbuf[pl.ds(src_row, 8), :].astype(F32)
        hv = _rb(_layernorm(xv) * modb[1]) + modb[0]
        dst[pl.ds(dst_row, 8), :] = hv.astype(BF)

    def finish_rows(row, attn):
        xv = xbuf[pl.ds(row, 8), :].astype(F32)
        x1 = _rb(xv + _rb(modb[2] * _rb(attn)))
        h2 = _rb(_rb(_layernorm(x1) * modb[4]) + modb[3])
        xbuf[pl.ds(row, 8), :] = x1.astype(BF)
        outbuf[pl.ds(row, 8), :] = (x1 + _rb(modb[5] * h2)).astype(BF)
        r = _rb(jnp.sum(h2 * modb[6], axis=-1, keepdims=True))
        rbuf[pl.ds(row, 8), :] = jnp.broadcast_to(r, (8, 128))

    cp_c.wait()
    cv = cbuf[...].astype(F32)
    sc16 = jnp.broadcast_to(_rb(cv * _rb(jax.nn.sigmoid(cv))), (16, D)).astype(BF)
    for c_ in cp_moda:
        c_.wait()
    moda = mod_part(sc16, 0, 16)
    modb[0] = moda[:, 0:D]
    modb[1] = _rb(1.0 + moda[:, D:2 * D])
    cp_x0.wait()

    def ln_pre(g, carry):
        for u in range(8):
            row = pl.multiple_of(g * 64 + u * 8, 8)
            ln1_rows(row, h0buf, row)
        return carry
    lax.fori_loop(0, PRE // 64, ln_pre, 0)

    w_copy(0, 0).wait()
    w_copy(2, 0).start()
    relayout(0, 0)
    for c_ in cp_wo:
        c_.start()
    for c_ in cp_modb:
        c_.start()
    cp_x1.wait()

    def pre_matmul(t, g):
        for i in range(4):
            w = pltpu.bitcast(
                jnp.concatenate([w_vs[t][g * 8 + 2 * i], w_vs[t][g * 8 + 2 * i + 1]], axis=1), BF)
            for rc in range(PRE // 128):
                y = jnp.dot(h0buf[rc * 128:(rc + 1) * 128, :], w, preferred_element_type=F32)
                yb = y.astype(BF)
                for sg in range(4):
                    for hh in range(2):
                        qkvbufs[i][rc * 4 + sg, g * 3 + t, hh * 32:(hh + 1) * 32, :] = (
                            yb[sg * 32:(sg + 1) * 32, hh * 128:(hh + 1) * 128])

    def ln_ride(j):
        for u in range(16):
            gi = j * 16 + u
            ln1_rows(pl.multiple_of(PRE + gi * 8, 8), hbuf,
                     pl.multiple_of((gi // 3) * 32 + 8 + (gi % 3) * 8, 8))

    def pre_body(g, carry):
        gn = jnp.minimum(g + 1, 3)
        for t in range(3):
            @pl.when(g < 3)
            def _():
                w_copy(t, gn).start()
            if t < 2:
                w_copy(t + 1, g).wait()
                pre_matmul(t, g)
                relayout(t + 1, g)
            else:
                @pl.when(g < 3)
                def _():
                    w_copy(0, gn).wait()
                pre_matmul(t, g)
                relayout(0, gn)
            ln_ride(g * 3 + t)
        return carry
    lax.fori_loop(0, 4, pre_body, 0)

    for c_ in cp_modb:
        c_.wait()
    for c_ in cp_wo:
        c_.wait()
    cp_mem.wait()
    cp_wr.wait()
    for c_ in cp_ffn:
        c_.start()
    modc = mod_part(sc16, 16, 48)
    modb[2] = modc[:, 0:D]
    modb[3] = modc[:, D:2 * D]
    modb[4] = _rb(1.0 + modc[:, 2 * D:3 * D])
    modb[5] = modc[:, 3 * D:4 * D]
    modb[6] = jnp.broadcast_to(wrbuf[...].astype(F32), (8, D))
    abuf[...] = jnp.zeros(abuf.shape, F32)

    ri = lax.broadcasted_iota(jnp.int32, (80, 80), 0)
    ci = lax.broadcasted_iota(jnp.int32, (80, 80), 1)

    def head_pos(i):
        hd = jnp.where(i < 16, i // 8, (i - 16) // 32)
        pos = jnp.where(i < 16, i % 8, 8 + (i - 16) % 32)
        return hd, pos
    rh, rp = head_pos(ri)
    ch, cpos = head_pos(ci)
    same = rh == ch
    valid = same & ((rp < M) | (rp >= cpos))
    fill = jnp.where(same, -1e9, -jnp.inf).astype(F32)

    def wo_w(h0, h1, n0, n1):
        return jnp.concatenate(
            [wo_v[n, h0:h1].reshape((h1 - h0) * DH, 128) for n in range(n0, n1)], axis=1)

    def step(s, carry):
        hrow = pl.multiple_of(s * 32, 32)
        lhs = hbuf[pl.ds(hrow, 32), :]
        slot = s % NSLOT
        dsts = []
        for j in range(3):
            gi = PRE // 8 + 3 * s + j
            dsts.append(((gi // 4) % NSLOT, pl.multiple_of((gi % 4) * 8, 8)))
        odst = []
        for j in range(4):
            gi = 4 * s + j
            row = jnp.where(gi < 3 * NSEG, ((gi // 3) % NOSLOT) * 32 + 8 + (gi % 3) * 8,
                            NOSLOT * 32 + (gi - 3 * NSEG) * 8)
            odst.append(pl.multiple_of(row, 8))
        orow = pl.multiple_of((s % NOSLOT) * 32, 32)
        mems = {}
        probs = {}

        erow = jnp.maximum(s - 1, 0) * RIDE
        for j in range(3):
            finish_rows(pl.multiple_of(erow + 8 * j, 8), abuf[8 * j:8 * j + 8, :])

        def qkv(p):
            w = pltpu.bitcast(jnp.concatenate(
                [w_vs[u // 2][2 * p + u % 2] for u in range(6)], axis=1), BF)
            y = jnp.dot(lhs, w, preferred_element_type=F32)
            buf = qkvbufs[p % NB]
            ms = []
            for t in range(3):
                bi = (p // NB) * 3 + t
                for hh in range(2):
                    col = t * 256 + hh * 128
                    for j in range(3):
                        sl, off = dsts[j]
                        buf[sl, bi, pl.ds(hh * 32 + off, 8), :] = (
                            y[8 + 8 * j:16 + 8 * j, col:col + 128].astype(BF))
                ms.append(jnp.concatenate(
                    [y[0:8, t * 256:t * 256 + 128], y[0:8, t * 256 + 128:t * 256 + 256]],
                    axis=0).astype(BF))
            mems[p] = ms

        def ld(p, t):
            return jnp.concatenate(
                [mems[p][t], qkvbufs[p % NB][slot, (p // NB) * 3 + t]], axis=0)

        def sc(p):
            s2 = lax.dot_general(ld(p, 0), ld(p, 1), (((1,), (1,)), ((), ())),
                                 preferred_element_type=F32) * SCALE
            s2 = jnp.where(valid, s2, fill)
            m = jnp.max(s2, axis=-1, keepdims=True)
            e = jnp.exp(s2 - m)
            l = jnp.sum(e, axis=-1, keepdims=True)
            rl = pl.reciprocal(l, approx=True)
            rl = rl * (2.0 - l * rl)
            probs[p] = (e * rl).astype(BF)

        def pv(p):
            o2 = jnp.dot(probs[p], ld(p, 2), preferred_element_type=F32)
            for hh in range(2):
                hcol = (2 * p + hh) * 128
                ob = obuf1
                if hcol >= KS:
                    ob = obuf2
                    hcol -= KS
                ob[pl.ds(orow, 8), hcol:hcol + 128] = o2[8 * hh:8 * hh + 8].astype(BF)
                for j in range(4):
                    r0 = 16 + 32 * hh + 8 * j
                    ob[pl.ds(odst[j], 8), hcol:hcol + 128] = o2[r0:r0 + 8].astype(BF)

        for p in range(NP):
            qkv(p)
            if p - LAG_S >= 0:
                sc(p - LAG_S)
            if p - LAG_P >= 0:
                pv(p - LAG_P)
        a1 = []
        for i in range(4):
            a1.append(jnp.dot(obuf1[pl.ds(orow, 32), :], wo_w(0, KS // DH, 2 * i, 2 * i + 2),
                              preferred_element_type=F32))
            p = NP + i
            if p - LAG_S < NP:
                sc(p - LAG_S)
            if p - LAG_P < NP:
                pv(p - LAG_P)
        a = jnp.concatenate(a1, axis=1) + jnp.dot(
            obuf2[pl.ds(orow, 32), :], wo_w(KS // DH, H, 0, 8), preferred_element_type=F32)
        hbuf[pl.ds(hrow + 32, 8), :] = a[0:8].astype(BF)
        abuf[...] = a[8:32]
        return carry
    lax.fori_loop(0, NSEG, step, 0)

    for j in range(3):
        finish_rows((NSEG - 1) * RIDE + 8 * j, abuf[8 * j:8 * j + 8, :])
    OUT0 = NSEG * RIDE
    cp_out = [cp(outbuf.at[0:OUT0], out_hbm.at[0, 0:OUT0], 9)]
    cp_out[0].start()
    ECH = 128
    for rc in range(PRE // ECH):
        r0 = NOSLOT * 32 + rc * ECH
        a = (jnp.dot(obuf1[r0:r0 + ECH, :], wo_w(0, KS // DH, 0, 8), preferred_element_type=F32)
             + jnp.dot(obuf2[r0:r0 + ECH, :], wo_w(KS // DH, H, 0, 8), preferred_element_type=F32))
        for j in range(ECH // 8):
            finish_rows(OUT0 + rc * ECH + 8 * j, a[8 * j:8 * j + 8])
    cp_out.append(cp(outbuf.at[OUT0:S], out_hbm.at[0, OUT0:S], 10))
    cp_out[1].start()

    r_all = rbuf[...]
    rows = lax.broadcasted_iota(jnp.int32, (S, 128), 0)
    m1 = jnp.max(r_all, axis=0, keepdims=True)
    i1v = jnp.min(jnp.where(r_all == m1, rows, S), axis=0, keepdims=True)
    r_rest = jnp.where(rows == i1v, -jnp.inf, r_all)
    m2 = jnp.max(r_rest, axis=0, keepdims=True)
    i2v = jnp.min(jnp.where((r_rest == m2) & (rows != i1v), rows, S), axis=0, keepdims=True)
    i1 = jnp.clip(jnp.max(i1v), 0, S - 1)
    i2 = jnp.clip(jnp.max(i2v), 0, S - 1)
    b1 = pl.multiple_of((i1 // 8) * 8, 8)
    b2 = pl.multiple_of((i2 // 8) * 8, 8)

    x1 = jnp.concatenate([xbuf[pl.ds(b1, 8), :].astype(F32), xbuf[pl.ds(b2, 8), :].astype(F32)],
                         axis=0)
    rr = jnp.concatenate([rbuf[pl.ds(b1, 8), :], rbuf[pl.ds(b2, 8), :]], axis=0)[:, 0:1]
    cb1 = jnp.concatenate([modb[4], modb[4]], axis=0)
    sb = jnp.concatenate([modb[3], modb[3]], axis=0)
    gb = jnp.concatenate([modb[5], modb[5]], axis=0)
    h2 = _rb(_rb(_layernorm(x1) * cb1) + sb)
    h2b = h2.astype(BF)
    for c_ in cp_ffn:
        c_.wait()
    gt = _rb(jnp.dot(h2b, jnp.concatenate([wg_v[n] for n in range(F // 128)], axis=1),
                     preferred_element_type=F32))
    up = _rb(jnp.dot(h2b, jnp.concatenate([wu_v[n] for n in range(F // 128)], axis=1),
                     preferred_element_type=F32))
    act = (_rb(gt * _rb(jax.nn.sigmoid(gt))) * up).astype(BF)
    y = _rb(jnp.dot(act, jnp.concatenate([wd_v[n] for n in range(8)], axis=1),
                    preferred_element_type=F32))
    y = _rb(y * _rb(jax.nn.sigmoid(rr)))
    sub = lax.broadcasted_iota(jnp.int32, (16, 1), 0)
    grow = jnp.where(sub < 8, b1 + sub, b2 + sub - 8)
    sel = (grow == i1) | (grow == i2)
    res = (x1 + _rb(gb * _rb(h2 + jnp.where(sel, y, 0.0)))).astype(BF)
    for c_ in cp_out:
        c_.wait()
    outbuf[pl.ds(b1, 8), :] = res[0:8]
    outbuf[pl.ds(b2, 8), :] = res[8:16]
    fix1 = cp(outbuf.at[pl.ds(b1, 8)], out_hbm.at[0, pl.ds(b1, 8)], 11)
    fix2 = cp(outbuf.at[pl.ds(b2, 8)], out_hbm.at[0, pl.ds(b2, 8)], 12)
    fix1.start()

    @pl.when(b1 != b2)
    def _():
        fix2.start()
        fix2.wait()
    fix1.wait()


@jax.jit
def pallas_adaLN_cond__memory_aug_recurrent_mem_tr__moe_arch_mod__prompt_kernel(
    A_x: jax.Array,
    A_mem0: jax.Array,
    A_Wq: jax.Array,
    A_Wk: jax.Array,
    A_Wv: jax.Array,
    A_Wo: jax.Array,
    A_seg_len,
    B_x: jax.Array,
    B_w_r: jax.Array,
    B_w_gate: jax.Array,
    B_w_up: jax.Array,
    B_w_down: jax.Array,
    c: jax.Array,
    w_mod: jax.Array,
):
    del B_x
    del A_seg_len
    assert A_x.shape == (1, S, D) and A_Wq.shape == (D, H, DH) and A_mem0.shape == (1, M, D)
    any_spec = pl.BlockSpec(memory_space=pl.ANY)
    scratch = [
        pltpu.VMEM((S, D), BF),
        pltpu.VMEM((PRE, D), BF),
        pltpu.VMEM(((NSEG + 1) * 32, D), BF),
        pltpu.VMEM((S, D), BF),
        pltpu.VMEM((S, 128), F32),
        pltpu.VMEM((RIDE, D), F32),
        pltpu.VMEM((7, 8, D), F32),
        pltpu.VMEM((1, D), BF),
        pltpu.VMEM((1, D), BF),
        pltpu.VMEM((H, D // 2, 128), U32),
        pltpu.VMEM((H, D // 2, 128), U32),
        pltpu.VMEM((H, D // 2, 128), U32),
        pltpu.VMEM((8, H, DH, 128), BF),
        pltpu.VMEM((48, D, 128), BF),
        pltpu.VMEM((F // 128, D, 128), BF),
        pltpu.VMEM((F // 128, D, 128), BF),
        pltpu.VMEM((8, F, 128), BF),
        pltpu.VMEM((NSTAGE, D, 8, DH), BF),
        pltpu.VMEM((4 * D, 128), U32),
        pltpu.VMEM((NOSLOT * 32 + PRE, KS), BF),
        pltpu.VMEM((NOSLOT * 32 + PRE, H * DH - KS), BF),
    ] + [pltpu.VMEM((NSLOT, 3 * NP // NB, 64, 128), BF) for _ in range(NB)] + [
        pltpu.SemaphoreType.DMA((13,)),
        pltpu.SemaphoreType.DMA((NSTAGE,)),
    ]
    return pl.pallas_call(
        _kernel,
        out_shape=jax.ShapeDtypeStruct((1, S, D), BF),
        in_specs=[any_spec] * 12,
        out_specs=any_spec,
        scratch_shapes=scratch,
        compiler_params=pltpu.CompilerParams(vmem_limit_bytes=120 * 1024 * 1024),
    )(A_x, A_mem0, A_Wq, A_Wk, A_Wv, A_Wo, B_w_r.reshape(1, D), B_w_gate, B_w_up, B_w_down,
      c, w_mod)
```

```python
import os
import jax
import jax.numpy as jnp
from jax import lax
import jax.experimental.pallas as pl
import jax.experimental.pallas.tpu as pltpu

BF = jnp.bfloat16
F32 = jnp.float32
U32 = jnp.uint32

S = 2048
D = 1024
H = 32
DH = 128
M = 8
SEG = 32
NSEG = S // SEG
F = 3584
NP = H // 2
RIDE = 24
PRE = S - NSEG * RIDE
NSLOT = 17
NOSLOT = 17
NB = 4
KS = 3072
LAG_S = 1
LAG_P = 3
EPS = 1e-5
SCALE = DH ** -0.5
OOFF = S
HOFF = 2 * S
PRE_U = int(os.environ.get('PRE_U', 1))
E_AT = (1, 3, 5)
L_AT = (7, 9, 11)
EPI_CHUNKS = (128, 128, 128, 96, 32)


def _rb(v):
    return v.astype(BF).astype(F32)


def _layernorm(x):
    mu = jnp.sum(x, axis=-1, keepdims=True) * (1.0 / D)
    xc = x - mu
    var = jnp.sum(xc * xc, axis=-1, keepdims=True) * (1.0 / D)
    sd = _rb(jnp.sqrt(_rb(_rb(var) + EPS)))
    return _rb(_rb(x - _rb(mu)) / sd)


def _kernel(x_hbm, mem0_hbm, wq_hbm, wk_hbm, wv_hbm, wo_hbm, wr_hbm, wg_hbm, wu_hbm,
            wd_hbm, c_hbm, wmod_hbm, out_hbm,
            act, h0buf, rmat, abuf, modb, cbuf, wrbuf,
            w_v, wo_v, wmod_v, wg_v, wu_v, wd_v,
            obuf1, obuf2, qkv0, qkv1, qkv2, qkv3, sems, wsems):
    qkvbufs = (qkv0, qkv1, qkv2, qkv3)
    w_hbms = tuple(w.bitcast(U32) for w in (wq_hbm, wk_hbm, wv_hbm))

    def cp(src, dst, i):
        return pltpu.make_async_copy(src, dst, sems.at[i])

    wmod_b = wmod_v.bitcast(BF)
    cp_c = cp(c_hbm, cbuf, 0)
    cp_mem = cp(mem0_hbm.at[0], act.at[HOFF:HOFF + M], 1)
    cp_wr = cp(wr_hbm, wrbuf, 2)
    cp_x0 = cp(x_hbm.at[0, 0:PRE], act.at[0:PRE], 3)
    cp_x1 = cp(x_hbm.at[0, PRE:S], act.at[PRE:S], 4)
    cp_moda = [cp(wmod_hbm.at[:, n * 512:(n + 1) * 512], wmod_b.at[:, n * 512:(n + 1) * 512],
                  13 + n) for n in range(4)]
    cp_modb = cp(wmod_hbm.at[:, 2 * D:6 * D], wmod_b.at[:, 2 * D:6 * D], 6)
    cp_wo = cp(wo_hbm, wo_v.bitcast(BF), 7)
    cp_ffn = [cp(wg_hbm, wg_v.bitcast(BF), 8), cp(wu_hbm, wu_v.bitcast(BF), 8),
              cp(wd_hbm, wd_v.bitcast(BF), 8)]

    def w_copies(g, t):
        return [pltpu.make_async_copy(w_hbms[t].at[:, par, g * 4 + i, :],
                                      w_v.at[(g * 4 + i) * 6 + t * 2 + par], wsems.at[g * 3 + t])
                for i in range(4) for par in range(2)]

    def w_start(g):
        for t in range(3):
            for c_ in w_copies(g, t):
                c_.start()

    cp_c.start()
    cp_x0.start()
    for c_ in cp_moda:
        c_.start()
    w_start(0)
    cp_mem.start()
    cp_wr.start()
    w_start(1)

    def mod_part(sc16, lo, hi):
        w = pltpu.bitcast(wmod_v[:, lo:hi], BF)
        return _rb(jnp.dot(sc16, w, preferred_element_type=F32))[0:8]

    def ln1_rows(src_row, dst_row):
        xv = act[pl.ds(src_row, 8), :].astype(F32)
        hv = _rb(_layernorm(xv) * modb[1]) + modb[0]
        act[pl.ds(dst_row, 8), :] = hv.astype(BF)

    lane256 = lax.broadcasted_iota(jnp.int32, (8, 256), 1)

    def finish_rows(row, attn):
        xv = act[pl.ds(row, 8), :].astype(F32)
        x1 = _rb(xv + _rb(modb[2] * _rb(attn)))
        h2 = _rb(_rb(_layernorm(x1) * modb[4]) + modb[3])
        act[pl.ds(row, 8), :] = x1.astype(BF)
        act[pl.ds(OOFF + row, 8), :] = (x1 + _rb(modb[5] * h2)).astype(BF)
        r = _rb(jnp.sum(h2 * modb[6], axis=-1, keepdims=True))
        rmat[...] = jnp.where(lane256 == row // 8, r, rmat[...])

    rmat[...] = jnp.zeros(rmat.shape, F32)
    abuf[...] = jnp.zeros(abuf.shape, F32)
    cp_c.wait()
    cv = cbuf[...].astype(F32)
    sc16 = jnp.broadcast_to(_rb(cv * _rb(jax.nn.sigmoid(cv))), (16, D)).astype(BF)
    cp_x0.wait()

    def ln_pre(g, carry):
        row = pl.multiple_of(g * 64, 64)
        h0buf[pl.ds(row, 64), :] = _layernorm(act[pl.ds(row, 64), :].astype(F32)).astype(BF)
        return carry
    lax.fori_loop(0, PRE // 64, ln_pre, 0)

    for n in range(4):
        cp_moda[n].wait()
        mv = mod_part(sc16, n * 512, (n + 1) * 512)
        if n >= 2:
            mv = _rb(1.0 + mv)
        modb[n // 2, :, (n % 2) * 512:(n % 2 + 1) * 512] = mv

    def mod_pre(g, carry):
        for u in range(8):
            row = pl.multiple_of(g * 64 + u * 8, 8)
            nv = h0buf[pl.ds(row, 8), :].astype(F32)
            h0buf[pl.ds(row, 8), :] = (_rb(nv * modb[1]) + modb[0]).astype(BF)
        return carry
    lax.fori_loop(0, PRE // 64, mod_pre, 0)

    def pre_unit(j, i):
        blk = (j // 3) * 24 + (j % 3) * 2 + i * 6
        a = w_v[blk]
        b = w_v[blk + 1]
        lo = (a & U32(0xFFFF)) | (b << 16)
        hi = (a >> 16) | (b & U32(0xFFFF0000))
        w_v[blk] = lo
        w_v[blk + 1] = hi
        for rc in range(PRE // 128):
            if rc > 0:
                lo = w_v[blk]
                hi = w_v[blk + 1]
            w = pltpu.bitcast(jnp.concatenate([lo, hi], axis=1), BF)
            y = jnp.dot(h0buf[rc * 128:(rc + 1) * 128, :], w, preferred_element_type=F32)
            for sg in range(4):
                for hh in range(2):
                    qkvbufs[i][rc * 4 + sg, j, hh * 32:(hh + 1) * 32, :] = (
                        y[sg * 32:(sg + 1) * 32, hh * 128:(hh + 1) * 128].astype(BF))

    def pre_body(jj, carry):
        @pl.when(jj == 0)
        def _():
            w_start(2)

        @pl.when(jj == 3 // PRE_U)
        def _():
            w_start(3)
            cp_wo.start()

        @pl.when(jj == 6 // PRE_U)
        def _():
            cp_x1.start()
            cp_modb.start()
        for u in range(PRE_U):
            j = jj * PRE_U + u
            blk0 = (j // 3) * 24 + (j % 3) * 2
            for i in range(4):
                for par in range(2):
                    pltpu.make_async_copy(w_hbms[0].at[:, 0, 0, :], w_v.at[blk0 + i * 6 + par],
                                          wsems.at[j]).wait()
            for i in range(4):
                pre_unit(j, i)
        return carry
    lax.fori_loop(0, 12 // PRE_U, pre_body, 0)

    cp_mem.wait()
    cp_wr.wait()
    cp_wo.wait()
    cp_x1.wait()
    cp_modb.wait()
    for c_ in cp_ffn:
        c_.start()
    modc = mod_part(sc16, 2 * D, 6 * D)
    modb[2] = modc[:, 0:D]
    modb[3] = modc[:, D:2 * D]
    modb[4] = _rb(1.0 + modc[:, 2 * D:3 * D])
    modb[5] = modc[:, 3 * D:4 * D]
    modb[6] = jnp.broadcast_to(wrbuf[...].astype(F32), (8, D))
    for j in range(3):
        ln1_rows(PRE + 8 * j, HOFF + 8 + 8 * j)

    ri = lax.broadcasted_iota(jnp.int32, (80, 80), 0)
    ci = lax.broadcasted_iota(jnp.int32, (80, 80), 1)

    def head_pos(i):
        hd = jnp.where(i < 16, i // 8, (i - 16) // 32)
        pos = jnp.where(i < 16, i % 8, 8 + (i - 16) % 32)
        return hd, pos
    rh, rp = head_pos(ri)
    ch, cpos = head_pos(ci)
    same = rh == ch
    valid = same & ((rp < M) | (rp >= cpos))
    fill = jnp.where(same, -1e9, -jnp.inf).astype(F32)

    def wo_w(h0, h1, n0, n1):
        w = wo_v[h0:h1, :, n0 * 128:n1 * 128].reshape((h1 - h0) * (DH // 2), (n1 - n0) * 128)
        return pltpu.bitcast(w, BF)

    def step(s, carry):
        hrow = pl.multiple_of(HOFF + (s % 2) * 32, 32)
        hnext = pl.multiple_of(HOFF + ((s + 1) % 2) * 32, 32)
        slot = s % NSLOT
        dsts = []
        for j in range(3):
            gi = PRE // 8 + 3 * s + j
            dsts.append(((gi // 4) % NSLOT, pl.multiple_of((gi % 4) * 8, 8)))
        odst = []
        for j in range(4):
            gi = 4 * s + j
            row = jnp.where(gi < 3 * NSEG, ((gi // 3) % NOSLOT) * 32 + 8 + (gi % 3) * 8,
                            NOSLOT * 32 + (gi - 3 * NSEG) * 8)
            odst.append(pl.multiple_of(row, 8))
        orow = pl.multiple_of((s % NOSLOT) * 32, 32)
        erow = jnp.maximum(s - 1, 0) * RIDE
        lrow = PRE + jnp.minimum(s + 1, NSEG - 1) * RIDE
        mems = {}
        probs = {}

        def side(p):
            if p in E_AT:
                j = E_AT.index(p)
                finish_rows(pl.multiple_of(erow + 8 * j, 8), abuf[8 * j:8 * j + 8, :])
            if p in L_AT:
                j = L_AT.index(p)
                ln1_rows(pl.multiple_of(lrow + 8 * j, 8), pl.multiple_of(hnext + 8 + 8 * j, 8))

        def qkv(p):
            w = pltpu.bitcast(jnp.concatenate([w_v[p * 6 + u] for u in range(6)], axis=1), BF)
            y = jnp.dot(act[pl.ds(hrow, 32), :], w, preferred_element_type=F32)
            buf = qkvbufs[p % NB]
            ms = []
            for t in range(3):
                bi = (p // NB) * 3 + t
                for hh in range(2):
                    col = t * 256 + hh * 128
                    for j in range(3):
                        sl, off = dsts[j]
                        buf[sl, bi, pl.ds(hh * 32 + off, 8), :] = (
                            y[8 + 8 * j:16 + 8 * j, col:col + 128].astype(BF))
                ms.append(jnp.concatenate(
                    [y[0:8, t * 256:t * 256 + 128], y[0:8, t * 256 + 128:t * 256 + 256]],
                    axis=0).astype(BF))
            mems[p] = ms

        def ld(p, t):
            return jnp.concatenate(
                [mems[p][t], qkvbufs[p % NB][slot, (p // NB) * 3 + t]], axis=0)

        def sc(p):
            s2 = lax.dot_general(ld(p, 0), ld(p, 1), (((1,), (1,)), ((), ())),
                                 preferred_element_type=F32) * SCALE
            s2 = jnp.where(valid, s2, fill)
            m = jnp.max(s2, axis=-1, keepdims=True)
            e = jnp.exp(s2 - m)
            l = jnp.sum(e, axis=-1, keepdims=True)
            rl = pl.reciprocal(l, approx=True)
            rl = rl * (2.0 - l * rl)
            probs[p] = (e * rl).astype(BF)

        def pv(p):
            o2 = jnp.dot(probs[p], ld(p, 2), preferred_element_type=F32)
            for hh in range(2):
                hcol = (2 * p + hh) * 128
                ob = obuf1
                if hcol >= KS:
                    ob = obuf2
                    hcol -= KS
                ob[pl.ds(orow, 8), hcol:hcol + 128] = o2[8 * hh:8 * hh + 8].astype(BF)
                for j in range(4):
                    r0 = 16 + 32 * hh + 8 * j
                    ob[pl.ds(odst[j], 8), hcol:hcol + 128] = o2[r0:r0 + 8].astype(BF)

        for p in range(NP):
            qkv(p)
            side(p)
            if p - LAG_S >= 0:
                sc(p - LAG_S)
            if p - LAG_P >= 0:
                pv(p - LAG_P)
        a1 = []
        for i in range(4):
            a1.append(jnp.dot(obuf1[pl.ds(orow, 32), :], wo_w(0, KS // DH, 2 * i, 2 * i + 2),
                              preferred_element_type=F32))
            p = NP + i
            if p - LAG_S < NP:
                sc(p - LAG_S)
            if p - LAG_P < NP:
                pv(p - LAG_P)
        a = jnp.concatenate(a1, axis=1) + jnp.dot(
            obuf2[pl.ds(orow, 32), :], wo_w(KS // DH, H, 0, 8), preferred_element_type=F32)
        act[pl.ds(hnext, 8), :] = a[0:8].astype(BF)
        abuf[...] = a[8:32]
        return carry
    lax.fori_loop(0, NSEG, step, 0)

    for j in range(3):
        finish_rows((NSEG - 1) * RIDE + 8 * j, abuf[8 * j:8 * j + 8, :])
    OUT0 = NSEG * RIDE
    cp_out = [cp(act.at[OOFF:OOFF + OUT0], out_hbm.at[0, 0:OUT0], 9)]
    cp_out[0].start()
    r0 = 0
    for ech in EPI_CHUNKS:
        o0 = NOSLOT * 32 + r0
        a = (jnp.dot(obuf1[o0:o0 + ech, :], wo_w(0, KS // DH, 0, 8), preferred_element_type=F32)
             + jnp.dot(obuf2[o0:o0 + ech, :], wo_w(KS // DH, H, 0, 8), preferred_element_type=F32))
        for j in range(ech // 8):
            finish_rows(OUT0 + r0 + 8 * j, a[8 * j:8 * j + 8])
        r0 += ech
    cp_out.append(cp(act.at[OOFF + OUT0:OOFF + S], out_hbm.at[0, OUT0:S], 10))
    cp_out[1].start()

    r_all = rmat[...]
    rows = lane256 * 8 + lax.broadcasted_iota(jnp.int32, (8, 256), 0)

    def allmax(v):
        return jnp.max(jnp.max(v, axis=1, keepdims=True), axis=0, keepdims=True)

    def allmin(v):
        return jnp.min(jnp.min(v, axis=1, keepdims=True), axis=0, keepdims=True)
    rowsf = rows.astype(F32)
    i1v = allmin(jnp.where(r_all == allmax(r_all), rowsf, float(S)))
    r_rest = jnp.where(rowsf == i1v, -jnp.inf, r_all)
    i2v = allmin(jnp.where((r_rest == allmax(r_rest)) & (rowsf != i1v), rowsf, float(S)))
    i1 = jnp.clip(i1v[0, 0].astype(jnp.int32), 0, S - 1)
    i2 = jnp.clip(i2v[0, 0].astype(jnp.int32), 0, S - 1)
    b1 = pl.multiple_of((i1 // 8) * 8, 8)
    b2 = pl.multiple_of((i2 // 8) * 8, 8)

    x1 = jnp.concatenate([act[pl.ds(b1, 8), :].astype(F32), act[pl.ds(b2, 8), :].astype(F32)],
                         axis=0)

    def two(i):
        return jnp.concatenate([modb[i], modb[i]], axis=0)
    h2 = _rb(_rb(_layernorm(x1) * two(4)) + two(3))
    rr = _rb(jnp.sum(h2 * two(6), axis=-1, keepdims=True))
    h2b = h2.astype(BF)
    for c_ in cp_ffn:
        c_.wait()
    gt = _rb(jnp.dot(h2b, pltpu.bitcast(wg_v[...], BF), preferred_element_type=F32))
    up = _rb(jnp.dot(h2b, pltpu.bitcast(wu_v[...], BF), preferred_element_type=F32))
    hid = (_rb(gt * _rb(jax.nn.sigmoid(gt))) * up).astype(BF)
    y = _rb(jnp.dot(hid, pltpu.bitcast(wd_v[...], BF), preferred_element_type=F32))
    y = _rb(y * _rb(jax.nn.sigmoid(rr)))
    sub = lax.broadcasted_iota(jnp.int32, (16, 1), 0)
    grow = jnp.where(sub < 8, b1 + sub, b2 + sub - 8)
    sel = (grow == i1) | (grow == i2)
    res = (x1 + _rb(two(5) * _rb(h2 + jnp.where(sel, y, 0.0)))).astype(BF)
    for c_ in cp_out:
        c_.wait()
    act[pl.ds(OOFF + b1, 8), :] = res[0:8]
    act[pl.ds(OOFF + b2, 8), :] = res[8:16]
    fix1 = cp(act.at[pl.ds(OOFF + b1, 8)], out_hbm.at[0, pl.ds(b1, 8)], 11)
    fix2 = cp(act.at[pl.ds(OOFF + b2, 8)], out_hbm.at[0, pl.ds(b2, 8)], 12)
    fix1.start()

    @pl.when(b1 != b2)
    def _():
        fix2.start()
        fix2.wait()
    fix1.wait()


@jax.jit
def pallas_adaLN_cond__memory_aug_recurrent_mem_tr__moe_arch_mod__prompt_kernel(
    A_x: jax.Array,
    A_mem0: jax.Array,
    A_Wq: jax.Array,
    A_Wk: jax.Array,
    A_Wv: jax.Array,
    A_Wo: jax.Array,
    A_seg_len,
    B_x: jax.Array,
    B_w_r: jax.Array,
    B_w_gate: jax.Array,
    B_w_up: jax.Array,
    B_w_down: jax.Array,
    c: jax.Array,
    w_mod: jax.Array,
):
    del B_x
    del A_seg_len
    assert A_x.shape == (1, S, D) and A_Wq.shape == (D, H, DH) and A_mem0.shape == (1, M, D)
    any_spec = pl.BlockSpec(memory_space=pl.ANY)
    scratch = [
        pltpu.VMEM((2 * S + 64, D), BF),
        pltpu.VMEM((PRE, D), BF),
        pltpu.VMEM((8, 256), F32),
        pltpu.VMEM((RIDE, D), F32),
        pltpu.VMEM((7, 8, D), F32),
        pltpu.VMEM((1, D), BF),
        pltpu.VMEM((1, D), BF),
        pltpu.VMEM((3 * H, D // 2, 128), U32),
        pltpu.VMEM((H, DH // 2, D), U32),
        pltpu.VMEM((D // 2, 6 * D), U32),
        pltpu.VMEM((D // 2, F), U32),
        pltpu.VMEM((D // 2, F), U32),
        pltpu.VMEM((F // 2, D), U32),
        pltpu.VMEM((NOSLOT * 32 + PRE, KS), BF),
        pltpu.VMEM((NOSLOT * 32 + PRE, H * DH - KS), BF),
    ] + [pltpu.VMEM((NSLOT, 3 * NP // NB, 64, 128), BF) for _ in range(NB)] + [
        pltpu.SemaphoreType.DMA((17,)),
        pltpu.SemaphoreType.DMA((12,)),
    ]
    wq, wk, wv = (w.reshape(D // 2, 2, H, DH) for w in (A_Wq, A_Wk, A_Wv))
    return pl.pallas_call(
        _kernel,
        out_shape=jax.ShapeDtypeStruct((1, S, D), BF),
        in_specs=[any_spec] * 12,
        out_specs=any_spec,
        scratch_shapes=scratch,
        compiler_params=pltpu.CompilerParams(vmem_limit_bytes=120 * 1024 * 1024),
    )(A_x, A_mem0, wq, wk, wv, A_Wo, B_w_r.reshape(1, D), B_w_gate, B_w_up, B_w_down,
      c, w_mod)
```

```python
import os
import jax
import jax.numpy as jnp
from jax import lax
import jax.experimental.pallas as pl
import jax.experimental.pallas.tpu as pltpu

BF = jnp.bfloat16
F32 = jnp.float32
U32 = jnp.uint32

S = 2048
D = 1024
H = 32
DH = 128
M = 8
SEG = 32
NSEG = S // SEG
F = 3584
NP = H // 2
RIDE = 24
PRE = S - NSEG * RIDE
NSLOT = 17
NOSLOT = 17
NB = int(os.environ.get('NB', 8))
KS = int(os.environ.get('KS', 2560))
LAG_S = 1
LAG_P = 3
EPS = 1e-5
SCALE = DH ** -0.5
OOFF = S
HOFF = 2 * S
ROFF = HOFF + 64
XOFF = ROFF + 16
PRE_SPLIT = 3
E_AT = tuple(int(v) for v in os.environ.get('E_AT', '2,3,4').split(','))
L_AT = tuple(int(v) for v in os.environ.get('L_AT', '8,10,12').split(','))
E_AT2 = tuple(int(v) for v in os.environ.get('E_AT2', '2,3,4').split(','))
L_AT2 = tuple(int(v) for v in os.environ.get('L_AT2', '8,10,12').split(','))


def _att_schedule(mode):
    att = {}
    if mode == 'lag':
        for p in range(NP):
            att.setdefault(p + LAG_S, []).append(('s', p))
        for p in range(NP):
            att.setdefault(p + LAG_P, []).append(('p', p))
    elif mode == 'q2':
        for p in range(0, NP, 2):
            att.setdefault(p + 2, []).extend([('s', p), ('s', p + 1)])
        for p in range(0, NP, 2):
            att.setdefault(p + 4, []).extend([('p', p), ('p', p + 1)])
    elif mode == 'q2b':
        for p in range(0, NP, 2):
            att.setdefault(p + 4, []).extend([('p', p), ('p', p + 1)])
        for p in range(0, NP, 2):
            att.setdefault(p + 2, []).extend([('s', p), ('s', p + 1)])
    elif mode == 'q2c':
        att[4] = [('s', i) for i in range(4)]
        for p in range(4, NP, 2):
            att[p + 2] = [('s', p), ('s', p + 1), ('p', p - 4), ('p', p - 3)]
        att[18] = [('p', i) for i in range(12, 16)]
    elif mode == 'q2d':
        att[3] = [('s', i) for i in range(3)]
        att[4] = [('s', 3)]
        att[3] = []
        att[4] = [('s', i) for i in range(4)]
        for p in range(4, NP, 2):
            att[p + 2] = [('p', p - 4), ('p', p - 3), ('s', p), ('s', p + 1)]
        att[18] = [('p', i) for i in range(12, 16)]
    elif mode == 'q4':
        for p in range(0, NP, 4):
            att.setdefault(p + 4, []).extend([('s', p + i) for i in range(4)])
            att.setdefault(p + 6, []).extend([('p', p + i) for i in range(4)])
    elif mode == 'q4b':
        for p in range(0, NP, 4):
            att.setdefault(min(p + 8, 18), []).extend([('p', p + i) for i in range(4)])
        for p in range(0, NP, 4):
            att.setdefault(p + 4, []).extend([('s', p + i) for i in range(4)])
    return att


ATT = _att_schedule(os.environ.get('ATT', 'q2c'))
XACT = int(os.environ.get('XACT', 0))
UNR = int(os.environ.get('UNR', 2))
EPI_CHUNKS = (128, 128, 128, 96, 32)


NTAB = 16


def _step_indices(s):
    t = [s % NSLOT]
    for j in range(3):
        gi = PRE // 8 + 3 * s + j
        t += [(gi // 4) % NSLOT, (gi % 4) * 8]
    for j in range(4):
        gi = 4 * s + j
        t.append(((gi // 3) % NOSLOT) * 32 + 8 + (gi % 3) * 8 if gi < 3 * NSEG
                 else NOSLOT * 32 + (gi - 3 * NSEG) * 8)
    t.append((s % NOSLOT) * 32)
    t.append(max(s - 1, 0) * RIDE)
    t.append(PRE + min(s + 1, NSEG - 1) * RIDE)
    return t


def _rb(v):
    return v.astype(BF).astype(F32)


def _layernorm(x):
    mu = jnp.sum(x, axis=-1, keepdims=True) * (1.0 / D)
    xc = x - mu
    var = jnp.sum(xc * xc, axis=-1, keepdims=True) * (1.0 / D)
    sd = _rb(jnp.sqrt(_rb(_rb(var) + EPS)))
    return _rb(_rb(x - _rb(mu)) / sd)


def _kernel(x_hbm, mem0_hbm, wq_hbm, wk_hbm, wv_hbm, wo_hbm, wr_hbm, wg_hbm, wu_hbm,
            wd_hbm, c_hbm, wmod_hbm, out_hbm,
            xbuf, act, h0buf, abuf, ybuf, tab, modb, cbuf, wrbuf,
            w_v, wo_v, wmod_v, wg_v, wu_v, wd_v,
            obuf1, obuf2, sems, wsems, *qkvbufs):
    qkv32 = tuple(b.bitcast(U32) for b in qkvbufs)
    if XACT:
        xbuf = act.at[pl.ds(XOFF, S)]
    w_hbms = tuple(w.bitcast(U32) for w in (wq_hbm, wk_hbm, wv_hbm))

    def cp(src, dst, i):
        return pltpu.make_async_copy(src, dst, sems.at[i])

    wmod_b = wmod_v.bitcast(BF)
    cp_c = cp(c_hbm, cbuf, 0)
    cp_mem = cp(mem0_hbm.at[0], act.at[HOFF:HOFF + M], 1)
    cp_wr = cp(wr_hbm, wrbuf, 2)
    cp_x0 = cp(x_hbm.at[0, 0:PRE], xbuf.at[0:PRE], 3)
    cp_x1 = cp(x_hbm.at[0, PRE:S], xbuf.at[PRE:S], 4)
    cp_moda = [cp(wmod_hbm.at[:, n * 512:(n + 1) * 512], wmod_b.at[:, n * 512:(n + 1) * 512],
                  13 + n) for n in range(4)]
    cp_modb = cp(wmod_hbm.at[:, 2 * D:6 * D], wmod_b.at[:, 2 * D:6 * D], 6)
    cp_wo = cp(wo_hbm, wo_v.bitcast(BF), 7)
    cp_ffn = [cp(wg_hbm, wg_v.bitcast(BF), 8), cp(wu_hbm, wu_v.bitcast(BF), 8),
              cp(wd_hbm, wd_v.bitcast(BF), 8)]

    def w_start(j):
        gg, t = j // 3, j % 3
        for i in range(NB):
            for par in range(2):
                pltpu.make_async_copy(w_hbms[t].at[:, par, gg * NB + i, :],
                                      w_v.at[(gg * NB + i) * 6 + t * 2 + par],
                                      wsems.at[2 * j + (i >= PRE_SPLIT)]).start()

    cp_c.start()
    cp_x0.start()
    for c_ in cp_moda:
        c_.start()
    w_start(0)
    cp_mem.start()
    cp_wr.start()
    w_start(1)
    w_start(2)

    def mod_part(sc16, lo, hi):
        w = pltpu.bitcast(wmod_v[:, lo:hi], BF)
        return _rb(jnp.dot(sc16, w, preferred_element_type=F32))[0:8]

    def ln1_rows(src_row, dst_row):
        xv = xbuf[pl.ds(src_row, 8), :].astype(F32)
        hv = _rb(_layernorm(xv) * modb[1]) + modb[0]
        act[pl.ds(dst_row, 8), :] = hv.astype(BF)

    lane256 = lax.broadcasted_iota(jnp.int32, (8, 256), 1)

    def finish_rows(row, attn):
        xv = xbuf[pl.ds(row, 8), :].astype(F32)
        x1 = _rb(xv + _rb(modb[2] * _rb(attn)))
        h2 = _rb(_rb(_layernorm(x1) * modb[4]) + modb[3])
        act[pl.ds(row, 8), :] = x1.astype(BF)
        act[pl.ds(OOFF + row, 8), :] = (x1 + _rb(modb[5] * h2)).astype(BF)
        r = jnp.sum(h2 * modb[6], axis=-1, keepdims=True)
        act[ROFF:ROFF + 8, 0:256] = jnp.where(
            lane256 * 8 == row, r, act[ROFF:ROFF + 8, 0:256].astype(F32)).astype(BF)

    act[ROFF:ROFF + 8, 0:256] = jnp.zeros((8, 256), BF)
    abuf[...] = jnp.zeros(abuf.shape, F32)
    for s_ in range(NSEG):
        for k, v in enumerate(_step_indices(s_)):
            tab[s_ * NTAB + k] = v
    cp_c.wait()
    cv = cbuf[...].astype(F32)
    sc16 = jnp.broadcast_to(_rb(cv * _rb(jax.nn.sigmoid(cv))), (16, D)).astype(BF)
    cp_x0.wait()

    def ln_pre(g, carry):
        row = pl.multiple_of(g * 64, 64)
        h0buf[pl.ds(row, 64), :] = _layernorm(xbuf[pl.ds(row, 64), :].astype(F32)).astype(BF)
        return carry
    lax.fori_loop(0, PRE // 64, ln_pre, 0)

    for n in range(4):
        cp_moda[n].wait()
        mv = mod_part(sc16, n * 512, (n + 1) * 512)
        if n >= 2:
            mv = _rb(1.0 + mv)
        modb[n // 2, :, (n % 2) * 512:(n % 2 + 1) * 512] = mv

    def mod_pre(g, carry):
        for u in range(8):
            row = pl.multiple_of(g * 64 + u * 8, 8)
            nv = h0buf[pl.ds(row, 8), :].astype(F32)
            h0buf[pl.ds(row, 8), :] = (_rb(nv * modb[1]) + modb[0]).astype(BF)
        return carry
    lax.fori_loop(0, PRE // 64, mod_pre, 0)

    def pre_unit(j, i):
        blk = (j // 3) * (6 * NB) + (j % 3) * 2 + i * 6
        a = w_v[blk]
        b = w_v[blk + 1]
        lo = (a & U32(0xFFFF)) | (b << 16)
        hi = (a >> 16) | (b & U32(0xFFFF0000))
        w_v[blk] = lo
        w_v[blk + 1] = hi
        for rc in range(PRE // 128):
            if rc > 0:
                lo = w_v[blk]
                hi = w_v[blk + 1]
            w = pltpu.bitcast(jnp.concatenate([lo, hi], axis=1), BF)
            y = jnp.dot(h0buf[rc * 128:(rc + 1) * 128, :], w, preferred_element_type=F32)
            for sg in range(4):
                for hh in range(2):
                    qkvbufs[i][rc * 4 + sg, j, 16 + hh * 32:16 + (hh + 1) * 32, :] = (
                        y[sg * 32:(sg + 1) * 32, hh * 128:(hh + 1) * 128].astype(BF))

    def pre_body(j, carry):
        @pl.when(j == 1)
        def _():
            w_start(3)
            w_start(4)

        @pl.when(j == 2)
        def _():
            w_start(5)
            cp_wo.start()

        @pl.when(j == 3)
        def _():
            cp_x1.start()
            cp_modb.start()
        blk0 = (j // 3) * (6 * NB) + (j % 3) * 2
        for half, (i0, i1) in enumerate(((0, PRE_SPLIT), (PRE_SPLIT, NB))):
            for i in range(i0, i1):
                for par in range(2):
                    pltpu.make_async_copy(w_hbms[0].at[:, 0, 0, :], w_v.at[blk0 + i * 6 + par],
                                          wsems.at[2 * j + half]).wait()
            for i in range(i0, i1):
                pre_unit(j, i)
        return carry
    lax.fori_loop(0, 6, pre_body, 0)

    cp_mem.wait()
    cp_wr.wait()
    cp_wo.wait()
    cp_x1.wait()
    cp_modb.wait()
    for c_ in cp_ffn:
        c_.start()
    modc = mod_part(sc16, 2 * D, 6 * D)
    modb[2] = modc[:, 0:D]
    modb[3] = modc[:, D:2 * D]
    modb[4] = _rb(1.0 + modc[:, 2 * D:3 * D])
    modb[5] = modc[:, 3 * D:4 * D]
    modb[6] = jnp.broadcast_to(wrbuf[...].astype(F32), (8, D))
    for j in range(3):
        ln1_rows(PRE + 8 * j, HOFF + 8 + 8 * j)

    ri = lax.broadcasted_iota(jnp.int32, (80, 80), 0)
    ci = lax.broadcasted_iota(jnp.int32, (80, 80), 1)

    def head_pos(i):
        hd = jnp.where(i < 16, i // 8, (i - 16) // 32)
        pos = jnp.where(i < 16, i % 8, 8 + (i - 16) % 32)
        return hd, pos
    rh, rp = head_pos(ri)
    ch, cpos = head_pos(ci)
    same = rh == ch
    valid = same & ((rp < M) | (rp >= cpos))
    fill = jnp.where(same, -1e9, -jnp.inf).astype(F32)

    def wo_w(h0, h1, n0, n1):
        w = wo_v[h0:h1, :, n0 * 128:n1 * 128].reshape((h1 - h0) * (DH // 2), (n1 - n0) * 128)
        return pltpu.bitcast(w, BF)

    HD = D // 2

    def emit_step(s, pend, last):
        hrow = pl.multiple_of(HOFF + (s & 1) * 32, 32)
        hnext = pl.multiple_of(HOFF + 32 - (s & 1) * 32, 32)
        tv = [tab[s * NTAB + k] for k in range(14)]
        slot = tv[0]
        dsts = [(tv[1 + 2 * j], pl.multiple_of(tv[2 + 2 * j], 8)) for j in range(3)]
        odst = [pl.multiple_of(tv[7 + j], 8) for j in range(4)]
        orow = pl.multiple_of(tv[11], 32)
        erow = tv[12]
        lrow = tv[13]
        e_at, l_at = (E_AT, L_AT) if pend is None else (E_AT2, L_AT2)
        probs = {}

        def wqkv(p, k0, k1):
            return pltpu.bitcast(jnp.concatenate(
                [w_v[p * 6 + u, k0 // 2:k1 // 2, :] for u in range(6)], axis=1), BF)

        lhs_lo = act[pl.ds(hrow, 32), 0:HD]
        if pend is not None:
            ybuf[...] = jnp.dot(lhs_lo, wqkv(0, 0, HD), preferred_element_type=F32)
            pend()
        lhs_hi = act[pl.ds(hrow, 32), HD:D]
        if pend is not None:
            y0 = ybuf[...] + jnp.dot(lhs_hi, wqkv(0, HD, D), preferred_element_type=F32)
        lhs_rest = jnp.concatenate([lhs_lo[:, 128:], lhs_hi], axis=1)
        lhs = [jnp.concatenate([lhs_lo, lhs_hi], axis=1)]

        def side(p):
            for j in range(3):
                if e_at[j] == p:
                    finish_rows(pl.multiple_of(erow + 8 * j, 8), abuf[8 * j:8 * j + 8, :])
            for j in range(3):
                if l_at[j] == p:
                    ln1_rows(pl.multiple_of(lrow + 8 * j, 8),
                             pl.multiple_of(hnext + 8 + 8 * j, 8))
            if (p in e_at or p in l_at) and p < NP - 1:
                lhs[0] = jnp.concatenate([act[pl.ds(hrow, 32), 0:128], lhs_rest], axis=1)

        def qkv(p):
            if p == 0 and pend is not None:
                y = y0
            else:
                y = jnp.dot(lhs[0], wqkv(p, 0, D), preferred_element_type=F32)
            buf = qkvbufs[p % NB]
            for u in range(6):
                t, hh = u // 2, u % 2
                bi = (p // NB) * 3 + t
                yu = y[:, u * 128:(u + 1) * 128]
                buf[slot, bi, hh * 8:hh * 8 + 8, :] = yu[0:8].astype(BF)
                for j in range(3):
                    sl, off = dsts[j]
                    buf[sl, bi, pl.ds(16 + hh * 32 + off, 8), :] = (
                        yu[8 + 8 * j:16 + 8 * j].astype(BF))

        def ld(p, t):
            return pltpu.bitcast(qkv32[p % NB][slot, (p // NB) * 3 + t], BF)

        def sc(p):
            s2 = lax.dot_general(ld(p, 0), ld(p, 1), (((1,), (1,)), ((), ())),
                                 preferred_element_type=F32) * SCALE
            s2 = jnp.where(valid, s2, fill)
            m = jnp.max(s2, axis=-1, keepdims=True)
            e = jnp.exp(s2 - m)
            l = jnp.sum(e, axis=-1, keepdims=True)
            rl = pl.reciprocal(l, approx=True)
            rl = rl * (2.0 - l * rl)
            probs[p] = (e * rl).astype(BF)

        def pv(p):
            o2 = jnp.dot(probs[p], ld(p, 2), preferred_element_type=F32)
            for hh in range(2):
                hcol = (2 * p + hh) * 128
                ob = obuf1
                if hcol >= KS:
                    ob = obuf2
                    hcol -= KS
                ob[pl.ds(orow, 8), hcol:hcol + 128] = o2[8 * hh:8 * hh + 8].astype(BF)
                for j in range(4):
                    r0 = 16 + 32 * hh + 8 * j
                    ob[pl.ds(odst[j], 8), hcol:hcol + 128] = o2[r0:r0 + 8].astype(BF)

        def attn(pos):
            for kind, p in ATT.get(pos, ()):
                (sc if kind == 's' else pv)(p)

        for p in range(NP):
            qkv(p)
            side(p)
            attn(p)
        a1 = []
        for i in range(4):
            a1.append(jnp.dot(obuf1[pl.ds(orow, 32), :], wo_w(0, KS // DH, 2 * i, 2 * i + 2),
                              preferred_element_type=F32))
            attn(NP + i)
            side(NP + i)
        o2lhs = obuf2[pl.ds(orow, 32), :]
        a_lo = jnp.concatenate(a1[0:2], axis=1) + jnp.dot(
            o2lhs, wo_w(KS // DH, H, 0, 4), preferred_element_type=F32)
        act[pl.ds(hnext, 8), 0:HD] = a_lo[0:8].astype(BF)
        abuf[:, 0:HD] = a_lo[8:32]
        a_hi = jnp.concatenate(a1[2:4], axis=1) + jnp.dot(
            o2lhs, wo_w(KS // DH, H, 4, 8), preferred_element_type=F32)

        def finish():
            act[pl.ds(hnext, 8), HD:D] = a_hi[0:8].astype(BF)
            abuf[:, HD:D] = a_hi[8:32]
        if last:
            finish()
        return finish

    def steps(it, carry):
        pend = None
        for u in range(UNR):
            pend = emit_step(it * UNR + u, pend, u == UNR - 1)
        return carry
    lax.fori_loop(0, NSEG // UNR, steps, 0)

    for j in range(3):
        finish_rows((NSEG - 1) * RIDE + 8 * j, abuf[8 * j:8 * j + 8, :])
    OUT0 = NSEG * RIDE
    cp_out = [cp(act.at[OOFF:OOFF + OUT0], out_hbm.at[0, 0:OUT0], 9)]
    cp_out[0].start()
    r0 = 0
    for ech in EPI_CHUNKS:
        o0 = NOSLOT * 32 + r0
        a = (jnp.dot(obuf1[o0:o0 + ech, :], wo_w(0, KS // DH, 0, 8), preferred_element_type=F32)
             + jnp.dot(obuf2[o0:o0 + ech, :], wo_w(KS // DH, H, 0, 8), preferred_element_type=F32))
        for j in range(ech // 8):
            finish_rows(OUT0 + r0 + 8 * j, a[8 * j:8 * j + 8])
        r0 += ech
    cp_out.append(cp(act.at[OOFF + OUT0:OOFF + S], out_hbm.at[0, OUT0:S], 10))
    cp_out[1].start()

    r_all = act[ROFF:ROFF + 8, 0:256].astype(F32)
    rows = lane256 * 8 + lax.broadcasted_iota(jnp.int32, (8, 256), 0)

    def allmax(v):
        return jnp.max(jnp.max(v, axis=1, keepdims=True), axis=0, keepdims=True)

    def allmin(v):
        return jnp.min(jnp.min(v, axis=1, keepdims=True), axis=0, keepdims=True)
    rowsf = rows.astype(F32)
    i1v = allmin(jnp.where(r_all == allmax(r_all), rowsf, float(S)))
    r_rest = jnp.where(rowsf == i1v, -jnp.inf, r_all)
    i2v = allmin(jnp.where((r_rest == allmax(r_rest)) & (rowsf != i1v), rowsf, float(S)))
    i1 = jnp.clip(i1v[0, 0].astype(jnp.int32), 0, S - 1)
    i2 = jnp.clip(i2v[0, 0].astype(jnp.int32), 0, S - 1)
    b1 = pl.multiple_of((i1 // 8) * 8, 8)
    b2 = pl.multiple_of((i2 // 8) * 8, 8)

    x1 = jnp.concatenate([act[pl.ds(b1, 8), :].astype(F32), act[pl.ds(b2, 8), :].astype(F32)],
                         axis=0)

    def two(i):
        return jnp.concatenate([modb[i], modb[i]], axis=0)
    h2 = _rb(_rb(_layernorm(x1) * two(4)) + two(3))
    rr = _rb(jnp.sum(h2 * two(6), axis=-1, keepdims=True))
    h2b = h2.astype(BF)
    for c_ in cp_ffn:
        c_.wait()
    gt = _rb(jnp.dot(h2b, pltpu.bitcast(wg_v[...], BF), preferred_element_type=F32))
    up = _rb(jnp.dot(h2b, pltpu.bitcast(wu_v[...], BF), preferred_element_type=F32))
    hid = (_rb(gt * _rb(jax.nn.sigmoid(gt))) * up).astype(BF)
    y = _rb(jnp.dot(hid, pltpu.bitcast(wd_v[...], BF), preferred_element_type=F32))
    y = _rb(y * _rb(jax.nn.sigmoid(rr)))
    sub = lax.broadcasted_iota(jnp.int32, (16, 1), 0)
    grow = jnp.where(sub < 8, b1 + sub, b2 + sub - 8)
    sel = (grow == i1) | (grow == i2)
    res = (x1 + _rb(two(5) * _rb(h2 + jnp.where(sel, y, 0.0)))).astype(BF)
    for c_ in cp_out:
        c_.wait()
    act[pl.ds(OOFF + b1, 8), :] = res[0:8]
    act[pl.ds(OOFF + b2, 8), :] = res[8:16]
    fix1 = cp(act.at[pl.ds(OOFF + b1, 8)], out_hbm.at[0, pl.ds(b1, 8)], 11)
    fix2 = cp(act.at[pl.ds(OOFF + b2, 8)], out_hbm.at[0, pl.ds(b2, 8)], 12)
    fix1.start()

    @pl.when(b1 != b2)
    def _():
        fix2.start()
        fix2.wait()
    fix1.wait()


@jax.jit
def pallas_adaLN_cond__memory_aug_recurrent_mem_tr__moe_arch_mod__prompt_kernel(
    A_x: jax.Array,
    A_mem0: jax.Array,
    A_Wq: jax.Array,
    A_Wk: jax.Array,
    A_Wv: jax.Array,
    A_Wo: jax.Array,
    A_seg_len,
    B_x: jax.Array,
    B_w_r: jax.Array,
    B_w_gate: jax.Array,
    B_w_up: jax.Array,
    B_w_down: jax.Array,
    c: jax.Array,
    w_mod: jax.Array,
):
    del B_x
    del A_seg_len
    assert A_x.shape == (1, S, D) and A_Wq.shape == (D, H, DH) and A_mem0.shape == (1, M, D)
    any_spec = pl.BlockSpec(memory_space=pl.ANY)
    scratch = [
        pltpu.VMEM((S if not XACT else 8, D), BF),
        pltpu.VMEM((XOFF + S * XACT, D), BF),
        pltpu.VMEM((PRE, D), BF),
        pltpu.VMEM((RIDE, D), F32),
        pltpu.VMEM((32, 768), F32),
        pltpu.SMEM((NSEG * NTAB,), jnp.int32),
        pltpu.VMEM((7, 8, D), F32),
        pltpu.VMEM((1, D), BF),
        pltpu.VMEM((1, D), BF),
        pltpu.VMEM((3 * H, D // 2, 128), U32),
        pltpu.VMEM((H, DH // 2, D), U32),
        pltpu.VMEM((D // 2, 6 * D), U32),
        pltpu.VMEM((D // 2, F), U32),
        pltpu.VMEM((D // 2, F), U32),
        pltpu.VMEM((F // 2, D), U32),
        pltpu.VMEM((NOSLOT * 32 + PRE, KS), BF),
        pltpu.VMEM((NOSLOT * 32 + PRE, H * DH - KS), BF),
        pltpu.SemaphoreType.DMA((17,)),
        pltpu.SemaphoreType.DMA((12,)),
    ] + [pltpu.VMEM((NSLOT, 3 * NP // NB, 80, 128), BF) for _ in range(NB)]
    wq, wk, wv = (w.reshape(D // 2, 2, H, DH) for w in (A_Wq, A_Wk, A_Wv))
    return pl.pallas_call(
        _kernel,
        out_shape=jax.ShapeDtypeStruct((1, S, D), BF),
        in_specs=[any_spec] * 12,
        out_specs=any_spec,
        scratch_shapes=scratch,
        compiler_params=pltpu.CompilerParams(vmem_limit_bytes=120 * 1024 * 1024),
    )(A_x, A_mem0, wq, wk, wv, A_Wo, B_w_r.reshape(1, D), B_w_gate, B_w_up, B_w_down,
      c, w_mod)
```

```python
import os
import jax
import jax.numpy as jnp
from jax import lax
import jax.experimental.pallas as pl
import jax.experimental.pallas.tpu as pltpu

BF = jnp.bfloat16
F32 = jnp.float32
U32 = jnp.uint32

S = 2048
D = 1024
H = 32
DH = 128
M = 8
SEG = 32
NSEG = S // SEG
F = 3584
NP = H // 2
RIDE = 24
PRE = S - NSEG * RIDE
NSLOT = 17
NOSLOT = 17
NB = int(os.environ.get('NB', 8))
KS = int(os.environ.get('KS', 2560))
LAG_S = 1
LAG_P = 3
EPS = 1e-5
SCALE = DH ** -0.5
OOFF = S
HOFF = 2 * S
ROFF = HOFF + 64
XOFF = ROFF + 16
PRE_SPLIT = 3
E_AT = tuple(int(v) for v in os.environ.get('E_AT', '2,3,4').split(','))
L_AT = tuple(int(v) for v in os.environ.get('L_AT', '8,10,12').split(','))
E_AT2 = tuple(int(v) for v in os.environ.get('E_AT2', '2,3,4').split(','))
L_AT2 = tuple(int(v) for v in os.environ.get('L_AT2', '8,10,12').split(','))


def _att_schedule(mode):
    att = {}
    if mode == 'lag':
        for p in range(NP):
            att.setdefault(p + LAG_S, []).append(('s', p))
        for p in range(NP):
            att.setdefault(p + LAG_P, []).append(('p', p))
    elif mode == 'q2':
        for p in range(0, NP, 2):
            att.setdefault(p + 2, []).extend([('s', p), ('s', p + 1)])
        for p in range(0, NP, 2):
            att.setdefault(p + 4, []).extend([('p', p), ('p', p + 1)])
    elif mode == 'q2b':
        for p in range(0, NP, 2):
            att.setdefault(p + 4, []).extend([('p', p), ('p', p + 1)])
        for p in range(0, NP, 2):
            att.setdefault(p + 2, []).extend([('s', p), ('s', p + 1)])
    elif mode == 'q2c':
        att[4] = [('s', i) for i in range(4)]
        for p in range(4, NP, 2):
            att[p + 2] = [('s', p), ('s', p + 1), ('p', p - 4), ('p', p - 3)]
        att[18] = [('p', i) for i in range(12, 16)]
    elif mode == 'q2d':
        att[3] = [('s', i) for i in range(3)]
        att[4] = [('s', 3)]
        att[3] = []
        att[4] = [('s', i) for i in range(4)]
        for p in range(4, NP, 2):
            att[p + 2] = [('p', p - 4), ('p', p - 3), ('s', p), ('s', p + 1)]
        att[18] = [('p', i) for i in range(12, 16)]
    elif mode == 'q4':
        for p in range(0, NP, 4):
            att.setdefault(p + 4, []).extend([('s', p + i) for i in range(4)])
            att.setdefault(p + 6, []).extend([('p', p + i) for i in range(4)])
    elif mode == 'q4b':
        for p in range(0, NP, 4):
            att.setdefault(min(p + 8, 18), []).extend([('p', p + i) for i in range(4)])
        for p in range(0, NP, 4):
            att.setdefault(p + 4, []).extend([('s', p + i) for i in range(4)])
    return att


ATT = _att_schedule(os.environ.get('ATT', 'q2c'))
XACT = int(os.environ.get('XACT', 0))
FFN_MODE = int(os.environ.get('FFN_MODE', 0))
LD32 = int(os.environ.get('LD32', 1))
UNR = int(os.environ.get('UNR', 2))
EPI_CHUNKS = (128, 128, 128, 96, 32)


NTAB = 16


def _step_indices(s):
    t = [s % NSLOT]
    for j in range(3):
        gi = PRE // 8 + 3 * s + j
        t += [(gi // 4) % NSLOT, (gi % 4) * 8]
    for j in range(4):
        gi = 4 * s + j
        t.append(((gi // 3) % NOSLOT) * 32 + 8 + (gi % 3) * 8 if gi < 3 * NSEG
                 else NOSLOT * 32 + (gi - 3 * NSEG) * 8)
    t.append((s % NOSLOT) * 32)
    t.append(max(s - 1, 0) * RIDE)
    t.append(PRE + min(s + 1, NSEG - 1) * RIDE)
    return t


def _rb(v):
    return v.astype(BF).astype(F32)


def _layernorm(x):
    mu = jnp.sum(x, axis=-1, keepdims=True) * (1.0 / D)
    xc = x - mu
    var = jnp.sum(xc * xc, axis=-1, keepdims=True) * (1.0 / D)
    sd = _rb(jnp.sqrt(_rb(_rb(var) + EPS)))
    return _rb(_rb(x - _rb(mu)) / sd)


def _kernel(x_hbm, mem0_hbm, wq_hbm, wk_hbm, wv_hbm, wo_hbm, wr_hbm, wg_hbm, wu_hbm,
            wd_hbm, c_hbm, wmod_hbm, out_hbm,
            xbuf, act, h0buf, abuf, ybuf, tab, modb, small,
            w_v, wo_v, wmod_v, wg_v, wu_v, wd_v,
            obuf1, obuf2, sems, wsems, *qkvbufs):
    qkv32 = tuple(b.bitcast(U32) for b in qkvbufs)
    if XACT:
        xbuf = act.at[pl.ds(XOFF, S)]
    w_hbms = tuple(w.bitcast(U32) for w in (wq_hbm, wk_hbm, wv_hbm))

    def cp(src, dst, i):
        return pltpu.make_async_copy(src, dst, sems.at[i])

    wmod_b = wmod_v.bitcast(BF)
    cp_c = cp(c_hbm, small.at[0], 0)
    cp_mem = cp(mem0_hbm.at[0], act.at[HOFF:HOFF + M], 1)
    cp_wr = cp(wr_hbm, small.at[1], 2)
    cp_x0 = cp(x_hbm.at[0, 0:PRE], xbuf.at[0:PRE], 3)
    cp_x1 = cp(x_hbm.at[0, PRE:S], xbuf.at[PRE:S], 4)
    cp_moda = [cp(wmod_hbm.at[:, n * 512:(n + 1) * 512], wmod_b.at[:, n * 512:(n + 1) * 512],
                  13 + n) for n in range(4)]
    cp_modb = cp(wmod_hbm.at[:, 2 * D:6 * D], wmod_b.at[:, 2 * D:6 * D], 6)
    cp_wo = cp(wo_hbm, wo_v.bitcast(BF), 7)
    cp_ffn = [cp(wg_hbm, wg_v.bitcast(BF), 8), cp(wu_hbm, wu_v.bitcast(BF), 8),
              cp(wd_hbm, wd_v.bitcast(BF), 8)]

    def w_start(j):
        gg, t = j // 3, j % 3
        for i in range(NB):
            for par in range(2):
                pltpu.make_async_copy(w_hbms[t].at[:, par, gg * NB + i, :],
                                      w_v.at[(gg * NB + i) * 6 + t * 2 + par],
                                      wsems.at[2 * j + (i >= PRE_SPLIT)]).start()

    cp_c.start()
    cp_x0.start()
    for c_ in cp_moda:
        c_.start()
    w_start(0)
    cp_mem.start()
    cp_wr.start()
    w_start(1)
    w_start(2)

    def mod_part(sc16, lo, hi):
        w = pltpu.bitcast(wmod_v[:, lo:hi], BF)
        return _rb(jnp.dot(sc16, w, preferred_element_type=F32))[0:8]

    def ln1_rows(src_row, dst_row):
        xv = xbuf[pl.ds(src_row, 8), :].astype(F32)
        hv = _rb(_layernorm(xv) * modb[1]) + modb[0]
        act[pl.ds(dst_row, 8), :] = hv.astype(BF)

    lane256 = lax.broadcasted_iota(jnp.int32, (8, 256), 1)

    def finish_rows(row, attn):
        xv = xbuf[pl.ds(row, 8), :].astype(F32)
        x1 = _rb(xv + _rb(modb[2] * _rb(attn)))
        h2 = _rb(_rb(_layernorm(x1) * modb[4]) + modb[3])
        act[pl.ds(row, 8), :] = x1.astype(BF)
        act[pl.ds(OOFF + row, 8), :] = (x1 + _rb(modb[5] * h2)).astype(BF)
        r = jnp.sum(h2 * modb[6], axis=-1, keepdims=True)
        act[ROFF:ROFF + 8, 0:256] = jnp.where(
            lane256 * 8 == row, r, act[ROFF:ROFF + 8, 0:256].astype(F32)).astype(BF)

    act[ROFF:ROFF + 8, 0:256] = jnp.zeros((8, 256), BF)
    abuf[...] = jnp.zeros(abuf.shape, F32)
    for s_ in range(NSEG):
        for k, v in enumerate(_step_indices(s_)):
            tab[s_ * NTAB + k] = v
    cp_c.wait()
    cv = small[0].astype(F32)
    sc16 = jnp.broadcast_to(_rb(cv * _rb(jax.nn.sigmoid(cv))), (16, D)).astype(BF)
    cp_x0.wait()

    def ln_pre(g, carry):
        row = pl.multiple_of(g * 64, 64)
        h0buf[pl.ds(row, 64), :] = _layernorm(xbuf[pl.ds(row, 64), :].astype(F32)).astype(BF)
        return carry
    lax.fori_loop(0, PRE // 64, ln_pre, 0)

    for n in range(4):
        cp_moda[n].wait()
        mv = mod_part(sc16, n * 512, (n + 1) * 512)
        if n >= 2:
            mv = _rb(1.0 + mv)
        modb[n // 2, :, (n % 2) * 512:(n % 2 + 1) * 512] = mv

    def mod_pre(g, carry):
        for u in range(8):
            row = pl.multiple_of(g * 64 + u * 8, 8)
            nv = h0buf[pl.ds(row, 8), :].astype(F32)
            h0buf[pl.ds(row, 8), :] = (_rb(nv * modb[1]) + modb[0]).astype(BF)
        return carry
    lax.fori_loop(0, PRE // 64, mod_pre, 0)

    def pre_unit(j, i):
        blk = (j // 3) * (6 * NB) + (j % 3) * 2 + i * 6
        jrow = pl.multiple_of(j * 80, 16)
        a = w_v[blk]
        b = w_v[blk + 1]
        lo = (a & U32(0xFFFF)) | (b << 16)
        hi = (a >> 16) | (b & U32(0xFFFF0000))
        w_v[blk] = lo
        w_v[blk + 1] = hi
        for rc in range(PRE // 128):
            if rc > 0:
                lo = w_v[blk]
                hi = w_v[blk + 1]
            w = pltpu.bitcast(jnp.concatenate([lo, hi], axis=1), BF)
            y = jnp.dot(h0buf[rc * 128:(rc + 1) * 128, :], w, preferred_element_type=F32)
            for sg in range(4):
                for hh in range(2):
                    qkvbufs[i][rc * 4 + sg, pl.ds(jrow + 16 + hh * 32, 32), :] = (
                        y[sg * 32:(sg + 1) * 32, hh * 128:(hh + 1) * 128].astype(BF))

    def pre_body(j, carry):
        @pl.when(j == 1)
        def _():
            w_start(3)
            w_start(4)

        @pl.when(j == 2)
        def _():
            w_start(5)
            cp_wo.start()

        @pl.when(j == 3)
        def _():
            cp_x1.start()
            cp_modb.start()
        blk0 = (j // 3) * (6 * NB) + (j % 3) * 2
        for half, (i0, i1) in enumerate(((0, PRE_SPLIT), (PRE_SPLIT, NB))):
            for i in range(i0, i1):
                for par in range(2):
                    pltpu.make_async_copy(w_hbms[0].at[:, 0, 0, :], w_v.at[blk0 + i * 6 + par],
                                          wsems.at[2 * j + half]).wait()
            for i in range(i0, i1):
                pre_unit(j, i)
        return carry
    lax.fori_loop(0, 6, pre_body, 0)

    cp_mem.wait()
    cp_wr.wait()
    cp_wo.wait()
    cp_x1.wait()
    cp_modb.wait()
    if FFN_MODE == 0:
        for c_ in cp_ffn:
            c_.start()
    modc = mod_part(sc16, 2 * D, 6 * D)
    modb[2] = modc[:, 0:D]
    modb[3] = modc[:, D:2 * D]
    modb[4] = _rb(1.0 + modc[:, 2 * D:3 * D])
    modb[5] = modc[:, 3 * D:4 * D]
    modb[6] = jnp.broadcast_to(small[1].astype(F32), (8, D))
    for j in range(3):
        ln1_rows(PRE + 8 * j, HOFF + 8 + 8 * j)

    ri = lax.broadcasted_iota(jnp.int32, (80, 80), 0)
    ci = lax.broadcasted_iota(jnp.int32, (80, 80), 1)

    def head_pos(i):
        hd = jnp.where(i < 16, i // 8, (i - 16) // 32)
        pos = jnp.where(i < 16, i % 8, 8 + (i - 16) % 32)
        return hd, pos
    rh, rp = head_pos(ri)
    ch, cpos = head_pos(ci)
    same = rh == ch
    valid = same & ((rp < M) | (rp >= cpos))
    fill = jnp.where(same, -1e9, -jnp.inf).astype(F32)

    def wo_w(h0, h1, n0, n1):
        w = wo_v[h0:h1, :, n0 * 128:n1 * 128].reshape((h1 - h0) * (DH // 2), (n1 - n0) * 128)
        return pltpu.bitcast(w, BF)

    HD = D // 2

    def emit_step(s, pend, last):
        hrow = pl.multiple_of(HOFF + (s & 1) * 32, 32)
        hnext = pl.multiple_of(HOFF + 32 - (s & 1) * 32, 32)
        tv = [tab[s * NTAB + k] for k in range(14)]
        slot = tv[0]
        dsts = [(tv[1 + 2 * j], pl.multiple_of(tv[2 + 2 * j], 8)) for j in range(3)]
        odst = [pl.multiple_of(tv[7 + j], 8) for j in range(4)]
        orow = pl.multiple_of(tv[11], 32)
        erow = tv[12]
        lrow = tv[13]
        e_at, l_at = (E_AT, L_AT) if pend is None else (E_AT2, L_AT2)
        probs = {}

        def wqkv(p, k0, k1):
            return pltpu.bitcast(jnp.concatenate(
                [w_v[p * 6 + u, k0 // 2:k1 // 2, :] for u in range(6)], axis=1), BF)

        lhs_lo = act[pl.ds(hrow, 32), 0:HD]
        if pend is not None:
            ybuf[...] = jnp.dot(lhs_lo, wqkv(0, 0, HD), preferred_element_type=F32)
            pend()
        lhs_hi = act[pl.ds(hrow, 32), HD:D]
        if pend is not None:
            y0 = ybuf[...] + jnp.dot(lhs_hi, wqkv(0, HD, D), preferred_element_type=F32)
        lhs_rest = jnp.concatenate([lhs_lo[:, 128:], lhs_hi], axis=1)
        lhs = [jnp.concatenate([lhs_lo, lhs_hi], axis=1)]

        def side(p):
            for j in range(3):
                if e_at[j] == p:
                    finish_rows(pl.multiple_of(erow + 8 * j, 8), abuf[8 * j:8 * j + 8, :])
            for j in range(3):
                if l_at[j] == p:
                    ln1_rows(pl.multiple_of(lrow + 8 * j, 8),
                             pl.multiple_of(hnext + 8 + 8 * j, 8))
            if (p in e_at or p in l_at) and p < NP - 1:
                lhs[0] = jnp.concatenate([act[pl.ds(hrow, 32), 0:128], lhs_rest], axis=1)

        def qkv(p):
            if p == 0 and pend is not None:
                y = y0
            else:
                y = jnp.dot(lhs[0], wqkv(p, 0, D), preferred_element_type=F32)
            buf = qkvbufs[p % NB]
            for u in range(6):
                t, hh = u // 2, u % 2
                b0 = ((p // NB) * 3 + t) * 80
                yu = y[:, u * 128:(u + 1) * 128]
                buf[slot, b0 + hh * 8:b0 + hh * 8 + 8, :] = yu[0:8].astype(BF)
                for j in range(3):
                    sl, off = dsts[j]
                    buf[sl, pl.ds(b0 + 16 + hh * 32 + off, 8), :] = (
                        yu[8 + 8 * j:16 + 8 * j].astype(BF))

        def ld(p, t):
            b0 = ((p // NB) * 3 + t) * 40
            if not LD32:
                return qkvbufs[p % NB][slot, 2 * b0:2 * b0 + 80, :]
            return pltpu.bitcast(qkv32[p % NB][slot, b0:b0 + 40, :], BF)

        def sc(p):
            s2 = lax.dot_general(ld(p, 0), ld(p, 1), (((1,), (1,)), ((), ())),
                                 preferred_element_type=F32) * SCALE
            s2 = jnp.where(valid, s2, fill)
            m = jnp.max(s2, axis=-1, keepdims=True)
            e = jnp.exp(s2 - m)
            l = jnp.sum(e, axis=-1, keepdims=True)
            rl = pl.reciprocal(l, approx=True)
            rl = rl * (2.0 - l * rl)
            probs[p] = (e * rl).astype(BF)

        def pv(p):
            o2 = jnp.dot(probs[p], ld(p, 2), preferred_element_type=F32)
            for hh in range(2):
                hcol = (2 * p + hh) * 128
                ob = obuf1
                if hcol >= KS:
                    ob = obuf2
                    hcol -= KS
                ob[pl.ds(orow, 8), hcol:hcol + 128] = o2[8 * hh:8 * hh + 8].astype(BF)
                for j in range(4):
                    r0 = 16 + 32 * hh + 8 * j
                    ob[pl.ds(odst[j], 8), hcol:hcol + 128] = o2[r0:r0 + 8].astype(BF)

        def attn(pos):
            for kind, p in ATT.get(pos, ()):
                (sc if kind == 's' else pv)(p)

        for p in range(NP):
            qkv(p)
            side(p)
            attn(p)
        a1 = []
        for i in range(4):
            a1.append(jnp.dot(obuf1[pl.ds(orow, 32), :], wo_w(0, KS // DH, 2 * i, 2 * i + 2),
                              preferred_element_type=F32))
            attn(NP + i)
            side(NP + i)
        o2lhs = obuf2[pl.ds(orow, 32), :]
        a_lo = jnp.concatenate(a1[0:2], axis=1) + jnp.dot(
            o2lhs, wo_w(KS // DH, H, 0, 4), preferred_element_type=F32)
        act[pl.ds(hnext, 8), 0:HD] = a_lo[0:8].astype(BF)
        abuf[:, 0:HD] = a_lo[8:32]
        a_hi = jnp.concatenate(a1[2:4], axis=1) + jnp.dot(
            o2lhs, wo_w(KS // DH, H, 4, 8), preferred_element_type=F32)

        def finish():
            act[pl.ds(hnext, 8), HD:D] = a_hi[0:8].astype(BF)
            abuf[:, HD:D] = a_hi[8:32]
        if last:
            finish()
        return finish

    def steps(it, carry):
        pend = None
        for u in range(UNR):
            pend = emit_step(it * UNR + u, pend, u == UNR - 1)
        return carry
    lax.fori_loop(0, NSEG // UNR, steps, 0)

    if FFN_MODE == 1:
        for c_ in cp_ffn:
            c_.start()
    for j in range(3):
        finish_rows((NSEG - 1) * RIDE + 8 * j, abuf[8 * j:8 * j + 8, :])
    OUT0 = NSEG * RIDE
    cp_out = [cp(act.at[OOFF:OOFF + OUT0], out_hbm.at[0, 0:OUT0], 9)]
    cp_out[0].start()
    r0 = 0
    for ech in EPI_CHUNKS:
        o0 = NOSLOT * 32 + r0
        a = (jnp.dot(obuf1[o0:o0 + ech, :], wo_w(0, KS // DH, 0, 8), preferred_element_type=F32)
             + jnp.dot(obuf2[o0:o0 + ech, :], wo_w(KS // DH, H, 0, 8), preferred_element_type=F32))
        for j in range(ech // 8):
            finish_rows(OUT0 + r0 + 8 * j, a[8 * j:8 * j + 8])
        r0 += ech
    cp_out.append(cp(act.at[OOFF + OUT0:OOFF + S], out_hbm.at[0, OUT0:S], 10))
    cp_out[1].start()

    r_all = act[ROFF:ROFF + 8, 0:256].astype(F32)
    rows = lane256 * 8 + lax.broadcasted_iota(jnp.int32, (8, 256), 0)

    def allmax(v):
        return jnp.max(jnp.max(v, axis=1, keepdims=True), axis=0, keepdims=True)

    def allmin(v):
        return jnp.min(jnp.min(v, axis=1, keepdims=True), axis=0, keepdims=True)
    rowsf = rows.astype(F32)
    i1v = allmin(jnp.where(r_all == allmax(r_all), rowsf, float(S)))
    r_rest = jnp.where(rowsf == i1v, -jnp.inf, r_all)
    i2v = allmin(jnp.where((r_rest == allmax(r_rest)) & (rowsf != i1v), rowsf, float(S)))
    i1 = jnp.clip(i1v[0, 0].astype(jnp.int32), 0, S - 1)
    i2 = jnp.clip(i2v[0, 0].astype(jnp.int32), 0, S - 1)
    b1 = pl.multiple_of((i1 // 8) * 8, 8)
    b2 = pl.multiple_of((i2 // 8) * 8, 8)

    x1 = jnp.concatenate([act[pl.ds(b1, 8), :].astype(F32), act[pl.ds(b2, 8), :].astype(F32)],
                         axis=0)

    def two(i):
        return jnp.concatenate([modb[i], modb[i]], axis=0)
    h2 = _rb(_rb(_layernorm(x1) * two(4)) + two(3))
    rr = _rb(jnp.sum(h2 * two(6), axis=-1, keepdims=True))
    h2b = h2.astype(BF)
    for c_ in cp_ffn:
        c_.wait()
    gt = _rb(jnp.dot(h2b, pltpu.bitcast(wg_v[...], BF), preferred_element_type=F32))
    up = _rb(jnp.dot(h2b, pltpu.bitcast(wu_v[...], BF), preferred_element_type=F32))
    hid = (_rb(gt * _rb(jax.nn.sigmoid(gt))) * up).astype(BF)
    y = _rb(jnp.dot(hid, pltpu.bitcast(wd_v[...], BF), preferred_element_type=F32))
    y = _rb(y * _rb(jax.nn.sigmoid(rr)))
    sub = lax.broadcasted_iota(jnp.int32, (16, 1), 0)
    grow = jnp.where(sub < 8, b1 + sub, b2 + sub - 8)
    sel = (grow == i1) | (grow == i2)
    res = (x1 + _rb(two(5) * _rb(h2 + jnp.where(sel, y, 0.0)))).astype(BF)
    for c_ in cp_out:
        c_.wait()
    act[pl.ds(OOFF + b1, 8), :] = res[0:8]
    act[pl.ds(OOFF + b2, 8), :] = res[8:16]
    fix1 = cp(act.at[pl.ds(OOFF + b1, 8)], out_hbm.at[0, pl.ds(b1, 8)], 11)
    fix2 = cp(act.at[pl.ds(OOFF + b2, 8)], out_hbm.at[0, pl.ds(b2, 8)], 12)
    fix1.start()

    @pl.when(b1 != b2)
    def _():
        fix2.start()
        fix2.wait()
    fix1.wait()


@jax.jit
def pallas_adaLN_cond__memory_aug_recurrent_mem_tr__moe_arch_mod__prompt_kernel(
    A_x: jax.Array,
    A_mem0: jax.Array,
    A_Wq: jax.Array,
    A_Wk: jax.Array,
    A_Wv: jax.Array,
    A_Wo: jax.Array,
    A_seg_len,
    B_x: jax.Array,
    B_w_r: jax.Array,
    B_w_gate: jax.Array,
    B_w_up: jax.Array,
    B_w_down: jax.Array,
    c: jax.Array,
    w_mod: jax.Array,
):
    del B_x
    del A_seg_len
    assert A_x.shape == (1, S, D) and A_Wq.shape == (D, H, DH) and A_mem0.shape == (1, M, D)
    any_spec = pl.BlockSpec(memory_space=pl.ANY)
    scratch = [
        pltpu.VMEM((S if not XACT else 8, D), BF),
        pltpu.VMEM((XOFF + S * XACT, D), BF),
        pltpu.VMEM((PRE, D), BF),
        pltpu.VMEM((RIDE, D), F32),
        pltpu.VMEM((32, 768), F32),
        pltpu.SMEM((NSEG * NTAB,), jnp.int32),
        pltpu.VMEM((7, 8, D), F32),
        pltpu.VMEM((4, 1, D), BF),
        pltpu.VMEM((3 * H, D // 2, 128), U32),
        pltpu.VMEM((H, DH // 2, D), U32),
        pltpu.VMEM((D // 2, 6 * D), U32),
        pltpu.VMEM((D // 2, F), U32),
        pltpu.VMEM((D // 2, F), U32),
        pltpu.VMEM((F // 2, D), U32),
        pltpu.VMEM((NOSLOT * 32 + PRE, KS), BF),
        pltpu.VMEM((NOSLOT * 32 + PRE, H * DH - KS), BF),
        pltpu.SemaphoreType.DMA((17,)),
        pltpu.SemaphoreType.DMA((12,)),
    ] + [pltpu.VMEM((NSLOT, 512, 128), BF) for _ in range(NB)]
    wq, wk, wv = (w.reshape(D // 2, 2, H, DH) for w in (A_Wq, A_Wk, A_Wv))
    return pl.pallas_call(
        _kernel,
        out_shape=jax.ShapeDtypeStruct((1, S, D), BF),
        in_specs=[any_spec] * 12,
        out_specs=any_spec,
        scratch_shapes=scratch,
        compiler_params=pltpu.CompilerParams(vmem_limit_bytes=120 * 1024 * 1024),
    )(A_x, A_mem0, wq, wk, wv, A_Wo, B_w_r.reshape(1, D), B_w_gate, B_w_up, B_w_down,
      c, w_mod)
```

```python
import contextlib
import os
import jax
import jax.numpy as jnp
from jax import lax
import jax.experimental.pallas as pl
import jax.experimental.pallas.tpu as pltpu

BF = jnp.bfloat16
F32 = jnp.float32
U32 = jnp.uint32

S = 2048
D = 1024
H = 32
DH = 128
M = 8
SEG = 32
NSEG = S // SEG
F = 3584
NP = H // 2
RIDE = 24
PRE = S - NSEG * RIDE
NSLOT = 17
NOSLOT = 17
NB = int(os.environ.get('NB', 8))
KS = int(os.environ.get('KS', 2560))
LAG_S = 1
LAG_P = 3
EPS = 1e-5
SCALE = DH ** -0.5
OOFF = S
HOFF = 2 * S
ROFF = HOFF + 64
XOFF = ROFF + 16
PRE_SPLIT = 3
E_AT = tuple(int(v) for v in os.environ.get('E_AT', '2,3,4').split(','))
L_AT = tuple(int(v) for v in os.environ.get('L_AT', '8,10,12').split(','))
E_AT2 = tuple(int(v) for v in os.environ.get('E_AT2', '2,3,4').split(','))
L_AT2 = tuple(int(v) for v in os.environ.get('L_AT2', '8,10,12').split(','))


def _att_schedule(mode):
    att = {}
    if mode == 'lag':
        for p in range(NP):
            att.setdefault(p + LAG_S, []).append(('s', p))
        for p in range(NP):
            att.setdefault(p + LAG_P, []).append(('p', p))
    elif mode == 'q2':
        for p in range(0, NP, 2):
            att.setdefault(p + 2, []).extend([('s', p), ('s', p + 1)])
        for p in range(0, NP, 2):
            att.setdefault(p + 4, []).extend([('p', p), ('p', p + 1)])
    elif mode == 'q2b':
        for p in range(0, NP, 2):
            att.setdefault(p + 4, []).extend([('p', p), ('p', p + 1)])
        for p in range(0, NP, 2):
            att.setdefault(p + 2, []).extend([('s', p), ('s', p + 1)])
    elif mode == 'q2c':
        att[4] = [('s', i) for i in range(4)]
        for p in range(4, NP, 2):
            att[p + 2] = [('s', p), ('s', p + 1), ('p', p - 4), ('p', p - 3)]
        att[18] = [('p', i) for i in range(12, 16)]
    elif mode == 'q2d':
        att[3] = [('s', i) for i in range(3)]
        att[4] = [('s', 3)]
        att[3] = []
        att[4] = [('s', i) for i in range(4)]
        for p in range(4, NP, 2):
            att[p + 2] = [('p', p - 4), ('p', p - 3), ('s', p), ('s', p + 1)]
        att[18] = [('p', i) for i in range(12, 16)]
    elif mode == 'q4':
        for p in range(0, NP, 4):
            att.setdefault(p + 4, []).extend([('s', p + i) for i in range(4)])
            att.setdefault(p + 6, []).extend([('p', p + i) for i in range(4)])
    elif mode == 'q4b':
        for p in range(0, NP, 4):
            att.setdefault(min(p + 8, 18), []).extend([('p', p + i) for i in range(4)])
        for p in range(0, NP, 4):
            att.setdefault(p + 4, []).extend([('s', p + i) for i in range(4)])
    return att


ATT = _att_schedule(os.environ.get('ATT', 'q2c'))
XACT = int(os.environ.get('XACT', 0))
LD32 = int(os.environ.get('LD32', 1))
UNR = int(os.environ.get('UNR', 2))
EPI_CHUNKS = (128, 128, 128, 96, 32)


NTAB = 16


def _step_indices(s):
    t = [s % NSLOT]
    for j in range(3):
        gi = PRE // 8 + 3 * s + j
        t += [(gi // 4) % NSLOT, (gi % 4) * 8]
    for j in range(4):
        gi = 4 * s + j
        t.append(((gi // 3) % NOSLOT) * 32 + 8 + (gi % 3) * 8 if gi < 3 * NSEG
                 else NOSLOT * 32 + (gi - 3 * NSEG) * 8)
    t.append((s % NOSLOT) * 32)
    t.append(max(s - 1, 0) * RIDE)
    t.append(PRE + min(s + 1, NSEG - 1) * RIDE)
    return t


def _scope(name):
    return jax.named_scope(name) if os.environ.get('PROF') else contextlib.nullcontext()


def _rb(v):
    return v.astype(BF).astype(F32)


def _layernorm(x):
    mu = jnp.sum(x, axis=-1, keepdims=True) * (1.0 / D)
    xc = x - mu
    var = jnp.sum(xc * xc, axis=-1, keepdims=True) * (1.0 / D)
    sd = _rb(jnp.sqrt(_rb(_rb(var) + EPS)))
    return _rb(_rb(x - _rb(mu)) / sd)


def _kernel(x_hbm, mem0_hbm, wq_hbm, wk_hbm, wv_hbm, wo_hbm, wr_hbm, wg_hbm, wu_hbm,
            wd_hbm, c_hbm, wmod_hbm, out_hbm,
            xbuf, act, h0buf, abuf, ybuf, tab, modb, small,
            w_v, wo_v, wmod_v, wg_v, wu_v, wd_v,
            obuf1, obuf2, sems, wsems, ksems, *qkvbufs):
    qkv32 = tuple(b.bitcast(U32) for b in qkvbufs)
    if XACT:
        xbuf = act.at[pl.ds(XOFF, S)]
    w_hbms = tuple(w.bitcast(U32) for w in (wq_hbm, wk_hbm, wv_hbm))

    def cp(src, dst, i):
        return pltpu.make_async_copy(src, dst, sems.at[i])

    wmod_b = wmod_v.bitcast(BF)
    cp_c = cp(c_hbm, small.at[0], 0)
    cp_mem = cp(mem0_hbm.at[0], act.at[HOFF:HOFF + M], 1)
    cp_wr = cp(wr_hbm, small.at[1], 2)
    cp_x0 = [cp(x_hbm.at[0, n * 128:(n + 1) * 128], xbuf.at[n * 128:(n + 1) * 128], 13 + n)
             for n in range(PRE // 128)]
    cp_xr = cp(x_hbm.at[0, PRE:PRE + 32], xbuf.at[PRE:PRE + 32], 5)
    cp_x1 = cp(x_hbm.at[0, PRE + 32:S], xbuf.at[PRE + 32:S], 4)
    cp_wo = cp(wo_hbm, wo_v.bitcast(BF), 7)
    cp_ffn = [cp(wg_hbm, wg_v.bitcast(BF), 8), cp(wu_hbm, wu_v.bitcast(BF), 8),
              cp(wd_hbm, wd_v.bitcast(BF), 8)]

    def w_start(j):
        gg, t = j // 3, j % 3
        for i in range(NB):
            for par in range(2):
                pltpu.make_async_copy(w_hbms[t].at[:, par, gg * NB + i, :],
                                      w_v.at[(gg * NB + i) * 6 + t * 2 + par],
                                      wsems.at[2 * j + (i >= PRE_SPLIT)]).start()

    def mod_copy(j):
        return pltpu.make_async_copy(wmod_hbm.at[:, j * D:(j + 1) * D], wmod_b.at[j],
                                     wsems.at[2 * j + 1])

    def mult(v, m):
        return v if isinstance(v, int) else pl.multiple_of(v, m)

    def moda_copies(kc):
        col = mult(kc * 128, 128)
        return [pltpu.make_async_copy(wmod_hbm.at[:, pl.ds(v * D + col, 128)],
                                      wmod_b.at[v, :, pl.ds(col, 128)], ksems.at[8 + kc])
                for v in range(2)]

    def chunk_copies(kc):
        r0 = mult(kc * 64, 64)
        return [pltpu.make_async_copy(w_hbms[0].at[pl.ds(r0, 64), par, i, :],
                                      w_v.at[i * 6 + par, pl.ds(r0, 64), :], ksems.at[kc])
                for i in range(NB) for par in range(2)]

    cp_c.start()
    cp_mem.start()
    cp_wr.start()
    for c_ in (cp_x0 + moda_copies(0) + moda_copies(1) + chunk_copies(0) + moda_copies(2)
               + chunk_copies(1) + [cp_xr] + chunk_copies(2)):
        c_.start()

    def ln1_rows(src_row, dst_row):
        xv = xbuf[pl.ds(src_row, 8), :].astype(F32)
        hv = _rb(_layernorm(xv) * modb[1]) + modb[0]
        act[pl.ds(dst_row, 8), :] = hv.astype(BF)

    lane256 = lax.broadcasted_iota(jnp.int32, (8, 256), 1)

    def finish_rows(row, attn):
        xv = xbuf[pl.ds(row, 8), :].astype(F32)
        x1 = _rb(xv + _rb(modb[2] * _rb(attn)))
        h2 = _rb(_rb(_layernorm(x1) * modb[4]) + modb[3])
        act[pl.ds(row, 8), :] = x1.astype(BF)
        act[pl.ds(OOFF + row, 8), :] = (x1 + _rb(modb[5] * h2)).astype(BF)
        r = jnp.sum(h2 * modb[6], axis=-1, keepdims=True)
        act[ROFF:ROFF + 8, 0:256] = jnp.where(
            lane256 * 8 == row, r, act[ROFF:ROFF + 8, 0:256].astype(F32)).astype(BF)

    act[ROFF:ROFF + 8, 0:256] = jnp.zeros((8, 256), BF)
    abuf[...] = jnp.zeros(abuf.shape, F32)
    for s_ in range(NSEG):
        for k, v in enumerate(_step_indices(s_)):
            tab[s_ * NTAB + k] = v
    ri = lax.broadcasted_iota(jnp.int32, (80, 80), 0)
    ci = lax.broadcasted_iota(jnp.int32, (80, 80), 1)

    def head_pos(i):
        hd = jnp.where(i < 16, i // 8, (i - 16) // 32)
        pos = jnp.where(i < 16, i % 8, 8 + (i - 16) % 32)
        return hd, pos
    rh, rp = head_pos(ri)
    ch, cpos = head_pos(ci)
    same = rh == ch
    valid = same & ((rp < M) | (rp >= cpos))
    fill = jnp.where(same, -1e9, -jnp.inf).astype(F32)

    cp_mem.wait()
    cp_wr.wait()
    modb[6] = jnp.broadcast_to(small[1].astype(F32), (8, D))
    cp_c.wait()
    cv = small[0].astype(F32)
    sc16 = jnp.broadcast_to(_rb(cv * _rb(jax.nn.sigmoid(cv))), (16, D)).astype(BF)

    def ln_pre(g, carry):
        pltpu.make_async_copy(x_hbm.at[0, 0:128], xbuf.at[pl.ds(pl.multiple_of(g * 128, 128), 128)],
                              sems.at[13 + g]).wait()
        for u in range(2):
            row = pl.multiple_of(g * 128 + u * 64, 64)
            nv = _layernorm(xbuf[pl.ds(row, 64), :].astype(F32)).astype(BF)
            for k in range(8):
                h0buf[k, pl.ds(pl.multiple_of(row // 2, 32), 32), :] = pltpu.bitcast(
                    nv[:, k * 128:(k + 1) * 128], U32)
            wg_v[pl.ds(row, 64), 0:2 * D] = jnp.zeros((64, 2 * D), U32)
        return carry
    lax.fori_loop(0, PRE // 128, ln_pre, 0)

    def mod_tile(v, col):
        w = pltpu.bitcast(wmod_v[v, :, pl.ds(col, 128)], BF)
        return _rb(jnp.dot(sc16, w, preferred_element_type=F32))[0:8]

    def moda_store(kc, sa, ca):
        col = mult(kc * 128, 128)
        c1 = _rb(1.0 + ca)
        modb[0, :, pl.ds(col, 128)] = sa
        modb[1, :, pl.ds(col, 128)] = c1
        return sa, c1

    def moda_apply(kc, sa, c1, r0, r1):
        for r in range(r0, r1, 16):
            nv = pltpu.bitcast(h0buf[kc, r // 2:r // 2 + 8, :], BF).astype(F32).reshape(2, 8, 128)
            hv = (_rb(nv * c1[None]) + sa[None]).reshape(16, 128).astype(BF)
            h0buf[kc, r // 2:r // 2 + 8, :] = pltpu.bitcast(hv, U32)

    def repack(a, b):
        return (a & U32(0xFFFF)) | (b << 16), (a >> 16) | (b & U32(0xFFFF0000))

    def store_qkv(i, jrow, y, seg0):
        for sg in range(y.shape[0] // 32):
            for hh in range(2):
                qkvbufs[i][seg0 + sg, pl.ds(jrow + 16 + hh * 32, 32), :] = (
                    y[sg * 32:(sg + 1) * 32, hh * 128:(hh + 1) * 128].astype(BF))

    for c_ in moda_copies(0):
        c_.wait()
    moda_apply(0, *moda_store(0, mod_tile(0, 0), mod_tile(1, 0)), 0, PRE)

    def chunk_block(kc, last, issue):
        with _scope('w_chunk'):
            for c_ in chunk_copies(kc) + ([cp_xr] if last else moda_copies(kc + 1)):
                c_.wait()
        issue()
        r0 = mult(kc * 64, 64)
        mv = []
        for i in range(NB):
            lo, hi = repack(w_v[i * 6, pl.ds(r0, 64), :], w_v[i * 6 + 1, pl.ds(r0, 64), :])
            w_v[i * 6, pl.ds(r0, 64), :] = lo
            w_v[i * 6 + 1, pl.ds(r0, 64), :] = hi
            w = pltpu.bitcast(jnp.concatenate([lo, hi], axis=1), BF)
            y = (pltpu.bitcast(wg_v[0:PRE, i * 256:(i + 1) * 256], F32)
                 + jnp.dot(pltpu.bitcast(h0buf[kc], BF), w, preferred_element_type=F32))
            if last:
                store_qkv(i, 0, y, 0)
            else:
                wg_v[0:PRE, i * 256:(i + 1) * 256] = pltpu.bitcast(y, U32)
                if i in (1, 3):
                    mv.append(mod_tile(i // 2, mult((kc + 1) * 128, 128)))
                if i == 3:
                    mv = moda_store(kc + 1, mv[0], mv[1])
                if i >= 4:
                    moda_apply(kc + 1, mv[0], mv[1], (i - 4) * 128, (i - 3) * 128)
        if last:
            for j in range(3):
                ln1_rows(PRE + 8 * j, HOFF + 8 + 8 * j)

    def chunk_body_a(kc, carry):
        def issue():
            for c_ in moda_copies(kc + 3) + chunk_copies(kc + 3):
                c_.start()
        chunk_block(kc, False, issue)
        return carry

    def chunk_body_b(kc, carry):
        chunk_block(kc, False, lambda: None)
        return carry

    def issue_last():
        w_start(2)
        mod_copy(2).start()
    lax.fori_loop(0, 5, chunk_body_a, 0)
    w_start(1)
    lax.fori_loop(5, 7, chunk_body_b, 0)
    chunk_block(7, True, issue_last)

    def pre_unit(j, i, extra):
        blk = (j // 3) * (6 * NB) + (j % 3) * 2 + i * 6
        jrow = pl.multiple_of(j * 80, 16)
        lo, hi = repack(w_v[blk], w_v[blk + 1])
        w_v[blk] = lo
        w_v[blk + 1] = hi
        for rc in range(PRE // 128):
            if rc > 0:
                lo = w_v[blk]
                hi = w_v[blk + 1]
            w = pltpu.bitcast(jnp.concatenate([lo, hi], axis=1), BF)
            lhs = jnp.concatenate([h0buf[k, rc * 64:(rc + 1) * 64, :] for k in range(8)], axis=1)
            y = jnp.dot(pltpu.bitcast(lhs, BF), w, preferred_element_type=F32)
            store_qkv(i, jrow, y, rc * 4)
            extra(rc)

    def pre_body(j, carry):
        @pl.when(j == 1)
        def _():
            for jn in (3, 4):
                w_start(jn)
                mod_copy(jn).start()

        @pl.when(j == 2)
        def _():
            w_start(5)
            mod_copy(5).start()
            cp_wo.start()
            cp_x1.start()
        blk0 = (j // 3) * (6 * NB) + (j % 3) * 2
        one = jnp.where((j == 1) | (j == 4), 1.0, 0.0).astype(F32)
        for half, (i0, i1) in enumerate(((0, PRE_SPLIT), (PRE_SPLIT, NB))):
            with _scope('w_pre'):
                for i in range(i0, i1):
                    for par in range(2):
                        pltpu.make_async_copy(w_hbms[0].at[:, 0, 0, :],
                                              w_v.at[blk0 + i * 6 + par],
                                              wsems.at[2 * j + half]).wait()
            if half == 1:
                @pl.when(j > 1)
                def _():
                    pltpu.make_async_copy(wmod_hbm.at[:, 0:D], wmod_b.at[j],
                                          wsems.at[2 * j + 1]).wait()
            for i in range(i0, i1):
                def extra(rc, i=i):
                    n = (i - PRE_SPLIT) * 2 + rc // 2
                    if i >= PRE_SPLIT and rc % 2 == 0 and n < 8:
                        modb[j, :, n * 128:(n + 1) * 128] = _rb(one + mod_tile(j, n * 128))
                pre_unit(j, i, extra)
        return carry
    lax.fori_loop(1, 6, pre_body, 0)

    cp_wo.wait()
    cp_x1.wait()
    for c_ in cp_ffn:
        c_.start()

    def wo_w(h0, h1, n0, n1):
        w = wo_v[h0:h1, :, n0 * 128:n1 * 128].reshape((h1 - h0) * (DH // 2), (n1 - n0) * 128)
        return pltpu.bitcast(w, BF)

    HD = D // 2

    def emit_step(s, pend, last):
        hrow = pl.multiple_of(HOFF + (s & 1) * 32, 32)
        hnext = pl.multiple_of(HOFF + 32 - (s & 1) * 32, 32)
        tv = [tab[s * NTAB + k] for k in range(14)]
        slot = tv[0]
        dsts = [(tv[1 + 2 * j], pl.multiple_of(tv[2 + 2 * j], 8)) for j in range(3)]
        odst = [pl.multiple_of(tv[7 + j], 8) for j in range(4)]
        orow = pl.multiple_of(tv[11], 32)
        erow = tv[12]
        lrow = tv[13]
        e_at, l_at = (E_AT, L_AT) if pend is None else (E_AT2, L_AT2)
        probs = {}

        def wqkv(p, k0, k1):
            return pltpu.bitcast(jnp.concatenate(
                [w_v[p * 6 + u, k0 // 2:k1 // 2, :] for u in range(6)], axis=1), BF)

        lhs_lo = act[pl.ds(hrow, 32), 0:HD]
        if pend is not None:
            ybuf[...] = jnp.dot(lhs_lo, wqkv(0, 0, HD), preferred_element_type=F32)
            pend()
        lhs_hi = act[pl.ds(hrow, 32), HD:D]
        if pend is not None:
            y0 = ybuf[...] + jnp.dot(lhs_hi, wqkv(0, HD, D), preferred_element_type=F32)
        lhs_rest = jnp.concatenate([lhs_lo[:, 128:], lhs_hi], axis=1)
        lhs = [jnp.concatenate([lhs_lo, lhs_hi], axis=1)]

        def side(p):
            for j in range(3):
                if e_at[j] == p:
                    finish_rows(pl.multiple_of(erow + 8 * j, 8), abuf[8 * j:8 * j + 8, :])
            for j in range(3):
                if l_at[j] == p:
                    ln1_rows(pl.multiple_of(lrow + 8 * j, 8),
                             pl.multiple_of(hnext + 8 + 8 * j, 8))
            if (p in e_at or p in l_at) and p < NP - 1:
                lhs[0] = jnp.concatenate([act[pl.ds(hrow, 32), 0:128], lhs_rest], axis=1)

        def qkv(p):
            if p == 0 and pend is not None:
                y = y0
            else:
                y = jnp.dot(lhs[0], wqkv(p, 0, D), preferred_element_type=F32)
            buf = qkvbufs[p % NB]
            for u in range(6):
                t, hh = u // 2, u % 2
                b0 = ((p // NB) * 3 + t) * 80
                yu = y[:, u * 128:(u + 1) * 128]
                buf[slot, b0 + hh * 8:b0 + hh * 8 + 8, :] = yu[0:8].astype(BF)
                for j in range(3):
                    sl, off = dsts[j]
                    buf[sl, pl.ds(b0 + 16 + hh * 32 + off, 8), :] = (
                        yu[8 + 8 * j:16 + 8 * j].astype(BF))

        def ld(p, t):
            b0 = ((p // NB) * 3 + t) * 40
            if not LD32:
                return qkvbufs[p % NB][slot, 2 * b0:2 * b0 + 80, :]
            return pltpu.bitcast(qkv32[p % NB][slot, b0:b0 + 40, :], BF)

        def sc(p):
            s2 = lax.dot_general(ld(p, 0), ld(p, 1), (((1,), (1,)), ((), ())),
                                 preferred_element_type=F32) * SCALE
            s2 = jnp.where(valid, s2, fill)
            m = jnp.max(s2, axis=-1, keepdims=True)
            e = jnp.exp(s2 - m)
            l = jnp.sum(e, axis=-1, keepdims=True)
            rl = pl.reciprocal(l, approx=True)
            rl = rl * (2.0 - l * rl)
            probs[p] = (e * rl).astype(BF)

        def pv(p):
            o2 = jnp.dot(probs[p], ld(p, 2), preferred_element_type=F32)
            for hh in range(2):
                hcol = (2 * p + hh) * 128
                ob = obuf1
                if hcol >= KS:
                    ob = obuf2
                    hcol -= KS
                ob[pl.ds(orow, 8), hcol:hcol + 128] = o2[8 * hh:8 * hh + 8].astype(BF)
                for j in range(4):
                    r0 = 16 + 32 * hh + 8 * j
                    ob[pl.ds(odst[j], 8), hcol:hcol + 128] = o2[r0:r0 + 8].astype(BF)

        def attn(pos):
            for kind, p in ATT.get(pos, ()):
                (sc if kind == 's' else pv)(p)

        for p in range(NP):
            qkv(p)
            side(p)
            attn(p)
        a1 = []
        for i in range(4):
            a1.append(jnp.dot(obuf1[pl.ds(orow, 32), :], wo_w(0, KS // DH, 2 * i, 2 * i + 2),
                              preferred_element_type=F32))
            attn(NP + i)
            side(NP + i)
        o2lhs = obuf2[pl.ds(orow, 32), :]
        a_lo = jnp.concatenate(a1[0:2], axis=1) + jnp.dot(
            o2lhs, wo_w(KS // DH, H, 0, 4), preferred_element_type=F32)
        act[pl.ds(hnext, 8), 0:HD] = a_lo[0:8].astype(BF)
        abuf[:, 0:HD] = a_lo[8:32]
        a_hi = jnp.concatenate(a1[2:4], axis=1) + jnp.dot(
            o2lhs, wo_w(KS // DH, H, 4, 8), preferred_element_type=F32)

        def finish():
            act[pl.ds(hnext, 8), HD:D] = a_hi[0:8].astype(BF)
            abuf[:, HD:D] = a_hi[8:32]
        if last:
            finish()
        return finish

    def steps(it, carry):
        pend = None
        for u in range(UNR):
            pend = emit_step(it * UNR + u, pend, u == UNR - 1)
        return carry
    lax.fori_loop(0, NSEG // UNR, steps, 0)

    for j in range(3):
        finish_rows((NSEG - 1) * RIDE + 8 * j, abuf[8 * j:8 * j + 8, :])
    OUT0 = NSEG * RIDE
    cp_out = [cp(act.at[OOFF:OOFF + OUT0], out_hbm.at[0, 0:OUT0], 9)]
    cp_out[0].start()
    r0 = 0
    for ech in EPI_CHUNKS:
        o0 = NOSLOT * 32 + r0
        a = (jnp.dot(obuf1[o0:o0 + ech, :], wo_w(0, KS // DH, 0, 8), preferred_element_type=F32)
             + jnp.dot(obuf2[o0:o0 + ech, :], wo_w(KS // DH, H, 0, 8), preferred_element_type=F32))
        for j in range(ech // 8):
            finish_rows(OUT0 + r0 + 8 * j, a[8 * j:8 * j + 8])
        r0 += ech
    cp_out.append(cp(act.at[OOFF + OUT0:OOFF + S], out_hbm.at[0, OUT0:S], 10))
    cp_out[1].start()

    r_all = act[ROFF:ROFF + 8, 0:256].astype(F32)
    rows = lane256 * 8 + lax.broadcasted_iota(jnp.int32, (8, 256), 0)

    def allmax(v):
        return jnp.max(jnp.max(v, axis=1, keepdims=True), axis=0, keepdims=True)

    def allmin(v):
        return jnp.min(jnp.min(v, axis=1, keepdims=True), axis=0, keepdims=True)
    rowsf = rows.astype(F32)
    i1v = allmin(jnp.where(r_all == allmax(r_all), rowsf, float(S)))
    r_rest = jnp.where(rowsf == i1v, -jnp.inf, r_all)
    i2v = allmin(jnp.where((r_rest == allmax(r_rest)) & (rowsf != i1v), rowsf, float(S)))
    i1 = jnp.clip(i1v[0, 0].astype(jnp.int32), 0, S - 1)
    i2 = jnp.clip(i2v[0, 0].astype(jnp.int32), 0, S - 1)
    b1 = pl.multiple_of((i1 // 8) * 8, 8)
    b2 = pl.multiple_of((i2 // 8) * 8, 8)

    x1 = jnp.concatenate([act[pl.ds(b1, 8), :].astype(F32), act[pl.ds(b2, 8), :].astype(F32)],
                         axis=0)

    def two(i):
        return jnp.concatenate([modb[i], modb[i]], axis=0)
    h2 = _rb(_rb(_layernorm(x1) * two(4)) + two(3))
    rr = _rb(jnp.sum(h2 * two(6), axis=-1, keepdims=True))
    h2b = h2.astype(BF)
    for c_ in cp_ffn:
        c_.wait()
    gt = _rb(jnp.dot(h2b, pltpu.bitcast(wg_v[...], BF), preferred_element_type=F32))
    up = _rb(jnp.dot(h2b, pltpu.bitcast(wu_v[...], BF), preferred_element_type=F32))
    hid = (_rb(gt * _rb(jax.nn.sigmoid(gt))) * up).astype(BF)
    y = _rb(jnp.dot(hid, pltpu.bitcast(wd_v[...], BF), preferred_element_type=F32))
    y = _rb(y * _rb(jax.nn.sigmoid(rr)))
    sub = lax.broadcasted_iota(jnp.int32, (16, 1), 0)
    grow = jnp.where(sub < 8, b1 + sub, b2 + sub - 8)
    sel = (grow == i1) | (grow == i2)
    res = (x1 + _rb(two(5) * _rb(h2 + jnp.where(sel, y, 0.0)))).astype(BF)
    for c_ in cp_out:
        c_.wait()
    act[pl.ds(OOFF + b1, 8), :] = res[0:8]
    act[pl.ds(OOFF + b2, 8), :] = res[8:16]
    fix1 = cp(act.at[pl.ds(OOFF + b1, 8)], out_hbm.at[0, pl.ds(b1, 8)], 11)
    fix2 = cp(act.at[pl.ds(OOFF + b2, 8)], out_hbm.at[0, pl.ds(b2, 8)], 12)
    fix1.start()

    @pl.when(b1 != b2)
    def _():
        fix2.start()
        fix2.wait()
    fix1.wait()


@jax.jit
def pallas_adaLN_cond__memory_aug_recurrent_mem_tr__moe_arch_mod__prompt_kernel(
    A_x: jax.Array,
    A_mem0: jax.Array,
    A_Wq: jax.Array,
    A_Wk: jax.Array,
    A_Wv: jax.Array,
    A_Wo: jax.Array,
    A_seg_len,
    B_x: jax.Array,
    B_w_r: jax.Array,
    B_w_gate: jax.Array,
    B_w_up: jax.Array,
    B_w_down: jax.Array,
    c: jax.Array,
    w_mod: jax.Array,
):
    del B_x
    del A_seg_len
    assert A_x.shape == (1, S, D) and A_Wq.shape == (D, H, DH) and A_mem0.shape == (1, M, D)
    any_spec = pl.BlockSpec(memory_space=pl.ANY)
    scratch = [
        pltpu.VMEM((S if not XACT else 8, D), BF),
        pltpu.VMEM((XOFF + S * XACT, D), BF),
        pltpu.VMEM((8, PRE // 2, 128), U32),
        pltpu.VMEM((RIDE, D), F32),
        pltpu.VMEM((32, 768), F32),
        pltpu.SMEM((NSEG * NTAB,), jnp.int32),
        pltpu.VMEM((7, 8, D), F32),
        pltpu.VMEM((4, 1, D), BF),
        pltpu.VMEM((3 * H, D // 2, 128), U32),
        pltpu.VMEM((H, DH // 2, D), U32),
        pltpu.VMEM((6, D // 2, D), U32),
        pltpu.VMEM((D // 2, F), U32),
        pltpu.VMEM((D // 2, F), U32),
        pltpu.VMEM((F // 2, D), U32),
        pltpu.VMEM((NOSLOT * 32 + PRE, KS), BF),
        pltpu.VMEM((NOSLOT * 32 + PRE, H * DH - KS), BF),
        pltpu.SemaphoreType.DMA((17,)),
        pltpu.SemaphoreType.DMA((12,)),
        pltpu.SemaphoreType.DMA((16,)),
    ] + [pltpu.VMEM((NSLOT, 512, 128), BF) for _ in range(NB)]
    wq, wk, wv = (w.reshape(D // 2, 2, H, DH) for w in (A_Wq, A_Wk, A_Wv))
    return pl.pallas_call(
        _kernel,
        out_shape=jax.ShapeDtypeStruct((1, S, D), BF),
        in_specs=[any_spec] * 12,
        out_specs=any_spec,
        scratch_shapes=scratch,
        compiler_params=pltpu.CompilerParams(vmem_limit_bytes=120 * 1024 * 1024,
                                             disable_bounds_checks=True),
    )(A_x, A_mem0, wq, wk, wv, A_Wo, B_w_r.reshape(1, D), B_w_gate, B_w_up, B_w_down,
      c, w_mod)
```

```python
import contextlib
import os
import jax
import jax.numpy as jnp
from jax import lax
import jax.experimental.pallas as pl
import jax.experimental.pallas.tpu as pltpu

BF = jnp.bfloat16
F32 = jnp.float32
U32 = jnp.uint32

S = 2048
D = 1024
H = 32
DH = 128
M = 8
SEG = 32
NSEG = S // SEG
F = 3584
NP = H // 2
RIDE = 24
PRE = S - NSEG * RIDE
NSLOT = 17
NOSLOT = 17
NB = int(os.environ.get('NB', 8))
KS = int(os.environ.get('KS', 2560))
LAG_S = 1
LAG_P = 3
EPS = 1e-5
SCALE = DH ** -0.5
OOFF = S
HOFF = 2 * S
ROFF = HOFF + 64
ZOFF = ROFF + 16
XOFF = ZOFF + 16
PRE_SPLIT = 3
E_AT = tuple(int(v) for v in os.environ.get('E_AT', '2,3,4').split(','))
L_AT = tuple(int(v) for v in os.environ.get('L_AT', '8,10,12').split(','))
E_AT2 = tuple(int(v) for v in os.environ.get('E_AT2', '2,3,4').split(','))
L_AT2 = tuple(int(v) for v in os.environ.get('L_AT2', '8,10,12').split(','))


def _att_schedule(mode):
    att = {}
    if mode == 'lag':
        for p in range(NP):
            att.setdefault(p + LAG_S, []).append(('s', p))
        for p in range(NP):
            att.setdefault(p + LAG_P, []).append(('p', p))
    elif mode == 'q2':
        for p in range(0, NP, 2):
            att.setdefault(p + 2, []).extend([('s', p), ('s', p + 1)])
        for p in range(0, NP, 2):
            att.setdefault(p + 4, []).extend([('p', p), ('p', p + 1)])
    elif mode == 'q2b':
        for p in range(0, NP, 2):
            att.setdefault(p + 4, []).extend([('p', p), ('p', p + 1)])
        for p in range(0, NP, 2):
            att.setdefault(p + 2, []).extend([('s', p), ('s', p + 1)])
    elif mode == 'q2c':
        att[4] = [('s', i) for i in range(4)]
        for p in range(4, NP, 2):
            att[p + 2] = [('s', p), ('s', p + 1), ('p', p - 4), ('p', p - 3)]
        att[18] = [('p', i) for i in range(12, 16)]
    elif mode == 'q2d':
        att[3] = [('s', i) for i in range(3)]
        att[4] = [('s', 3)]
        att[3] = []
        att[4] = [('s', i) for i in range(4)]
        for p in range(4, NP, 2):
            att[p + 2] = [('p', p - 4), ('p', p - 3), ('s', p), ('s', p + 1)]
        att[18] = [('p', i) for i in range(12, 16)]
    elif mode == 'q4':
        for p in range(0, NP, 4):
            att.setdefault(p + 4, []).extend([('s', p + i) for i in range(4)])
            att.setdefault(p + 6, []).extend([('p', p + i) for i in range(4)])
    elif mode == 'q4b':
        for p in range(0, NP, 4):
            att.setdefault(min(p + 8, 18), []).extend([('p', p + i) for i in range(4)])
        for p in range(0, NP, 4):
            att.setdefault(p + 4, []).extend([('s', p + i) for i in range(4)])
    return att


ATT = _att_schedule(os.environ.get('ATT', 'q2c'))
XACT = int(os.environ.get('XACT', 0))
LD32 = int(os.environ.get('LD32', 1))
K2 = H * DH - KS
OPAD = int(os.environ.get('OPAD', 1))
OW1 = -(-KS // 1024) * 1024 if OPAD else KS
OW2 = -(-K2 // 1024) * 1024 if OPAD else K2
UNR = int(os.environ.get('UNR', 2))
EPI_CHUNKS = tuple(int(v) for v in os.environ.get('EPI', '64,64,64,64,64,64,48,48,32').split(','))
EMAX = max(EPI_CHUNKS)
EPI_PIN = int(os.environ.get('EPI_PIN', 0))
EPI_SPARE = int(os.environ.get('EPI_SPARE', 0))
EPI_NSUB = int(os.environ.get('EPI_NSUB', 8))


NTAB = 16


def _step_indices(s):
    t = [s % NSLOT]
    for j in range(3):
        gi = PRE // 8 + 3 * s + j
        t += [(gi // 4) % NSLOT, (gi % 4) * 8]
    for j in range(4):
        gi = 4 * s + j
        t.append(((gi // 3) % NOSLOT) * 32 + 8 + (gi % 3) * 8 if gi < 3 * NSEG
                 else NOSLOT * 32 + (gi - 3 * NSEG) * 8)
    t.append((s % NOSLOT) * 32)
    t.append(max(s - 1, 0) * RIDE)
    t.append(PRE + min(s + 1, NSEG - 1) * RIDE)
    return t


def _scope(name):
    return jax.named_scope(name) if os.environ.get('PROF') else contextlib.nullcontext()


def _rb(v):
    return v.astype(BF).astype(F32)


def _layernorm(x):
    mu = jnp.sum(x, axis=-1, keepdims=True) * (1.0 / D)
    xc = x - mu
    var = jnp.sum(xc * xc, axis=-1, keepdims=True) * (1.0 / D)
    sd = _rb(jnp.sqrt(_rb(_rb(var) + EPS)))
    return _rb(_rb(x - _rb(mu)) / sd)


def _kernel(x_hbm, mem0_hbm, wq_hbm, wk_hbm, wv_hbm, wo_hbm, wr_hbm, wg_hbm, wu_hbm,
            wd_hbm, c_hbm, wmod_hbm, out_hbm,
            xbuf, act, h0buf, abuf, ybuf, ebuf, tab, modb, small,
            w_v, wo_v, wmod_v, wg_v, wu_v, wd_v,
            obuf1, obuf2, sems, wsems, ksems, *qkvbufs):
    qkv32 = tuple(b.bitcast(U32) for b in qkvbufs)
    if XACT:
        xbuf = act.at[pl.ds(XOFF, S)]
    w_hbms = tuple(w.bitcast(U32) for w in (wq_hbm, wk_hbm, wv_hbm))

    def cp(src, dst, i):
        return pltpu.make_async_copy(src, dst, sems.at[i])

    wmod_b = wmod_v.bitcast(BF)
    cp_c = cp(c_hbm, small.at[0], 0)
    cp_mem = cp(mem0_hbm.at[0], act.at[HOFF:HOFF + M], 1)
    cp_wr = cp(wr_hbm, small.at[1], 2)
    cp_x0 = [cp(x_hbm.at[0, n * 128:(n + 1) * 128], xbuf.at[n * 128:(n + 1) * 128], 13 + n)
             for n in range(PRE // 128)]
    cp_xr = cp(x_hbm.at[0, PRE:PRE + 32], xbuf.at[PRE:PRE + 32], 5)
    cp_x1 = cp(x_hbm.at[0, PRE + 32:S], xbuf.at[PRE + 32:S], 4)
    cp_wo = cp(wo_hbm, wo_v.bitcast(BF), 7)
    cp_ffn = [cp(wg_hbm, wg_v.bitcast(BF), 8), cp(wu_hbm, wu_v.bitcast(BF), 8),
              cp(wd_hbm, wd_v.bitcast(BF), 8)]

    def w_start(j):
        gg, t = j // 3, j % 3
        for i in range(NB):
            for par in range(2):
                pltpu.make_async_copy(w_hbms[t].at[:, par, gg * NB + i, :],
                                      w_v.at[(gg * NB + i) * 6 + t * 2 + par],
                                      wsems.at[2 * j + (i >= PRE_SPLIT)]).start()

    def mod_copy(j):
        return pltpu.make_async_copy(wmod_hbm.at[:, j * D:(j + 1) * D], wmod_b.at[j],
                                     wsems.at[2 * j + 1])

    def mult(v, m):
        return v if isinstance(v, int) else pl.multiple_of(v, m)

    def moda_copies(kc):
        col = mult(kc * 128, 128)
        return [pltpu.make_async_copy(wmod_hbm.at[:, pl.ds(v * D + col, 128)],
                                      wmod_b.at[v, :, pl.ds(col, 128)], ksems.at[8 + kc])
                for v in range(2)]

    def chunk_copies(kc):
        r0 = mult(kc * 64, 64)
        return [pltpu.make_async_copy(w_hbms[0].at[pl.ds(r0, 64), par, i, :],
                                      w_v.at[i * 6 + par, pl.ds(r0, 64), :], ksems.at[kc])
                for i in range(NB) for par in range(2)]

    cp_c.start()
    cp_mem.start()
    cp_wr.start()
    for c_ in (cp_x0 + moda_copies(0) + moda_copies(1) + chunk_copies(0) + moda_copies(2)
               + chunk_copies(1) + [cp_xr] + chunk_copies(2)):
        c_.start()

    def ln1_rows(src_row, dst_row):
        xv = xbuf[pl.ds(src_row, 8), :].astype(F32)
        hv = _rb(_layernorm(xv) * modb[1]) + modb[0]
        act[pl.ds(dst_row, 8), :] = hv.astype(BF)

    lane256 = lax.broadcasted_iota(jnp.int32, (8, 256), 1)

    def finish_rows(row, attn):
        xv = xbuf[pl.ds(row, 8), :].astype(F32)
        x1 = _rb(xv + _rb(modb[2] * _rb(attn)))
        h2 = _rb(_rb(_layernorm(x1) * modb[4]) + modb[3])
        act[pl.ds(row, 8), :] = x1.astype(BF)
        act[pl.ds(OOFF + row, 8), :] = (x1 + _rb(modb[5] * h2)).astype(BF)
        r = jnp.sum(h2 * modb[6], axis=-1, keepdims=True)
        act[ROFF:ROFF + 8, 0:256] = jnp.where(
            lane256 * 8 == row, r, act[ROFF:ROFF + 8, 0:256].astype(F32)).astype(BF)

    act[ROFF:ROFF + 8, 0:256] = jnp.zeros((8, 256), BF)
    act[ZOFF:ZOFF + 16, 0:128] = jnp.zeros((16, 128), BF)
    tab[14] = ZOFF
    tab[15] = 0
    abuf[...] = jnp.zeros(abuf.shape, F32)
    for s_ in range(NSEG):
        for k, v in enumerate(_step_indices(s_)):
            tab[s_ * NTAB + k] = v
    ri = lax.broadcasted_iota(jnp.int32, (80, 80), 0)
    ci = lax.broadcasted_iota(jnp.int32, (80, 80), 1)

    def head_pos(i):
        hd = jnp.where(i < 16, i // 8, (i - 16) // 32)
        pos = jnp.where(i < 16, i % 8, 8 + (i - 16) % 32)
        return hd, pos
    rh, rp = head_pos(ri)
    ch, cpos = head_pos(ci)
    same = rh == ch
    valid = same & ((rp < M) | (rp >= cpos))
    fill = jnp.where(same, -1e9, -jnp.inf).astype(F32)

    cp_mem.wait()
    cp_wr.wait()
    modb[6] = jnp.broadcast_to(small[1].astype(F32), (8, D))
    cp_c.wait()
    cv = small[0].astype(F32)
    sc16 = jnp.broadcast_to(_rb(cv * _rb(jax.nn.sigmoid(cv))), (16, D)).astype(BF)

    def ln_pre(g, carry):
        pltpu.make_async_copy(x_hbm.at[0, 0:128], xbuf.at[pl.ds(pl.multiple_of(g * 128, 128), 128)],
                              sems.at[13 + g]).wait()
        for u in range(2):
            row = pl.multiple_of(g * 128 + u * 64, 64)
            nv = _layernorm(xbuf[pl.ds(row, 64), :].astype(F32)).astype(BF)
            for k in range(8):
                h0buf[k, pl.ds(pl.multiple_of(row // 2, 32), 32), :] = pltpu.bitcast(
                    nv[:, k * 128:(k + 1) * 128], U32)
            wg_v[pl.ds(row, 64), 0:2 * D] = jnp.zeros((64, 2 * D), U32)
        return carry
    lax.fori_loop(0, PRE // 128, ln_pre, 0)

    def mod_tile(v, col):
        w = pltpu.bitcast(wmod_v[v, :, pl.ds(col, 128)], BF)
        return _rb(jnp.dot(sc16, w, preferred_element_type=F32))[0:8]

    def moda_store(kc, sa, ca):
        col = mult(kc * 128, 128)
        c1 = _rb(1.0 + ca)
        modb[0, :, pl.ds(col, 128)] = sa
        modb[1, :, pl.ds(col, 128)] = c1
        return sa, c1

    def moda_apply(kc, sa, c1, r0, r1):
        for r in range(r0, r1, 16):
            nv = pltpu.bitcast(h0buf[kc, r // 2:r // 2 + 8, :], BF).astype(F32).reshape(2, 8, 128)
            hv = (_rb(nv * c1[None]) + sa[None]).reshape(16, 128).astype(BF)
            h0buf[kc, r // 2:r // 2 + 8, :] = pltpu.bitcast(hv, U32)

    def repack(a, b):
        return (a & U32(0xFFFF)) | (b << 16), (a >> 16) | (b & U32(0xFFFF0000))

    def store_qkv(i, jrow, y, seg0):
        for sg in range(y.shape[0] // 32):
            for hh in range(2):
                qkvbufs[i][seg0 + sg, pl.ds(jrow + 16 + hh * 32, 32), :] = (
                    y[sg * 32:(sg + 1) * 32, hh * 128:(hh + 1) * 128].astype(BF))

    for c_ in moda_copies(0):
        c_.wait()
    moda_apply(0, *moda_store(0, mod_tile(0, 0), mod_tile(1, 0)), 0, PRE)

    def chunk_block(kc, last, issue):
        with _scope('w_chunk'):
            for c_ in chunk_copies(kc) + ([cp_xr] if last else moda_copies(kc + 1)):
                c_.wait()
        issue()
        r0 = mult(kc * 64, 64)
        mv = []
        for i in range(NB):
            lo, hi = repack(w_v[i * 6, pl.ds(r0, 64), :], w_v[i * 6 + 1, pl.ds(r0, 64), :])
            w_v[i * 6, pl.ds(r0, 64), :] = lo
            w_v[i * 6 + 1, pl.ds(r0, 64), :] = hi
            w = pltpu.bitcast(jnp.concatenate([lo, hi], axis=1), BF)
            y = (pltpu.bitcast(wg_v[0:PRE, i * 256:(i + 1) * 256], F32)
                 + jnp.dot(pltpu.bitcast(h0buf[kc], BF), w, preferred_element_type=F32))
            if last:
                store_qkv(i, 0, y, 0)
            else:
                wg_v[0:PRE, i * 256:(i + 1) * 256] = pltpu.bitcast(y, U32)
                if i in (1, 3):
                    mv.append(mod_tile(i // 2, mult((kc + 1) * 128, 128)))
                if i == 3:
                    mv = moda_store(kc + 1, mv[0], mv[1])
                if i >= 4:
                    moda_apply(kc + 1, mv[0], mv[1], (i - 4) * 128, (i - 3) * 128)
        if last:
            for j in range(3):
                ln1_rows(PRE + 8 * j, HOFF + 8 + 8 * j)

    def chunk_body_a(kc, carry):
        def issue():
            for c_ in moda_copies(kc + 3) + chunk_copies(kc + 3):
                c_.start()
        chunk_block(kc, False, issue)
        return carry

    def chunk_body_b(kc, carry):
        chunk_block(kc, False, lambda: None)
        return carry

    def issue_last():
        w_start(2)
        mod_copy(2).start()
    lax.fori_loop(0, 5, chunk_body_a, 0)
    w_start(1)
    lax.fori_loop(5, 7, chunk_body_b, 0)
    chunk_block(7, True, issue_last)

    def pre_unit(j, i, extra):
        blk = (j // 3) * (6 * NB) + (j % 3) * 2 + i * 6
        jrow = pl.multiple_of(j * 80, 16)
        lo, hi = repack(w_v[blk], w_v[blk + 1])
        w_v[blk] = lo
        w_v[blk + 1] = hi
        for rc in range(PRE // 128):
            if rc > 0:
                lo = w_v[blk]
                hi = w_v[blk + 1]
            w = pltpu.bitcast(jnp.concatenate([lo, hi], axis=1), BF)
            lhs = jnp.concatenate([h0buf[k, rc * 64:(rc + 1) * 64, :] for k in range(8)], axis=1)
            y = jnp.dot(pltpu.bitcast(lhs, BF), w, preferred_element_type=F32)
            store_qkv(i, jrow, y, rc * 4)
            extra(rc)

    def pre_body(j, carry):
        @pl.when(j == 1)
        def _():
            for jn in (3, 4):
                w_start(jn)
                mod_copy(jn).start()

        @pl.when(j == 2)
        def _():
            w_start(5)
            mod_copy(5).start()
            cp_wo.start()
            cp_x1.start()
        blk0 = (j // 3) * (6 * NB) + (j % 3) * 2
        one = jnp.where((j == 1) | (j == 4), 1.0, 0.0).astype(F32)
        for half, (i0, i1) in enumerate(((0, PRE_SPLIT), (PRE_SPLIT, NB))):
            with _scope('w_pre'):
                for i in range(i0, i1):
                    for par in range(2):
                        pltpu.make_async_copy(w_hbms[0].at[:, 0, 0, :],
                                              w_v.at[blk0 + i * 6 + par],
                                              wsems.at[2 * j + half]).wait()
            if half == 1:
                @pl.when(j > 1)
                def _():
                    pltpu.make_async_copy(wmod_hbm.at[:, 0:D], wmod_b.at[j],
                                          wsems.at[2 * j + 1]).wait()
            for i in range(i0, i1):
                def extra(rc, i=i):
                    n = (i - PRE_SPLIT) * 2 + rc // 2
                    if i >= PRE_SPLIT and rc % 2 == 0 and n < 8:
                        modb[j, :, n * 128:(n + 1) * 128] = _rb(one + mod_tile(j, n * 128))
                pre_unit(j, i, extra)
        return carry
    lax.fori_loop(1, 6, pre_body, 0)

    cp_wo.wait()
    cp_x1.wait()
    for c_ in cp_ffn:
        c_.start()

    def wo_w(h0, h1, n0, n1):
        w = wo_v[h0:h1, :, n0 * 128:n1 * 128].reshape((h1 - h0) * (DH // 2), (n1 - n0) * 128)
        return pltpu.bitcast(w, BF)

    HD = D // 2

    def emit_step(s, pend, last):
        hrow = pl.multiple_of(HOFF + (s & 1) * 32, 32)
        hnext = pl.multiple_of(HOFF + 32 - (s & 1) * 32, 32)
        tv = [tab[s * NTAB + k] for k in range(14)]
        slot = tv[0]
        dsts = [(tv[1 + 2 * j], pl.multiple_of(tv[2 + 2 * j], 8)) for j in range(3)]
        odst = [pl.multiple_of(tv[7 + j], 8) for j in range(4)]
        orow = pl.multiple_of(tv[11], 32)
        erow = tv[12]
        lrow = tv[13]
        e_at, l_at = (E_AT, L_AT) if pend is None else (E_AT2, L_AT2)
        probs = {}

        def wqkv(p, k0, k1):
            return pltpu.bitcast(jnp.concatenate(
                [w_v[p * 6 + u, k0 // 2:k1 // 2, :] for u in range(6)], axis=1), BF)

        lhs_lo = act[pl.ds(hrow, 32), 0:HD]
        if pend is not None:
            ybuf[...] = jnp.dot(lhs_lo, wqkv(0, 0, HD), preferred_element_type=F32)
            pend()
        lhs_hi = act[pl.ds(hrow, 32), HD:D]
        if pend is not None:
            y0 = ybuf[...] + jnp.dot(lhs_hi, wqkv(0, HD, D), preferred_element_type=F32)
        lhs_rest = jnp.concatenate([lhs_lo[:, 128:], lhs_hi], axis=1)
        lhs = [jnp.concatenate([lhs_lo, lhs_hi], axis=1)]

        def side(p):
            for j in range(3):
                if e_at[j] == p:
                    finish_rows(pl.multiple_of(erow + 8 * j, 8), abuf[8 * j:8 * j + 8, :])
            for j in range(3):
                if l_at[j] == p:
                    ln1_rows(pl.multiple_of(lrow + 8 * j, 8),
                             pl.multiple_of(hnext + 8 + 8 * j, 8))
            if (p in e_at or p in l_at) and p < NP - 1:
                lhs[0] = jnp.concatenate([act[pl.ds(hrow, 32), 0:128], lhs_rest], axis=1)

        def qkv(p):
            if p == 0 and pend is not None:
                y = y0
            else:
                y = jnp.dot(lhs[0], wqkv(p, 0, D), preferred_element_type=F32)
            buf = qkvbufs[p % NB]
            for u in range(6):
                t, hh = u // 2, u % 2
                b0 = ((p // NB) * 3 + t) * 80
                yu = y[:, u * 128:(u + 1) * 128]
                buf[slot, b0 + hh * 8:b0 + hh * 8 + 8, :] = yu[0:8].astype(BF)
                for j in range(3):
                    sl, off = dsts[j]
                    buf[sl, pl.ds(b0 + 16 + hh * 32 + off, 8), :] = (
                        yu[8 + 8 * j:16 + 8 * j].astype(BF))

        def ld(p, t):
            b0 = ((p // NB) * 3 + t) * 40
            if not LD32:
                return qkvbufs[p % NB][slot, 2 * b0:2 * b0 + 80, :]
            return pltpu.bitcast(qkv32[p % NB][slot, b0:b0 + 40, :], BF)

        def sc(p):
            s2 = lax.dot_general(ld(p, 0), ld(p, 1), (((1,), (1,)), ((), ())),
                                 preferred_element_type=F32) * SCALE
            s2 = jnp.where(valid, s2, fill)
            m = jnp.max(s2, axis=-1, keepdims=True)
            e = jnp.exp(s2 - m)
            l = jnp.sum(e, axis=-1, keepdims=True)
            rl = pl.reciprocal(l, approx=True)
            rl = rl * (2.0 - l * rl)
            probs[p] = (e * rl).astype(BF)

        def pv(p):
            o2 = jnp.dot(probs[p], ld(p, 2), preferred_element_type=F32)
            for hh in range(2):
                hcol = (2 * p + hh) * 128
                ob = obuf1
                if hcol >= KS:
                    ob = obuf2
                    hcol -= KS
                ob[pl.ds(orow, 8), hcol:hcol + 128] = o2[8 * hh:8 * hh + 8].astype(BF)
                for j in range(4):
                    r0 = 16 + 32 * hh + 8 * j
                    ob[pl.ds(odst[j], 8), hcol:hcol + 128] = o2[r0:r0 + 8].astype(BF)

        def attn(pos):
            for kind, p in ATT.get(pos, ()):
                (sc if kind == 's' else pv)(p)

        for p in range(NP):
            qkv(p)
            side(p)
            attn(p)
        a1 = []
        for i in range(4):
            a1.append(jnp.dot(obuf1[pl.ds(orow, 32), 0:KS], wo_w(0, KS // DH, 2 * i, 2 * i + 2),
                              preferred_element_type=F32))
            attn(NP + i)
            side(NP + i)
        o2lhs = obuf2[pl.ds(orow, 32), 0:K2]
        a_lo = jnp.concatenate(a1[0:2], axis=1) + jnp.dot(
            o2lhs, wo_w(KS // DH, H, 0, 4), preferred_element_type=F32)
        act[pl.ds(hnext, 8), 0:HD] = a_lo[0:8].astype(BF)
        abuf[:, 0:HD] = a_lo[8:32]
        a_hi = jnp.concatenate(a1[2:4], axis=1) + jnp.dot(
            o2lhs, wo_w(KS // DH, H, 4, 8), preferred_element_type=F32)

        def finish():
            act[pl.ds(hnext, 8), HD:D] = a_hi[0:8].astype(BF)
            abuf[:, HD:D] = a_hi[8:32]
        if last:
            finish()
        return finish

    def steps(it, carry):
        pend = None
        for u in range(UNR):
            pend = emit_step(it * UNR + u, pend, u == UNR - 1)
        return carry
    lax.fori_loop(0, NSEG // UNR, steps, 0)

    OUT0 = (NSEG - 1) * RIDE
    cp_out = [cp(act.at[OOFF:OOFF + OUT0], out_hbm.at[0, 0:OUT0], 9)]
    cp_out[0].start()
    zrow = pl.multiple_of(tab[14], 16)
    zero = pl.multiple_of(tab[15], 8)
    ebuf[EMAX:EMAX + RIDE, :] = abuf[...]
    todo = [(OUT0 + 8 * j, EMAX + 8 * j) for j in range(3)]
    r0 = 0
    nw = 8 // EPI_NSUB
    for ci, ech in enumerate(EPI_CHUNKS):
        o0 = NOSLOT * 32 + r0
        e0 = (ci % 2) * EMAX
        per = -(-len(todo) // (EPI_NSUB - EPI_SPARE))
        for n in range(EPI_NSUB):
            first = obuf1[o0:o0 + 16, 0:128]
            if n == 0 and ci > 0 and EPI_PIN:
                first = pltpu.bitcast(
                    pltpu.bitcast(first, U32) | pltpu.bitcast(act[pl.ds(zrow, 16), 0:128], U32), BF)
            col0 = jnp.concatenate([first, obuf1[o0 + 16:o0 + ech, 0:128]], axis=0)
            lhs = jnp.concatenate(
                [col0, obuf1[o0:o0 + ech, 128:KS], obuf2[o0:o0 + ech, 0:K2]], axis=1)
            ebuf[e0:e0 + ech, n * nw * 128:(n + 1) * nw * 128] = jnp.dot(
                lhs, wo_w(0, H, n * nw, (n + 1) * nw), preferred_element_type=F32)
            for row, er in todo[:per]:
                finish_rows(row, ebuf[pl.ds(zero + er, 8), :])
            todo = todo[per:]
        todo = [(OUT0 + RIDE + r0 + 8 * j, e0 + 8 * j) for j in range(ech // 8)]
        r0 += ech
    for row, er in todo:
        finish_rows(row, ebuf[er:er + 8, :])
    cp_out.append(cp(act.at[OOFF + OUT0:OOFF + S], out_hbm.at[0, OUT0:S], 10))
    cp_out[1].start()

    r_all = act[ROFF:ROFF + 8, 0:256].astype(F32)
    rows = lane256 * 8 + lax.broadcasted_iota(jnp.int32, (8, 256), 0)

    def allmax(v):
        return jnp.max(jnp.max(v, axis=1, keepdims=True), axis=0, keepdims=True)

    def allmin(v):
        return jnp.min(jnp.min(v, axis=1, keepdims=True), axis=0, keepdims=True)
    rowsf = rows.astype(F32)
    i1v = allmin(jnp.where(r_all == allmax(r_all), rowsf, float(S)))
    r_rest = jnp.where(rowsf == i1v, -jnp.inf, r_all)
    i2v = allmin(jnp.where((r_rest == allmax(r_rest)) & (rowsf != i1v), rowsf, float(S)))
    i1 = jnp.clip(i1v[0, 0].astype(jnp.int32), 0, S - 1)
    i2 = jnp.clip(i2v[0, 0].astype(jnp.int32), 0, S - 1)
    b1 = pl.multiple_of((i1 // 8) * 8, 8)
    b2 = pl.multiple_of((i2 // 8) * 8, 8)

    x1 = jnp.concatenate([act[pl.ds(b1, 8), :].astype(F32), act[pl.ds(b2, 8), :].astype(F32)],
                         axis=0)

    def two(i):
        return jnp.concatenate([modb[i], modb[i]], axis=0)
    h2 = _rb(_rb(_layernorm(x1) * two(4)) + two(3))
    rr = _rb(jnp.sum(h2 * two(6), axis=-1, keepdims=True))
    h2b = h2.astype(BF)
    for c_ in cp_ffn:
        c_.wait()
    gt = _rb(jnp.dot(h2b, pltpu.bitcast(wg_v[...], BF), preferred_element_type=F32))
    up = _rb(jnp.dot(h2b, pltpu.bitcast(wu_v[...], BF), preferred_element_type=F32))
    hid = (_rb(gt * _rb(jax.nn.sigmoid(gt))) * up).astype(BF)
    y = _rb(jnp.dot(hid, pltpu.bitcast(wd_v[...], BF), preferred_element_type=F32))
    y = _rb(y * _rb(jax.nn.sigmoid(rr)))
    sub = lax.broadcasted_iota(jnp.int32, (16, 1), 0)
    grow = jnp.where(sub < 8, b1 + sub, b2 + sub - 8)
    sel = (grow == i1) | (grow == i2)
    res = (x1 + _rb(two(5) * _rb(h2 + jnp.where(sel, y, 0.0)))).astype(BF)
    for c_ in cp_out:
        c_.wait()
    act[pl.ds(OOFF + b1, 8), :] = res[0:8]
    act[pl.ds(OOFF + b2, 8), :] = res[8:16]
    fix1 = cp(act.at[pl.ds(OOFF + b1, 8)], out_hbm.at[0, pl.ds(b1, 8)], 11)
    fix2 = cp(act.at[pl.ds(OOFF + b2, 8)], out_hbm.at[0, pl.ds(b2, 8)], 12)
    fix1.start()

    @pl.when(b1 != b2)
    def _():
        fix2.start()
        fix2.wait()
    fix1.wait()


@jax.jit
def pallas_adaLN_cond__memory_aug_recurrent_mem_tr__moe_arch_mod__prompt_kernel(
    A_x: jax.Array,
    A_mem0: jax.Array,
    A_Wq: jax.Array,
    A_Wk: jax.Array,
    A_Wv: jax.Array,
    A_Wo: jax.Array,
    A_seg_len,
    B_x: jax.Array,
    B_w_r: jax.Array,
    B_w_gate: jax.Array,
    B_w_up: jax.Array,
    B_w_down: jax.Array,
    c: jax.Array,
    w_mod: jax.Array,
):
    del B_x
    del A_seg_len
    assert A_x.shape == (1, S, D) and A_Wq.shape == (D, H, DH) and A_mem0.shape == (1, M, D)
    any_spec = pl.BlockSpec(memory_space=pl.ANY)
    scratch = [
        pltpu.VMEM((S if not XACT else 8, D), BF),
        pltpu.VMEM((XOFF + S * XACT, D), BF),
        pltpu.VMEM((8, PRE // 2, 128), U32),
        pltpu.VMEM((RIDE, D), F32),
        pltpu.VMEM((32, 768), F32),
        pltpu.VMEM((2 * EMAX, D), F32),
        pltpu.SMEM((NSEG * NTAB,), jnp.int32),
        pltpu.VMEM((7, 8, D), F32),
        pltpu.VMEM((4, 1, D), BF),
        pltpu.VMEM((3 * H, D // 2, 128), U32),
        pltpu.VMEM((H, DH // 2, D), U32),
        pltpu.VMEM((6, D // 2, D), U32),
        pltpu.VMEM((D // 2, F), U32),
        pltpu.VMEM((D // 2, F), U32),
        pltpu.VMEM((F // 2, D), U32),
        pltpu.VMEM((NOSLOT * 32 + PRE, OW1), BF),
        pltpu.VMEM((NOSLOT * 32 + PRE, OW2), BF),
        pltpu.SemaphoreType.DMA((17,)),
        pltpu.SemaphoreType.DMA((12,)),
        pltpu.SemaphoreType.DMA((16,)),
    ] + [pltpu.VMEM((NSLOT, 512, 128), BF) for _ in range(NB)]
    wq, wk, wv = (w.reshape(D // 2, 2, H, DH) for w in (A_Wq, A_Wk, A_Wv))
    return pl.pallas_call(
        _kernel,
        out_shape=jax.ShapeDtypeStruct((1, S, D), BF),
        in_specs=[any_spec] * 12,
        out_specs=any_spec,
        scratch_shapes=scratch,
        compiler_params=pltpu.CompilerParams(vmem_limit_bytes=120 * 1024 * 1024,
                                             disable_bounds_checks=True),
    )(A_x, A_mem0, wq, wk, wv, A_Wo, B_w_r.reshape(1, D), B_w_gate, B_w_up, B_w_down,
      c, w_mod)
```

```python
import contextlib
import os
import jax
import jax.numpy as jnp
from jax import lax
import jax.experimental.pallas as pl
import jax.experimental.pallas.tpu as pltpu

BF = jnp.bfloat16
F32 = jnp.float32
U32 = jnp.uint32

S = 2048
D = 1024
H = 32
DH = 128
M = 8
SEG = 32
NSEG = S // SEG
F = 3584
NP = H // 2
RIDE = 24
PRE = S - NSEG * RIDE
NSLOT = 17
NOSLOT = 17
NB = int(os.environ.get('NB', 8))
KS = int(os.environ.get('KS', 2560))
LAG_S = 1
LAG_P = 3
EPS = 1e-5
SCALE = DH ** -0.5
OOFF = S
HOFF = 2 * S
ROFF = HOFF + 64
ZOFF = ROFF + 16
XOFF = ZOFF + 16
PRE_SPLIT = 3
E_AT = tuple(int(v) for v in os.environ.get('E_AT', '2,3,4').split(','))
L_AT = tuple(int(v) for v in os.environ.get('L_AT', '8,10,12').split(','))
E_AT2 = tuple(int(v) for v in os.environ.get('E_AT2', '2,3,4').split(','))
L_AT2 = tuple(int(v) for v in os.environ.get('L_AT2', '8,10,12').split(','))


def _att_schedule(mode):
    att = {}
    if mode == 'lag':
        for p in range(NP):
            att.setdefault(p + LAG_S, []).append(('s', p))
        for p in range(NP):
            att.setdefault(p + LAG_P, []).append(('p', p))
    elif mode == 'q2':
        for p in range(0, NP, 2):
            att.setdefault(p + 2, []).extend([('s', p), ('s', p + 1)])
        for p in range(0, NP, 2):
            att.setdefault(p + 4, []).extend([('p', p), ('p', p + 1)])
    elif mode == 'q2b':
        for p in range(0, NP, 2):
            att.setdefault(p + 4, []).extend([('p', p), ('p', p + 1)])
        for p in range(0, NP, 2):
            att.setdefault(p + 2, []).extend([('s', p), ('s', p + 1)])
    elif mode == 'q2c':
        att[4] = [('s', i) for i in range(4)]
        for p in range(4, NP, 2):
            att[p + 2] = [('s', p), ('s', p + 1), ('p', p - 4), ('p', p - 3)]
        att[18] = [('p', i) for i in range(12, 16)]
    elif mode == 'q2d':
        att[3] = [('s', i) for i in range(3)]
        att[4] = [('s', 3)]
        att[3] = []
        att[4] = [('s', i) for i in range(4)]
        for p in range(4, NP, 2):
            att[p + 2] = [('p', p - 4), ('p', p - 3), ('s', p), ('s', p + 1)]
        att[18] = [('p', i) for i in range(12, 16)]
    elif mode == 'q4':
        for p in range(0, NP, 4):
            att.setdefault(p + 4, []).extend([('s', p + i) for i in range(4)])
            att.setdefault(p + 6, []).extend([('p', p + i) for i in range(4)])
    elif mode == 'q4b':
        for p in range(0, NP, 4):
            att.setdefault(min(p + 8, 18), []).extend([('p', p + i) for i in range(4)])
        for p in range(0, NP, 4):
            att.setdefault(p + 4, []).extend([('s', p + i) for i in range(4)])
    return att


ATT = _att_schedule(os.environ.get('ATT', 'q2c'))
XACT = int(os.environ.get('XACT', 0))
LD32 = int(os.environ.get('LD32', 1))
K2 = H * DH - KS
OPAD = int(os.environ.get('OPAD', 1))
OW1 = -(-KS // 1024) * 1024 if OPAD else KS
OW2 = -(-K2 // 1024) * 1024 if OPAD else K2
UNR = int(os.environ.get('UNR', 2))
EPI_CHUNKS = tuple(int(v) for v in os.environ.get('EPI', '64,64,64,64,64,64,48,48,32').split(','))
EMAX = max(EPI_CHUNKS)
EPI_PIN = int(os.environ.get('EPI_PIN', 0))
EPI_SPARE = int(os.environ.get('EPI_SPARE', 0))
EPI_NSUB = int(os.environ.get('EPI_NSUB', 8))


NTAB = 16


def _step_indices(s):
    t = [s % NSLOT]
    for j in range(3):
        gi = PRE // 8 + 3 * s + j
        t += [(gi // 4) % NSLOT, (gi % 4) * 8]
    for j in range(4):
        gi = 4 * s + j
        t.append(((gi // 3) % NOSLOT) * 32 + 8 + (gi % 3) * 8 if gi < 3 * NSEG
                 else NOSLOT * 32 + (gi - 3 * NSEG) * 8)
    t.append((s % NOSLOT) * 32)
    t.append(max(s - 1, 0) * RIDE)
    t.append(PRE + min(s + 1, NSEG - 1) * RIDE)
    return t


def _scope(name):
    return jax.named_scope(name) if os.environ.get('PROF') else contextlib.nullcontext()


def _rb(v):
    return v.astype(BF).astype(F32)


def _layernorm(x):
    mu = jnp.sum(x, axis=-1, keepdims=True) * (1.0 / D)
    xc = x - mu
    var = jnp.sum(xc * xc, axis=-1, keepdims=True) * (1.0 / D)
    sd = _rb(jnp.sqrt(_rb(_rb(var) + EPS)))
    return _rb(_rb(x - _rb(mu)) / sd)


def _kernel(x_hbm, mem0_hbm, wq_hbm, wk_hbm, wv_hbm, wo_hbm, wr_hbm, wg_hbm, wu_hbm,
            wd_hbm, c_hbm, wmod_hbm, out_hbm,
            xbuf, act, h0buf, abuf, ybuf, ebuf, tab, modb, small,
            w_v, wo_v, wmod_v, wg_v, wu_v, wd_v,
            obuf1, obuf2, sems, wsems, ksems, *rest):
    qkvbufs, wrbuf = rest[:NB], rest[NB]
    qkv32 = tuple(b.bitcast(U32) for b in qkvbufs)
    if XACT:
        xbuf = act.at[pl.ds(XOFF, S)]
    w_hbms = tuple(w.bitcast(U32) for w in (wq_hbm, wk_hbm, wv_hbm))

    def cp(src, dst, i):
        return pltpu.make_async_copy(src, dst, sems.at[i])

    wmod_b = wmod_v.bitcast(BF)
    cp_c = cp(c_hbm, small.at[0], 0)
    cp_mem = cp(mem0_hbm.at[0], act.at[HOFF:HOFF + M], 1)
    cp_wr = cp(wr_hbm, wrbuf, 2)
    cp_x0 = [cp(x_hbm.at[0, n * 128:(n + 1) * 128], xbuf.at[n * 128:(n + 1) * 128], 13 + n)
             for n in range(PRE // 128)]
    cp_xr = cp(x_hbm.at[0, PRE:PRE + 32], xbuf.at[PRE:PRE + 32], 5)
    cp_x1 = cp(x_hbm.at[0, PRE + 32:S], xbuf.at[PRE + 32:S], 4)
    cp_wo = cp(wo_hbm, wo_v.bitcast(BF), 7)
    cp_ffn = [cp(wg_hbm, wg_v.bitcast(BF), 8), cp(wu_hbm, wu_v.bitcast(BF), 8),
              cp(wd_hbm, wd_v.bitcast(BF), 8)]

    def w_start(j):
        gg, t = j // 3, j % 3
        for i in range(NB):
            for par in range(2):
                pltpu.make_async_copy(w_hbms[t].at[:, par, gg * NB + i, :],
                                      w_v.at[(gg * NB + i) * 6 + t * 2 + par],
                                      wsems.at[2 * j + (i >= PRE_SPLIT)]).start()

    def mod_copy(j):
        return pltpu.make_async_copy(wmod_hbm.at[:, j * D:(j + 1) * D], wmod_b.at[j],
                                     wsems.at[2 * j + 1])

    def mult(v, m):
        return v if isinstance(v, int) else pl.multiple_of(v, m)

    def moda_copies(kc):
        col = mult(kc * 128, 128)
        return [pltpu.make_async_copy(wmod_hbm.at[:, pl.ds(v * D + col, 128)],
                                      wmod_b.at[v, :, pl.ds(col, 128)], ksems.at[8 + kc])
                for v in range(2)]

    def chunk_copies(kc):
        r0 = mult(kc * 64, 64)
        return [pltpu.make_async_copy(w_hbms[0].at[pl.ds(r0, 64), par, i, :],
                                      w_v.at[i * 6 + par, pl.ds(r0, 64), :], ksems.at[kc])
                for i in range(NB) for par in range(2)]

    cp_c.start()
    cp_mem.start()
    cp_wr.start()
    for c_ in (cp_x0 + moda_copies(0) + moda_copies(1) + chunk_copies(0) + moda_copies(2)
               + chunk_copies(1) + [cp_xr] + chunk_copies(2)):
        c_.start()

    def ln1_rows(src_row, dst_row):
        xv = xbuf[pl.ds(src_row, 8), :].astype(F32)
        hv = _rb(_layernorm(xv) * modb[1]) + modb[0]
        act[pl.ds(dst_row, 8), :] = hv.astype(BF)

    lane256 = lax.broadcasted_iota(jnp.int32, (8, 256), 1)

    def finish_rows(row, attn):
        xv = xbuf[pl.ds(row, 8), :].astype(F32)
        x1 = _rb(xv + _rb(modb[2] * _rb(attn)))
        h2 = _rb(_rb(_layernorm(x1) * modb[4]) + modb[3])
        act[pl.ds(row, 8), :] = x1.astype(BF)
        act[pl.ds(OOFF + row, 8), :] = (x1 + _rb(modb[5] * h2)).astype(BF)
        r = jnp.sum(h2 * modb[6], axis=-1, keepdims=True)
        act[ROFF:ROFF + 8, 0:256] = jnp.where(
            lane256 * 8 == row, r, act[ROFF:ROFF + 8, 0:256].astype(F32)).astype(BF)

    act[ROFF:ROFF + 8, 0:256] = jnp.zeros((8, 256), BF)
    act[ZOFF:ZOFF + 16, 0:128] = jnp.zeros((16, 128), BF)
    tab[14] = ZOFF
    tab[15] = 0
    abuf[...] = jnp.zeros(abuf.shape, F32)
    for s_ in range(NSEG):
        for k, v in enumerate(_step_indices(s_)):
            tab[s_ * NTAB + k] = v
    ri = lax.broadcasted_iota(jnp.int32, (80, 80), 0)
    ci = lax.broadcasted_iota(jnp.int32, (80, 80), 1)

    def head_pos(i):
        hd = jnp.where(i < 16, i // 8, (i - 16) // 32)
        pos = jnp.where(i < 16, i % 8, 8 + (i - 16) % 32)
        return hd, pos
    rh, rp = head_pos(ri)
    ch, cpos = head_pos(ci)
    same = rh == ch
    valid = same & ((rp < M) | (rp >= cpos))
    fill = jnp.where(same, -1e9, -jnp.inf).astype(F32)

    cp_mem.wait()
    cp_wr.wait()
    modb[6] = jnp.broadcast_to(wrbuf[...].astype(F32).reshape(1, D), (8, D))
    cp_c.wait()
    cv = small[0].astype(F32)
    sc16 = jnp.broadcast_to(_rb(cv * _rb(jax.nn.sigmoid(cv))), (16, D)).astype(BF)

    def ln_pre(g, carry):
        pltpu.make_async_copy(x_hbm.at[0, 0:128], xbuf.at[pl.ds(pl.multiple_of(g * 128, 128), 128)],
                              sems.at[13 + g]).wait()
        for u in range(2):
            row = pl.multiple_of(g * 128 + u * 64, 64)
            nv = _layernorm(xbuf[pl.ds(row, 64), :].astype(F32)).astype(BF)
            for k in range(8):
                h0buf[k, pl.ds(pl.multiple_of(row // 2, 32), 32), :] = pltpu.bitcast(
                    nv[:, k * 128:(k + 1) * 128], U32)
            wg_v[pl.ds(row, 64), 0:2 * D] = jnp.zeros((64, 2 * D), U32)
        return carry
    lax.fori_loop(0, PRE // 128, ln_pre, 0)

    def mod_tile(v, col):
        w = pltpu.bitcast(wmod_v[v, :, pl.ds(col, 128)], BF)
        return _rb(jnp.dot(sc16, w, preferred_element_type=F32))[0:8]

    def moda_store(kc, sa, ca):
        col = mult(kc * 128, 128)
        c1 = _rb(1.0 + ca)
        modb[0, :, pl.ds(col, 128)] = sa
        modb[1, :, pl.ds(col, 128)] = c1
        return sa, c1

    def moda_apply(kc, sa, c1, r0, r1):
        for r in range(r0, r1, 16):
            nv = pltpu.bitcast(h0buf[kc, r // 2:r // 2 + 8, :], BF).astype(F32).reshape(2, 8, 128)
            hv = (_rb(nv * c1[None]) + sa[None]).reshape(16, 128).astype(BF)
            h0buf[kc, r // 2:r // 2 + 8, :] = pltpu.bitcast(hv, U32)

    def repack(a, b):
        return (a & U32(0xFFFF)) | (b << 16), (a >> 16) | (b & U32(0xFFFF0000))

    def store_qkv(i, jrow, y, seg0):
        for sg in range(y.shape[0] // 32):
            for hh in range(2):
                qkvbufs[i][seg0 + sg, pl.ds(jrow + 16 + hh * 32, 32), :] = (
                    y[sg * 32:(sg + 1) * 32, hh * 128:(hh + 1) * 128].astype(BF))

    for c_ in moda_copies(0):
        c_.wait()
    moda_apply(0, *moda_store(0, mod_tile(0, 0), mod_tile(1, 0)), 0, PRE)

    def chunk_block(kc, last, issue):
        with _scope('w_chunk'):
            for c_ in chunk_copies(kc) + ([cp_xr] if last else moda_copies(kc + 1)):
                c_.wait()
        issue()
        r0 = mult(kc * 64, 64)
        mv = []
        for i in range(NB):
            lo, hi = repack(w_v[i * 6, pl.ds(r0, 64), :], w_v[i * 6 + 1, pl.ds(r0, 64), :])
            w_v[i * 6, pl.ds(r0, 64), :] = lo
            w_v[i * 6 + 1, pl.ds(r0, 64), :] = hi
            w = pltpu.bitcast(jnp.concatenate([lo, hi], axis=1), BF)
            y = (pltpu.bitcast(wg_v[0:PRE, i * 256:(i + 1) * 256], F32)
                 + jnp.dot(pltpu.bitcast(h0buf[kc], BF), w, preferred_element_type=F32))
            if last:
                store_qkv(i, 0, y, 0)
            else:
                wg_v[0:PRE, i * 256:(i + 1) * 256] = pltpu.bitcast(y, U32)
                if i in (1, 3):
                    mv.append(mod_tile(i // 2, mult((kc + 1) * 128, 128)))
                if i == 3:
                    mv = moda_store(kc + 1, mv[0], mv[1])
                if i >= 4:
                    moda_apply(kc + 1, mv[0], mv[1], (i - 4) * 128, (i - 3) * 128)
        if last:
            for j in range(3):
                ln1_rows(PRE + 8 * j, HOFF + 8 + 8 * j)

    def chunk_body_a(kc, carry):
        def issue():
            for c_ in moda_copies(kc + 3) + chunk_copies(kc + 3):
                c_.start()
        chunk_block(kc, False, issue)
        return carry

    def chunk_body_b(kc, carry):
        chunk_block(kc, False, lambda: None)
        return carry

    def issue_last():
        w_start(2)
        mod_copy(2).start()
    lax.fori_loop(0, 5, chunk_body_a, 0)
    w_start(1)
    lax.fori_loop(5, 7, chunk_body_b, 0)
    chunk_block(7, True, issue_last)

    def pre_unit(j, i, extra):
        blk = (j // 3) * (6 * NB) + (j % 3) * 2 + i * 6
        jrow = pl.multiple_of(j * 80, 16)
        lo, hi = repack(w_v[blk], w_v[blk + 1])
        w_v[blk] = lo
        w_v[blk + 1] = hi
        for rc in range(PRE // 128):
            if rc > 0:
                lo = w_v[blk]
                hi = w_v[blk + 1]
            w = pltpu.bitcast(jnp.concatenate([lo, hi], axis=1), BF)
            lhs = jnp.concatenate([h0buf[k, rc * 64:(rc + 1) * 64, :] for k in range(8)], axis=1)
            y = jnp.dot(pltpu.bitcast(lhs, BF), w, preferred_element_type=F32)
            store_qkv(i, jrow, y, rc * 4)
            extra(rc)

    def pre_body(j, carry):
        @pl.when(j == 1)
        def _():
            for jn in (3, 4):
                w_start(jn)
                mod_copy(jn).start()

        @pl.when(j == 2)
        def _():
            w_start(5)
            mod_copy(5).start()
            cp_wo.start()
            cp_x1.start()
        blk0 = (j // 3) * (6 * NB) + (j % 3) * 2
        one = jnp.where((j == 1) | (j == 4), 1.0, 0.0).astype(F32)
        for half, (i0, i1) in enumerate(((0, PRE_SPLIT), (PRE_SPLIT, NB))):
            with _scope('w_pre'):
                for i in range(i0, i1):
                    for par in range(2):
                        pltpu.make_async_copy(w_hbms[0].at[:, 0, 0, :],
                                              w_v.at[blk0 + i * 6 + par],
                                              wsems.at[2 * j + half]).wait()
            if half == 1:
                @pl.when(j > 1)
                def _():
                    pltpu.make_async_copy(wmod_hbm.at[:, 0:D], wmod_b.at[j],
                                          wsems.at[2 * j + 1]).wait()
            for i in range(i0, i1):
                def extra(rc, i=i):
                    n = (i - PRE_SPLIT) * 2 + rc // 2
                    if i >= PRE_SPLIT and rc % 2 == 0 and n < 8:
                        modb[j, :, n * 128:(n + 1) * 128] = _rb(one + mod_tile(j, n * 128))
                pre_unit(j, i, extra)
        return carry
    lax.fori_loop(1, 6, pre_body, 0)

    cp_wo.wait()
    cp_x1.wait()
    for c_ in cp_ffn:
        c_.start()

    def wo_w(h0, h1, n0, n1):
        w = wo_v[h0:h1, :, n0 * 128:n1 * 128].reshape((h1 - h0) * (DH // 2), (n1 - n0) * 128)
        return pltpu.bitcast(w, BF)

    HD = D // 2

    def emit_step(s, pend, last):
        hrow = pl.multiple_of(HOFF + (s & 1) * 32, 32)
        hnext = pl.multiple_of(HOFF + 32 - (s & 1) * 32, 32)
        tv = [tab[s * NTAB + k] for k in range(14)]
        slot = tv[0]
        dsts = [(tv[1 + 2 * j], pl.multiple_of(tv[2 + 2 * j], 8)) for j in range(3)]
        odst = [pl.multiple_of(tv[7 + j], 8) for j in range(4)]
        orow = pl.multiple_of(tv[11], 32)
        erow = tv[12]
        lrow = tv[13]
        e_at, l_at = (E_AT, L_AT) if pend is None else (E_AT2, L_AT2)
        probs = {}

        def wqkv(p, k0, k1):
            return pltpu.bitcast(jnp.concatenate(
                [w_v[p * 6 + u, k0 // 2:k1 // 2, :] for u in range(6)], axis=1), BF)

        lhs_lo = act[pl.ds(hrow, 32), 0:HD]
        if pend is not None:
            ybuf[...] = jnp.dot(lhs_lo, wqkv(0, 0, HD), preferred_element_type=F32)
            pend()
        lhs_hi = act[pl.ds(hrow, 32), HD:D]
        if pend is not None:
            y0 = ybuf[...] + jnp.dot(lhs_hi, wqkv(0, HD, D), preferred_element_type=F32)
        lhs_rest = jnp.concatenate([lhs_lo[:, 128:], lhs_hi], axis=1)
        lhs = [jnp.concatenate([lhs_lo, lhs_hi], axis=1)]

        def side(p):
            for j in range(3):
                if e_at[j] == p:
                    finish_rows(pl.multiple_of(erow + 8 * j, 8), abuf[8 * j:8 * j + 8, :])
            for j in range(3):
                if l_at[j] == p:
                    ln1_rows(pl.multiple_of(lrow + 8 * j, 8),
                             pl.multiple_of(hnext + 8 + 8 * j, 8))
            if (p in e_at or p in l_at) and p < NP - 1:
                lhs[0] = jnp.concatenate([act[pl.ds(hrow, 32), 0:128], lhs_rest], axis=1)

        def qkv(p):
            if p == 0 and pend is not None:
                y = y0
            else:
                y = jnp.dot(lhs[0], wqkv(p, 0, D), preferred_element_type=F32)
            buf = qkvbufs[p % NB]
            for u in range(6):
                t, hh = u // 2, u % 2
                b0 = ((p // NB) * 3 + t) * 80
                yu = y[:, u * 128:(u + 1) * 128]
                buf[slot, b0 + hh * 8:b0 + hh * 8 + 8, :] = yu[0:8].astype(BF)
                for j in range(3):
                    sl, off = dsts[j]
                    buf[sl, pl.ds(b0 + 16 + hh * 32 + off, 8), :] = (
                        yu[8 + 8 * j:16 + 8 * j].astype(BF))

        def ld(p, t):
            b0 = ((p // NB) * 3 + t) * 40
            if not LD32:
                return qkvbufs[p % NB][slot, 2 * b0:2 * b0 + 80, :]
            return pltpu.bitcast(qkv32[p % NB][slot, b0:b0 + 40, :], BF)

        def sc(p):
            s2 = lax.dot_general(ld(p, 0), ld(p, 1), (((1,), (1,)), ((), ())),
                                 preferred_element_type=F32) * SCALE
            s2 = jnp.where(valid, s2, fill)
            m = jnp.max(s2, axis=-1, keepdims=True)
            e = jnp.exp(s2 - m)
            l = jnp.sum(e, axis=-1, keepdims=True)
            rl = pl.reciprocal(l, approx=True)
            rl = rl * (2.0 - l * rl)
            probs[p] = (e * rl).astype(BF)

        def pv(p):
            o2 = jnp.dot(probs[p], ld(p, 2), preferred_element_type=F32)
            for hh in range(2):
                hcol = (2 * p + hh) * 128
                ob = obuf1
                if hcol >= KS:
                    ob = obuf2
                    hcol -= KS
                ob[pl.ds(orow, 8), hcol:hcol + 128] = o2[8 * hh:8 * hh + 8].astype(BF)
                for j in range(4):
                    r0 = 16 + 32 * hh + 8 * j
                    ob[pl.ds(odst[j], 8), hcol:hcol + 128] = o2[r0:r0 + 8].astype(BF)

        def attn(pos):
            for kind, p in ATT.get(pos, ()):
                (sc if kind == 's' else pv)(p)

        for p in range(NP):
            qkv(p)
            side(p)
            attn(p)
        a1 = []
        for i in range(4):
            a1.append(jnp.dot(obuf1[pl.ds(orow, 32), 0:KS], wo_w(0, KS // DH, 2 * i, 2 * i + 2),
                              preferred_element_type=F32))
            attn(NP + i)
            side(NP + i)
        o2lhs = obuf2[pl.ds(orow, 32), 0:K2]
        a_lo = jnp.concatenate(a1[0:2], axis=1) + jnp.dot(
            o2lhs, wo_w(KS // DH, H, 0, 4), preferred_element_type=F32)
        act[pl.ds(hnext, 8), 0:HD] = a_lo[0:8].astype(BF)
        abuf[:, 0:HD] = a_lo[8:32]
        a_hi = jnp.concatenate(a1[2:4], axis=1) + jnp.dot(
            o2lhs, wo_w(KS // DH, H, 4, 8), preferred_element_type=F32)

        def finish():
            act[pl.ds(hnext, 8), HD:D] = a_hi[0:8].astype(BF)
            abuf[:, HD:D] = a_hi[8:32]
        if last:
            finish()
        return finish

    def steps(it, carry):
        pend = None
        for u in range(UNR):
            pend = emit_step(it * UNR + u, pend, u == UNR - 1)
        return carry
    lax.fori_loop(0, NSEG // UNR, steps, 0)

    OUT0 = (NSEG - 1) * RIDE
    cp_out = [cp(act.at[OOFF:OOFF + OUT0], out_hbm.at[0, 0:OUT0], 9)]
    cp_out[0].start()
    zrow = pl.multiple_of(tab[14], 16)
    zero = pl.multiple_of(tab[15], 8)
    ebuf[EMAX:EMAX + RIDE, :] = abuf[...]
    todo = [(OUT0 + 8 * j, EMAX + 8 * j) for j in range(3)]
    r0 = 0
    nw = 8 // EPI_NSUB
    for ci, ech in enumerate(EPI_CHUNKS):
        o0 = NOSLOT * 32 + r0
        e0 = (ci % 2) * EMAX
        per = -(-len(todo) // (EPI_NSUB - EPI_SPARE))
        for n in range(EPI_NSUB):
            first = obuf1[o0:o0 + 16, 0:128]
            if n == 0 and ci > 0 and EPI_PIN:
                first = pltpu.bitcast(
                    pltpu.bitcast(first, U32) | pltpu.bitcast(act[pl.ds(zrow, 16), 0:128], U32), BF)
            col0 = jnp.concatenate([first, obuf1[o0 + 16:o0 + ech, 0:128]], axis=0)
            lhs = jnp.concatenate(
                [col0, obuf1[o0:o0 + ech, 128:KS], obuf2[o0:o0 + ech, 0:K2]], axis=1)
            ebuf[e0:e0 + ech, n * nw * 128:(n + 1) * nw * 128] = jnp.dot(
                lhs, wo_w(0, H, n * nw, (n + 1) * nw), preferred_element_type=F32)
            for row, er in todo[:per]:
                finish_rows(row, ebuf[pl.ds(zero + er, 8), :])
            todo = todo[per:]
        todo = [(OUT0 + RIDE + r0 + 8 * j, e0 + 8 * j) for j in range(ech // 8)]
        r0 += ech
    for row, er in todo:
        finish_rows(row, ebuf[er:er + 8, :])
    cp_out.append(cp(act.at[OOFF + OUT0:OOFF + S], out_hbm.at[0, OUT0:S], 10))
    cp_out[1].start()

    r_all = act[ROFF:ROFF + 8, 0:256].astype(F32)
    rows = lane256 * 8 + lax.broadcasted_iota(jnp.int32, (8, 256), 0)

    def allmax(v):
        return jnp.max(jnp.max(v, axis=1, keepdims=True), axis=0, keepdims=True)

    def allmin(v):
        return jnp.min(jnp.min(v, axis=1, keepdims=True), axis=0, keepdims=True)
    rowsf = rows.astype(F32)
    i1v = allmin(jnp.where(r_all == allmax(r_all), rowsf, float(S)))
    r_rest = jnp.where(rowsf == i1v, -jnp.inf, r_all)
    i2v = allmin(jnp.where((r_rest == allmax(r_rest)) & (rowsf != i1v), rowsf, float(S)))
    i1 = jnp.clip(i1v[0, 0].astype(jnp.int32), 0, S - 1)
    i2 = jnp.clip(i2v[0, 0].astype(jnp.int32), 0, S - 1)
    b1 = pl.multiple_of((i1 // 8) * 8, 8)
    b2 = pl.multiple_of((i2 // 8) * 8, 8)

    x1 = jnp.concatenate([act[pl.ds(b1, 8), :].astype(F32), act[pl.ds(b2, 8), :].astype(F32)],
                         axis=0)

    def two(i):
        return jnp.concatenate([modb[i], modb[i]], axis=0)
    h2 = _rb(_rb(_layernorm(x1) * two(4)) + two(3))
    rr = _rb(jnp.sum(h2 * two(6), axis=-1, keepdims=True))
    h2b = h2.astype(BF)
    for c_ in cp_ffn:
        c_.wait()
    gt = _rb(jnp.dot(h2b, pltpu.bitcast(wg_v[...], BF), preferred_element_type=F32))
    up = _rb(jnp.dot(h2b, pltpu.bitcast(wu_v[...], BF), preferred_element_type=F32))
    hid = (_rb(gt * _rb(jax.nn.sigmoid(gt))) * up).astype(BF)
    y = _rb(jnp.dot(hid, pltpu.bitcast(wd_v[...], BF), preferred_element_type=F32))
    y = _rb(y * _rb(jax.nn.sigmoid(rr)))
    sub = lax.broadcasted_iota(jnp.int32, (16, 1), 0)
    grow = jnp.where(sub < 8, b1 + sub, b2 + sub - 8)
    sel = (grow == i1) | (grow == i2)
    res = (x1 + _rb(two(5) * _rb(h2 + jnp.where(sel, y, 0.0)))).astype(BF)
    for c_ in cp_out:
        c_.wait()
    act[pl.ds(OOFF + b1, 8), :] = res[0:8]
    act[pl.ds(OOFF + b2, 8), :] = res[8:16]
    fix1 = cp(act.at[pl.ds(OOFF + b1, 8)], out_hbm.at[0, pl.ds(b1, 8)], 11)
    fix2 = cp(act.at[pl.ds(OOFF + b2, 8)], out_hbm.at[0, pl.ds(b2, 8)], 12)
    fix1.start()

    @pl.when(b1 != b2)
    def _():
        fix2.start()
        fix2.wait()
    fix1.wait()


@jax.jit
def pallas_adaLN_cond__memory_aug_recurrent_mem_tr__moe_arch_mod__prompt_kernel(
    A_x: jax.Array,
    A_mem0: jax.Array,
    A_Wq: jax.Array,
    A_Wk: jax.Array,
    A_Wv: jax.Array,
    A_Wo: jax.Array,
    A_seg_len,
    B_x: jax.Array,
    B_w_r: jax.Array,
    B_w_gate: jax.Array,
    B_w_up: jax.Array,
    B_w_down: jax.Array,
    c: jax.Array,
    w_mod: jax.Array,
):
    del B_x
    del A_seg_len
    assert A_x.shape == (1, S, D) and A_Wq.shape == (D, H, DH) and A_mem0.shape == (1, M, D)
    any_spec = pl.BlockSpec(memory_space=pl.ANY)
    scratch = [
        pltpu.VMEM((S if not XACT else 8, D), BF),
        pltpu.VMEM((XOFF + S * XACT, D), BF),
        pltpu.VMEM((8, PRE // 2, 128), U32),
        pltpu.VMEM((RIDE, D), F32),
        pltpu.VMEM((32, 768), F32),
        pltpu.VMEM((2 * EMAX, D), F32),
        pltpu.SMEM((NSEG * NTAB,), jnp.int32),
        pltpu.VMEM((7, 8, D), F32),
        pltpu.VMEM((4, 1, D), BF),
        pltpu.VMEM((3 * H, D // 2, 128), U32),
        pltpu.VMEM((H, DH // 2, D), U32),
        pltpu.VMEM((6, D // 2, D), U32),
        pltpu.VMEM((D // 2, F), U32),
        pltpu.VMEM((D // 2, F), U32),
        pltpu.VMEM((F // 2, D), U32),
        pltpu.VMEM((NOSLOT * 32 + PRE, OW1), BF),
        pltpu.VMEM((NOSLOT * 32 + PRE, OW2), BF),
        pltpu.SemaphoreType.DMA((17,)),
        pltpu.SemaphoreType.DMA((12,)),
        pltpu.SemaphoreType.DMA((16,)),
    ] + [pltpu.VMEM((NSLOT, 512, 128), BF) for _ in range(NB)] + [
        pltpu.VMEM((D,), BF),
    ]
    wq, wk, wv = (w.reshape(D // 2, 2, H, DH) for w in (A_Wq, A_Wk, A_Wv))
    return pl.pallas_call(
        _kernel,
        out_shape=jax.ShapeDtypeStruct((1, S, D), BF),
        in_specs=[any_spec] * 12,
        out_specs=any_spec,
        scratch_shapes=scratch,
        compiler_params=pltpu.CompilerParams(vmem_limit_bytes=120 * 1024 * 1024,
                                             disable_bounds_checks=True,
                                             disable_semaphore_checks=True),
    )(A_x, A_mem0, wq, wk, wv, A_Wo, B_w_r, B_w_gate, B_w_up, B_w_down,
      c, w_mod)
```

```python
import contextlib
import os
import jax
import jax.numpy as jnp
from jax import lax
import jax.experimental.pallas as pl
import jax.experimental.pallas.tpu as pltpu

BF = jnp.bfloat16
F32 = jnp.float32
U32 = jnp.uint32

S = 2048
D = 1024
H = 32
DH = 128
M = 8
SEG = 32
NSEG = S // SEG
F = 3584
NP = H // 2
RIDE = 24
PRE = S - NSEG * RIDE
NSLOT = 17
NOSLOT = 17
NB = int(os.environ.get('NB', 8))
KS = int(os.environ.get('KS', 2560))
LAG_S = 1
LAG_P = 3
EPS = 1e-5
SCALE = DH ** -0.5
OOFF = S
HOFF = 2 * S
ROFF = HOFF + 64
ZOFF = ROFF + 16
XOFF = ZOFF + 16
PRE_SPLIT = 3
E_AT = tuple(int(v) for v in os.environ.get('E_AT', '2,3,4').split(','))
L_AT = tuple(int(v) for v in os.environ.get('L_AT', '8,10,12').split(','))
E_AT2 = tuple(int(v) for v in os.environ.get('E_AT2', '2,3,4').split(','))
L_AT2 = tuple(int(v) for v in os.environ.get('L_AT2', '8,10,12').split(','))


def _att_schedule(mode):
    att = {}
    if mode == 'lag':
        for p in range(NP):
            att.setdefault(p + LAG_S, []).append(('s', p))
        for p in range(NP):
            att.setdefault(p + LAG_P, []).append(('p', p))
    elif mode == 'q2':
        for p in range(0, NP, 2):
            att.setdefault(p + 2, []).extend([('s', p), ('s', p + 1)])
        for p in range(0, NP, 2):
            att.setdefault(p + 4, []).extend([('p', p), ('p', p + 1)])
    elif mode == 'q2b':
        for p in range(0, NP, 2):
            att.setdefault(p + 4, []).extend([('p', p), ('p', p + 1)])
        for p in range(0, NP, 2):
            att.setdefault(p + 2, []).extend([('s', p), ('s', p + 1)])
    elif mode == 'q2c':
        att[4] = [('s', i) for i in range(4)]
        for p in range(4, NP, 2):
            att[p + 2] = [('s', p), ('s', p + 1), ('p', p - 4), ('p', p - 3)]
        att[18] = [('p', i) for i in range(12, 16)]
    elif mode == 'q2d':
        att[3] = [('s', i) for i in range(3)]
        att[4] = [('s', 3)]
        att[3] = []
        att[4] = [('s', i) for i in range(4)]
        for p in range(4, NP, 2):
            att[p + 2] = [('p', p - 4), ('p', p - 3), ('s', p), ('s', p + 1)]
        att[18] = [('p', i) for i in range(12, 16)]
    elif mode == 'q4':
        for p in range(0, NP, 4):
            att.setdefault(p + 4, []).extend([('s', p + i) for i in range(4)])
            att.setdefault(p + 6, []).extend([('p', p + i) for i in range(4)])
    elif mode == 'q4b':
        for p in range(0, NP, 4):
            att.setdefault(min(p + 8, 18), []).extend([('p', p + i) for i in range(4)])
        for p in range(0, NP, 4):
            att.setdefault(p + 4, []).extend([('s', p + i) for i in range(4)])
    return att


ATT = _att_schedule(os.environ.get('ATT', 'q2c'))
XACT = int(os.environ.get('XACT', 0))
K2 = H * DH - KS
OPAD = int(os.environ.get('OPAD', 1))
OW1 = -(-KS // 1024) * 1024 if OPAD else KS
OW2 = -(-K2 // 1024) * 1024 if OPAD else K2
UNR = int(os.environ.get('UNR', 2))
EPI_CHUNKS = tuple(int(v) for v in os.environ.get('EPI', '64,64,64,64,64,64,48,48,32').split(','))
EMAX = max(EPI_CHUNKS)
EPI_PIN = int(os.environ.get('EPI_PIN', 0))
EPI_SPARE = int(os.environ.get('EPI_SPARE', 0))
EPI_NSUB = int(os.environ.get('EPI_NSUB', 8))


NTAB = 16


def _step_indices(s):
    t = [s % NSLOT]
    for j in range(3):
        gi = PRE // 8 + 3 * s + j
        t += [(gi // 4) % NSLOT, (gi % 4) * 4]
    for j in range(4):
        gi = 4 * s + j
        t.append(((gi // 3) % NOSLOT) * 32 + 8 + (gi % 3) * 8 if gi < 3 * NSEG
                 else NOSLOT * 32 + (gi - 3 * NSEG) * 8)
    t.append((s % NOSLOT) * 32)
    t.append(max(s - 1, 0) * RIDE)
    t.append(PRE + min(s + 1, NSEG - 1) * RIDE)
    return t


def _scope(name):
    return jax.named_scope(name) if os.environ.get('PROF') else contextlib.nullcontext()


def _rb(v):
    return v.astype(BF).astype(F32)


def _pack(v):
    return pltpu.bitcast(v.astype(BF), U32)


def _layernorm(x):
    mu = jnp.sum(x, axis=-1, keepdims=True) * (1.0 / D)
    xc = x - mu
    var = jnp.sum(xc * xc, axis=-1, keepdims=True) * (1.0 / D)
    sd = _rb(jnp.sqrt(_rb(_rb(var) + EPS)))
    return _rb(_rb(x - _rb(mu)) / sd)


def _kernel(x_hbm, mem0_hbm, wq_hbm, wk_hbm, wv_hbm, wo_hbm, wr_hbm, wg_hbm, wu_hbm,
            wd_hbm, c_hbm, wmod_hbm, out_hbm,
            xbuf, act, h0buf, abuf, ybuf, ebuf, tab, modb, small,
            w_v, wo_v, wmod_v, wg_v, wu_v, wd_v,
            obuf1, obuf2, sems, wsems, ksems, *rest):
    qkvbufs, wrbuf = rest[:NB], rest[NB]
    if XACT:
        xbuf = act.at[pl.ds(XOFF, S)]
    w_hbms = tuple(w.bitcast(U32) for w in (wq_hbm, wk_hbm, wv_hbm))

    def cp(src, dst, i):
        return pltpu.make_async_copy(src, dst, sems.at[i])

    wmod32 = wmod_hbm.bitcast(U32)
    cp_c = cp(c_hbm, small.at[0], 0)
    cp_mem = cp(mem0_hbm.at[0], act.at[HOFF:HOFF + M], 1)
    cp_wr = cp(wr_hbm, wrbuf, 2)
    cp_x0 = [cp(x_hbm.at[0, n * 128:(n + 1) * 128], xbuf.at[n * 128:(n + 1) * 128], 13 + n)
             for n in range(PRE // 128)]
    cp_xr = cp(x_hbm.at[0, PRE:PRE + 32], xbuf.at[PRE:PRE + 32], 5)
    cp_x1 = cp(x_hbm.at[0, PRE + 32:S], xbuf.at[PRE + 32:S], 4)
    cp_wo = cp(wo_hbm.bitcast(U32), wo_v, 7)
    cp_ffn = [cp(wg_hbm.bitcast(U32), wg_v, 8), cp(wu_hbm.bitcast(U32), wu_v, 8),
              cp(wd_hbm.bitcast(U32), wd_v, 8)]

    def w_start(j):
        gg, t = j // 3, j % 3
        for i in range(NB):
            for par in range(2):
                pltpu.make_async_copy(w_hbms[t].at[:, par, gg * NB + i, :],
                                      w_v.at[(gg * NB + i) * 6 + t * 2 + par],
                                      wsems.at[2 * j + (i >= PRE_SPLIT)]).start()

    def mod_copy(j):
        return pltpu.make_async_copy(wmod32.at[:, j * D:(j + 1) * D], wmod_v.at[j],
                                     wsems.at[2 * j + 1])

    def mult(v, m):
        return v if isinstance(v, int) else pl.multiple_of(v, m)

    def moda_copies(kc):
        col = mult(kc * 128, 128)
        return [pltpu.make_async_copy(wmod32.at[:, pl.ds(v * D + col, 128)],
                                      wmod_v.at[v, :, pl.ds(col, 128)], ksems.at[8 + kc])
                for v in range(2)]

    def chunk_copies(kc):
        r0 = mult(kc * 64, 64)
        return [pltpu.make_async_copy(w_hbms[0].at[pl.ds(r0, 64), par, i, :],
                                      w_v.at[i * 6 + par, pl.ds(r0, 64), :], ksems.at[kc])
                for i in range(NB) for par in range(2)]

    cp_c.start()
    cp_mem.start()
    cp_wr.start()
    for c_ in (cp_x0 + moda_copies(0) + moda_copies(1) + chunk_copies(0) + moda_copies(2)
               + chunk_copies(1) + [cp_xr] + chunk_copies(2)):
        c_.start()

    def ln1_rows(src_row, dst_row):
        xv = xbuf[pl.ds(src_row, 8), :].astype(F32)
        hv = _rb(_layernorm(xv) * modb[1]) + modb[0]
        act[pl.ds(dst_row, 8), :] = hv.astype(BF)

    lane256 = lax.broadcasted_iota(jnp.int32, (8, 256), 1)

    def finish_rows(row, attn):
        xv = xbuf[pl.ds(row, 8), :].astype(F32)
        x1 = _rb(xv + _rb(modb[2] * _rb(attn)))
        h2 = _rb(_rb(_layernorm(x1) * modb[4]) + modb[3])
        act[pl.ds(row, 8), :] = x1.astype(BF)
        act[pl.ds(OOFF + row, 8), :] = (x1 + _rb(modb[5] * h2)).astype(BF)
        r = jnp.sum(h2 * modb[6], axis=-1, keepdims=True)
        act[ROFF:ROFF + 8, 0:256] = jnp.where(
            lane256 * 8 == row, r, act[ROFF:ROFF + 8, 0:256].astype(F32)).astype(BF)

    act[ROFF:ROFF + 8, 0:256] = jnp.zeros((8, 256), BF)
    act[ZOFF:ZOFF + 16, 0:128] = jnp.zeros((16, 128), BF)
    tab[14] = ZOFF
    tab[15] = 0
    abuf[...] = jnp.zeros(abuf.shape, F32)
    for s_ in range(NSEG):
        for k, v in enumerate(_step_indices(s_)):
            tab[s_ * NTAB + k] = v
    ri = lax.broadcasted_iota(jnp.int32, (80, 80), 0)
    ci = lax.broadcasted_iota(jnp.int32, (80, 80), 1)

    def head_pos(i):
        hd = jnp.where(i < 16, i // 8, (i - 16) // 32)
        pos = jnp.where(i < 16, i % 8, 8 + (i - 16) % 32)
        return hd, pos
    rh, rp = head_pos(ri)
    ch, cpos = head_pos(ci)
    same = rh == ch
    valid = same & ((rp < M) | (rp >= cpos))
    fill = jnp.where(same, -1e9, -jnp.inf).astype(F32)

    cp_mem.wait()
    cp_wr.wait()
    modb[6] = jnp.broadcast_to(wrbuf[...].astype(F32).reshape(1, D), (8, D))
    cp_c.wait()
    cv = small[0].astype(F32)
    sc16 = jnp.broadcast_to(_rb(cv * _rb(jax.nn.sigmoid(cv))), (16, D)).astype(BF)

    def ln_pre(g, carry):
        pltpu.make_async_copy(x_hbm.at[0, 0:128], xbuf.at[pl.ds(pl.multiple_of(g * 128, 128), 128)],
                              sems.at[13 + g]).wait()
        for u in range(2):
            row = pl.multiple_of(g * 128 + u * 64, 64)
            nv = _layernorm(xbuf[pl.ds(row, 64), :].astype(F32)).astype(BF)
            for k in range(8):
                h0buf[k, pl.ds(pl.multiple_of(row // 2, 32), 32), :] = pltpu.bitcast(
                    nv[:, k * 128:(k + 1) * 128], U32)
            wg_v[pl.ds(row, 64), 0:2 * D] = jnp.zeros((64, 2 * D), U32)
        return carry
    lax.fori_loop(0, PRE // 128, ln_pre, 0)

    def mod_tile(v, col):
        w = pltpu.bitcast(wmod_v[v, :, pl.ds(col, 128)], BF)
        return _rb(jnp.dot(sc16, w, preferred_element_type=F32))[0:8]

    def moda_store(kc, sa, ca):
        col = mult(kc * 128, 128)
        c1 = _rb(1.0 + ca)
        modb[0, :, pl.ds(col, 128)] = sa
        modb[1, :, pl.ds(col, 128)] = c1
        return sa, c1

    def moda_apply(kc, sa, c1, r0, r1):
        for r in range(r0, r1, 16):
            nv = pltpu.bitcast(h0buf[kc, r // 2:r // 2 + 8, :], BF).astype(F32).reshape(2, 8, 128)
            hv = (_rb(nv * c1[None]) + sa[None]).reshape(16, 128).astype(BF)
            h0buf[kc, r // 2:r // 2 + 8, :] = pltpu.bitcast(hv, U32)

    def repack(a, b):
        return (a & U32(0xFFFF)) | (b << 16), (a >> 16) | (b & U32(0xFFFF0000))

    def store_qkv(i, jrow, y, seg0):
        for sg in range(y.shape[0] // 32):
            for hh in range(2):
                qkvbufs[i][seg0 + sg, pl.ds(jrow + 8 + hh * 16, 16), :] = _pack(
                    y[sg * 32:(sg + 1) * 32, hh * 128:(hh + 1) * 128])

    for c_ in moda_copies(0):
        c_.wait()
    moda_apply(0, *moda_store(0, mod_tile(0, 0), mod_tile(1, 0)), 0, PRE)

    def chunk_block(kc, last, issue):
        with _scope('w_chunk'):
            for c_ in chunk_copies(kc) + ([cp_xr] if last else moda_copies(kc + 1)):
                c_.wait()
        issue()
        r0 = mult(kc * 64, 64)
        mv = []
        for i in range(NB):
            lo, hi = repack(w_v[i * 6, pl.ds(r0, 64), :], w_v[i * 6 + 1, pl.ds(r0, 64), :])
            w_v[i * 6, pl.ds(r0, 64), :] = lo
            w_v[i * 6 + 1, pl.ds(r0, 64), :] = hi
            w = pltpu.bitcast(jnp.concatenate([lo, hi], axis=1), BF)
            y = (pltpu.bitcast(wg_v[0:PRE, i * 256:(i + 1) * 256], F32)
                 + jnp.dot(pltpu.bitcast(h0buf[kc], BF), w, preferred_element_type=F32))
            if last:
                store_qkv(i, 0, y, 0)
            else:
                wg_v[0:PRE, i * 256:(i + 1) * 256] = pltpu.bitcast(y, U32)
                if i in (1, 3):
                    mv.append(mod_tile(i // 2, mult((kc + 1) * 128, 128)))
                if i == 3:
                    mv = moda_store(kc + 1, mv[0], mv[1])
                if i >= 4:
                    moda_apply(kc + 1, mv[0], mv[1], (i - 4) * 128, (i - 3) * 128)
        if last:
            for j in range(3):
                ln1_rows(PRE + 8 * j, HOFF + 8 + 8 * j)

    def chunk_body_a(kc, carry):
        def issue():
            for c_ in moda_copies(kc + 3) + chunk_copies(kc + 3):
                c_.start()
        chunk_block(kc, False, issue)
        return carry

    def chunk_body_b(kc, carry):
        chunk_block(kc, False, lambda: None)
        return carry

    def issue_last():
        w_start(2)
        mod_copy(2).start()
    lax.fori_loop(0, 5, chunk_body_a, 0)
    w_start(1)
    lax.fori_loop(5, 7, chunk_body_b, 0)
    chunk_block(7, True, issue_last)

    def pre_unit(j, i, extra):
        blk = (j // 3) * (6 * NB) + (j % 3) * 2 + i * 6
        jrow = pl.multiple_of(j * 40, 8)
        lo, hi = repack(w_v[blk], w_v[blk + 1])
        w_v[blk] = lo
        w_v[blk + 1] = hi
        for rc in range(PRE // 128):
            if rc > 0:
                lo = w_v[blk]
                hi = w_v[blk + 1]
            w = pltpu.bitcast(jnp.concatenate([lo, hi], axis=1), BF)
            lhs = jnp.concatenate([h0buf[k, rc * 64:(rc + 1) * 64, :] for k in range(8)], axis=1)
            y = jnp.dot(pltpu.bitcast(lhs, BF), w, preferred_element_type=F32)
            store_qkv(i, jrow, y, rc * 4)
            extra(rc)

    def pre_body(j, carry):
        @pl.when(j == 1)
        def _():
            for jn in (3, 4):
                w_start(jn)
                mod_copy(jn).start()

        @pl.when(j == 2)
        def _():
            w_start(5)
            mod_copy(5).start()
            cp_wo.start()
            cp_x1.start()
        blk0 = (j // 3) * (6 * NB) + (j % 3) * 2
        one = jnp.where((j == 1) | (j == 4), 1.0, 0.0).astype(F32)
        for half, (i0, i1) in enumerate(((0, PRE_SPLIT), (PRE_SPLIT, NB))):
            with _scope('w_pre'):
                for i in range(i0, i1):
                    for par in range(2):
                        pltpu.make_async_copy(w_hbms[0].at[:, 0, 0, :],
                                              w_v.at[blk0 + i * 6 + par],
                                              wsems.at[2 * j + half]).wait()
            if half == 1:
                @pl.when(j > 1)
                def _():
                    pltpu.make_async_copy(wmod32.at[:, 0:D], wmod_v.at[j],
                                          wsems.at[2 * j + 1]).wait()
            for i in range(i0, i1):
                def extra(rc, i=i):
                    n = (i - PRE_SPLIT) * 2 + rc // 2
                    if i >= PRE_SPLIT and rc % 2 == 0 and n < 8:
                        modb[j, :, n * 128:(n + 1) * 128] = _rb(one + mod_tile(j, n * 128))
                pre_unit(j, i, extra)
        return carry
    lax.fori_loop(1, 6, pre_body, 0)

    cp_wo.wait()
    cp_x1.wait()
    for c_ in cp_ffn:
        c_.start()

    def wo_w(h0, h1, n0, n1):
        w = wo_v[h0:h1, :, n0 * 128:n1 * 128].reshape((h1 - h0) * (DH // 2), (n1 - n0) * 128)
        return pltpu.bitcast(w, BF)

    HD = D // 2

    def emit_step(s, pend, last):
        hrow = pl.multiple_of(HOFF + (s & 1) * 32, 32)
        hnext = pl.multiple_of(HOFF + 32 - (s & 1) * 32, 32)
        tv = [tab[s * NTAB + k] for k in range(14)]
        slot = tv[0]
        dsts = [(tv[1 + 2 * j], pl.multiple_of(tv[2 + 2 * j], 4)) for j in range(3)]
        odst = [pl.multiple_of(tv[7 + j], 8) for j in range(4)]
        orow = pl.multiple_of(tv[11], 32)
        erow = tv[12]
        lrow = tv[13]
        e_at, l_at = (E_AT, L_AT) if pend is None else (E_AT2, L_AT2)
        probs = {}

        def wqkv(p, k0, k1):
            return pltpu.bitcast(jnp.concatenate(
                [w_v[p * 6 + u, k0 // 2:k1 // 2, :] for u in range(6)], axis=1), BF)

        lhs_lo = act[pl.ds(hrow, 32), 0:HD]
        if pend is not None:
            ybuf[...] = jnp.dot(lhs_lo, wqkv(0, 0, HD), preferred_element_type=F32)
            pend()
        lhs_hi = act[pl.ds(hrow, 32), HD:D]
        if pend is not None:
            y0 = ybuf[...] + jnp.dot(lhs_hi, wqkv(0, HD, D), preferred_element_type=F32)
        lhs_rest = jnp.concatenate([lhs_lo[:, 128:], lhs_hi], axis=1)
        lhs = [jnp.concatenate([lhs_lo, lhs_hi], axis=1)]

        def side(p):
            for j in range(3):
                if e_at[j] == p:
                    finish_rows(pl.multiple_of(erow + 8 * j, 8), abuf[8 * j:8 * j + 8, :])
            for j in range(3):
                if l_at[j] == p:
                    ln1_rows(pl.multiple_of(lrow + 8 * j, 8),
                             pl.multiple_of(hnext + 8 + 8 * j, 8))
            if (p in e_at or p in l_at) and p < NP - 1:
                lhs[0] = jnp.concatenate([act[pl.ds(hrow, 32), 0:128], lhs_rest], axis=1)

        def qkv(p):
            if p == 0 and pend is not None:
                y = y0
            else:
                y = jnp.dot(lhs[0], wqkv(p, 0, D), preferred_element_type=F32)
            buf = qkvbufs[p % NB]
            for u in range(6):
                t, hh = u // 2, u % 2
                b0 = ((p // NB) * 3 + t) * 40
                yu = y[:, u * 128:(u + 1) * 128]
                buf[slot, b0 + hh * 4:b0 + hh * 4 + 4, :] = _pack(yu[0:8])
                for j in range(3):
                    sl, off = dsts[j]
                    buf[sl, pl.ds(b0 + 8 + hh * 16 + off, 4), :] = _pack(yu[8 + 8 * j:16 + 8 * j])

        def ld(p, t):
            b0 = ((p // NB) * 3 + t) * 40
            return pltpu.bitcast(qkvbufs[p % NB][slot, b0:b0 + 40, :], BF)

        def sc(p):
            s2 = lax.dot_general(ld(p, 0), ld(p, 1), (((1,), (1,)), ((), ())),
                                 preferred_element_type=F32) * SCALE
            s2 = jnp.where(valid, s2, fill)
            m = jnp.max(s2, axis=-1, keepdims=True)
            e = jnp.exp(s2 - m)
            l = jnp.sum(e, axis=-1, keepdims=True)
            rl = pl.reciprocal(l, approx=True)
            rl = rl * (2.0 - l * rl)
            probs[p] = (e * rl).astype(BF)

        def pv(p):
            o2 = jnp.dot(probs[p], ld(p, 2), preferred_element_type=F32)
            for hh in range(2):
                hcol = (2 * p + hh) * 128
                ob = obuf1
                if hcol >= KS:
                    ob = obuf2
                    hcol -= KS
                ob[pl.ds(orow, 8), hcol:hcol + 128] = o2[8 * hh:8 * hh + 8].astype(BF)
                for j in range(4):
                    r0 = 16 + 32 * hh + 8 * j
                    ob[pl.ds(odst[j], 8), hcol:hcol + 128] = o2[r0:r0 + 8].astype(BF)

        def attn(pos):
            for kind, p in ATT.get(pos, ()):
                (sc if kind == 's' else pv)(p)

        for p in range(NP):
            qkv(p)
            side(p)
            attn(p)
        a1 = []
        for i in range(4):
            a1.append(jnp.dot(obuf1[pl.ds(orow, 32), 0:KS], wo_w(0, KS // DH, 2 * i, 2 * i + 2),
                              preferred_element_type=F32))
            attn(NP + i)
            side(NP + i)
        o2lhs = obuf2[pl.ds(orow, 32), 0:K2]
        a_lo = jnp.concatenate(a1[0:2], axis=1) + jnp.dot(
            o2lhs, wo_w(KS // DH, H, 0, 4), preferred_element_type=F32)
        act[pl.ds(hnext, 8), 0:HD] = a_lo[0:8].astype(BF)
        abuf[:, 0:HD] = a_lo[8:32]
        a_hi = jnp.concatenate(a1[2:4], axis=1) + jnp.dot(
            o2lhs, wo_w(KS // DH, H, 4, 8), preferred_element_type=F32)

        def finish():
            act[pl.ds(hnext, 8), HD:D] = a_hi[0:8].astype(BF)
            abuf[:, HD:D] = a_hi[8:32]
        if last:
            finish()
        return finish

    def steps(it, carry):
        pend = None
        for u in range(UNR):
            pend = emit_step(it * UNR + u, pend, u == UNR - 1)
        return carry
    lax.fori_loop(0, NSEG // UNR, steps, 0)

    OUT0 = (NSEG - 1) * RIDE
    cp_out = [cp(act.at[OOFF:OOFF + OUT0], out_hbm.at[0, 0:OUT0], 9)]
    cp_out[0].start()
    zrow = pl.multiple_of(tab[14], 16)
    zero = pl.multiple_of(tab[15], 8)
    ebuf[EMAX:EMAX + RIDE, :] = abuf[...]
    todo = [(OUT0 + 8 * j, EMAX + 8 * j) for j in range(3)]
    r0 = 0
    nw = 8 // EPI_NSUB
    for ci, ech in enumerate(EPI_CHUNKS):
        o0 = NOSLOT * 32 + r0
        e0 = (ci % 2) * EMAX
        per = -(-len(todo) // (EPI_NSUB - EPI_SPARE))
        for n in range(EPI_NSUB):
            first = obuf1[o0:o0 + 16, 0:128]
            if n == 0 and ci > 0 and EPI_PIN:
                first = pltpu.bitcast(
                    pltpu.bitcast(first, U32) | pltpu.bitcast(act[pl.ds(zrow, 16), 0:128], U32), BF)
            col0 = jnp.concatenate([first, obuf1[o0 + 16:o0 + ech, 0:128]], axis=0)
            lhs = jnp.concatenate(
                [col0, obuf1[o0:o0 + ech, 128:KS], obuf2[o0:o0 + ech, 0:K2]], axis=1)
            ebuf[e0:e0 + ech, n * nw * 128:(n + 1) * nw * 128] = jnp.dot(
                lhs, wo_w(0, H, n * nw, (n + 1) * nw), preferred_element_type=F32)
            for row, er in todo[:per]:
                finish_rows(row, ebuf[pl.ds(zero + er, 8), :])
            todo = todo[per:]
        todo = [(OUT0 + RIDE + r0 + 8 * j, e0 + 8 * j) for j in range(ech // 8)]
        r0 += ech
    for row, er in todo:
        finish_rows(row, ebuf[er:er + 8, :])
    cp_out.append(cp(act.at[OOFF + OUT0:OOFF + S], out_hbm.at[0, OUT0:S], 10))
    cp_out[1].start()

    r_all = act[ROFF:ROFF + 8, 0:256].astype(F32)
    rows = lane256 * 8 + lax.broadcasted_iota(jnp.int32, (8, 256), 0)

    def allmax(v):
        return jnp.max(jnp.max(v, axis=1, keepdims=True), axis=0, keepdims=True)

    def allmin(v):
        return jnp.min(jnp.min(v, axis=1, keepdims=True), axis=0, keepdims=True)
    rowsf = rows.astype(F32)
    i1v = allmin(jnp.where(r_all == allmax(r_all), rowsf, float(S)))
    r_rest = jnp.where(rowsf == i1v, -jnp.inf, r_all)
    i2v = allmin(jnp.where((r_rest == allmax(r_rest)) & (rowsf != i1v), rowsf, float(S)))
    i1 = jnp.clip(i1v[0, 0].astype(jnp.int32), 0, S - 1)
    i2 = jnp.clip(i2v[0, 0].astype(jnp.int32), 0, S - 1)
    b1 = pl.multiple_of((i1 // 8) * 8, 8)
    b2 = pl.multiple_of((i2 // 8) * 8, 8)

    x1 = jnp.concatenate([act[pl.ds(b1, 8), :].astype(F32), act[pl.ds(b2, 8), :].astype(F32)],
                         axis=0)

    def two(i):
        return jnp.concatenate([modb[i], modb[i]], axis=0)
    h2 = _rb(_rb(_layernorm(x1) * two(4)) + two(3))
    rr = _rb(jnp.sum(h2 * two(6), axis=-1, keepdims=True))
    h2b = h2.astype(BF)
    for c_ in cp_ffn:
        c_.wait()
    gt = _rb(jnp.dot(h2b, pltpu.bitcast(wg_v[...], BF), preferred_element_type=F32))
    up = _rb(jnp.dot(h2b, pltpu.bitcast(wu_v[...], BF), preferred_element_type=F32))
    hid = (_rb(gt * _rb(jax.nn.sigmoid(gt))) * up).astype(BF)
    y = _rb(jnp.dot(hid, pltpu.bitcast(wd_v[...], BF), preferred_element_type=F32))
    y = _rb(y * _rb(jax.nn.sigmoid(rr)))
    sub = lax.broadcasted_iota(jnp.int32, (16, 1), 0)
    grow = jnp.where(sub < 8, b1 + sub, b2 + sub - 8)
    sel = (grow == i1) | (grow == i2)
    res = (x1 + _rb(two(5) * _rb(h2 + jnp.where(sel, y, 0.0)))).astype(BF)
    for c_ in cp_out:
        c_.wait()
    act[pl.ds(OOFF + b1, 8), :] = res[0:8]
    act[pl.ds(OOFF + b2, 8), :] = res[8:16]
    fix1 = cp(act.at[pl.ds(OOFF + b1, 8)], out_hbm.at[0, pl.ds(b1, 8)], 11)
    fix2 = cp(act.at[pl.ds(OOFF + b2, 8)], out_hbm.at[0, pl.ds(b2, 8)], 12)
    fix1.start()

    @pl.when(b1 != b2)
    def _():
        fix2.start()
        fix2.wait()
    fix1.wait()


@jax.jit
def pallas_adaLN_cond__memory_aug_recurrent_mem_tr__moe_arch_mod__prompt_kernel(
    A_x: jax.Array,
    A_mem0: jax.Array,
    A_Wq: jax.Array,
    A_Wk: jax.Array,
    A_Wv: jax.Array,
    A_Wo: jax.Array,
    A_seg_len,
    B_x: jax.Array,
    B_w_r: jax.Array,
    B_w_gate: jax.Array,
    B_w_up: jax.Array,
    B_w_down: jax.Array,
    c: jax.Array,
    w_mod: jax.Array,
):
    del B_x
    del A_seg_len
    assert A_x.shape == (1, S, D) and A_Wq.shape == (D, H, DH) and A_mem0.shape == (1, M, D)
    any_spec = pl.BlockSpec(memory_space=pl.ANY)
    scratch = [
        pltpu.VMEM((S if not XACT else 8, D), BF),
        pltpu.VMEM((XOFF + S * XACT, D), BF),
        pltpu.VMEM((8, PRE // 2, 128), U32),
        pltpu.VMEM((RIDE, D), F32),
        pltpu.VMEM((32, 768), F32),
        pltpu.VMEM((2 * EMAX, D), F32),
        pltpu.SMEM((NSEG * NTAB,), jnp.int32),
        pltpu.VMEM((7, 8, D), F32),
        pltpu.VMEM((4, 1, D), BF),
        pltpu.VMEM((3 * H, D // 2, 128), U32),
        pltpu.VMEM((H, DH // 2, D), U32),
        pltpu.VMEM((6, D // 2, D), U32),
        pltpu.VMEM((D // 2, F), U32),
        pltpu.VMEM((D // 2, F), U32),
        pltpu.VMEM((F // 2, D), U32),
        pltpu.VMEM((NOSLOT * 32 + PRE, OW1), BF),
        pltpu.VMEM((NOSLOT * 32 + PRE, OW2), BF),
        pltpu.SemaphoreType.DMA((17,)),
        pltpu.SemaphoreType.DMA((12,)),
        pltpu.SemaphoreType.DMA((16,)),
    ] + [pltpu.VMEM((NSLOT, 256, 128), U32) for _ in range(NB)] + [
        pltpu.VMEM((D,), BF),
    ]
    wq, wk, wv = (w.reshape(D // 2, 2, H, DH) for w in (A_Wq, A_Wk, A_Wv))
    return pl.pallas_call(
        _kernel,
        out_shape=jax.ShapeDtypeStruct((1, S, D), BF),
        in_specs=[any_spec] * 12,
        out_specs=any_spec,
        scratch_shapes=scratch,
        compiler_params=pltpu.CompilerParams(vmem_limit_bytes=120 * 1024 * 1024,
                                             disable_bounds_checks=True,
                                             disable_semaphore_checks=True),
    )(A_x, A_mem0, wq, wk, wv, A_Wo, B_w_r, B_w_gate, B_w_up, B_w_down,
      c, w_mod)
```

```python
import contextlib
import os
import jax
import jax.numpy as jnp
from jax import lax
import jax.experimental.pallas as pl
import jax.experimental.pallas.tpu as pltpu

BF = jnp.bfloat16
F32 = jnp.float32
U32 = jnp.uint32

S = 2048
D = 1024
H = 32
DH = 128
M = 8
SEG = 32
NSEG = S // SEG
F = 3584
NP = H // 2
RIDE = 24
PRE = S - NSEG * RIDE
NSLOT = 17
NOSLOT = 17
NB = int(os.environ.get('NB', 8))
KS = int(os.environ.get('KS', 2560))
LAG_S = 1
LAG_P = 3
EPS = 1e-5
SCALE = DH ** -0.5
OOFF = S
HOFF = 2 * S
ROFF = HOFF + 64
ZOFF = ROFF + 16
XOFF = ZOFF + 16
PRE_SPLIT = 3
E_AT = tuple(int(v) for v in os.environ.get('E_AT', '2,3,4').split(','))
L_AT = tuple(int(v) for v in os.environ.get('L_AT', '8,10,12').split(','))
E_AT2 = tuple(int(v) for v in os.environ.get('E_AT2', '2,3,4').split(','))
L_AT2 = tuple(int(v) for v in os.environ.get('L_AT2', '8,10,12').split(','))


def _att_schedule(mode):
    att = {}
    if mode == 'lag':
        for p in range(NP):
            att.setdefault(p + LAG_S, []).append(('s', p))
        for p in range(NP):
            att.setdefault(p + LAG_P, []).append(('p', p))
    elif mode == 'q2':
        for p in range(0, NP, 2):
            att.setdefault(p + 2, []).extend([('s', p), ('s', p + 1)])
        for p in range(0, NP, 2):
            att.setdefault(p + 4, []).extend([('p', p), ('p', p + 1)])
    elif mode == 'q2b':
        for p in range(0, NP, 2):
            att.setdefault(p + 4, []).extend([('p', p), ('p', p + 1)])
        for p in range(0, NP, 2):
            att.setdefault(p + 2, []).extend([('s', p), ('s', p + 1)])
    elif mode == 'q2c':
        att[4] = [('s', i) for i in range(4)]
        for p in range(4, NP, 2):
            att[p + 2] = [('s', p), ('s', p + 1), ('p', p - 4), ('p', p - 3)]
        att[18] = [('p', i) for i in range(12, 16)]
    elif mode == 'q2d':
        att[3] = [('s', i) for i in range(3)]
        att[4] = [('s', 3)]
        att[3] = []
        att[4] = [('s', i) for i in range(4)]
        for p in range(4, NP, 2):
            att[p + 2] = [('p', p - 4), ('p', p - 3), ('s', p), ('s', p + 1)]
        att[18] = [('p', i) for i in range(12, 16)]
    elif mode == 'q4':
        for p in range(0, NP, 4):
            att.setdefault(p + 4, []).extend([('s', p + i) for i in range(4)])
            att.setdefault(p + 6, []).extend([('p', p + i) for i in range(4)])
    elif mode == 'q4b':
        for p in range(0, NP, 4):
            att.setdefault(min(p + 8, 18), []).extend([('p', p + i) for i in range(4)])
        for p in range(0, NP, 4):
            att.setdefault(p + 4, []).extend([('s', p + i) for i in range(4)])
    return att


ATT = _att_schedule(os.environ.get('ATT', 'q2c'))
XACT = int(os.environ.get('XACT', 0))
K2 = H * DH - KS
OPAD = int(os.environ.get('OPAD', 1))
OW1 = -(-KS // 1024) * 1024 if OPAD else KS
OW2 = -(-K2 // 1024) * 1024 if OPAD else K2
SMX = int(os.environ.get('SMX', 0))
LOG2E = 1.4426950408889634
SKIP = int(os.environ.get('SKIP', 0))
A_BUF = tuple(int(v) for v in os.environ.get('A_BUF', '0,1,2').split(','))
ECOL = int(os.environ.get('ECOL', 0))
UNR = int(os.environ.get('UNR', 2))
EPI_CHUNKS = tuple(int(v) for v in os.environ.get('EPI', '64,64,64,64,64,64,48,48,32').split(','))
EMAX = max(EPI_CHUNKS)
EPI_PIN = int(os.environ.get('EPI_PIN', 0))
EPI_SPARE = int(os.environ.get('EPI_SPARE', 0))
EPI_NSUB = int(os.environ.get('EPI_NSUB', 8))


NTAB = 16


def _step_indices(s):
    t = [s % NSLOT]
    for j in range(3):
        gi = PRE // 8 + 3 * s + j
        t += [(gi // 4) % NSLOT, (gi % 4) * 4]
    for j in range(4):
        gi = 4 * s + j
        t.append(((gi // 3) % NOSLOT) * 32 + 8 + (gi % 3) * 8 if gi < 3 * NSEG
                 else NOSLOT * 32 + (gi - 3 * NSEG) * 8)
    t.append((s % NOSLOT) * 32)
    t.append(max(s - 1, 0) * RIDE)
    t.append(PRE + min(s + 1, NSEG - 1) * RIDE)
    t.append(max(s - 1, 0) * RIDE)
    return t


def _scope(name):
    return jax.named_scope(name) if os.environ.get('PROF') else contextlib.nullcontext()


def _rb(v):
    return v.astype(BF).astype(F32)


def _pack(v):
    return pltpu.bitcast(v.astype(BF), U32)


def _ln_stats(x):
    mu = jnp.sum(x, axis=-1, keepdims=True) * (1.0 / D)
    xc = x - mu
    var = jnp.sum(xc * xc, axis=-1, keepdims=True) * (1.0 / D)
    return _rb(mu), _rb(jnp.sqrt(_rb(_rb(var) + EPS)))


def _layernorm(x):
    mu, sd = _ln_stats(x)
    return _rb(_rb(x - mu) / sd)


def _kernel(x_hbm, mem0_hbm, wq_hbm, wk_hbm, wv_hbm, wo_hbm, wr_hbm, wg_hbm, wu_hbm,
            wd_hbm, c_hbm, wmod_hbm, out_hbm,
            xbuf, act, h0buf, ybuf, ebuf, tab, modb, small,
            w_v, wo_v, wmod_v, wg_v, wu_v, wd_v,
            obuf1, obuf2, sems, wsems, ksems, *rest):
    qkvbufs, wrbuf = rest[:NB], rest[NB]
    if XACT:
        xbuf = act.at[pl.ds(XOFF, S)]
    w_hbms = tuple(w.bitcast(U32) for w in (wq_hbm, wk_hbm, wv_hbm))

    def cp(src, dst, i):
        return pltpu.make_async_copy(src, dst, sems.at[i])

    wmod32 = wmod_hbm.bitcast(U32)
    cp_c = cp(c_hbm, small.at[0], 0)
    cp_mem = cp(mem0_hbm.at[0], act.at[HOFF:HOFF + M], 1)
    cp_wr = cp(wr_hbm, wrbuf, 2)
    cp_x0 = [cp(x_hbm.at[0, n * 128:(n + 1) * 128], xbuf.at[n * 128:(n + 1) * 128], 13 + n)
             for n in range(PRE // 128)]
    cp_xr = cp(x_hbm.at[0, PRE:PRE + 32], xbuf.at[PRE:PRE + 32], 5)
    cp_x1 = cp(x_hbm.at[0, PRE + 32:S], xbuf.at[PRE + 32:S], 4)
    cp_wo = cp(wo_hbm.bitcast(U32), wo_v, 7)
    cp_ffn = [cp(wg_hbm.bitcast(U32), wg_v, 8), cp(wu_hbm.bitcast(U32), wu_v, 8),
              cp(wd_hbm.bitcast(U32), wd_v, 8)]

    def w_start(j):
        gg, t = j // 3, j % 3
        for i in range(NB):
            for par in range(2):
                pltpu.make_async_copy(w_hbms[t].at[:, par, gg * NB + i, :],
                                      w_v.at[(gg * NB + i) * 6 + t * 2 + par],
                                      wsems.at[2 * j + (i >= PRE_SPLIT)]).start()

    def mod_copy(j):
        return pltpu.make_async_copy(wmod32.at[:, j * D:(j + 1) * D], wmod_v.at[j],
                                     wsems.at[2 * j + 1])

    def mult(v, m):
        return v if isinstance(v, int) else pl.multiple_of(v, m)

    def moda_copies(kc):
        col = mult(kc * 128, 128)
        return [pltpu.make_async_copy(wmod32.at[:, pl.ds(v * D + col, 128)],
                                      wmod_v.at[v, :, pl.ds(col, 128)], ksems.at[8 + kc])
                for v in range(2)]

    def chunk_copies(kc):
        r0 = mult(kc * 64, 64)
        return [pltpu.make_async_copy(w_hbms[0].at[pl.ds(r0, 64), par, i, :],
                                      w_v.at[i * 6 + par, pl.ds(r0, 64), :], ksems.at[kc])
                for i in range(NB) for par in range(2)]

    cp_c.start()
    cp_mem.start()
    cp_wr.start()
    for c_ in (cp_x0 + moda_copies(0) + moda_copies(1) + chunk_copies(0) + moda_copies(2)
               + chunk_copies(1) + [cp_xr] + chunk_copies(2)):
        c_.start()

    def ln1_rows(src_row, dst_row):
        xv = xbuf[pl.ds(src_row, 8), :].astype(F32)
        hv = _rb(_layernorm(xv) * modb[1]) + modb[0]
        act[pl.ds(dst_row, 8), :] = hv.astype(BF)

    lane256 = lax.broadcasted_iota(jnp.int32, (8, 256), 1)

    def finish_rows(row, attn, row2=None):
        xv = xbuf[pl.ds(row, 8), :].astype(F32)
        x1 = _rb(xv + _rb(modb[2] * _rb(attn)))
        act[pl.ds(row, 8), :] = x1.astype(BF)
        if row2 is None:
            h2 = _rb(_rb(_layernorm(x1) * modb[4]) + modb[3])
            act[pl.ds(OOFF + row, 8), :] = (x1 + _rb(modb[5] * h2)).astype(BF)
            hw = h2 * modb[6]
        else:
            mu, sd = _ln_stats(x1)
            hw = None
            for c0 in range(0, D, ECOL):
                cs = slice(c0, c0 + ECOL)
                xb = act[pl.ds(row2, 8), cs].astype(F32)
                h2 = _rb(_rb(_rb(_rb(xb - mu) / sd) * modb[4, :, cs]) + modb[3, :, cs])
                act[pl.ds(OOFF + row, 8), cs] = (xb + _rb(modb[5, :, cs] * h2)).astype(BF)
                t = h2 * modb[6, :, cs]
                hw = t if hw is None else hw + t
        r = jnp.sum(hw, axis=-1, keepdims=True)
        act[ROFF:ROFF + 8, 0:256] = jnp.where(
            lane256 * 8 == row, r, act[ROFF:ROFF + 8, 0:256].astype(F32)).astype(BF)

    def attn_store(a, k0):
        for j in range(3):
            for k in range(a.shape[1] // 128):
                qkvbufs[A_BUF[j]][NSLOT, (k0 + k) * 8:(k0 + k + 1) * 8, :] = pltpu.bitcast(
                    a[8 * j:8 * j + 8, k * 128:(k + 1) * 128], U32)

    def attn_load(j):
        return pltpu.bitcast(jnp.concatenate(
            [qkvbufs[A_BUF[j]][NSLOT, k * 8:(k + 1) * 8, :] for k in range(8)], axis=1), F32)

    act[ROFF:ROFF + 8, 0:256] = jnp.zeros((8, 256), BF)
    act[ZOFF:ZOFF + 16, 0:128] = jnp.zeros((16, 128), BF)
    tab[31] = ZOFF
    tab[15] = 0
    attn_store(jnp.zeros((RIDE, D), F32), 0)
    for s_ in range(NSEG):
        for k, v in enumerate(_step_indices(s_)):
            tab[s_ * NTAB + k] = v
    ri = lax.broadcasted_iota(jnp.int32, (80, 80), 0)
    ci = lax.broadcasted_iota(jnp.int32, (80, 80), 1)

    def head_pos(i):
        hd = jnp.where(i < 16, i // 8, (i - 16) // 32)
        pos = jnp.where(i < 16, i % 8, 8 + (i - 16) % 32)
        return hd, pos
    rh, rp = head_pos(ri)
    ch, cpos = head_pos(ci)
    same = rh == ch
    valid = same & ((rp < M) | (rp >= cpos))
    fill = jnp.where(same, -1e9, -jnp.inf).astype(F32)

    cp_mem.wait()
    cp_wr.wait()
    modb[6] = jnp.broadcast_to(wrbuf[...].astype(F32).reshape(1, D), (8, D))
    cp_c.wait()
    cv = small[0].astype(F32)
    sc16 = jnp.broadcast_to(_rb(cv * _rb(jax.nn.sigmoid(cv))), (16, D)).astype(BF)

    def ln_pre(g, carry):
        pltpu.make_async_copy(x_hbm.at[0, 0:128], xbuf.at[pl.ds(pl.multiple_of(g * 128, 128), 128)],
                              sems.at[13 + g]).wait()
        for u in range(2):
            row = pl.multiple_of(g * 128 + u * 64, 64)
            nv = _layernorm(xbuf[pl.ds(row, 64), :].astype(F32)).astype(BF)
            for k in range(8):
                h0buf[k, pl.ds(pl.multiple_of(row // 2, 32), 32), :] = pltpu.bitcast(
                    nv[:, k * 128:(k + 1) * 128], U32)
            wg_v[pl.ds(row, 64), 0:2 * D] = jnp.zeros((64, 2 * D), U32)
        return carry
    lax.fori_loop(0, PRE // 128, ln_pre, 0)

    def mod_tile(v, col):
        w = pltpu.bitcast(wmod_v[v, :, pl.ds(col, 128)], BF)
        return _rb(jnp.dot(sc16, w, preferred_element_type=F32))[0:8]

    def moda_store(kc, sa, ca):
        col = mult(kc * 128, 128)
        c1 = _rb(1.0 + ca)
        modb[0, :, pl.ds(col, 128)] = sa
        modb[1, :, pl.ds(col, 128)] = c1
        return sa, c1

    def moda_apply(kc, sa, c1, r0, r1):
        for r in range(r0, r1, 16):
            nv = pltpu.bitcast(h0buf[kc, r // 2:r // 2 + 8, :], BF).astype(F32).reshape(2, 8, 128)
            hv = (_rb(nv * c1[None]) + sa[None]).reshape(16, 128).astype(BF)
            h0buf[kc, r // 2:r // 2 + 8, :] = pltpu.bitcast(hv, U32)

    def repack(a, b):
        return (a & U32(0xFFFF)) | (b << 16), (a >> 16) | (b & U32(0xFFFF0000))

    def store_qkv(i, jrow, y, seg0):
        for sg in range(y.shape[0] // 32):
            for hh in range(2):
                qkvbufs[i][seg0 + sg, pl.ds(jrow + 8 + hh * 16, 16), :] = _pack(
                    y[sg * 32:(sg + 1) * 32, hh * 128:(hh + 1) * 128])

    for c_ in moda_copies(0):
        c_.wait()
    moda_apply(0, *moda_store(0, mod_tile(0, 0), mod_tile(1, 0)), 0, PRE)

    def chunk_block(kc, last, issue):
        with _scope('w_chunk'):
            for c_ in chunk_copies(kc) + ([cp_xr] if last else moda_copies(kc + 1)):
                c_.wait()
        issue()
        r0 = mult(kc * 64, 64)
        mv = []
        for i in range(NB):
            lo, hi = repack(w_v[i * 6, pl.ds(r0, 64), :], w_v[i * 6 + 1, pl.ds(r0, 64), :])
            w_v[i * 6, pl.ds(r0, 64), :] = lo
            w_v[i * 6 + 1, pl.ds(r0, 64), :] = hi
            w = pltpu.bitcast(jnp.concatenate([lo, hi], axis=1), BF)
            y = (pltpu.bitcast(wg_v[0:PRE, i * 256:(i + 1) * 256], F32)
                 + jnp.dot(pltpu.bitcast(h0buf[kc], BF), w, preferred_element_type=F32))
            if last:
                store_qkv(i, 0, y, 0)
            else:
                wg_v[0:PRE, i * 256:(i + 1) * 256] = pltpu.bitcast(y, U32)
                if i in (1, 3):
                    mv.append(mod_tile(i // 2, mult((kc + 1) * 128, 128)))
                if i == 3:
                    mv = moda_store(kc + 1, mv[0], mv[1])
                if i >= 4:
                    moda_apply(kc + 1, mv[0], mv[1], (i - 4) * 128, (i - 3) * 128)
        if last:
            for j in range(3):
                ln1_rows(PRE + 8 * j, HOFF + 8 + 8 * j)

    def chunk_body_a(kc, carry):
        def issue():
            for c_ in moda_copies(kc + 3) + chunk_copies(kc + 3):
                c_.start()
        chunk_block(kc, False, issue)
        return carry

    def chunk_body_b(kc, carry):
        chunk_block(kc, False, lambda: None)
        return carry

    def issue_last():
        w_start(2)
        mod_copy(2).start()
    lax.fori_loop(0, 5, chunk_body_a, 0)
    w_start(1)
    lax.fori_loop(5, 7, chunk_body_b, 0)
    chunk_block(7, True, issue_last)

    def pre_unit(j, i, extra):
        blk = (j // 3) * (6 * NB) + (j % 3) * 2 + i * 6
        jrow = pl.multiple_of(j * 40, 8)
        lo, hi = repack(w_v[blk], w_v[blk + 1])
        w_v[blk] = lo
        w_v[blk + 1] = hi
        for rc in range(PRE // 128):
            if rc > 0:
                lo = w_v[blk]
                hi = w_v[blk + 1]
            w = pltpu.bitcast(jnp.concatenate([lo, hi], axis=1), BF)
            lhs = jnp.concatenate([h0buf[k, rc * 64:(rc + 1) * 64, :] for k in range(8)], axis=1)
            y = jnp.dot(pltpu.bitcast(lhs, BF), w, preferred_element_type=F32)
            store_qkv(i, jrow, y, rc * 4)
            extra(rc)

    def pre_body(j, carry):
        @pl.when(j == 1)
        def _():
            for jn in (3, 4):
                w_start(jn)
                mod_copy(jn).start()

        @pl.when(j == 2)
        def _():
            w_start(5)
            mod_copy(5).start()
            cp_wo.start()
            cp_x1.start()
        blk0 = (j // 3) * (6 * NB) + (j % 3) * 2
        one = jnp.where((j == 1) | (j == 4), 1.0, 0.0).astype(F32)
        for half, (i0, i1) in enumerate(((0, PRE_SPLIT), (PRE_SPLIT, NB))):
            with _scope('w_pre'):
                for i in range(i0, i1):
                    for par in range(2):
                        pltpu.make_async_copy(w_hbms[0].at[:, 0, 0, :],
                                              w_v.at[blk0 + i * 6 + par],
                                              wsems.at[2 * j + half]).wait()
            if half == 1:
                @pl.when(j > 1)
                def _():
                    pltpu.make_async_copy(wmod32.at[:, 0:D], wmod_v.at[j],
                                          wsems.at[2 * j + 1]).wait()
            for i in range(i0, i1):
                def extra(rc, i=i):
                    n = (i - PRE_SPLIT) * 2 + rc // 2
                    if i >= PRE_SPLIT and rc % 2 == 0 and n < 8:
                        modb[j, :, n * 128:(n + 1) * 128] = _rb(one + mod_tile(j, n * 128))
                pre_unit(j, i, extra)
        return carry
    lax.fori_loop(1, 6, pre_body, 0)

    cp_wo.wait()
    cp_x1.wait()
    for c_ in cp_ffn:
        c_.start()

    def wo_w(h0, h1, n0, n1):
        w = wo_v[h0:h1, :, n0 * 128:n1 * 128].reshape((h1 - h0) * (DH // 2), (n1 - n0) * 128)
        return pltpu.bitcast(w, BF)

    HD = D // 2

    def emit_step(s, pend, last):
        hrow = pl.multiple_of(HOFF + (s & 1) * 32, 32)
        hnext = pl.multiple_of(HOFF + 32 - (s & 1) * 32, 32)
        tv = [tab[s * NTAB + k] for k in range(15)]
        slot = tv[0]
        dsts = [(tv[1 + 2 * j], pl.multiple_of(tv[2 + 2 * j], 4)) for j in range(3)]
        odst = [pl.multiple_of(tv[7 + j], 8) for j in range(4)]
        orow = pl.multiple_of(tv[11], 32)
        erow = tv[12]
        lrow = tv[13]
        erow2 = tv[14]
        e_at, l_at = (E_AT, L_AT) if pend is None else (E_AT2, L_AT2)
        probs = {}

        def wqkv(p, k0, k1):
            return pltpu.bitcast(jnp.concatenate(
                [w_v[p * 6 + u, k0 // 2:k1 // 2, :] for u in range(6)], axis=1), BF)

        lhs_lo = act[pl.ds(hrow, 32), 0:HD]
        if pend is not None:
            ybuf[...] = jnp.dot(lhs_lo, wqkv(0, 0, HD), preferred_element_type=F32)
            pend()
        lhs_hi = act[pl.ds(hrow, 32), HD:D]
        if pend is not None:
            y0 = ybuf[...] + jnp.dot(lhs_hi, wqkv(0, HD, D), preferred_element_type=F32)
        lhs_rest = jnp.concatenate([lhs_lo[:, 128:], lhs_hi], axis=1)
        lhs = [jnp.concatenate([lhs_lo, lhs_hi], axis=1)]

        def side(p):
            for j in range(3):
                if e_at[j] == p:
                    finish_rows(pl.multiple_of(erow + 8 * j, 8), attn_load(j),
                                pl.multiple_of(erow2 + 8 * j, 8) if ECOL else None)
            for j in range(3):
                if l_at[j] == p:
                    ln1_rows(pl.multiple_of(lrow + 8 * j, 8),
                             pl.multiple_of(hnext + 8 + 8 * j, 8))
            if (p in e_at or p in l_at) and p < NP - 1:
                lhs[0] = jnp.concatenate([act[pl.ds(hrow, 32), 0:128], lhs_rest], axis=1)

        def qkv(p):
            if p == 0 and pend is not None:
                y = y0
            else:
                y = jnp.dot(lhs[0], wqkv(p, 0, D), preferred_element_type=F32)
            buf = qkvbufs[p % NB]
            for u in range(6):
                t, hh = u // 2, u % 2
                b0 = ((p // NB) * 3 + t) * 40
                yu = y[:, u * 128:(u + 1) * 128]
                buf[slot, b0 + hh * 4:b0 + hh * 4 + 4, :] = _pack(yu[0:8])
                for j in range(3):
                    sl, off = dsts[j]
                    buf[sl, pl.ds(b0 + 8 + hh * 16 + off, 4), :] = _pack(yu[8 + 8 * j:16 + 8 * j])

        def ld(p, t):
            b0 = ((p // NB) * 3 + t) * 40
            return pltpu.bitcast(qkvbufs[p % NB][slot, b0:b0 + 40, :], BF)

        def sc(p):
            s2 = lax.dot_general(ld(p, 0), ld(p, 1), (((1,), (1,)), ((), ())),
                                 preferred_element_type=F32)
            if SMX == 0:
                s2 = jnp.where(valid, s2 * SCALE, fill)
                m = jnp.max(s2, axis=-1, keepdims=True)
                e = jnp.exp(s2 - m)
            else:
                s2 = jnp.where(valid, s2, fill * (1.0 / SCALE))
                m = jnp.max(s2, axis=-1, keepdims=True)
                e = jnp.exp2((s2 - m) * (SCALE * LOG2E))
            l = jnp.sum(e, axis=-1, keepdims=True)
            rl = pl.reciprocal(l, approx=True)
            rl = rl * (2.0 - l * rl)
            probs[p] = (e * rl).astype(BF)

        def pv(p):
            o2 = jnp.dot(probs[p], ld(p, 2), preferred_element_type=F32)
            for hh in range(2):
                hcol = (2 * p + hh) * 128
                ob = obuf1
                if hcol >= KS:
                    ob = obuf2
                    hcol -= KS
                ob[pl.ds(orow, 8), hcol:hcol + 128] = o2[8 * hh:8 * hh + 8].astype(BF)
                for j in range(4):
                    r0 = 16 + 32 * hh + 8 * j
                    ob[pl.ds(odst[j], 8), hcol:hcol + 128] = o2[r0:r0 + 8].astype(BF)

        def attn(pos):
            for kind, p in ATT.get(pos, ()):
                (sc if kind == 's' else pv)(p)

        for p in range(NP):
            qkv(p)
            side(p)
            attn(p)
        a1 = []
        for i in range(4):
            a1.append(jnp.dot(obuf1[pl.ds(orow, 32), 0:KS], wo_w(0, KS // DH, 2 * i, 2 * i + 2),
                              preferred_element_type=F32))
            attn(NP + i)
            side(NP + i)
        o2lhs = obuf2[pl.ds(orow, 32), 0:K2]
        a_lo = jnp.concatenate(a1[0:2], axis=1) + jnp.dot(
            o2lhs, wo_w(KS // DH, H, 0, 4), preferred_element_type=F32)
        act[pl.ds(hnext, 8), 0:HD] = a_lo[0:8].astype(BF)
        attn_store(a_lo[8:32], 0)
        a_hi = jnp.concatenate(a1[2:4], axis=1) + jnp.dot(
            o2lhs, wo_w(KS // DH, H, 4, 8), preferred_element_type=F32)

        def finish():
            act[pl.ds(hnext, 8), HD:D] = a_hi[0:8].astype(BF)
            attn_store(a_hi[8:32], 4)
        if last:
            finish()
        return finish

    def steps(it, carry):
        pend = None
        for u in range(UNR):
            pend = emit_step(it * UNR + u, pend, u == UNR - 1)
        return carry
    lax.fori_loop(0, NSEG // UNR, steps, 0)

    if SKIP:
        return
    OUT0 = (NSEG - 1) * RIDE
    cp_out = [cp(act.at[OOFF:OOFF + OUT0], out_hbm.at[0, 0:OUT0], 9)]
    cp_out[0].start()
    zrow = pl.multiple_of(tab[31], 16)
    zero = pl.multiple_of(tab[15], 8)
    for j in range(3):
        ebuf[EMAX + 8 * j:EMAX + 8 * j + 8, :] = attn_load(j)
    todo = [(OUT0 + 8 * j, EMAX + 8 * j) for j in range(3)]
    r0 = 0
    nw = 8 // EPI_NSUB
    for ci, ech in enumerate(EPI_CHUNKS):
        o0 = NOSLOT * 32 + r0
        e0 = (ci % 2) * EMAX
        per = -(-len(todo) // (EPI_NSUB - EPI_SPARE))
        for n in range(EPI_NSUB):
            first = obuf1[o0:o0 + 16, 0:128]
            if n == 0 and ci > 0 and EPI_PIN:
                first = pltpu.bitcast(
                    pltpu.bitcast(first, U32) | pltpu.bitcast(act[pl.ds(zrow, 16), 0:128], U32), BF)
            col0 = jnp.concatenate([first, obuf1[o0 + 16:o0 + ech, 0:128]], axis=0)
            lhs = jnp.concatenate(
                [col0, obuf1[o0:o0 + ech, 128:KS], obuf2[o0:o0 + ech, 0:K2]], axis=1)
            ebuf[e0:e0 + ech, n * nw * 128:(n + 1) * nw * 128] = jnp.dot(
                lhs, wo_w(0, H, n * nw, (n + 1) * nw), preferred_element_type=F32)
            for row, er in todo[:per]:
                finish_rows(row, ebuf[pl.ds(zero + er, 8), :])
            todo = todo[per:]
        todo = [(OUT0 + RIDE + r0 + 8 * j, e0 + 8 * j) for j in range(ech // 8)]
        r0 += ech
    for row, er in todo:
        finish_rows(row, ebuf[er:er + 8, :])
    cp_out.append(cp(act.at[OOFF + OUT0:OOFF + S], out_hbm.at[0, OUT0:S], 10))
    cp_out[1].start()

    r_all = act[ROFF:ROFF + 8, 0:256].astype(F32)
    rows = lane256 * 8 + lax.broadcasted_iota(jnp.int32, (8, 256), 0)

    def allmax(v):
        return jnp.max(jnp.max(v, axis=1, keepdims=True), axis=0, keepdims=True)

    def allmin(v):
        return jnp.min(jnp.min(v, axis=1, keepdims=True), axis=0, keepdims=True)
    rowsf = rows.astype(F32)
    i1v = allmin(jnp.where(r_all == allmax(r_all), rowsf, float(S)))
    r_rest = jnp.where(rowsf == i1v, -jnp.inf, r_all)
    i2v = allmin(jnp.where((r_rest == allmax(r_rest)) & (rowsf != i1v), rowsf, float(S)))
    i1 = jnp.clip(i1v[0, 0].astype(jnp.int32), 0, S - 1)
    i2 = jnp.clip(i2v[0, 0].astype(jnp.int32), 0, S - 1)
    b1 = pl.multiple_of((i1 // 8) * 8, 8)
    b2 = pl.multiple_of((i2 // 8) * 8, 8)

    x1 = jnp.concatenate([act[pl.ds(b1, 8), :].astype(F32), act[pl.ds(b2, 8), :].astype(F32)],
                         axis=0)

    def two(i):
        return jnp.concatenate([modb[i], modb[i]], axis=0)
    h2 = _rb(_rb(_layernorm(x1) * two(4)) + two(3))
    rr = _rb(jnp.sum(h2 * two(6), axis=-1, keepdims=True))
    h2b = h2.astype(BF)
    for c_ in cp_ffn:
        c_.wait()
    gt = _rb(jnp.dot(h2b, pltpu.bitcast(wg_v[...], BF), preferred_element_type=F32))
    up = _rb(jnp.dot(h2b, pltpu.bitcast(wu_v[...], BF), preferred_element_type=F32))
    hid = (_rb(gt * _rb(jax.nn.sigmoid(gt))) * up).astype(BF)
    y = _rb(jnp.dot(hid, pltpu.bitcast(wd_v[...], BF), preferred_element_type=F32))
    y = _rb(y * _rb(jax.nn.sigmoid(rr)))
    sub = lax.broadcasted_iota(jnp.int32, (16, 1), 0)
    grow = jnp.where(sub < 8, b1 + sub, b2 + sub - 8)
    sel = (grow == i1) | (grow == i2)
    res = (x1 + _rb(two(5) * _rb(h2 + jnp.where(sel, y, 0.0)))).astype(BF)
    for c_ in cp_out:
        c_.wait()
    act[pl.ds(OOFF + b1, 8), :] = res[0:8]
    act[pl.ds(OOFF + b2, 8), :] = res[8:16]
    fix1 = cp(act.at[pl.ds(OOFF + b1, 8)], out_hbm.at[0, pl.ds(b1, 8)], 11)
    fix2 = cp(act.at[pl.ds(OOFF + b2, 8)], out_hbm.at[0, pl.ds(b2, 8)], 12)
    fix1.start()

    @pl.when(b1 != b2)
    def _():
        fix2.start()
        fix2.wait()
    fix1.wait()


@jax.jit
def pallas_adaLN_cond__memory_aug_recurrent_mem_tr__moe_arch_mod__prompt_kernel(
    A_x: jax.Array,
    A_mem0: jax.Array,
    A_Wq: jax.Array,
    A_Wk: jax.Array,
    A_Wv: jax.Array,
    A_Wo: jax.Array,
    A_seg_len,
    B_x: jax.Array,
    B_w_r: jax.Array,
    B_w_gate: jax.Array,
    B_w_up: jax.Array,
    B_w_down: jax.Array,
    c: jax.Array,
    w_mod: jax.Array,
):
    del B_x
    del A_seg_len
    assert A_x.shape == (1, S, D) and A_Wq.shape == (D, H, DH) and A_mem0.shape == (1, M, D)
    any_spec = pl.BlockSpec(memory_space=pl.ANY)
    scratch = [
        pltpu.VMEM((S if not XACT else 8, D), BF),
        pltpu.VMEM((XOFF + S * XACT, D), BF),
        pltpu.VMEM((8, PRE // 2, 128), U32),
        pltpu.VMEM((32, 768), F32),
        pltpu.VMEM((2 * EMAX, D), F32),
        pltpu.SMEM((NSEG * NTAB,), jnp.int32),
        pltpu.VMEM((7, 8, D), F32),
        pltpu.VMEM((4, 1, D), BF),
        pltpu.VMEM((3 * H, D // 2, 128), U32),
        pltpu.VMEM((H, DH // 2, D), U32),
        pltpu.VMEM((6, D // 2, D), U32),
        pltpu.VMEM((D // 2, F), U32),
        pltpu.VMEM((D // 2, F), U32),
        pltpu.VMEM((F // 2, D), U32),
        pltpu.VMEM((NOSLOT * 32 + PRE, OW1), BF),
        pltpu.VMEM((NOSLOT * 32 + PRE, OW2), BF),
        pltpu.SemaphoreType.DMA((17,)),
        pltpu.SemaphoreType.DMA((12,)),
        pltpu.SemaphoreType.DMA((16,)),
    ] + [pltpu.VMEM((NSLOT + 1, 256, 128), U32) for _ in range(NB)] + [
        pltpu.VMEM((D,), BF),
    ]
    wq, wk, wv = (w.reshape(D // 2, 2, H, DH) for w in (A_Wq, A_Wk, A_Wv))
    return pl.pallas_call(
        _kernel,
        out_shape=jax.ShapeDtypeStruct((1, S, D), BF),
        in_specs=[any_spec] * 12,
        out_specs=any_spec,
        scratch_shapes=scratch,
        compiler_params=pltpu.CompilerParams(vmem_limit_bytes=120 * 1024 * 1024,
                                             disable_bounds_checks=True,
                                             disable_semaphore_checks=True),
    )(A_x, A_mem0, wq, wk, wv, A_Wo, B_w_r, B_w_gate, B_w_up, B_w_down,
      c, w_mod)
```

```python
import contextlib
import os
import jax
import jax.numpy as jnp
from jax import lax
import jax.experimental.pallas as pl
import jax.experimental.pallas.tpu as pltpu

BF = jnp.bfloat16
F32 = jnp.float32
U32 = jnp.uint32

S = 2048
D = 1024
H = 32
DH = 128
M = 8
SEG = 32
NSEG = S // SEG
F = 3584
NP = H // 2
RIDE = 24
PRE = S - NSEG * RIDE
NSLOT = 17
NOSLOT = 17
NB = int(os.environ.get('NB', 8))
KS = int(os.environ.get('KS', 2560))
LAG_S = 1
LAG_P = 3
EPS = 1e-5
SCALE = DH ** -0.5
OOFF = S
HOFF = 2 * S
ROFF = HOFF + 64
XOFF = ROFF + 16
PRE_SPLIT = 3
E_AT = tuple(int(v) for v in os.environ.get('E_AT', '2,3,4').split(','))
L_AT = tuple(int(v) for v in os.environ.get('L_AT', '8,10,12').split(','))
E_AT2 = tuple(int(v) for v in os.environ.get('E_AT2', '2,3,4').split(','))
L_AT2 = tuple(int(v) for v in os.environ.get('L_AT2', '8,10,12').split(','))


def _att_schedule(mode):
    att = {}
    if mode == 'lag':
        for p in range(NP):
            att.setdefault(p + LAG_S, []).append(('s', p))
        for p in range(NP):
            att.setdefault(p + LAG_P, []).append(('p', p))
    elif mode == 'q2':
        for p in range(0, NP, 2):
            att.setdefault(p + 2, []).extend([('s', p), ('s', p + 1)])
        for p in range(0, NP, 2):
            att.setdefault(p + 4, []).extend([('p', p), ('p', p + 1)])
    elif mode == 'q2b':
        for p in range(0, NP, 2):
            att.setdefault(p + 4, []).extend([('p', p), ('p', p + 1)])
        for p in range(0, NP, 2):
            att.setdefault(p + 2, []).extend([('s', p), ('s', p + 1)])
    elif mode == 'q2c':
        att[4] = [('s', i) for i in range(4)]
        for p in range(4, NP, 2):
            att[p + 2] = [('s', p), ('s', p + 1), ('p', p - 4), ('p', p - 3)]
        att[18] = [('p', i) for i in range(12, 16)]
    elif mode == 'q2d':
        att[3] = [('s', i) for i in range(3)]
        att[4] = [('s', 3)]
        att[3] = []
        att[4] = [('s', i) for i in range(4)]
        for p in range(4, NP, 2):
            att[p + 2] = [('p', p - 4), ('p', p - 3), ('s', p), ('s', p + 1)]
        att[18] = [('p', i) for i in range(12, 16)]
    elif mode == 'q4':
        for p in range(0, NP, 4):
            att.setdefault(p + 4, []).extend([('s', p + i) for i in range(4)])
            att.setdefault(p + 6, []).extend([('p', p + i) for i in range(4)])
    elif mode == 'q4b':
        for p in range(0, NP, 4):
            att.setdefault(min(p + 8, 18), []).extend([('p', p + i) for i in range(4)])
        for p in range(0, NP, 4):
            att.setdefault(p + 4, []).extend([('s', p + i) for i in range(4)])
    return att


ATT = _att_schedule(os.environ.get('ATT', 'q2c'))
XACT = int(os.environ.get('XACT', 0))
K2 = H * DH - KS
OPAD = int(os.environ.get('OPAD', 1))
OW1 = -(-KS // 1024) * 1024 if OPAD else KS
OW2 = -(-K2 // 1024) * 1024 if OPAD else K2
SMX = int(os.environ.get('SMX', 0))
LOG2E = 1.4426950408889634
SKIP = int(os.environ.get('SKIP', 0))
A_BUF = tuple(int(v) for v in os.environ.get('A_BUF', '0,1,2').split(','))
ECOL = int(os.environ.get('ECOL', 0))
UNR = int(os.environ.get('UNR', 2))
EPI_CHUNKS = tuple(int(v) for v in os.environ.get('EPI', '64,64,64,64,64,64,64,32,32').split(','))
EMAX = max(EPI_CHUNKS)
NEW = 24
EPI_LASTPER = int(os.environ.get('EPI_LASTPER', 2))
FFN_NB = int(os.environ.get('FFN_NB', 512))


NTAB = 16


def _step_indices(s):
    t = [s % NSLOT]
    for j in range(3):
        gi = PRE // 8 + 3 * s + j
        t += [(gi // 4) % NSLOT, (gi % 4) * 4]
    for j in range(4):
        gi = 4 * s + j
        if gi < 3 * NSEG:
            t.append(((gi // 3) % NOSLOT) * 32 + 8 + (gi % 3) * 8)
        elif gi == 3 * NSEG:
            t.append(((NSEG - 1) % NOSLOT) * 32)
        else:
            t.append(NOSLOT * 32 + (gi - 3 * NSEG - 1) * 8)
    t.append((s % NOSLOT) * 32)
    t.append(max(s - 1, 0) * RIDE)
    t.append(PRE + min(s + 1, NSEG - 1) * RIDE)
    t.append(max(s - 1, 0) * RIDE)
    t.append((s % NOSLOT) * 32 if s < NSEG - 1 else NOSLOT * 32 + PRE - 8)
    return t


def _scope(name):
    return jax.named_scope(name) if os.environ.get('PROF') else contextlib.nullcontext()


def _rb(v):
    return v.astype(BF).astype(F32)


def _pack(v):
    return pltpu.bitcast(v.astype(BF), U32)


def _ln_stats(x):
    mu = jnp.sum(x, axis=-1, keepdims=True) * (1.0 / D)
    xc = x - mu
    var = jnp.sum(xc * xc, axis=-1, keepdims=True) * (1.0 / D)
    return _rb(mu), _rb(jnp.sqrt(_rb(_rb(var) + EPS)))


def _layernorm(x):
    mu, sd = _ln_stats(x)
    return _rb(_rb(x - mu) / sd)


def _kernel(x_hbm, mem0_hbm, wq_hbm, wk_hbm, wv_hbm, wo_hbm, wr_hbm, wg_hbm, wu_hbm,
            wd_hbm, c_hbm, wmod_hbm, out_hbm,
            xbuf, act, h0buf, ybuf, ebuf, tab, modb, small,
            w_v, wo_v, wmod_v, wg_v, wu_v, wd_v,
            obuf1, obuf2, sems, wsems, ksems, *rest):
    qkvbufs, wrbuf = rest[:NB], rest[NB]
    if XACT:
        xbuf = act.at[pl.ds(XOFF, S)]
    w_hbms = tuple(w.bitcast(U32) for w in (wq_hbm, wk_hbm, wv_hbm))

    def cp(src, dst, i):
        return pltpu.make_async_copy(src, dst, sems.at[i])

    wmod32 = wmod_hbm.bitcast(U32)
    cp_c = cp(c_hbm, small.at[0], 0)
    cp_mem = cp(mem0_hbm.at[0], act.at[HOFF:HOFF + M], 1)
    cp_wr = cp(wr_hbm, wrbuf, 2)
    cp_x0 = [cp(x_hbm.at[0, n * 128:(n + 1) * 128], xbuf.at[n * 128:(n + 1) * 128], 13 + n)
             for n in range(PRE // 128)]
    cp_xr = cp(x_hbm.at[0, PRE:PRE + 32], xbuf.at[PRE:PRE + 32], 5)
    cp_x1 = cp(x_hbm.at[0, PRE + 32:S], xbuf.at[PRE + 32:S], 4)
    cp_wo = cp(wo_hbm.bitcast(U32), wo_v, 7)
    cp_ffn = [cp(wg_hbm.bitcast(U32), wg_v, 8), cp(wu_hbm.bitcast(U32), wu_v, 8),
              cp(wd_hbm.bitcast(U32), wd_v, 8)]

    def w_start(j):
        gg, t = j // 3, j % 3
        for i in range(NB):
            for par in range(2):
                pltpu.make_async_copy(w_hbms[t].at[:, par, gg * NB + i, :],
                                      w_v.at[(gg * NB + i) * 6 + t * 2 + par],
                                      wsems.at[2 * j + (i >= PRE_SPLIT)]).start()

    def mod_copy(j):
        return pltpu.make_async_copy(wmod32.at[:, j * D:(j + 1) * D], wmod_v.at[j],
                                     wsems.at[2 * j + 1])

    def mult(v, m):
        return v if isinstance(v, int) else pl.multiple_of(v, m)

    def moda_copies(kc):
        col = mult(kc * 128, 128)
        return [pltpu.make_async_copy(wmod32.at[:, pl.ds(v * D + col, 128)],
                                      wmod_v.at[v, :, pl.ds(col, 128)], ksems.at[8 + kc])
                for v in range(2)]

    def chunk_copies(kc):
        r0 = mult(kc * 64, 64)
        return [pltpu.make_async_copy(w_hbms[0].at[pl.ds(r0, 64), par, i, :],
                                      w_v.at[i * 6 + par, pl.ds(r0, 64), :], ksems.at[kc])
                for i in range(NB) for par in range(2)]

    cp_c.start()
    cp_mem.start()
    cp_wr.start()
    for c_ in (cp_x0 + moda_copies(0) + moda_copies(1) + chunk_copies(0) + moda_copies(2)
               + chunk_copies(1) + [cp_xr] + chunk_copies(2)):
        c_.start()

    def ln1_rows(src_row, dst_row):
        xv = xbuf[pl.ds(src_row, 8), :].astype(F32)
        hv = _rb(_layernorm(xv) * modb[1]) + modb[0]
        act[pl.ds(dst_row, 8), :] = hv.astype(BF)

    lane256 = lax.broadcasted_iota(jnp.int32, (8, 256), 1)

    def finish_rows(row, attn, row2=None):
        xv = xbuf[pl.ds(row, 8), :].astype(F32)
        x1 = _rb(xv + _rb(modb[2] * _rb(attn)))
        act[pl.ds(row, 8), :] = x1.astype(BF)
        if row2 is None:
            h2 = _rb(_rb(_layernorm(x1) * modb[4]) + modb[3])
            act[pl.ds(OOFF + row, 8), :] = (x1 + _rb(modb[5] * h2)).astype(BF)
            hw = h2 * modb[6]
        else:
            mu, sd = _ln_stats(x1)
            hw = None
            for c0 in range(0, D, ECOL):
                cs = slice(c0, c0 + ECOL)
                xb = act[pl.ds(row2, 8), cs].astype(F32)
                h2 = _rb(_rb(_rb(_rb(xb - mu) / sd) * modb[4, :, cs]) + modb[3, :, cs])
                act[pl.ds(OOFF + row, 8), cs] = (xb + _rb(modb[5, :, cs] * h2)).astype(BF)
                t = h2 * modb[6, :, cs]
                hw = t if hw is None else hw + t
        r = jnp.sum(hw, axis=-1, keepdims=True)
        act[ROFF:ROFF + 8, 0:256] = jnp.where(
            lane256 * 8 == row, r, act[ROFF:ROFF + 8, 0:256].astype(F32)).astype(BF)

    def attn_store(a, k0):
        for j in range(3):
            for k in range(a.shape[1] // 128):
                qkvbufs[A_BUF[j]][NSLOT, (k0 + k) * 8:(k0 + k + 1) * 8, :] = pltpu.bitcast(
                    a[8 * j:8 * j + 8, k * 128:(k + 1) * 128], U32)

    def attn_load(j):
        return pltpu.bitcast(jnp.concatenate(
            [qkvbufs[A_BUF[j]][NSLOT, k * 8:(k + 1) * 8, :] for k in range(8)], axis=1), F32)

    act[ROFF:ROFF + 8, 0:256] = jnp.zeros((8, 256), BF)
    tab[NSEG * NTAB] = 0
    attn_store(jnp.zeros((RIDE, D), F32), 0)
    for s_ in range(NSEG):
        for k, v in enumerate(_step_indices(s_)):
            tab[s_ * NTAB + k] = v
    ri = lax.broadcasted_iota(jnp.int32, (80, 80), 0)
    ci = lax.broadcasted_iota(jnp.int32, (80, 80), 1)

    def head_pos(i):
        hd = jnp.where(i < 16, i // 8, (i - 16) // 32)
        pos = jnp.where(i < 16, i % 8, 8 + (i - 16) % 32)
        return hd, pos
    rh, rp = head_pos(ri)
    ch, cpos = head_pos(ci)
    same = rh == ch
    valid = same & ((rp < M) | (rp >= cpos))
    fill = jnp.where(same, -1e9, -jnp.inf).astype(F32)

    cp_mem.wait()
    cp_wr.wait()
    modb[6] = jnp.broadcast_to(wrbuf[...].astype(F32).reshape(1, D), (8, D))
    cp_c.wait()
    cv = small[0].astype(F32)
    sc16 = jnp.broadcast_to(_rb(cv * _rb(jax.nn.sigmoid(cv))), (16, D)).astype(BF)

    def ln_pre(g, carry):
        pltpu.make_async_copy(x_hbm.at[0, 0:128], xbuf.at[pl.ds(pl.multiple_of(g * 128, 128), 128)],
                              sems.at[13 + g]).wait()
        for u in range(2):
            row = pl.multiple_of(g * 128 + u * 64, 64)
            nv = _layernorm(xbuf[pl.ds(row, 64), :].astype(F32)).astype(BF)
            for k in range(8):
                h0buf[k, pl.ds(pl.multiple_of(row // 2, 32), 32), :] = pltpu.bitcast(
                    nv[:, k * 128:(k + 1) * 128], U32)
            wg_v[pl.ds(row, 64), 0:2 * D] = jnp.zeros((64, 2 * D), U32)
        return carry
    lax.fori_loop(0, PRE // 128, ln_pre, 0)

    def mod_tile(v, col):
        w = pltpu.bitcast(wmod_v[v, :, pl.ds(col, 128)], BF)
        return _rb(jnp.dot(sc16, w, preferred_element_type=F32))[0:8]

    def moda_store(kc, sa, ca):
        col = mult(kc * 128, 128)
        c1 = _rb(1.0 + ca)
        modb[0, :, pl.ds(col, 128)] = sa
        modb[1, :, pl.ds(col, 128)] = c1
        return sa, c1

    def moda_apply(kc, sa, c1, r0, r1):
        for r in range(r0, r1, 16):
            nv = pltpu.bitcast(h0buf[kc, r // 2:r // 2 + 8, :], BF).astype(F32).reshape(2, 8, 128)
            hv = (_rb(nv * c1[None]) + sa[None]).reshape(16, 128).astype(BF)
            h0buf[kc, r // 2:r // 2 + 8, :] = pltpu.bitcast(hv, U32)

    def repack(a, b):
        return (a & U32(0xFFFF)) | (b << 16), (a >> 16) | (b & U32(0xFFFF0000))

    def store_qkv(i, jrow, y, seg0):
        for sg in range(y.shape[0] // 32):
            for hh in range(2):
                qkvbufs[i][seg0 + sg, pl.ds(jrow + 8 + hh * 16, 16), :] = _pack(
                    y[sg * 32:(sg + 1) * 32, hh * 128:(hh + 1) * 128])

    for c_ in moda_copies(0):
        c_.wait()
    moda_apply(0, *moda_store(0, mod_tile(0, 0), mod_tile(1, 0)), 0, PRE)

    def chunk_block(kc, last, issue):
        with _scope('w_chunk'):
            for c_ in chunk_copies(kc) + ([cp_xr] if last else moda_copies(kc + 1)):
                c_.wait()
        issue()
        r0 = mult(kc * 64, 64)
        mv = []
        for i in range(NB):
            lo, hi = repack(w_v[i * 6, pl.ds(r0, 64), :], w_v[i * 6 + 1, pl.ds(r0, 64), :])
            w_v[i * 6, pl.ds(r0, 64), :] = lo
            w_v[i * 6 + 1, pl.ds(r0, 64), :] = hi
            w = pltpu.bitcast(jnp.concatenate([lo, hi], axis=1), BF)
            y = (pltpu.bitcast(wg_v[0:PRE, i * 256:(i + 1) * 256], F32)
                 + jnp.dot(pltpu.bitcast(h0buf[kc], BF), w, preferred_element_type=F32))
            if last:
                store_qkv(i, 0, y, 0)
            else:
                wg_v[0:PRE, i * 256:(i + 1) * 256] = pltpu.bitcast(y, U32)
                if i in (1, 3):
                    mv.append(mod_tile(i // 2, mult((kc + 1) * 128, 128)))
                if i == 3:
                    mv = moda_store(kc + 1, mv[0], mv[1])
                if i >= 4:
                    moda_apply(kc + 1, mv[0], mv[1], (i - 4) * 128, (i - 3) * 128)
        if last:
            for j in range(3):
                ln1_rows(PRE + 8 * j, HOFF + 8 + 8 * j)

    def chunk_body_a(kc, carry):
        def issue():
            for c_ in moda_copies(kc + 3) + chunk_copies(kc + 3):
                c_.start()
        chunk_block(kc, False, issue)
        return carry

    def chunk_body_b(kc, carry):
        chunk_block(kc, False, lambda: None)
        return carry

    def issue_last():
        w_start(2)
        mod_copy(2).start()
    lax.fori_loop(0, 5, chunk_body_a, 0)
    w_start(1)
    lax.fori_loop(5, 7, chunk_body_b, 0)
    chunk_block(7, True, issue_last)

    def pre_unit(j, i, extra):
        blk = (j // 3) * (6 * NB) + (j % 3) * 2 + i * 6
        jrow = pl.multiple_of(j * 40, 8)
        lo, hi = repack(w_v[blk], w_v[blk + 1])
        w_v[blk] = lo
        w_v[blk + 1] = hi
        for rc in range(PRE // 128):
            if rc > 0:
                lo = w_v[blk]
                hi = w_v[blk + 1]
            w = pltpu.bitcast(jnp.concatenate([lo, hi], axis=1), BF)
            lhs = jnp.concatenate([h0buf[k, rc * 64:(rc + 1) * 64, :] for k in range(8)], axis=1)
            y = jnp.dot(pltpu.bitcast(lhs, BF), w, preferred_element_type=F32)
            store_qkv(i, jrow, y, rc * 4)
            extra(rc)

    def pre_body(j, carry):
        @pl.when(j == 1)
        def _():
            for jn in (3, 4):
                w_start(jn)
                mod_copy(jn).start()

        @pl.when(j == 2)
        def _():
            w_start(5)
            mod_copy(5).start()
            cp_wo.start()
            cp_x1.start()
        blk0 = (j // 3) * (6 * NB) + (j % 3) * 2
        one = jnp.where((j == 1) | (j == 4), 1.0, 0.0).astype(F32)
        for half, (i0, i1) in enumerate(((0, PRE_SPLIT), (PRE_SPLIT, NB))):
            with _scope('w_pre'):
                for i in range(i0, i1):
                    for par in range(2):
                        pltpu.make_async_copy(w_hbms[0].at[:, 0, 0, :],
                                              w_v.at[blk0 + i * 6 + par],
                                              wsems.at[2 * j + half]).wait()
            if half == 1:
                @pl.when(j > 1)
                def _():
                    pltpu.make_async_copy(wmod32.at[:, 0:D], wmod_v.at[j],
                                          wsems.at[2 * j + 1]).wait()
            for i in range(i0, i1):
                def extra(rc, i=i):
                    n = (i - PRE_SPLIT) * 2 + rc // 2
                    if i >= PRE_SPLIT and rc % 2 == 0 and n < 8:
                        modb[j, :, n * 128:(n + 1) * 128] = _rb(one + mod_tile(j, n * 128))
                pre_unit(j, i, extra)
        return carry
    lax.fori_loop(1, 6, pre_body, 0)

    cp_wo.wait()
    cp_x1.wait()
    for c_ in cp_ffn:
        c_.start()

    def wo_w(h0, h1, n0, n1):
        w = wo_v[h0:h1, :, n0 * 128:n1 * 128].reshape((h1 - h0) * (DH // 2), (n1 - n0) * 128)
        return pltpu.bitcast(w, BF)

    HD = D // 2

    def emit_step(s, pend, last):
        hrow = pl.multiple_of(HOFF + (s & 1) * 32, 32)
        hnext = pl.multiple_of(HOFF + 32 - (s & 1) * 32, 32)
        tv = [tab[s * NTAB + k] for k in range(16)]
        slot = tv[0]
        dsts = [(tv[1 + 2 * j], pl.multiple_of(tv[2 + 2 * j], 4)) for j in range(3)]
        odst = [pl.multiple_of(tv[7 + j], 8) for j in range(4)]
        orow = pl.multiple_of(tv[11], 32)
        erow = tv[12]
        lrow = tv[13]
        erow2 = tv[14]
        mrow = pl.multiple_of(tv[15], 8)
        e_at, l_at = (E_AT, L_AT) if pend is None else (E_AT2, L_AT2)
        probs = {}

        def wqkv(p, k0, k1):
            return pltpu.bitcast(jnp.concatenate(
                [w_v[p * 6 + u, k0 // 2:k1 // 2, :] for u in range(6)], axis=1), BF)

        lhs_lo = act[pl.ds(hrow, 32), 0:HD]
        if pend is not None:
            ybuf[...] = jnp.dot(lhs_lo, wqkv(0, 0, HD), preferred_element_type=F32)
            pend()
        lhs_hi = act[pl.ds(hrow, 32), HD:D]
        if pend is not None:
            y0 = ybuf[...] + jnp.dot(lhs_hi, wqkv(0, HD, D), preferred_element_type=F32)
        lhs_rest = jnp.concatenate([lhs_lo[:, 128:], lhs_hi], axis=1)
        lhs = [jnp.concatenate([lhs_lo, lhs_hi], axis=1)]

        def side(p):
            for j in range(3):
                if e_at[j] == p:
                    finish_rows(pl.multiple_of(erow + 8 * j, 8), attn_load(j),
                                pl.multiple_of(erow2 + 8 * j, 8) if ECOL else None)
            for j in range(3):
                if l_at[j] == p:
                    ln1_rows(pl.multiple_of(lrow + 8 * j, 8),
                             pl.multiple_of(hnext + 8 + 8 * j, 8))
            if (p in e_at or p in l_at) and p < NP - 1:
                lhs[0] = jnp.concatenate([act[pl.ds(hrow, 32), 0:128], lhs_rest], axis=1)

        def qkv(p):
            if p == 0 and pend is not None:
                y = y0
            else:
                y = jnp.dot(lhs[0], wqkv(p, 0, D), preferred_element_type=F32)
            buf = qkvbufs[p % NB]
            for u in range(6):
                t, hh = u // 2, u % 2
                b0 = ((p // NB) * 3 + t) * 40
                yu = y[:, u * 128:(u + 1) * 128]
                buf[slot, b0 + hh * 4:b0 + hh * 4 + 4, :] = _pack(yu[0:8])
                for j in range(3):
                    sl, off = dsts[j]
                    buf[sl, pl.ds(b0 + 8 + hh * 16 + off, 4), :] = _pack(yu[8 + 8 * j:16 + 8 * j])

        def ld(p, t):
            b0 = ((p // NB) * 3 + t) * 40
            return pltpu.bitcast(qkvbufs[p % NB][slot, b0:b0 + 40, :], BF)

        def sc(p):
            s2 = lax.dot_general(ld(p, 0), ld(p, 1), (((1,), (1,)), ((), ())),
                                 preferred_element_type=F32)
            if SMX == 0:
                s2 = jnp.where(valid, s2 * SCALE, fill)
                m = jnp.max(s2, axis=-1, keepdims=True)
                e = jnp.exp(s2 - m)
            else:
                s2 = jnp.where(valid, s2, fill * (1.0 / SCALE))
                m = jnp.max(s2, axis=-1, keepdims=True)
                e = jnp.exp2((s2 - m) * (SCALE * LOG2E))
            l = jnp.sum(e, axis=-1, keepdims=True)
            rl = pl.reciprocal(l, approx=True)
            rl = rl * (2.0 - l * rl)
            probs[p] = (e * rl).astype(BF)

        def pv(p):
            o2 = jnp.dot(probs[p], ld(p, 2), preferred_element_type=F32)
            for hh in range(2):
                hcol = (2 * p + hh) * 128
                ob = obuf1
                if hcol >= KS:
                    ob = obuf2
                    hcol -= KS
                ob[pl.ds(mrow, 8), hcol:hcol + 128] = o2[8 * hh:8 * hh + 8].astype(BF)
                for j in range(4):
                    r0 = 16 + 32 * hh + 8 * j
                    ob[pl.ds(odst[j], 8), hcol:hcol + 128] = o2[r0:r0 + 8].astype(BF)

        def attn(pos):
            for kind, p in ATT.get(pos, ()):
                (sc if kind == 's' else pv)(p)

        for p in range(NP):
            qkv(p)
            side(p)
            attn(p)
        a1 = []
        for i in range(4):
            a1.append(jnp.dot(obuf1[pl.ds(orow, 32), 0:KS], wo_w(0, KS // DH, 2 * i, 2 * i + 2),
                              preferred_element_type=F32))
            attn(NP + i)
            side(NP + i)
        o2lhs = obuf2[pl.ds(orow, 32), 0:K2]
        a_lo = jnp.concatenate(a1[0:2], axis=1) + jnp.dot(
            o2lhs, wo_w(KS // DH, H, 0, 4), preferred_element_type=F32)
        act[pl.ds(hnext, 8), 0:HD] = a_lo[0:8].astype(BF)
        attn_store(a_lo[8:32], 0)
        a_hi = jnp.concatenate(a1[2:4], axis=1) + jnp.dot(
            o2lhs, wo_w(KS // DH, H, 4, 8), preferred_element_type=F32)

        def finish():
            act[pl.ds(hnext, 8), HD:D] = a_hi[0:8].astype(BF)
            attn_store(a_hi[8:32], 4)
        if last:
            finish()
        return finish

    def steps(it, carry):
        pend = None
        for u in range(UNR):
            pend = emit_step(it * UNR + u, pend, u == UNR - 1)
        return carry
    lax.fori_loop(0, NSEG // UNR, steps, 0)

    if SKIP:
        return
    for c_ in cp_ffn:
        c_.wait()
    OUT0 = (NSEG - 1) * RIDE
    NEW0 = S - NEW
    cp_out = [cp(act.at[OOFF:OOFF + OUT0], out_hbm.at[0, 0:OUT0], 9)]
    cp_out[0].start()
    zero = pl.multiple_of(tab[NSEG * NTAB], 8)
    for j in range(3):
        ebuf[EMAX + 8 * j:EMAX + 8 * j + 8, :] = attn_load(j)
    ebuf[EMAX + RIDE:EMAX + RIDE + 8, :] = act[HOFF:HOFF + 8, :].astype(F32)
    todo = [(OUT0 + 8 * j, EMAX + 8 * j) for j in range(4)]
    r0 = 0
    for ci, ech in enumerate(EPI_CHUNKS):
        o0 = NOSLOT * 32 + r0
        e0 = (ci % 2) * EMAX
        per = -(-len(todo) // 8)
        if ci == len(EPI_CHUNKS) - 1:
            per = EPI_LASTPER
        for n in range(8):
            lhs = jnp.concatenate([obuf1[o0:o0 + ech, 0:KS], obuf2[o0:o0 + ech, 0:K2]], axis=1)
            ebuf[e0:e0 + ech, n * 128:(n + 1) * 128] = jnp.dot(
                lhs, wo_w(0, H, n, n + 1), preferred_element_type=F32)
            for row, er in todo[:per]:
                finish_rows(row, ebuf[pl.ds(zero + er, 8), :])
            todo = todo[per:]
        todo = [(OUT0 + RIDE + 8 + r0 + 8 * j, e0 + 8 * j) for j in range(ech // 8)]
        r0 += ech

    rowsf = (lane256 * 8 + lax.broadcasted_iota(jnp.int32, (8, 256), 0)).astype(F32)
    r_old = jnp.where(rowsf < NEW0, act[ROFF:ROFF + 8, 0:256].astype(F32), -jnp.inf)

    def allmax(v):
        return jnp.max(jnp.max(v, axis=1, keepdims=True), axis=0, keepdims=True)

    def allmin(v):
        return jnp.min(jnp.min(v, axis=1, keepdims=True), axis=0, keepdims=True)
    m1 = allmax(r_old)
    i1v = allmin(jnp.where(r_old == m1, rowsf, float(S)))
    r_rest = jnp.where(rowsf == i1v, -jnp.inf, r_old)
    m2 = allmax(r_rest)
    i2v = allmin(jnp.where((r_rest == m2) & (rowsf != i1v), rowsf, float(S)))
    i1 = jnp.clip(i1v[0, 0].astype(jnp.int32), 0, NEW0 - 1)
    i2 = jnp.clip(i2v[0, 0].astype(jnp.int32), 0, NEW0 - 1)
    b1 = pl.multiple_of((i1 // 8) * 8, 8)
    b2 = pl.multiple_of((i2 // 8) * 8, 8)
    sub8 = lax.broadcasted_iota(jnp.int32, (8, 1), 0)

    def rep(i, n):
        return jnp.concatenate([modb[i]] * n, axis=0)
    x1c = jnp.concatenate([act[pl.ds(b1, 8), :].astype(F32), act[pl.ds(b2, 8), :].astype(F32)],
                          axis=0)
    h2c = _rb(_rb(_layernorm(x1c) * rep(4, 2)) + rep(3, 2))
    row1 = jnp.sum(jnp.where(sub8 == i1 - b1, h2c[0:8], 0.0), axis=0, keepdims=True)
    row2 = jnp.sum(jnp.where(sub8 == i2 - b2, h2c[8:16], 0.0), axis=0, keepdims=True)
    cand = jnp.where(sub8 == 0, row1, jnp.where(sub8 == 1, row2, 0.0))

    e0 = ((len(EPI_CHUNKS) - 1) % 2) * EMAX
    ng = NEW // 8
    x1n = _rb(xbuf[NEW0:S, :].astype(F32) + _rb(rep(2, ng) * _rb(ebuf[e0:e0 + NEW, :])))
    h2n = _rb(_rb(_layernorm(x1n) * rep(4, ng)) + rep(3, ng))
    h2b = jnp.concatenate([cand, h2n], axis=0).astype(BF)
    cp_out.append(cp(act.at[OOFF + OUT0:OOFF + NEW0], out_hbm.at[0, OUT0:NEW0], 10))
    cp_out[1].start()
    hid = []
    for n in range(0, F, FFN_NB):
        gt = _rb(jnp.dot(h2b, pltpu.bitcast(wg_v[:, n:n + FFN_NB], BF), preferred_element_type=F32))
        up = _rb(jnp.dot(h2b, pltpu.bitcast(wu_v[:, n:n + FFN_NB], BF), preferred_element_type=F32))
        hid.append((_rb(gt * _rb(jax.nn.sigmoid(gt))) * up).astype(BF))
    y = _rb(jnp.dot(jnp.concatenate(hid, axis=1), pltpu.bitcast(wd_v[...], BF),
                    preferred_element_type=F32))
    val = jnp.concatenate(
        [jnp.where(sub8 == 0, m1, jnp.where(sub8 == 1, m2, -jnp.inf)),
         _rb(jnp.sum(h2n * rep(6, ng), axis=-1, keepdims=True))], axis=0)
    pos = lax.broadcasted_iota(jnp.int32, (8 + NEW, 1), 0).astype(F32)
    p1 = jnp.min(jnp.where(val == jnp.max(val, axis=0, keepdims=True), pos, float(S)),
                 axis=0, keepdims=True)
    val2 = jnp.where(pos == p1, -jnp.inf, val)
    p2 = jnp.min(jnp.where((val2 == jnp.max(val2, axis=0, keepdims=True)) & (pos != p1), pos,
                           float(S)), axis=0, keepdims=True)
    upd = jnp.where((pos == p1) | (pos == p2), _rb(y * _rb(jax.nn.sigmoid(val))), 0.0)
    act[OOFF + NEW0:OOFF + S, :] = (x1n + _rb(rep(5, ng) * _rb(h2n + upd[8:]))).astype(BF)
    sub16 = lax.broadcasted_iota(jnp.int32, (16, 1), 0)
    grow = jnp.where(sub16 < 8, b1 + sub16, b2 + sub16 - 8)
    updc = jnp.where(grow == i1, upd[0:1], jnp.where(grow == i2, upd[1:2], 0.0))
    res = (x1c + _rb(rep(5, 2) * _rb(h2c + updc))).astype(BF)
    for c_ in cp_out:
        c_.wait()
    act[pl.ds(OOFF + b1, 8), :] = res[0:8]
    act[pl.ds(OOFF + b2, 8), :] = res[8:16]
    fix0 = cp(act.at[OOFF + NEW0:OOFF + S], out_hbm.at[0, NEW0:S], 6)
    fix1 = cp(act.at[pl.ds(OOFF + b1, 8)], out_hbm.at[0, pl.ds(b1, 8)], 11)
    fix2 = cp(act.at[pl.ds(OOFF + b2, 8)], out_hbm.at[0, pl.ds(b2, 8)], 12)
    fix0.start()
    fix1.start()

    @pl.when(b1 != b2)
    def _():
        fix2.start()
        fix2.wait()
    fix0.wait()
    fix1.wait()


@jax.jit
def pallas_adaLN_cond__memory_aug_recurrent_mem_tr__moe_arch_mod__prompt_kernel(
    A_x: jax.Array,
    A_mem0: jax.Array,
    A_Wq: jax.Array,
    A_Wk: jax.Array,
    A_Wv: jax.Array,
    A_Wo: jax.Array,
    A_seg_len,
    B_x: jax.Array,
    B_w_r: jax.Array,
    B_w_gate: jax.Array,
    B_w_up: jax.Array,
    B_w_down: jax.Array,
    c: jax.Array,
    w_mod: jax.Array,
):
    del B_x
    del A_seg_len
    assert A_x.shape == (1, S, D) and A_Wq.shape == (D, H, DH) and A_mem0.shape == (1, M, D)
    any_spec = pl.BlockSpec(memory_space=pl.ANY)
    scratch = [
        pltpu.VMEM((S if not XACT else 8, D), BF),
        pltpu.VMEM((XOFF + S * XACT, D), BF),
        pltpu.VMEM((8, PRE // 2, 128), U32),
        pltpu.VMEM((32, 768), F32),
        pltpu.VMEM((2 * EMAX, D), F32),
        pltpu.SMEM((NSEG * NTAB + 1,), jnp.int32),
        pltpu.VMEM((7, 8, D), F32),
        pltpu.VMEM((4, 1, D), BF),
        pltpu.VMEM((3 * H, D // 2, 128), U32),
        pltpu.VMEM((H, DH // 2, D), U32),
        pltpu.VMEM((6, D // 2, D), U32),
        pltpu.VMEM((D // 2, F), U32),
        pltpu.VMEM((D // 2, F), U32),
        pltpu.VMEM((F // 2, D), U32),
        pltpu.VMEM((NOSLOT * 32 + PRE, OW1), BF),
        pltpu.VMEM((NOSLOT * 32 + PRE, OW2), BF),
        pltpu.SemaphoreType.DMA((17,)),
        pltpu.SemaphoreType.DMA((12,)),
        pltpu.SemaphoreType.DMA((16,)),
    ] + [pltpu.VMEM((NSLOT + 1, 256, 128), U32) for _ in range(NB)] + [
        pltpu.VMEM((D,), BF),
    ]
    wq, wk, wv = (w.reshape(D // 2, 2, H, DH) for w in (A_Wq, A_Wk, A_Wv))
    return pl.pallas_call(
        _kernel,
        out_shape=jax.ShapeDtypeStruct((1, S, D), BF),
        in_specs=[any_spec] * 12,
        out_specs=any_spec,
        scratch_shapes=scratch,
        compiler_params=pltpu.CompilerParams(vmem_limit_bytes=120 * 1024 * 1024,
                                             disable_bounds_checks=True,
                                             disable_semaphore_checks=True),
    )(A_x, A_mem0, wq, wk, wv, A_Wo, B_w_r, B_w_gate, B_w_up, B_w_down,
      c, w_mod)
```

```python
import contextlib
import os
import jax
import jax.numpy as jnp
from jax import lax
import jax.experimental.pallas as pl
import jax.experimental.pallas.tpu as pltpu

BF = jnp.bfloat16
F32 = jnp.float32
U32 = jnp.uint32

S = 2048
D = 1024
H = 32
DH = 128
M = 8
SEG = 32
NSEG = S // SEG
F = 3584
NP = H // 2
RIDE = 24
PRE = S - NSEG * RIDE
NSLOT = 17
NOSLOT = 17
NB = int(os.environ.get('NB', 8))
KS = int(os.environ.get('KS', 2304))
LAG_S = 1
LAG_P = 3
EPS = 1e-5
SCALE = DH ** -0.5
OOFF = S
HOFF = 2 * S
ROFF = HOFF + 64
XOFF = ROFF + 16
PRE_SPLIT = 3
E_AT = tuple(int(v) for v in os.environ.get('E_AT', '2,3,5').split(','))
L_AT = tuple(int(v) for v in os.environ.get('L_AT', '8,10,12').split(','))
E_AT2 = tuple(int(v) for v in os.environ.get('E_AT2', '3,5,6').split(','))
L_AT2 = tuple(int(v) for v in os.environ.get('L_AT2', '8,10,12').split(','))


def _att_schedule(mode):
    att = {}
    if mode == 'lag':
        for p in range(NP):
            att.setdefault(p + LAG_S, []).append(('s', p))
        for p in range(NP):
            att.setdefault(p + LAG_P, []).append(('p', p))
    elif mode == 'q2':
        for p in range(0, NP, 2):
            att.setdefault(p + 2, []).extend([('s', p), ('s', p + 1)])
        for p in range(0, NP, 2):
            att.setdefault(p + 4, []).extend([('p', p), ('p', p + 1)])
    elif mode == 'q2b':
        for p in range(0, NP, 2):
            att.setdefault(p + 4, []).extend([('p', p), ('p', p + 1)])
        for p in range(0, NP, 2):
            att.setdefault(p + 2, []).extend([('s', p), ('s', p + 1)])
    elif mode == 'q2c':
        att[4] = [('s', i) for i in range(4)]
        for p in range(4, NP, 2):
            att[p + 2] = [('s', p), ('s', p + 1), ('p', p - 4), ('p', p - 3)]
        att[18] = [('p', i) for i in range(12, 16)]
    elif mode == 'q2d':
        att[3] = [('s', i) for i in range(3)]
        att[4] = [('s', 3)]
        att[3] = []
        att[4] = [('s', i) for i in range(4)]
        for p in range(4, NP, 2):
            att[p + 2] = [('p', p - 4), ('p', p - 3), ('s', p), ('s', p + 1)]
        att[18] = [('p', i) for i in range(12, 16)]
    elif mode == 'q4':
        for p in range(0, NP, 4):
            att.setdefault(p + 4, []).extend([('s', p + i) for i in range(4)])
            att.setdefault(p + 6, []).extend([('p', p + i) for i in range(4)])
    elif mode == 'q4b':
        for p in range(0, NP, 4):
            att.setdefault(min(p + 8, 18), []).extend([('p', p + i) for i in range(4)])
        for p in range(0, NP, 4):
            att.setdefault(p + 4, []).extend([('s', p + i) for i in range(4)])
    return att


ATT = _att_schedule(os.environ.get('ATT', 'q2c'))
XACT = int(os.environ.get('XACT', 0))
K2 = H * DH - KS
OPAD = int(os.environ.get('OPAD', 1))
OW1 = -(-KS // 1024) * 1024 if OPAD else KS
OW2 = -(-K2 // 1024) * 1024 if OPAD else K2
SMX = int(os.environ.get('SMX', 0))
LOG2E = 1.4426950408889634
SKIP = int(os.environ.get('SKIP', 0))
A_BUF = tuple(int(v) for v in os.environ.get('A_BUF', '7,0,1').split(','))
ECOL = int(os.environ.get('ECOL', 0))
UNR = int(os.environ.get('UNR', 2))
EPI_CHUNKS = tuple(int(v) for v in os.environ.get('EPI', '64,64,64,64,64,64,48,48,32').split(','))
EMAX = max(EPI_CHUNKS)
NEW = 24
EPI_LASTPER = int(os.environ.get('EPI_LASTPER', 2))
FFN_NB = int(os.environ.get('FFN_NB', 512))


NTAB = 16


def _step_indices(s):
    t = [s % NSLOT]
    for j in range(3):
        gi = PRE // 8 + 3 * s + j
        t += [(gi // 4) % NSLOT, (gi % 4) * 4]
    for j in range(4):
        gi = 4 * s + j
        if gi < 3 * NSEG:
            t.append(((gi // 3) % NOSLOT) * 32 + 8 + (gi % 3) * 8)
        elif gi == 3 * NSEG:
            t.append(((NSEG - 1) % NOSLOT) * 32)
        else:
            t.append(NOSLOT * 32 + (gi - 3 * NSEG - 1) * 8)
    t.append((s % NOSLOT) * 32)
    t.append(max(s - 1, 0) * RIDE)
    t.append(PRE + min(s + 1, NSEG - 1) * RIDE)
    t.append(max(s - 1, 0) * RIDE)
    t.append((s % NOSLOT) * 32 if s < NSEG - 1 else NOSLOT * 32 + PRE - 8)
    return t


def _scope(name):
    return jax.named_scope(name) if os.environ.get('PROF') else contextlib.nullcontext()


def _rb(v):
    return v.astype(BF).astype(F32)


def _pack(v):
    return pltpu.bitcast(v.astype(BF), U32)


def _ln_stats(x):
    mu = jnp.sum(x, axis=-1, keepdims=True) * (1.0 / D)
    xc = x - mu
    var = jnp.sum(xc * xc, axis=-1, keepdims=True) * (1.0 / D)
    return _rb(mu), _rb(jnp.sqrt(_rb(_rb(var) + EPS)))


def _layernorm(x):
    mu, sd = _ln_stats(x)
    return _rb(_rb(x - mu) / sd)


def _kernel(x_hbm, mem0_hbm, wq_hbm, wk_hbm, wv_hbm, wo_hbm, wr_hbm, wg_hbm, wu_hbm,
            wd_hbm, c_hbm, wmod_hbm, out_hbm,
            xbuf, act, h0buf, ybuf, ebuf, tab, modb, small,
            w_v, wo_v, wmod_v, wg_v, wu_v, wd_v,
            obuf1, obuf2, sems, wsems, ksems, *rest):
    qkvbufs, wrbuf = rest[:NB], rest[NB]
    if XACT:
        xbuf = act.at[pl.ds(XOFF, S)]
    w_hbms = tuple(w.bitcast(U32) for w in (wq_hbm, wk_hbm, wv_hbm))

    def cp(src, dst, i):
        return pltpu.make_async_copy(src, dst, sems.at[i])

    wmod32 = wmod_hbm.bitcast(U32)
    cp_c = cp(c_hbm, small.at[0], 0)
    cp_mem = cp(mem0_hbm.at[0], act.at[HOFF:HOFF + M], 1)
    cp_wr = cp(wr_hbm, wrbuf, 2)
    cp_x0 = [cp(x_hbm.at[0, n * 128:(n + 1) * 128], xbuf.at[n * 128:(n + 1) * 128], 13 + n)
             for n in range(PRE // 128)]
    cp_xr = cp(x_hbm.at[0, PRE:PRE + 32], xbuf.at[PRE:PRE + 32], 5)
    cp_x1 = cp(x_hbm.at[0, PRE + 32:S], xbuf.at[PRE + 32:S], 4)
    cp_wo = cp(wo_hbm.bitcast(U32), wo_v, 7)
    cp_ffn = [cp(wg_hbm.bitcast(U32), wg_v, 8), cp(wu_hbm.bitcast(U32), wu_v, 8),
              cp(wd_hbm.bitcast(U32), wd_v, 8)]

    def w_start(j):
        gg, t = j // 3, j % 3
        for i in range(NB):
            for par in range(2):
                pltpu.make_async_copy(w_hbms[t].at[:, par, gg * NB + i, :],
                                      w_v.at[(gg * NB + i) * 6 + t * 2 + par],
                                      wsems.at[2 * j + (i >= PRE_SPLIT)]).start()

    def mod_copy(j):
        return pltpu.make_async_copy(wmod32.at[:, j * D:(j + 1) * D], wmod_v.at[j],
                                     wsems.at[2 * j + 1])

    def mult(v, m):
        return v if isinstance(v, int) else pl.multiple_of(v, m)

    def moda_copies(kc):
        col = mult(kc * 128, 128)
        return [pltpu.make_async_copy(wmod32.at[:, pl.ds(v * D + col, 128)],
                                      wmod_v.at[v, :, pl.ds(col, 128)], ksems.at[8 + kc])
                for v in range(2)]

    def chunk_copies(kc):
        r0 = mult(kc * 64, 64)
        return [pltpu.make_async_copy(w_hbms[0].at[pl.ds(r0, 64), par, i, :],
                                      w_v.at[i * 6 + par, pl.ds(r0, 64), :], ksems.at[kc])
                for i in range(NB) for par in range(2)]

    cp_c.start()
    cp_mem.start()
    cp_wr.start()
    for c_ in (cp_x0 + moda_copies(0) + moda_copies(1) + chunk_copies(0) + moda_copies(2)
               + chunk_copies(1) + [cp_xr] + chunk_copies(2)):
        c_.start()

    def ln1_rows(src_row, dst_row):
        xv = xbuf[pl.ds(src_row, 8), :].astype(F32)
        hv = _rb(_layernorm(xv) * modb[1]) + modb[0]
        act[pl.ds(dst_row, 8), :] = hv.astype(BF)

    lane256 = lax.broadcasted_iota(jnp.int32, (8, 256), 1)

    def finish_rows(row, attn, row2=None):
        xv = xbuf[pl.ds(row, 8), :].astype(F32)
        x1 = _rb(xv + _rb(modb[2] * _rb(attn)))
        act[pl.ds(row, 8), :] = x1.astype(BF)
        if row2 is None:
            h2 = _rb(_rb(_layernorm(x1) * modb[4]) + modb[3])
            act[pl.ds(OOFF + row, 8), :] = (x1 + _rb(modb[5] * h2)).astype(BF)
            hw = h2 * modb[6]
        else:
            mu, sd = _ln_stats(x1)
            hw = None
            for c0 in range(0, D, ECOL):
                cs = slice(c0, c0 + ECOL)
                xb = act[pl.ds(row2, 8), cs].astype(F32)
                h2 = _rb(_rb(_rb(_rb(xb - mu) / sd) * modb[4, :, cs]) + modb[3, :, cs])
                act[pl.ds(OOFF + row, 8), cs] = (xb + _rb(modb[5, :, cs] * h2)).astype(BF)
                t = h2 * modb[6, :, cs]
                hw = t if hw is None else hw + t
        r = jnp.sum(hw, axis=-1, keepdims=True)
        act[ROFF:ROFF + 8, 0:256] = jnp.where(
            lane256 * 8 == row, r, act[ROFF:ROFF + 8, 0:256].astype(F32)).astype(BF)

    def attn_store(a, k0):
        for j in range(3):
            for k in range(a.shape[1] // 128):
                qkvbufs[A_BUF[j]][NSLOT, (k0 + k) * 8:(k0 + k + 1) * 8, :] = pltpu.bitcast(
                    a[8 * j:8 * j + 8, k * 128:(k + 1) * 128], U32)

    def attn_load(j):
        return pltpu.bitcast(jnp.concatenate(
            [qkvbufs[A_BUF[j]][NSLOT, k * 8:(k + 1) * 8, :] for k in range(8)], axis=1), F32)

    act[ROFF:ROFF + 8, 0:256] = jnp.zeros((8, 256), BF)
    tab[NSEG * NTAB] = 0
    attn_store(jnp.zeros((RIDE, D), F32), 0)
    for s_ in range(NSEG):
        for k, v in enumerate(_step_indices(s_)):
            tab[s_ * NTAB + k] = v
    ri = lax.broadcasted_iota(jnp.int32, (80, 80), 0)
    ci = lax.broadcasted_iota(jnp.int32, (80, 80), 1)

    def head_pos(i):
        hd = jnp.where(i < 16, i // 8, (i - 16) // 32)
        pos = jnp.where(i < 16, i % 8, 8 + (i - 16) % 32)
        return hd, pos
    rh, rp = head_pos(ri)
    ch, cpos = head_pos(ci)
    same = rh == ch
    valid = same & ((rp < M) | (rp >= cpos))
    fill = jnp.where(same, -1e9, -jnp.inf).astype(F32)

    cp_mem.wait()
    cp_wr.wait()
    modb[6] = jnp.broadcast_to(wrbuf[...].astype(F32).reshape(1, D), (8, D))
    cp_c.wait()
    cv = small[0].astype(F32)
    sc16 = jnp.broadcast_to(_rb(cv * _rb(jax.nn.sigmoid(cv))), (16, D)).astype(BF)

    def ln_pre(g, carry):
        pltpu.make_async_copy(x_hbm.at[0, 0:128], xbuf.at[pl.ds(pl.multiple_of(g * 128, 128), 128)],
                              sems.at[13 + g]).wait()
        for u in range(2):
            row = pl.multiple_of(g * 128 + u * 64, 64)
            nv = _layernorm(xbuf[pl.ds(row, 64), :].astype(F32)).astype(BF)
            for k in range(8):
                h0buf[k, pl.ds(pl.multiple_of(row // 2, 32), 32), :] = pltpu.bitcast(
                    nv[:, k * 128:(k + 1) * 128], U32)
            wg_v[pl.ds(row, 64), 0:2 * D] = jnp.zeros((64, 2 * D), U32)
        return carry
    lax.fori_loop(0, PRE // 128, ln_pre, 0)

    def mod_tile(v, col):
        w = pltpu.bitcast(wmod_v[v, :, pl.ds(col, 128)], BF)
        return _rb(jnp.dot(sc16, w, preferred_element_type=F32))[0:8]

    def moda_store(kc, sa, ca):
        col = mult(kc * 128, 128)
        c1 = _rb(1.0 + ca)
        modb[0, :, pl.ds(col, 128)] = sa
        modb[1, :, pl.ds(col, 128)] = c1
        return sa, c1

    def moda_apply(kc, sa, c1, r0, r1):
        for r in range(r0, r1, 16):
            nv = pltpu.bitcast(h0buf[kc, r // 2:r // 2 + 8, :], BF).astype(F32).reshape(2, 8, 128)
            hv = (_rb(nv * c1[None]) + sa[None]).reshape(16, 128).astype(BF)
            h0buf[kc, r // 2:r // 2 + 8, :] = pltpu.bitcast(hv, U32)

    def repack(a, b):
        return (a & U32(0xFFFF)) | (b << 16), (a >> 16) | (b & U32(0xFFFF0000))

    def store_qkv(i, jrow, y, seg0):
        for sg in range(y.shape[0] // 32):
            for hh in range(2):
                qkvbufs[i][seg0 + sg, pl.ds(jrow + 8 + hh * 16, 16), :] = _pack(
                    y[sg * 32:(sg + 1) * 32, hh * 128:(hh + 1) * 128])

    for c_ in moda_copies(0):
        c_.wait()
    moda_apply(0, *moda_store(0, mod_tile(0, 0), mod_tile(1, 0)), 0, PRE)

    def chunk_block(kc, last, issue):
        with _scope('w_chunk'):
            for c_ in chunk_copies(kc) + ([cp_xr] if last else moda_copies(kc + 1)):
                c_.wait()
        issue()
        r0 = mult(kc * 64, 64)
        mv = []
        for i in range(NB):
            lo, hi = repack(w_v[i * 6, pl.ds(r0, 64), :], w_v[i * 6 + 1, pl.ds(r0, 64), :])
            w_v[i * 6, pl.ds(r0, 64), :] = lo
            w_v[i * 6 + 1, pl.ds(r0, 64), :] = hi
            w = pltpu.bitcast(jnp.concatenate([lo, hi], axis=1), BF)
            y = (pltpu.bitcast(wg_v[0:PRE, i * 256:(i + 1) * 256], F32)
                 + jnp.dot(pltpu.bitcast(h0buf[kc], BF), w, preferred_element_type=F32))
            if last:
                store_qkv(i, 0, y, 0)
            else:
                wg_v[0:PRE, i * 256:(i + 1) * 256] = pltpu.bitcast(y, U32)
                if i in (1, 3):
                    mv.append(mod_tile(i // 2, mult((kc + 1) * 128, 128)))
                if i == 3:
                    mv = moda_store(kc + 1, mv[0], mv[1])
                if i >= 4:
                    moda_apply(kc + 1, mv[0], mv[1], (i - 4) * 128, (i - 3) * 128)
        if last:
            for j in range(3):
                ln1_rows(PRE + 8 * j, HOFF + 8 + 8 * j)

    def chunk_body_a(kc, carry):
        def issue():
            for c_ in moda_copies(kc + 3) + chunk_copies(kc + 3):
                c_.start()
        chunk_block(kc, False, issue)
        return carry

    def chunk_body_b(kc, carry):
        chunk_block(kc, False, lambda: None)
        return carry

    def issue_last():
        w_start(2)
        mod_copy(2).start()
    lax.fori_loop(0, 5, chunk_body_a, 0)
    w_start(1)
    lax.fori_loop(5, 7, chunk_body_b, 0)
    chunk_block(7, True, issue_last)

    def pre_unit(j, i, extra):
        blk = (j // 3) * (6 * NB) + (j % 3) * 2 + i * 6
        jrow = pl.multiple_of(j * 40, 8)
        lo, hi = repack(w_v[blk], w_v[blk + 1])
        w_v[blk] = lo
        w_v[blk + 1] = hi
        for rc in range(PRE // 128):
            if rc > 0:
                lo = w_v[blk]
                hi = w_v[blk + 1]
            w = pltpu.bitcast(jnp.concatenate([lo, hi], axis=1), BF)
            lhs = jnp.concatenate([h0buf[k, rc * 64:(rc + 1) * 64, :] for k in range(8)], axis=1)
            y = jnp.dot(pltpu.bitcast(lhs, BF), w, preferred_element_type=F32)
            store_qkv(i, jrow, y, rc * 4)
            extra(rc)

    def pre_body(j, carry):
        @pl.when(j == 1)
        def _():
            for jn in (3, 4):
                w_start(jn)
                mod_copy(jn).start()

        @pl.when(j == 2)
        def _():
            w_start(5)
            mod_copy(5).start()
            cp_wo.start()
            cp_x1.start()
        blk0 = (j // 3) * (6 * NB) + (j % 3) * 2
        one = jnp.where((j == 1) | (j == 4), 1.0, 0.0).astype(F32)
        for half, (i0, i1) in enumerate(((0, PRE_SPLIT), (PRE_SPLIT, NB))):
            with _scope('w_pre'):
                for i in range(i0, i1):
                    for par in range(2):
                        pltpu.make_async_copy(w_hbms[0].at[:, 0, 0, :],
                                              w_v.at[blk0 + i * 6 + par],
                                              wsems.at[2 * j + half]).wait()
            if half == 1:
                @pl.when(j > 1)
                def _():
                    pltpu.make_async_copy(wmod32.at[:, 0:D], wmod_v.at[j],
                                          wsems.at[2 * j + 1]).wait()
            for i in range(i0, i1):
                def extra(rc, i=i):
                    n = (i - PRE_SPLIT) * 2 + rc // 2
                    if i >= PRE_SPLIT and rc % 2 == 0 and n < 8:
                        modb[j, :, n * 128:(n + 1) * 128] = _rb(one + mod_tile(j, n * 128))
                pre_unit(j, i, extra)
        return carry
    lax.fori_loop(1, 6, pre_body, 0)

    cp_wo.wait()
    cp_x1.wait()
    for c_ in cp_ffn:
        c_.start()

    def wo_w(h0, h1, n0, n1):
        w = wo_v[h0:h1, :, n0 * 128:n1 * 128].reshape((h1 - h0) * (DH // 2), (n1 - n0) * 128)
        return pltpu.bitcast(w, BF)

    HD = D // 2

    def emit_step(s, pend, last):
        hrow = pl.multiple_of(HOFF + (s & 1) * 32, 32)
        hnext = pl.multiple_of(HOFF + 32 - (s & 1) * 32, 32)
        tv = [tab[s * NTAB + k] for k in range(16)]
        slot = tv[0]
        dsts = [(tv[1 + 2 * j], pl.multiple_of(tv[2 + 2 * j], 4)) for j in range(3)]
        odst = [pl.multiple_of(tv[7 + j], 8) for j in range(4)]
        orow = pl.multiple_of(tv[11], 32)
        erow = tv[12]
        lrow = tv[13]
        erow2 = tv[14]
        mrow = pl.multiple_of(tv[15], 8)
        e_at, l_at = (E_AT, L_AT) if pend is None else (E_AT2, L_AT2)
        probs = {}

        def wqkv(p, k0, k1):
            return pltpu.bitcast(jnp.concatenate(
                [w_v[p * 6 + u, k0 // 2:k1 // 2, :] for u in range(6)], axis=1), BF)

        lhs_lo = act[pl.ds(hrow, 32), 0:HD]
        if pend is not None:
            ybuf[...] = jnp.dot(lhs_lo, wqkv(0, 0, HD), preferred_element_type=F32)
            pend()
        lhs_hi = act[pl.ds(hrow, 32), HD:D]
        if pend is not None:
            y0 = ybuf[...] + jnp.dot(lhs_hi, wqkv(0, HD, D), preferred_element_type=F32)
        lhs_rest = jnp.concatenate([lhs_lo[:, 128:], lhs_hi], axis=1)
        lhs = [jnp.concatenate([lhs_lo, lhs_hi], axis=1)]

        def side(p):
            for j in range(3):
                if e_at[j] == p:
                    finish_rows(pl.multiple_of(erow + 8 * j, 8), attn_load(j),
                                pl.multiple_of(erow2 + 8 * j, 8) if ECOL else None)
            for j in range(3):
                if l_at[j] == p:
                    ln1_rows(pl.multiple_of(lrow + 8 * j, 8),
                             pl.multiple_of(hnext + 8 + 8 * j, 8))
            if (p in e_at or p in l_at) and p < NP - 1:
                lhs[0] = jnp.concatenate([act[pl.ds(hrow, 32), 0:128], lhs_rest], axis=1)

        def qkv(p):
            if p == 0 and pend is not None:
                y = y0
            else:
                y = jnp.dot(lhs[0], wqkv(p, 0, D), preferred_element_type=F32)
            buf = qkvbufs[p % NB]
            for u in range(6):
                t, hh = u // 2, u % 2
                b0 = ((p // NB) * 3 + t) * 40
                yu = y[:, u * 128:(u + 1) * 128]
                buf[slot, b0 + hh * 4:b0 + hh * 4 + 4, :] = _pack(yu[0:8])
                for j in range(3):
                    sl, off = dsts[j]
                    buf[sl, pl.ds(b0 + 8 + hh * 16 + off, 4), :] = _pack(yu[8 + 8 * j:16 + 8 * j])

        def ld(p, t):
            b0 = ((p // NB) * 3 + t) * 40
            return pltpu.bitcast(qkvbufs[p % NB][slot, b0:b0 + 40, :], BF)

        def sc(p):
            s2 = lax.dot_general(ld(p, 0), ld(p, 1), (((1,), (1,)), ((), ())),
                                 preferred_element_type=F32)
            if SMX == 0:
                s2 = jnp.where(valid, s2 * SCALE, fill)
                m = jnp.max(s2, axis=-1, keepdims=True)
                e = jnp.exp(s2 - m)
            else:
                s2 = jnp.where(valid, s2, fill * (1.0 / SCALE))
                m = jnp.max(s2, axis=-1, keepdims=True)
                e = jnp.exp2((s2 - m) * (SCALE * LOG2E))
            l = jnp.sum(e, axis=-1, keepdims=True)
            rl = pl.reciprocal(l, approx=True)
            rl = rl * (2.0 - l * rl)
            probs[p] = (e * rl).astype(BF)

        def pv(p):
            o2 = jnp.dot(probs[p], ld(p, 2), preferred_element_type=F32)
            for hh in range(2):
                hcol = (2 * p + hh) * 128
                ob = obuf1
                if hcol >= KS:
                    ob = obuf2
                    hcol -= KS
                ob[pl.ds(mrow, 8), hcol:hcol + 128] = o2[8 * hh:8 * hh + 8].astype(BF)
                for j in range(4):
                    r0 = 16 + 32 * hh + 8 * j
                    ob[pl.ds(odst[j], 8), hcol:hcol + 128] = o2[r0:r0 + 8].astype(BF)

        def attn(pos):
            for kind, p in ATT.get(pos, ()):
                (sc if kind == 's' else pv)(p)

        for p in range(NP):
            qkv(p)
            side(p)
            attn(p)
        a1 = []
        for i in range(4):
            a1.append(jnp.dot(obuf1[pl.ds(orow, 32), 0:KS], wo_w(0, KS // DH, 2 * i, 2 * i + 2),
                              preferred_element_type=F32))
            attn(NP + i)
            side(NP + i)
        o2lhs = obuf2[pl.ds(orow, 32), 0:K2]
        a_lo = jnp.concatenate(a1[0:2], axis=1) + jnp.dot(
            o2lhs, wo_w(KS // DH, H, 0, 4), preferred_element_type=F32)
        act[pl.ds(hnext, 8), 0:HD] = a_lo[0:8].astype(BF)
        attn_store(a_lo[8:32], 0)
        a_hi = jnp.concatenate(a1[2:4], axis=1) + jnp.dot(
            o2lhs, wo_w(KS // DH, H, 4, 8), preferred_element_type=F32)

        def finish():
            act[pl.ds(hnext, 8), HD:D] = a_hi[0:8].astype(BF)
            attn_store(a_hi[8:32], 4)
        if last:
            finish()
        return finish

    def steps(it, carry):
        pend = None
        for u in range(UNR):
            pend = emit_step(it * UNR + u, pend, u == UNR - 1)
        return carry
    lax.fori_loop(0, NSEG // UNR, steps, 0)

    if SKIP:
        return
    for c_ in cp_ffn:
        c_.wait()
    OUT0 = (NSEG - 1) * RIDE
    NEW0 = S - NEW
    cp_out = [cp(act.at[OOFF:OOFF + OUT0], out_hbm.at[0, 0:OUT0], 9)]
    cp_out[0].start()
    zero = pl.multiple_of(tab[NSEG * NTAB], 8)
    for j in range(3):
        ebuf[EMAX + 8 * j:EMAX + 8 * j + 8, :] = attn_load(j)
    ebuf[EMAX + RIDE:EMAX + RIDE + 8, :] = act[HOFF:HOFF + 8, :].astype(F32)
    todo = [(OUT0 + 8 * j, EMAX + 8 * j) for j in range(4)]
    r0 = 0
    for ci, ech in enumerate(EPI_CHUNKS):
        o0 = NOSLOT * 32 + r0
        e0 = (ci % 2) * EMAX
        per = -(-len(todo) // 8)
        if ci == len(EPI_CHUNKS) - 1:
            per = EPI_LASTPER
        for n in range(8):
            lhs = jnp.concatenate([obuf1[o0:o0 + ech, 0:KS], obuf2[o0:o0 + ech, 0:K2]], axis=1)
            ebuf[e0:e0 + ech, n * 128:(n + 1) * 128] = jnp.dot(
                lhs, wo_w(0, H, n, n + 1), preferred_element_type=F32)
            for row, er in todo[:per]:
                finish_rows(row, ebuf[pl.ds(zero + er, 8), :])
            todo = todo[per:]
        todo = [(OUT0 + RIDE + 8 + r0 + 8 * j, e0 + 8 * j) for j in range(ech // 8)]
        r0 += ech

    rowsf = (lane256 * 8 + lax.broadcasted_iota(jnp.int32, (8, 256), 0)).astype(F32)
    r_old = jnp.where(rowsf < NEW0, act[ROFF:ROFF + 8, 0:256].astype(F32), -jnp.inf)

    def allmax(v):
        return jnp.max(jnp.max(v, axis=1, keepdims=True), axis=0, keepdims=True)

    def allmin(v):
        return jnp.min(jnp.min(v, axis=1, keepdims=True), axis=0, keepdims=True)
    m1 = allmax(r_old)
    i1v = allmin(jnp.where(r_old == m1, rowsf, float(S)))
    r_rest = jnp.where(rowsf == i1v, -jnp.inf, r_old)
    m2 = allmax(r_rest)
    i2v = allmin(jnp.where((r_rest == m2) & (rowsf != i1v), rowsf, float(S)))
    i1 = jnp.clip(i1v[0, 0].astype(jnp.int32), 0, NEW0 - 1)
    i2 = jnp.clip(i2v[0, 0].astype(jnp.int32), 0, NEW0 - 1)
    b1 = pl.multiple_of((i1 // 8) * 8, 8)
    b2 = pl.multiple_of((i2 // 8) * 8, 8)
    sub8 = lax.broadcasted_iota(jnp.int32, (8, 1), 0)

    def rep(i, n):
        return jnp.concatenate([modb[i]] * n, axis=0)
    x1c = jnp.concatenate([act[pl.ds(b1, 8), :].astype(F32), act[pl.ds(b2, 8), :].astype(F32)],
                          axis=0)
    h2c = _rb(_rb(_layernorm(x1c) * rep(4, 2)) + rep(3, 2))
    row1 = jnp.sum(jnp.where(sub8 == i1 - b1, h2c[0:8], 0.0), axis=0, keepdims=True)
    row2 = jnp.sum(jnp.where(sub8 == i2 - b2, h2c[8:16], 0.0), axis=0, keepdims=True)
    cand = jnp.where(sub8 == 0, row1, jnp.where(sub8 == 1, row2, 0.0))

    e0 = ((len(EPI_CHUNKS) - 1) % 2) * EMAX
    ng = NEW // 8
    x1n = _rb(xbuf[NEW0:S, :].astype(F32) + _rb(rep(2, ng) * _rb(ebuf[e0:e0 + NEW, :])))
    h2n = _rb(_rb(_layernorm(x1n) * rep(4, ng)) + rep(3, ng))
    h2b = jnp.concatenate([cand, h2n], axis=0).astype(BF)
    cp_out.append(cp(act.at[OOFF + OUT0:OOFF + NEW0], out_hbm.at[0, OUT0:NEW0], 10))
    cp_out[1].start()
    hid = []
    for n in range(0, F, FFN_NB):
        gt = _rb(jnp.dot(h2b, pltpu.bitcast(wg_v[:, n:n + FFN_NB], BF), preferred_element_type=F32))
        up = _rb(jnp.dot(h2b, pltpu.bitcast(wu_v[:, n:n + FFN_NB], BF), preferred_element_type=F32))
        hid.append((_rb(gt * _rb(jax.nn.sigmoid(gt))) * up).astype(BF))
    y = _rb(jnp.dot(jnp.concatenate(hid, axis=1), pltpu.bitcast(wd_v[...], BF),
                    preferred_element_type=F32))
    val = jnp.concatenate(
        [jnp.where(sub8 == 0, m1, jnp.where(sub8 == 1, m2, -jnp.inf)),
         _rb(jnp.sum(h2n * rep(6, ng), axis=-1, keepdims=True))], axis=0)
    pos = lax.broadcasted_iota(jnp.int32, (8 + NEW, 1), 0).astype(F32)
    p1 = jnp.min(jnp.where(val == jnp.max(val, axis=0, keepdims=True), pos, float(S)),
                 axis=0, keepdims=True)
    val2 = jnp.where(pos == p1, -jnp.inf, val)
    p2 = jnp.min(jnp.where((val2 == jnp.max(val2, axis=0, keepdims=True)) & (pos != p1), pos,
                           float(S)), axis=0, keepdims=True)
    upd = jnp.where((pos == p1) | (pos == p2), _rb(y * _rb(jax.nn.sigmoid(val))), 0.0)
    act[OOFF + NEW0:OOFF + S, :] = (x1n + _rb(rep(5, ng) * _rb(h2n + upd[8:]))).astype(BF)
    sub16 = lax.broadcasted_iota(jnp.int32, (16, 1), 0)
    grow = jnp.where(sub16 < 8, b1 + sub16, b2 + sub16 - 8)
    updc = jnp.where(grow == i1, upd[0:1], jnp.where(grow == i2, upd[1:2], 0.0))
    res = (x1c + _rb(rep(5, 2) * _rb(h2c + updc))).astype(BF)
    for c_ in cp_out:
        c_.wait()
    act[pl.ds(OOFF + b1, 8), :] = res[0:8]
    act[pl.ds(OOFF + b2, 8), :] = res[8:16]
    fix0 = cp(act.at[OOFF + NEW0:OOFF + S], out_hbm.at[0, NEW0:S], 6)
    fix1 = cp(act.at[pl.ds(OOFF + b1, 8)], out_hbm.at[0, pl.ds(b1, 8)], 11)
    fix2 = cp(act.at[pl.ds(OOFF + b2, 8)], out_hbm.at[0, pl.ds(b2, 8)], 12)
    fix0.start()
    fix1.start()

    @pl.when(b1 != b2)
    def _():
        fix2.start()
        fix2.wait()
    fix0.wait()
    fix1.wait()


@jax.jit
def pallas_adaLN_cond__memory_aug_recurrent_mem_tr__moe_arch_mod__prompt_kernel(
    A_x: jax.Array,
    A_mem0: jax.Array,
    A_Wq: jax.Array,
    A_Wk: jax.Array,
    A_Wv: jax.Array,
    A_Wo: jax.Array,
    A_seg_len,
    B_x: jax.Array,
    B_w_r: jax.Array,
    B_w_gate: jax.Array,
    B_w_up: jax.Array,
    B_w_down: jax.Array,
    c: jax.Array,
    w_mod: jax.Array,
):
    del B_x
    del A_seg_len
    assert A_x.shape == (1, S, D) and A_Wq.shape == (D, H, DH) and A_mem0.shape == (1, M, D)
    any_spec = pl.BlockSpec(memory_space=pl.ANY)
    scratch = [
        pltpu.VMEM((S if not XACT else 8, D), BF),
        pltpu.VMEM((XOFF + S * XACT, D), BF),
        pltpu.VMEM((8, PRE // 2, 128), U32),
        pltpu.VMEM((32, 768), F32),
        pltpu.VMEM((2 * EMAX, D), F32),
        pltpu.SMEM((NSEG * NTAB + 1,), jnp.int32),
        pltpu.VMEM((7, 8, D), F32),
        pltpu.VMEM((4, 1, D), BF),
        pltpu.VMEM((3 * H, D // 2, 128), U32),
        pltpu.VMEM((H, DH // 2, D), U32),
        pltpu.VMEM((6, D // 2, D), U32),
        pltpu.VMEM((D // 2, F), U32),
        pltpu.VMEM((D // 2, F), U32),
        pltpu.VMEM((F // 2, D), U32),
        pltpu.VMEM((NOSLOT * 32 + PRE, OW1), BF),
        pltpu.VMEM((NOSLOT * 32 + PRE, OW2), BF),
        pltpu.SemaphoreType.DMA((17,)),
        pltpu.SemaphoreType.DMA((12,)),
        pltpu.SemaphoreType.DMA((16,)),
    ] + [pltpu.VMEM((NSLOT + 1, 256, 128), U32) for _ in range(NB)] + [
        pltpu.VMEM((D,), BF),
    ]
    wq, wk, wv = (w.reshape(D // 2, 2, H, DH) for w in (A_Wq, A_Wk, A_Wv))
    return pl.pallas_call(
        _kernel,
        out_shape=jax.ShapeDtypeStruct((1, S, D), BF),
        in_specs=[any_spec] * 12,
        out_specs=any_spec,
        scratch_shapes=scratch,
        compiler_params=pltpu.CompilerParams(vmem_limit_bytes=120 * 1024 * 1024,
                                             disable_bounds_checks=True,
                                             disable_semaphore_checks=True),
    )(A_x, A_mem0, wq, wk, wv, A_Wo, B_w_r, B_w_gate, B_w_up, B_w_down,
      c, w_mod)
```

```python
import contextlib
import os
import jax
import jax.numpy as jnp
from jax import lax
import jax.experimental.pallas as pl
import jax.experimental.pallas.tpu as pltpu

BF = jnp.bfloat16
F32 = jnp.float32
U32 = jnp.uint32

S = 2048
D = 1024
H = 32
DH = 128
M = 8
SEG = 32
NSEG = S // SEG
F = 3584
NP = H // 2
RIDE = 24
PRE = S - NSEG * RIDE
NSLOT = 17
NOSLOT = 17
NB = int(os.environ.get('NB', 8))
KS = int(os.environ.get('KS', 2304))
LAG_S = 1
LAG_P = 3
EPS = 1e-5
SCALE = DH ** -0.5
OOFF = S
HOFF = 2 * S
ROFF = HOFF + 64
XOFF = ROFF + 16
PRE_SPLIT = int(os.environ.get('PRE_SPLIT', 3))
E_AT = tuple(int(v) for v in os.environ.get('E_AT', '2,3,5').split(','))
L_AT = tuple(int(v) for v in os.environ.get('L_AT', '8,10,12').split(','))
E_AT2 = tuple(int(v) for v in os.environ.get('E_AT2', '3,5,6').split(','))
L_AT2 = tuple(int(v) for v in os.environ.get('L_AT2', '8,10,12').split(','))


def _att_schedule(mode):
    att = {}
    if mode == 'lag':
        for p in range(NP):
            att.setdefault(p + LAG_S, []).append(('s', p))
        for p in range(NP):
            att.setdefault(p + LAG_P, []).append(('p', p))
    elif mode == 'q2':
        for p in range(0, NP, 2):
            att.setdefault(p + 2, []).extend([('s', p), ('s', p + 1)])
        for p in range(0, NP, 2):
            att.setdefault(p + 4, []).extend([('p', p), ('p', p + 1)])
    elif mode == 'q2b':
        for p in range(0, NP, 2):
            att.setdefault(p + 4, []).extend([('p', p), ('p', p + 1)])
        for p in range(0, NP, 2):
            att.setdefault(p + 2, []).extend([('s', p), ('s', p + 1)])
    elif mode == 'q2c':
        att[4] = [('s', i) for i in range(4)]
        for p in range(4, NP, 2):
            att[p + 2] = [('s', p), ('s', p + 1), ('p', p - 4), ('p', p - 3)]
        att[18] = [('p', i) for i in range(12, 16)]
    elif mode == 'q2d':
        att[3] = [('s', i) for i in range(3)]
        att[4] = [('s', 3)]
        att[3] = []
        att[4] = [('s', i) for i in range(4)]
        for p in range(4, NP, 2):
            att[p + 2] = [('p', p - 4), ('p', p - 3), ('s', p), ('s', p + 1)]
        att[18] = [('p', i) for i in range(12, 16)]
    elif mode == 'q4':
        for p in range(0, NP, 4):
            att.setdefault(p + 4, []).extend([('s', p + i) for i in range(4)])
            att.setdefault(p + 6, []).extend([('p', p + i) for i in range(4)])
    elif mode == 'q4b':
        for p in range(0, NP, 4):
            att.setdefault(min(p + 8, 18), []).extend([('p', p + i) for i in range(4)])
        for p in range(0, NP, 4):
            att.setdefault(p + 4, []).extend([('s', p + i) for i in range(4)])
    return att


ATT = _att_schedule(os.environ.get('ATT', 'q2c'))
XACT = int(os.environ.get('XACT', 0))
K2 = H * DH - KS
OPAD = int(os.environ.get('OPAD', 1))
OW1 = -(-KS // 1024) * 1024 if OPAD else KS
OW2 = -(-K2 // 1024) * 1024 if OPAD else K2
SMX = int(os.environ.get('SMX', 0))
LOG2E = 1.4426950408889634
SKIP = int(os.environ.get('SKIP', 0))
A_BUF = tuple(int(v) for v in os.environ.get('A_BUF', '7,0,1').split(','))
ECOL = int(os.environ.get('ECOL', 0))
ONELOOP = int(os.environ.get('ONELOOP', 1))
BULK = int(os.environ.get('BULK', 0))
UNR = int(os.environ.get('UNR', 2))
EPI_CHUNKS = tuple(int(v) for v in os.environ.get('EPI', '64,64,64,64,64,64,48,48,32').split(','))
EMAX = max(EPI_CHUNKS)
NEW = 24
EPI_LASTPER = int(os.environ.get('EPI_LASTPER', 2))
FFN_NB = int(os.environ.get('FFN_NB', 512))


NTAB = 16


def _step_indices(s):
    t = [s % NSLOT]
    for j in range(3):
        gi = PRE // 8 + 3 * s + j
        t += [(gi // 4) % NSLOT, (gi % 4) * 4]
    for j in range(4):
        gi = 4 * s + j
        if gi < 3 * NSEG:
            t.append(((gi // 3) % NOSLOT) * 32 + 8 + (gi % 3) * 8)
        elif gi == 3 * NSEG:
            t.append(((NSEG - 1) % NOSLOT) * 32)
        else:
            t.append(NOSLOT * 32 + (gi - 3 * NSEG - 1) * 8)
    t.append((s % NOSLOT) * 32)
    t.append(max(s - 1, 0) * RIDE)
    t.append(PRE + min(s + 1, NSEG - 1) * RIDE)
    t.append(max(s - 1, 0) * RIDE)
    t.append((s % NOSLOT) * 32 if s < NSEG - 1 else NOSLOT * 32 + PRE - 8)
    return t


def _scope(name):
    return jax.named_scope(name) if os.environ.get('PROF') else contextlib.nullcontext()


def _rb(v):
    return v.astype(BF).astype(F32)


def _pack(v):
    return pltpu.bitcast(v.astype(BF), U32)


def _ln_stats(x):
    mu = jnp.sum(x, axis=-1, keepdims=True) * (1.0 / D)
    xc = x - mu
    var = jnp.sum(xc * xc, axis=-1, keepdims=True) * (1.0 / D)
    return _rb(mu), _rb(jnp.sqrt(_rb(_rb(var) + EPS)))


def _layernorm(x):
    mu, sd = _ln_stats(x)
    return _rb(_rb(x - mu) / sd)


def _kernel(x_hbm, mem0_hbm, wq_hbm, wk_hbm, wv_hbm, wo_hbm, wr_hbm, wg_hbm, wu_hbm,
            wd_hbm, c_hbm, wmod_hbm, out_hbm,
            xbuf, act, h0buf, ybuf, ebuf, tab, modb, small,
            w_v, wo_v, wmod_v, wg_v, wu_v, wd_v,
            obuf1, obuf2, sems, wsems, ksems, *rest):
    qkvbufs, wrbuf = rest[:NB], rest[NB]
    if XACT:
        xbuf = act.at[pl.ds(XOFF, S)]
    w_hbms = tuple(w.bitcast(U32) for w in (wq_hbm, wk_hbm, wv_hbm))

    def cp(src, dst, i):
        return pltpu.make_async_copy(src, dst, sems.at[i])

    wmod32 = wmod_hbm.bitcast(U32)
    cp_c = cp(c_hbm, small.at[0], 0)
    cp_mem = cp(mem0_hbm.at[0], act.at[HOFF:HOFF + M], 1)
    cp_wr = cp(wr_hbm, wrbuf, 2)
    cp_x0 = [cp(x_hbm.at[0, n * 128:(n + 1) * 128], xbuf.at[n * 128:(n + 1) * 128], 13 + n)
             for n in range(PRE // 128)]
    cp_xr = cp(x_hbm.at[0, PRE:PRE + 32], xbuf.at[PRE:PRE + 32], 5)
    cp_x1 = cp(x_hbm.at[0, PRE + 32:S], xbuf.at[PRE + 32:S], 4)
    cp_wo = cp(wo_hbm.bitcast(U32), wo_v, 7)
    cp_ffn = [cp(wg_hbm.bitcast(U32), wg_v, 8), cp(wu_hbm.bitcast(U32), wu_v, 8),
              cp(wd_hbm.bitcast(U32), wd_v, 8)]

    def w_start(j, prio=BULK, i0=0, i1=NB):
        gg, t = j // 3, j % 3
        for i in range(i0, i1):
            for par in range(2):
                pltpu.make_async_copy(w_hbms[t].at[:, par, gg * NB + i, :],
                                      w_v.at[(gg * NB + i) * 6 + t * 2 + par],
                                      wsems.at[2 * j + (i >= PRE_SPLIT)]).start(priority=prio)

    def mod_copy(j):
        return pltpu.make_async_copy(wmod32.at[:, j * D:(j + 1) * D], wmod_v.at[j],
                                     wsems.at[2 * j + 1])

    def mult(v, m):
        return v if isinstance(v, int) else pl.multiple_of(v, m)

    def moda_copies(kc):
        col = mult(kc * 128, 128)
        return [pltpu.make_async_copy(wmod32.at[:, pl.ds(v * D + col, 128)],
                                      wmod_v.at[v, :, pl.ds(col, 128)], ksems.at[8 + kc])
                for v in range(2)]

    def chunk_copies(kc):
        r0 = mult(kc * 64, 64)
        return [pltpu.make_async_copy(w_hbms[0].at[pl.ds(r0, 64), par, i, :],
                                      w_v.at[i * 6 + par, pl.ds(r0, 64), :], ksems.at[kc])
                for i in range(NB) for par in range(2)]

    cp_c.start()
    cp_mem.start()
    cp_wr.start()
    for c_ in (cp_x0 + moda_copies(0) + moda_copies(1) + chunk_copies(0) + moda_copies(2)
               + chunk_copies(1) + [cp_xr] + chunk_copies(2)):
        c_.start()

    def ln1_rows(src_row, dst_row):
        xv = xbuf[pl.ds(src_row, 8), :].astype(F32)
        hv = _rb(_layernorm(xv) * modb[1]) + modb[0]
        act[pl.ds(dst_row, 8), :] = hv.astype(BF)

    lane256 = lax.broadcasted_iota(jnp.int32, (8, 256), 1)

    def finish_rows(row, attn, row2=None):
        xv = xbuf[pl.ds(row, 8), :].astype(F32)
        x1 = _rb(xv + _rb(modb[2] * _rb(attn)))
        act[pl.ds(row, 8), :] = x1.astype(BF)
        if row2 is None:
            h2 = _rb(_rb(_layernorm(x1) * modb[4]) + modb[3])
            act[pl.ds(OOFF + row, 8), :] = (x1 + _rb(modb[5] * h2)).astype(BF)
            hw = h2 * modb[6]
        else:
            mu, sd = _ln_stats(x1)
            hw = None
            for c0 in range(0, D, ECOL):
                cs = slice(c0, c0 + ECOL)
                xb = act[pl.ds(row2, 8), cs].astype(F32)
                h2 = _rb(_rb(_rb(_rb(xb - mu) / sd) * modb[4, :, cs]) + modb[3, :, cs])
                act[pl.ds(OOFF + row, 8), cs] = (xb + _rb(modb[5, :, cs] * h2)).astype(BF)
                t = h2 * modb[6, :, cs]
                hw = t if hw is None else hw + t
        r = jnp.sum(hw, axis=-1, keepdims=True)
        act[ROFF:ROFF + 8, 0:256] = jnp.where(
            lane256 * 8 == row, r, act[ROFF:ROFF + 8, 0:256].astype(F32)).astype(BF)

    def attn_store(a, k0):
        for j in range(3):
            for k in range(a.shape[1] // 128):
                qkvbufs[A_BUF[j]][NSLOT, (k0 + k) * 8:(k0 + k + 1) * 8, :] = pltpu.bitcast(
                    a[8 * j:8 * j + 8, k * 128:(k + 1) * 128], U32)

    def attn_load(j):
        return pltpu.bitcast(jnp.concatenate(
            [qkvbufs[A_BUF[j]][NSLOT, k * 8:(k + 1) * 8, :] for k in range(8)], axis=1), F32)

    act[ROFF:ROFF + 8, 0:256] = jnp.zeros((8, 256), BF)
    attn_store(jnp.zeros((RIDE, D), F32), 0)
    for s_ in range(NSEG):
        for k, v in enumerate(_step_indices(s_)):
            tab[s_ * NTAB + k] = v
    tab[NSEG * NTAB] = 0
    ri = lax.broadcasted_iota(jnp.int32, (80, 80), 0)
    ci = lax.broadcasted_iota(jnp.int32, (80, 80), 1)

    def head_pos(i):
        hd = jnp.where(i < 16, i // 8, (i - 16) // 32)
        pos = jnp.where(i < 16, i % 8, 8 + (i - 16) % 32)
        return hd, pos
    rh, rp = head_pos(ri)
    ch, cpos = head_pos(ci)
    same = rh == ch
    valid = same & ((rp < M) | (rp >= cpos))
    fill = jnp.where(same, -1e9, -jnp.inf).astype(F32)

    cp_mem.wait()
    cp_wr.wait()
    modb[6] = jnp.broadcast_to(wrbuf[...].astype(F32).reshape(1, D), (8, D))
    cp_c.wait()
    cv = small[0].astype(F32)
    sc16 = jnp.broadcast_to(_rb(cv * _rb(jax.nn.sigmoid(cv))), (16, D)).astype(BF)

    def ln_pre(g, carry):
        pltpu.make_async_copy(x_hbm.at[0, 0:128], xbuf.at[pl.ds(pl.multiple_of(g * 128, 128), 128)],
                              sems.at[13 + g]).wait()
        for u in range(2):
            row = pl.multiple_of(g * 128 + u * 64, 64)
            nv = _layernorm(xbuf[pl.ds(row, 64), :].astype(F32)).astype(BF)
            for k in range(8):
                h0buf[k, pl.ds(pl.multiple_of(row // 2, 32), 32), :] = pltpu.bitcast(
                    nv[:, k * 128:(k + 1) * 128], U32)
            wg_v[pl.ds(row, 64), 0:2 * D] = jnp.zeros((64, 2 * D), U32)
        return carry
    lax.fori_loop(0, PRE // 128, ln_pre, 0)

    def mod_tile(v, col):
        w = pltpu.bitcast(wmod_v[v, :, pl.ds(col, 128)], BF)
        return _rb(jnp.dot(sc16, w, preferred_element_type=F32))[0:8]

    def moda_store(kc, sa, ca):
        col = mult(kc * 128, 128)
        c1 = _rb(1.0 + ca)
        modb[0, :, pl.ds(col, 128)] = sa
        modb[1, :, pl.ds(col, 128)] = c1
        return sa, c1

    def moda_apply(kc, sa, c1, r0, r1):
        for r in range(r0, r1, 16):
            nv = pltpu.bitcast(h0buf[kc, r // 2:r // 2 + 8, :], BF).astype(F32).reshape(2, 8, 128)
            hv = (_rb(nv * c1[None]) + sa[None]).reshape(16, 128).astype(BF)
            h0buf[kc, r // 2:r // 2 + 8, :] = pltpu.bitcast(hv, U32)

    def repack(a, b):
        return (a & U32(0xFFFF)) | (b << 16), (a >> 16) | (b & U32(0xFFFF0000))

    def store_qkv(i, jrow, y, seg0):
        for sg in range(y.shape[0] // 32):
            for hh in range(2):
                qkvbufs[i][seg0 + sg, pl.ds(jrow + 8 + hh * 16, 16), :] = _pack(
                    y[sg * 32:(sg + 1) * 32, hh * 128:(hh + 1) * 128])

    for c_ in moda_copies(0):
        c_.wait()
    moda_apply(0, *moda_store(0, mod_tile(0, 0), mod_tile(1, 0)), 0, PRE)

    def w_wait(j, i0, i1):
        blk0 = (j // 3) * (6 * NB) + (j % 3) * 2
        with _scope('w_pre'):
            for i in range(i0, i1):
                for par in range(2):
                    pltpu.make_async_copy(w_hbms[0].at[:, 0, 0, :], w_v.at[blk0 + i * 6 + par],
                                          wsems.at[2 * j + (i >= PRE_SPLIT)]).wait()

    def chunk_block(kc, last, issue):
        with _scope('w_chunk'):
            for c_ in chunk_copies(kc) + ([cp_xr] if last else moda_copies(kc + 1)):
                c_.wait()
        issue()
        r0 = mult(kc * 64, 64)
        mv = []
        for i in range(NB):
            lo, hi = repack(w_v[i * 6, pl.ds(r0, 64), :], w_v[i * 6 + 1, pl.ds(r0, 64), :])
            w_v[i * 6, pl.ds(r0, 64), :] = lo
            w_v[i * 6 + 1, pl.ds(r0, 64), :] = hi
            w = pltpu.bitcast(jnp.concatenate([lo, hi], axis=1), BF)
            y = (pltpu.bitcast(wg_v[0:PRE, i * 256:(i + 1) * 256], F32)
                 + jnp.dot(pltpu.bitcast(h0buf[kc], BF), w, preferred_element_type=F32))
            if last:
                store_qkv(i, 0, y, 0)
            else:
                wg_v[0:PRE, i * 256:(i + 1) * 256] = pltpu.bitcast(y, U32)
                if i in (1, 3):
                    mv.append(mod_tile(i // 2, mult((kc + 1) * 128, 128)))
                if i == 3:
                    mv = moda_store(kc + 1, mv[0], mv[1])
                if i >= 4:
                    moda_apply(kc + 1, mv[0], mv[1], (i - 4) * 128, (i - 3) * 128)
        if last:
            for j in range(3):
                ln1_rows(PRE + 8 * j, HOFF + 8 + 8 * j)

    def chunk_body_a(kc, carry):
        def issue():
            if ONELOOP:
                @pl.when(kc < 5)
                def _():
                    for c_ in moda_copies(kc + 3) + chunk_copies(kc + 3):
                        c_.start()
            else:
                for c_ in moda_copies(kc + 3) + chunk_copies(kc + 3):
                    c_.start()
        chunk_block(kc, False, issue)
        return carry

    def chunk_body_b(kc, carry):
        chunk_block(kc, False, lambda: None)
        return carry

    def issue_last():
        w_wait(1, 0, PRE_SPLIT)
        w_start(1, 0, PRE_SPLIT, NB)
        w_start(2)
        mod_copy(2).start(priority=BULK)
    if ONELOOP:
        w_start(1, 1, 0, PRE_SPLIT)
        lax.fori_loop(0, 7, chunk_body_a, 0)
    else:
        lax.fori_loop(0, 5, chunk_body_a, 0)
        w_start(1)
        lax.fori_loop(5, 7, chunk_body_b, 0)
    chunk_block(7, True, issue_last)

    def pre_unit(j, i, extra):
        blk = (j // 3) * (6 * NB) + (j % 3) * 2 + i * 6
        jrow = mult(j * 40, 8)
        lo, hi = repack(w_v[blk], w_v[blk + 1])
        w_v[blk] = lo
        w_v[blk + 1] = hi
        for rc in range(PRE // 128):
            if rc > 0:
                lo = w_v[blk]
                hi = w_v[blk + 1]
            w = pltpu.bitcast(jnp.concatenate([lo, hi], axis=1), BF)
            lhs = jnp.concatenate([h0buf[k, rc * 64:(rc + 1) * 64, :] for k in range(8)], axis=1)
            y = jnp.dot(pltpu.bitcast(lhs, BF), w, preferred_element_type=F32)
            store_qkv(i, jrow, y, rc * 4)
            extra(rc)

    for i in range(NB):
        if i == PRE_SPLIT:
            w_wait(1, PRE_SPLIT, NB)
            for jn in (3, 4):
                w_start(jn)
                mod_copy(jn).start(priority=BULK)
        pre_unit(1, i, lambda rc: None)
    w_start(5)
    mod_copy(5).start(priority=BULK)
    cp_wo.start(priority=BULK)
    cp_x1.start(priority=BULK)

    def pre_body(j, carry):
        w_wait(j, 0, NB)
        pltpu.make_async_copy(wmod32.at[:, 0:D], wmod_v.at[j], wsems.at[2 * j + 1]).wait()
        one = jnp.where(j == 4, 1.0, 0.0).astype(F32)
        for i in range(NB):
            def extra(rc, i=i):
                if rc == 1:
                    modb[j, :, i * 128:(i + 1) * 128] = _rb(one + mod_tile(j, i * 128))
            pre_unit(j, i, extra)
        return carry
    lax.fori_loop(2, 6, pre_body, 0)

    cp_wo.wait()
    cp_x1.wait()
    for c_ in cp_ffn:
        c_.start(priority=BULK)

    def wo_w(h0, h1, n0, n1):
        w = wo_v[h0:h1, :, n0 * 128:n1 * 128].reshape((h1 - h0) * (DH // 2), (n1 - n0) * 128)
        return pltpu.bitcast(w, BF)

    HD = D // 2

    def emit_step(s, pend, last):
        hrow = pl.multiple_of(HOFF + (s & 1) * 32, 32)
        hnext = pl.multiple_of(HOFF + 32 - (s & 1) * 32, 32)
        tv = [tab[s * NTAB + k] for k in range(16)]
        slot = tv[0]
        dsts = [(tv[1 + 2 * j], pl.multiple_of(tv[2 + 2 * j], 4)) for j in range(3)]
        odst = [pl.multiple_of(tv[7 + j], 8) for j in range(4)]
        orow = pl.multiple_of(tv[11], 32)
        erow = tv[12]
        lrow = tv[13]
        erow2 = tv[14]
        mrow = pl.multiple_of(tv[15], 8)
        e_at, l_at = (E_AT, L_AT) if pend is None else (E_AT2, L_AT2)
        probs = {}

        def wqkv(p, k0, k1):
            return pltpu.bitcast(jnp.concatenate(
                [w_v[p * 6 + u, k0 // 2:k1 // 2, :] for u in range(6)], axis=1), BF)

        lhs_lo = act[pl.ds(hrow, 32), 0:HD]
        if pend is not None:
            ybuf[...] = jnp.dot(lhs_lo, wqkv(0, 0, HD), preferred_element_type=F32)
            pend()
        lhs_hi = act[pl.ds(hrow, 32), HD:D]
        if pend is not None:
            y0 = ybuf[...] + jnp.dot(lhs_hi, wqkv(0, HD, D), preferred_element_type=F32)
        lhs_rest = jnp.concatenate([lhs_lo[:, 128:], lhs_hi], axis=1)
        lhs = [jnp.concatenate([lhs_lo, lhs_hi], axis=1)]

        def side(p):
            for j in range(3):
                if e_at[j] == p:
                    finish_rows(pl.multiple_of(erow + 8 * j, 8), attn_load(j),
                                pl.multiple_of(erow2 + 8 * j, 8) if ECOL else None)
            for j in range(3):
                if l_at[j] == p:
                    ln1_rows(pl.multiple_of(lrow + 8 * j, 8),
                             pl.multiple_of(hnext + 8 + 8 * j, 8))
            if (p in e_at or p in l_at) and p < NP - 1:
                lhs[0] = jnp.concatenate([act[pl.ds(hrow, 32), 0:128], lhs_rest], axis=1)

        def qkv(p):
            if p == 0 and pend is not None:
                y = y0
            else:
                y = jnp.dot(lhs[0], wqkv(p, 0, D), preferred_element_type=F32)
            buf = qkvbufs[p % NB]
            for u in range(6):
                t, hh = u // 2, u % 2
                b0 = ((p // NB) * 3 + t) * 40
                yu = y[:, u * 128:(u + 1) * 128]
                buf[slot, b0 + hh * 4:b0 + hh * 4 + 4, :] = _pack(yu[0:8])
                for j in range(3):
                    sl, off = dsts[j]
                    buf[sl, pl.ds(b0 + 8 + hh * 16 + off, 4), :] = _pack(yu[8 + 8 * j:16 + 8 * j])

        def ld(p, t):
            b0 = ((p // NB) * 3 + t) * 40
            return pltpu.bitcast(qkvbufs[p % NB][slot, b0:b0 + 40, :], BF)

        def sc(p):
            s2 = lax.dot_general(ld(p, 0), ld(p, 1), (((1,), (1,)), ((), ())),
                                 preferred_element_type=F32)
            if SMX == 0:
                s2 = jnp.where(valid, s2 * SCALE, fill)
                m = jnp.max(s2, axis=-1, keepdims=True)
                e = jnp.exp(s2 - m)
            else:
                s2 = jnp.where(valid, s2, fill * (1.0 / SCALE))
                m = jnp.max(s2, axis=-1, keepdims=True)
                e = jnp.exp2((s2 - m) * (SCALE * LOG2E))
            l = jnp.sum(e, axis=-1, keepdims=True)
            rl = pl.reciprocal(l, approx=True)
            rl = rl * (2.0 - l * rl)
            probs[p] = (e * rl).astype(BF)

        def pv(p):
            o2 = jnp.dot(probs[p], ld(p, 2), preferred_element_type=F32)
            for hh in range(2):
                hcol = (2 * p + hh) * 128
                ob = obuf1
                if hcol >= KS:
                    ob = obuf2
                    hcol -= KS
                ob[pl.ds(mrow, 8), hcol:hcol + 128] = o2[8 * hh:8 * hh + 8].astype(BF)
                for j in range(4):
                    r0 = 16 + 32 * hh + 8 * j
                    ob[pl.ds(odst[j], 8), hcol:hcol + 128] = o2[r0:r0 + 8].astype(BF)

        def attn(pos):
            for kind, p in ATT.get(pos, ()):
                (sc if kind == 's' else pv)(p)

        for p in range(NP):
            qkv(p)
            side(p)
            attn(p)
        a1 = []
        for i in range(4):
            a1.append(jnp.dot(obuf1[pl.ds(orow, 32), 0:KS], wo_w(0, KS // DH, 2 * i, 2 * i + 2),
                              preferred_element_type=F32))
            attn(NP + i)
            side(NP + i)
        o2lhs = obuf2[pl.ds(orow, 32), 0:K2]
        a_lo = jnp.concatenate(a1[0:2], axis=1) + jnp.dot(
            o2lhs, wo_w(KS // DH, H, 0, 4), preferred_element_type=F32)
        act[pl.ds(hnext, 8), 0:HD] = a_lo[0:8].astype(BF)
        attn_store(a_lo[8:32], 0)
        a_hi = jnp.concatenate(a1[2:4], axis=1) + jnp.dot(
            o2lhs, wo_w(KS // DH, H, 4, 8), preferred_element_type=F32)

        def finish():
            act[pl.ds(hnext, 8), HD:D] = a_hi[0:8].astype(BF)
            attn_store(a_hi[8:32], 4)
        if last:
            finish()
        return finish

    def steps(it, carry):
        pend = None
        for u in range(UNR):
            pend = emit_step(it * UNR + u, pend, u == UNR - 1)
        return carry
    lax.fori_loop(0, NSEG // UNR, steps, 0)

    if SKIP:
        return
    for c_ in cp_ffn:
        c_.wait()
    OUT0 = (NSEG - 1) * RIDE
    NEW0 = S - NEW
    cp_out = [cp(act.at[OOFF:OOFF + OUT0], out_hbm.at[0, 0:OUT0], 9)]
    cp_out[0].start()
    zero = pl.multiple_of(tab[NSEG * NTAB], 8)
    for j in range(3):
        ebuf[EMAX + 8 * j:EMAX + 8 * j + 8, :] = attn_load(j)
    ebuf[EMAX + RIDE:EMAX + RIDE + 8, :] = act[HOFF:HOFF + 8, :].astype(F32)
    todo = [(OUT0 + 8 * j, EMAX + 8 * j) for j in range(4)]
    r0 = 0
    for ci, ech in enumerate(EPI_CHUNKS):
        o0 = NOSLOT * 32 + r0
        e0 = (ci % 2) * EMAX
        per = -(-len(todo) // 8)
        if ci == len(EPI_CHUNKS) - 1:
            per = EPI_LASTPER
        for n in range(8):
            lhs = jnp.concatenate([obuf1[o0:o0 + ech, 0:KS], obuf2[o0:o0 + ech, 0:K2]], axis=1)
            ebuf[e0:e0 + ech, n * 128:(n + 1) * 128] = jnp.dot(
                lhs, wo_w(0, H, n, n + 1), preferred_element_type=F32)
            for row, er in todo[:per]:
                finish_rows(row, ebuf[pl.ds(zero + er, 8), :])
            todo = todo[per:]
        todo = [(OUT0 + RIDE + 8 + r0 + 8 * j, e0 + 8 * j) for j in range(ech // 8)]
        r0 += ech

    rowsf = (lane256 * 8 + lax.broadcasted_iota(jnp.int32, (8, 256), 0)).astype(F32)
    r_old = jnp.where(rowsf < NEW0, act[ROFF:ROFF + 8, 0:256].astype(F32), -jnp.inf)

    def allmax(v):
        return jnp.max(jnp.max(v, axis=1, keepdims=True), axis=0, keepdims=True)

    def allmin(v):
        return jnp.min(jnp.min(v, axis=1, keepdims=True), axis=0, keepdims=True)
    m1 = allmax(r_old)
    i1v = allmin(jnp.where(r_old == m1, rowsf, float(S)))
    r_rest = jnp.where(rowsf == i1v, -jnp.inf, r_old)
    m2 = allmax(r_rest)
    i2v = allmin(jnp.where((r_rest == m2) & (rowsf != i1v), rowsf, float(S)))
    i1 = jnp.clip(i1v[0, 0].astype(jnp.int32), 0, NEW0 - 1)
    i2 = jnp.clip(i2v[0, 0].astype(jnp.int32), 0, NEW0 - 1)
    b1 = pl.multiple_of((i1 // 8) * 8, 8)
    b2 = pl.multiple_of((i2 // 8) * 8, 8)
    sub8 = lax.broadcasted_iota(jnp.int32, (8, 1), 0)

    def rep(i, n):
        return jnp.concatenate([modb[i]] * n, axis=0)
    x1c = jnp.concatenate([act[pl.ds(b1, 8), :].astype(F32), act[pl.ds(b2, 8), :].astype(F32)],
                          axis=0)
    h2c = _rb(_rb(_layernorm(x1c) * rep(4, 2)) + rep(3, 2))
    row1 = jnp.sum(jnp.where(sub8 == i1 - b1, h2c[0:8], 0.0), axis=0, keepdims=True)
    row2 = jnp.sum(jnp.where(sub8 == i2 - b2, h2c[8:16], 0.0), axis=0, keepdims=True)
    cand = jnp.where(sub8 == 0, row1, jnp.where(sub8 == 1, row2, 0.0))

    e0 = ((len(EPI_CHUNKS) - 1) % 2) * EMAX
    ng = NEW // 8
    x1n = _rb(xbuf[NEW0:S, :].astype(F32) + _rb(rep(2, ng) * _rb(ebuf[e0:e0 + NEW, :])))
    h2n = _rb(_rb(_layernorm(x1n) * rep(4, ng)) + rep(3, ng))
    h2b = jnp.concatenate([cand, h2n], axis=0).astype(BF)
    cp_out.append(cp(act.at[OOFF + OUT0:OOFF + NEW0], out_hbm.at[0, OUT0:NEW0], 10))
    cp_out[1].start()
    hid = []
    for n in range(0, F, FFN_NB):
        gt = _rb(jnp.dot(h2b, pltpu.bitcast(wg_v[:, n:n + FFN_NB], BF), preferred_element_type=F32))
        up = _rb(jnp.dot(h2b, pltpu.bitcast(wu_v[:, n:n + FFN_NB], BF), preferred_element_type=F32))
        hid.append((_rb(gt * _rb(jax.nn.sigmoid(gt))) * up).astype(BF))
    y = _rb(jnp.dot(jnp.concatenate(hid, axis=1), pltpu.bitcast(wd_v[...], BF),
                    preferred_element_type=F32))
    val = jnp.concatenate(
        [jnp.where(sub8 == 0, m1, jnp.where(sub8 == 1, m2, -jnp.inf)),
         _rb(jnp.sum(h2n * rep(6, ng), axis=-1, keepdims=True))], axis=0)
    pos = lax.broadcasted_iota(jnp.int32, (8 + NEW, 1), 0).astype(F32)
    p1 = jnp.min(jnp.where(val == jnp.max(val, axis=0, keepdims=True), pos, float(S)),
                 axis=0, keepdims=True)
    val2 = jnp.where(pos == p1, -jnp.inf, val)
    p2 = jnp.min(jnp.where((val2 == jnp.max(val2, axis=0, keepdims=True)) & (pos != p1), pos,
                           float(S)), axis=0, keepdims=True)
    upd = jnp.where((pos == p1) | (pos == p2), _rb(y * _rb(jax.nn.sigmoid(val))), 0.0)
    act[OOFF + NEW0:OOFF + S, :] = (x1n + _rb(rep(5, ng) * _rb(h2n + upd[8:]))).astype(BF)
    sub16 = lax.broadcasted_iota(jnp.int32, (16, 1), 0)
    grow = jnp.where(sub16 < 8, b1 + sub16, b2 + sub16 - 8)
    updc = jnp.where(grow == i1, upd[0:1], jnp.where(grow == i2, upd[1:2], 0.0))
    res = (x1c + _rb(rep(5, 2) * _rb(h2c + updc))).astype(BF)
    for c_ in cp_out:
        c_.wait()
    act[pl.ds(OOFF + b1, 8), :] = res[0:8]
    act[pl.ds(OOFF + b2, 8), :] = res[8:16]
    fix0 = cp(act.at[OOFF + NEW0:OOFF + S], out_hbm.at[0, NEW0:S], 6)
    fix1 = cp(act.at[pl.ds(OOFF + b1, 8)], out_hbm.at[0, pl.ds(b1, 8)], 11)
    fix2 = cp(act.at[pl.ds(OOFF + b2, 8)], out_hbm.at[0, pl.ds(b2, 8)], 12)
    fix0.start()
    fix1.start()

    @pl.when(b1 != b2)
    def _():
        fix2.start()
        fix2.wait()
    fix0.wait()
    fix1.wait()


@jax.jit
def pallas_adaLN_cond__memory_aug_recurrent_mem_tr__moe_arch_mod__prompt_kernel(
    A_x: jax.Array,
    A_mem0: jax.Array,
    A_Wq: jax.Array,
    A_Wk: jax.Array,
    A_Wv: jax.Array,
    A_Wo: jax.Array,
    A_seg_len,
    B_x: jax.Array,
    B_w_r: jax.Array,
    B_w_gate: jax.Array,
    B_w_up: jax.Array,
    B_w_down: jax.Array,
    c: jax.Array,
    w_mod: jax.Array,
):
    del B_x
    del A_seg_len
    assert A_x.shape == (1, S, D) and A_Wq.shape == (D, H, DH) and A_mem0.shape == (1, M, D)
    any_spec = pl.BlockSpec(memory_space=pl.ANY)
    scratch = [
        pltpu.VMEM((S if not XACT else 8, D), BF),
        pltpu.VMEM((XOFF + S * XACT, D), BF),
        pltpu.VMEM((8, PRE // 2, 128), U32),
        pltpu.VMEM((32, 768), F32),
        pltpu.VMEM((2 * EMAX, D), F32),
        pltpu.SMEM((NSEG * NTAB + 1,), jnp.int32),
        pltpu.VMEM((7, 8, D), F32),
        pltpu.VMEM((4, 1, D), BF),
        pltpu.VMEM((3 * H, D // 2, 128), U32),
        pltpu.VMEM((H, DH // 2, D), U32),
        pltpu.VMEM((6, D // 2, D), U32),
        pltpu.VMEM((D // 2, F), U32),
        pltpu.VMEM((D // 2, F), U32),
        pltpu.VMEM((F // 2, D), U32),
        pltpu.VMEM((NOSLOT * 32 + PRE, OW1), BF),
        pltpu.VMEM((NOSLOT * 32 + PRE, OW2), BF),
        pltpu.SemaphoreType.DMA((17,)),
        pltpu.SemaphoreType.DMA((12,)),
        pltpu.SemaphoreType.DMA((16,)),
    ] + [pltpu.VMEM((NSLOT + 1, 256, 128), U32) for _ in range(NB)] + [
        pltpu.VMEM((D,), BF),
    ]
    wq, wk, wv = (w.reshape(D // 2, 2, H, DH) for w in (A_Wq, A_Wk, A_Wv))
    return pl.pallas_call(
        _kernel,
        out_shape=jax.ShapeDtypeStruct((1, S, D), BF),
        in_specs=[any_spec] * 12,
        out_specs=any_spec,
        scratch_shapes=scratch,
        compiler_params=pltpu.CompilerParams(vmem_limit_bytes=120 * 1024 * 1024,
                                             disable_bounds_checks=True,
                                             disable_semaphore_checks=True),
    )(A_x, A_mem0, wq, wk, wv, A_Wo, B_w_r, B_w_gate, B_w_up, B_w_down,
      c, w_mod)
```

```python
import jax
import jax.numpy as jnp
from jax import lax
import jax.experimental.pallas as pl
import jax.experimental.pallas.tpu as pltpu

BF = jnp.bfloat16
F32 = jnp.float32
U32 = jnp.uint32

S = 2048
D = 1024
H = 32
DH = 128
M = 8
SEG = 32
NSEG = S // SEG
F = 3584
NP = H // 2
EPS = 1e-5
SCALE = DH ** -0.5

RIDE = 24
PRE = S - NSEG * RIDE
NSLOT = 17
NOSLOT = 17
NB = 8
KS = 2304
K2 = H * DH - KS
OW1 = -(-KS // D) * D
OW2 = -(-K2 // D) * D
OOFF = S
HOFF = 2 * S
ROFF = HOFF + 64
ACT_ROWS = ROFF + 16
UNR = 2
PRE_SPLIT = 3
E_AT = (2, 3, 5)
E_AT2 = (3, 5, 6)
L_AT = (8, 10, 12)
L_AT2 = (8, 10, 12)
A_BUF = (7, 0, 1)
EPI_CHUNKS = (64, 64, 64, 64, 64, 64, 48, 48, 32)
EPI_LASTPER = 2
EMAX = max(EPI_CHUNKS)
NEW = 24
FFN_NB = 512
NTAB = 16

ATT = {4: [('s', i) for i in range(4)], 18: [('p', i) for i in range(12, 16)]}
for _p in range(4, NP, 2):
    ATT[_p + 2] = [('s', _p), ('s', _p + 1), ('p', _p - 4), ('p', _p - 3)]


def _step_indices(s):
    t = [s % NSLOT]
    for j in range(3):
        gi = PRE // 8 + 3 * s + j
        t += [(gi // 4) % NSLOT, (gi % 4) * 4]
    for j in range(4):
        gi = 4 * s + j
        if gi < 3 * NSEG:
            t.append(((gi // 3) % NOSLOT) * 32 + 8 + (gi % 3) * 8)
        elif gi == 3 * NSEG:
            t.append(((NSEG - 1) % NOSLOT) * 32)
        else:
            t.append(NOSLOT * 32 + (gi - 3 * NSEG - 1) * 8)
    t.append((s % NOSLOT) * 32)
    t.append(max(s - 1, 0) * RIDE)
    t.append(PRE + min(s + 1, NSEG - 1) * RIDE)
    t.append((s % NOSLOT) * 32 if s < NSEG - 1 else NOSLOT * 32 + PRE - 8)
    return t


def _rb(v):
    return v.astype(BF).astype(F32)


def _pack(v):
    return pltpu.bitcast(v.astype(BF), U32)


def _layernorm(x):
    mu = jnp.sum(x, axis=-1, keepdims=True) * (1.0 / D)
    xc = x - mu
    var = jnp.sum(xc * xc, axis=-1, keepdims=True) * (1.0 / D)
    sd = _rb(jnp.sqrt(_rb(_rb(var) + EPS)))
    return _rb(_rb(x - _rb(mu)) / sd)


def _kernel(x_hbm, mem0_hbm, wq_hbm, wk_hbm, wv_hbm, wo_hbm, wr_hbm, wg_hbm, wu_hbm,
            wd_hbm, c_hbm, wmod_hbm, out_hbm,
            xbuf, act, h0buf, ybuf, ebuf, tab, modb,
            w_v, wo_v, wmod_v, wg_v, wu_v, wd_v,
            obuf1, obuf2, sems, wsems, ksems, *rest):
    qkvbufs, cbuf, wrbuf = rest[:NB], rest[NB], rest[NB + 1]
    w_hbms = tuple(w.bitcast(U32) for w in (wq_hbm, wk_hbm, wv_hbm))

    def cp(src, dst, i):
        return pltpu.make_async_copy(src, dst, sems.at[i])

    wmod32 = wmod_hbm.bitcast(U32)
    cp_c = cp(c_hbm, cbuf, 0)
    cp_mem = cp(mem0_hbm.at[0], act.at[HOFF:HOFF + M], 1)
    cp_wr = cp(wr_hbm, wrbuf, 2)
    cp_x0 = [cp(x_hbm.at[0, n * 128:(n + 1) * 128], xbuf.at[n * 128:(n + 1) * 128], 13 + n)
             for n in range(PRE // 128)]
    cp_xr = cp(x_hbm.at[0, PRE:PRE + 32], xbuf.at[PRE:PRE + 32], 5)
    cp_x1 = cp(x_hbm.at[0, PRE + 32:S], xbuf.at[PRE + 32:S], 4)
    cp_wo = cp(wo_hbm.bitcast(U32), wo_v, 7)
    cp_ffn = [cp(wg_hbm.bitcast(U32), wg_v, 8), cp(wu_hbm.bitcast(U32), wu_v, 8),
              cp(wd_hbm.bitcast(U32), wd_v, 8)]

    def w_start(j, i0=0, i1=NB, prio=0):
        gg, t = j // 3, j % 3
        for i in range(i0, i1):
            for par in range(2):
                pltpu.make_async_copy(w_hbms[t].at[:, par, gg * NB + i, :],
                                      w_v.at[(gg * NB + i) * 6 + t * 2 + par],
                                      wsems.at[2 * j + (i >= PRE_SPLIT)]).start(priority=prio)

    def mod_copy(j):
        return pltpu.make_async_copy(wmod32.at[:, j * D:(j + 1) * D], wmod_v.at[j],
                                     wsems.at[2 * j + 1])

    def mult(v, m):
        return v if isinstance(v, int) else pl.multiple_of(v, m)

    def moda_copies(kc):
        col = mult(kc * 128, 128)
        return [pltpu.make_async_copy(wmod32.at[:, pl.ds(v * D + col, 128)],
                                      wmod_v.at[v, :, pl.ds(col, 128)], ksems.at[8 + kc])
                for v in range(2)]

    def chunk_copies(kc):
        r0 = mult(kc * 64, 64)
        return [pltpu.make_async_copy(w_hbms[0].at[pl.ds(r0, 64), par, i, :],
                                      w_v.at[i * 6 + par, pl.ds(r0, 64), :], ksems.at[kc])
                for i in range(NB) for par in range(2)]

    cp_c.start()
    cp_mem.start()
    cp_wr.start()
    for c_ in (cp_x0 + moda_copies(0) + moda_copies(1) + chunk_copies(0) + moda_copies(2)
               + chunk_copies(1) + [cp_xr] + chunk_copies(2)):
        c_.start()

    def ln1_rows(src_row, dst_row):
        xv = xbuf[pl.ds(src_row, 8), :].astype(F32)
        hv = _rb(_layernorm(xv) * modb[1]) + modb[0]
        act[pl.ds(dst_row, 8), :] = hv.astype(BF)

    lane256 = lax.broadcasted_iota(jnp.int32, (8, 256), 1)

    def finish_rows(row, attn):
        xv = xbuf[pl.ds(row, 8), :].astype(F32)
        x1 = _rb(xv + _rb(modb[2] * _rb(attn)))
        act[pl.ds(row, 8), :] = x1.astype(BF)
        h2 = _rb(_rb(_layernorm(x1) * modb[4]) + modb[3])
        act[pl.ds(OOFF + row, 8), :] = (x1 + _rb(modb[5] * h2)).astype(BF)
        r = jnp.sum(h2 * modb[6], axis=-1, keepdims=True)
        act[ROFF:ROFF + 8, 0:256] = jnp.where(
            lane256 * 8 == row, r, act[ROFF:ROFF + 8, 0:256].astype(F32)).astype(BF)

    def attn_store(a, k0):
        for j in range(3):
            for k in range(a.shape[1] // 128):
                qkvbufs[A_BUF[j]][NSLOT, (k0 + k) * 8:(k0 + k + 1) * 8, :] = pltpu.bitcast(
                    a[8 * j:8 * j + 8, k * 128:(k + 1) * 128], U32)

    def attn_load(j):
        return pltpu.bitcast(jnp.concatenate(
            [qkvbufs[A_BUF[j]][NSLOT, k * 8:(k + 1) * 8, :] for k in range(8)], axis=1), F32)

    act[ROFF:ROFF + 8, 0:256] = jnp.zeros((8, 256), BF)
    attn_store(jnp.zeros((RIDE, D), F32), 0)
    for s_ in range(NSEG):
        for k, v in enumerate(_step_indices(s_)):
            tab[s_ * NTAB + k] = v
    tab[NSEG * NTAB] = 0
    ri = lax.broadcasted_iota(jnp.int32, (80, 80), 0)
    ci = lax.broadcasted_iota(jnp.int32, (80, 80), 1)

    def head_pos(i):
        hd = jnp.where(i < 16, i // 8, (i - 16) // 32)
        pos = jnp.where(i < 16, i % 8, 8 + (i - 16) % 32)
        return hd, pos
    rh, rp = head_pos(ri)
    ch, cpos = head_pos(ci)
    same = rh == ch
    valid = same & ((rp < M) | (rp >= cpos))
    fill = jnp.where(same, -1e9, -jnp.inf).astype(F32)

    cp_mem.wait()
    cp_wr.wait()
    modb[6] = jnp.broadcast_to(wrbuf[...].astype(F32).reshape(1, D), (8, D))
    cp_c.wait()
    cv = cbuf[...].astype(F32)
    sc16 = jnp.broadcast_to(_rb(cv * _rb(jax.nn.sigmoid(cv))), (16, D)).astype(BF)

    def ln_pre(g, carry):
        pltpu.make_async_copy(x_hbm.at[0, 0:128], xbuf.at[pl.ds(pl.multiple_of(g * 128, 128), 128)],
                              sems.at[13 + g]).wait()
        for u in range(2):
            row = pl.multiple_of(g * 128 + u * 64, 64)
            nv = _layernorm(xbuf[pl.ds(row, 64), :].astype(F32)).astype(BF)
            for k in range(8):
                h0buf[k, pl.ds(pl.multiple_of(row // 2, 32), 32), :] = pltpu.bitcast(
                    nv[:, k * 128:(k + 1) * 128], U32)
            wg_v[pl.ds(row, 64), 0:2 * D] = jnp.zeros((64, 2 * D), U32)
        return carry
    lax.fori_loop(0, PRE // 128, ln_pre, 0)

    def mod_tile(v, col):
        w = pltpu.bitcast(wmod_v[v, :, pl.ds(col, 128)], BF)
        return _rb(jnp.dot(sc16, w, preferred_element_type=F32))[0:8]

    def moda_store(kc, sa, ca):
        col = mult(kc * 128, 128)
        c1 = _rb(1.0 + ca)
        modb[0, :, pl.ds(col, 128)] = sa
        modb[1, :, pl.ds(col, 128)] = c1
        return sa, c1

    def moda_apply(kc, sa, c1, r0, r1):
        for r in range(r0, r1, 16):
            nv = pltpu.bitcast(h0buf[kc, r // 2:r // 2 + 8, :], BF).astype(F32).reshape(2, 8, 128)
            hv = (_rb(nv * c1[None]) + sa[None]).reshape(16, 128).astype(BF)
            h0buf[kc, r // 2:r // 2 + 8, :] = pltpu.bitcast(hv, U32)

    def repack(a, b):
        return (a & U32(0xFFFF)) | (b << 16), (a >> 16) | (b & U32(0xFFFF0000))

    def store_qkv(i, jrow, y, seg0):
        for sg in range(y.shape[0] // 32):
            for hh in range(2):
                qkvbufs[i][seg0 + sg, pl.ds(jrow + 8 + hh * 16, 16), :] = _pack(
                    y[sg * 32:(sg + 1) * 32, hh * 128:(hh + 1) * 128])

    for c_ in moda_copies(0):
        c_.wait()
    moda_apply(0, *moda_store(0, mod_tile(0, 0), mod_tile(1, 0)), 0, PRE)

    def w_wait(j, i0, i1):
        blk0 = (j // 3) * (6 * NB) + (j % 3) * 2
        for i in range(i0, i1):
            for par in range(2):
                pltpu.make_async_copy(w_hbms[0].at[:, 0, 0, :], w_v.at[blk0 + i * 6 + par],
                                      wsems.at[2 * j + (i >= PRE_SPLIT)]).wait()

    def chunk_block(kc, last, issue):
        for c_ in chunk_copies(kc) + ([cp_xr] if last else moda_copies(kc + 1)):
            c_.wait()
        issue()
        r0 = mult(kc * 64, 64)
        mv = []
        for i in range(NB):
            lo, hi = repack(w_v[i * 6, pl.ds(r0, 64), :], w_v[i * 6 + 1, pl.ds(r0, 64), :])
            w_v[i * 6, pl.ds(r0, 64), :] = lo
            w_v[i * 6 + 1, pl.ds(r0, 64), :] = hi
            w = pltpu.bitcast(jnp.concatenate([lo, hi], axis=1), BF)
            y = (pltpu.bitcast(wg_v[0:PRE, i * 256:(i + 1) * 256], F32)
                 + jnp.dot(pltpu.bitcast(h0buf[kc], BF), w, preferred_element_type=F32))
            if last:
                store_qkv(i, 0, y, 0)
            else:
                wg_v[0:PRE, i * 256:(i + 1) * 256] = pltpu.bitcast(y, U32)
                if i in (1, 3):
                    mv.append(mod_tile(i // 2, mult((kc + 1) * 128, 128)))
                if i == 3:
                    mv = moda_store(kc + 1, mv[0], mv[1])
                if i >= 4:
                    moda_apply(kc + 1, mv[0], mv[1], (i - 4) * 128, (i - 3) * 128)
        if last:
            for j in range(3):
                ln1_rows(PRE + 8 * j, HOFF + 8 + 8 * j)

    def chunk_body(kc, carry):
        def issue():
            @pl.when(kc < 5)
            def _():
                for c_ in moda_copies(kc + 3) + chunk_copies(kc + 3):
                    c_.start()
        chunk_block(kc, False, issue)
        return carry

    def issue_last():
        w_wait(1, 0, PRE_SPLIT)
        w_start(1, PRE_SPLIT, NB)
        w_start(2)
        mod_copy(2).start()
    w_start(1, 0, PRE_SPLIT, prio=1)
    lax.fori_loop(0, 7, chunk_body, 0)
    chunk_block(7, True, issue_last)

    def pre_unit(j, i, extra):
        blk = (j // 3) * (6 * NB) + (j % 3) * 2 + i * 6
        jrow = mult(j * 40, 8)
        lo, hi = repack(w_v[blk], w_v[blk + 1])
        w_v[blk] = lo
        w_v[blk + 1] = hi
        for rc in range(PRE // 128):
            if rc > 0:
                lo = w_v[blk]
                hi = w_v[blk + 1]
            w = pltpu.bitcast(jnp.concatenate([lo, hi], axis=1), BF)
            lhs = jnp.concatenate([h0buf[k, rc * 64:(rc + 1) * 64, :] for k in range(8)], axis=1)
            y = jnp.dot(pltpu.bitcast(lhs, BF), w, preferred_element_type=F32)
            store_qkv(i, jrow, y, rc * 4)
            extra(rc)

    for i in range(NB):
        if i == PRE_SPLIT:
            w_wait(1, PRE_SPLIT, NB)
            for jn in (3, 4):
                w_start(jn)
                mod_copy(jn).start()
        pre_unit(1, i, lambda rc: None)
    w_start(5)
    mod_copy(5).start()
    cp_wo.start()
    cp_x1.start()

    def pre_body(j, carry):
        w_wait(j, 0, NB)
        pltpu.make_async_copy(wmod32.at[:, 0:D], wmod_v.at[j], wsems.at[2 * j + 1]).wait()
        one = jnp.where(j == 4, 1.0, 0.0).astype(F32)
        for i in range(NB):
            def extra(rc, i=i):
                if rc == 1:
                    modb[j, :, i * 128:(i + 1) * 128] = _rb(one + mod_tile(j, i * 128))
            pre_unit(j, i, extra)
        return carry
    lax.fori_loop(2, 6, pre_body, 0)

    cp_wo.wait()
    cp_x1.wait()
    for c_ in cp_ffn:
        c_.start()

    def wo_w(h0, h1, n0, n1):
        w = wo_v[h0:h1, :, n0 * 128:n1 * 128].reshape((h1 - h0) * (DH // 2), (n1 - n0) * 128)
        return pltpu.bitcast(w, BF)

    HD = D // 2

    def emit_step(s, pend, last):
        hrow = pl.multiple_of(HOFF + (s & 1) * 32, 32)
        hnext = pl.multiple_of(HOFF + 32 - (s & 1) * 32, 32)
        tv = [tab[s * NTAB + k] for k in range(15)]
        slot = tv[0]
        dsts = [(tv[1 + 2 * j], pl.multiple_of(tv[2 + 2 * j], 4)) for j in range(3)]
        odst = [pl.multiple_of(tv[7 + j], 8) for j in range(4)]
        orow = pl.multiple_of(tv[11], 32)
        erow = tv[12]
        lrow = tv[13]
        mrow = pl.multiple_of(tv[14], 8)
        e_at, l_at = (E_AT, L_AT) if pend is None else (E_AT2, L_AT2)
        probs = {}

        def wqkv(p, k0, k1):
            return pltpu.bitcast(jnp.concatenate(
                [w_v[p * 6 + u, k0 // 2:k1 // 2, :] for u in range(6)], axis=1), BF)

        lhs_lo = act[pl.ds(hrow, 32), 0:HD]
        if pend is not None:
            ybuf[...] = jnp.dot(lhs_lo, wqkv(0, 0, HD), preferred_element_type=F32)
            pend()
        lhs_hi = act[pl.ds(hrow, 32), HD:D]
        if pend is not None:
            y0 = ybuf[...] + jnp.dot(lhs_hi, wqkv(0, HD, D), preferred_element_type=F32)
        lhs_rest = jnp.concatenate([lhs_lo[:, 128:], lhs_hi], axis=1)
        lhs = [jnp.concatenate([lhs_lo, lhs_hi], axis=1)]

        def side(p):
            for j in range(3):
                if e_at[j] == p:
                    finish_rows(pl.multiple_of(erow + 8 * j, 8), attn_load(j))
            for j in range(3):
                if l_at[j] == p:
                    ln1_rows(pl.multiple_of(lrow + 8 * j, 8),
                             pl.multiple_of(hnext + 8 + 8 * j, 8))
            if p in e_at or p in l_at:
                lhs[0] = jnp.concatenate([act[pl.ds(hrow, 32), 0:128], lhs_rest], axis=1)

        def qkv(p):
            if p == 0 and pend is not None:
                y = y0
            else:
                y = jnp.dot(lhs[0], wqkv(p, 0, D), preferred_element_type=F32)
            buf = qkvbufs[p % NB]
            for u in range(6):
                t, hh = u // 2, u % 2
                b0 = ((p // NB) * 3 + t) * 40
                yu = y[:, u * 128:(u + 1) * 128]
                buf[slot, b0 + hh * 4:b0 + hh * 4 + 4, :] = _pack(yu[0:8])
                for j in range(3):
                    sl, off = dsts[j]
                    buf[sl, pl.ds(b0 + 8 + hh * 16 + off, 4), :] = _pack(yu[8 + 8 * j:16 + 8 * j])

        def ld(p, t):
            b0 = ((p // NB) * 3 + t) * 40
            return pltpu.bitcast(qkvbufs[p % NB][slot, b0:b0 + 40, :], BF)

        def sc(p):
            s2 = lax.dot_general(ld(p, 0), ld(p, 1), (((1,), (1,)), ((), ())),
                                 preferred_element_type=F32)
            s2 = jnp.where(valid, s2 * SCALE, fill)
            m = jnp.max(s2, axis=-1, keepdims=True)
            e = jnp.exp(s2 - m)
            l = jnp.sum(e, axis=-1, keepdims=True)
            rl = pl.reciprocal(l, approx=True)
            rl = rl * (2.0 - l * rl)
            probs[p] = (e * rl).astype(BF)

        def pv(p):
            o2 = jnp.dot(probs[p], ld(p, 2), preferred_element_type=F32)
            for hh in range(2):
                hcol = (2 * p + hh) * 128
                ob = obuf1
                if hcol >= KS:
                    ob = obuf2
                    hcol -= KS
                ob[pl.ds(mrow, 8), hcol:hcol + 128] = o2[8 * hh:8 * hh + 8].astype(BF)
                for j in range(4):
                    r0 = 16 + 32 * hh + 8 * j
                    ob[pl.ds(odst[j], 8), hcol:hcol + 128] = o2[r0:r0 + 8].astype(BF)

        def attn(pos):
            for kind, p in ATT.get(pos, ()):
                (sc if kind == 's' else pv)(p)

        for p in range(NP):
            qkv(p)
            side(p)
            attn(p)
        a1 = []
        for i in range(4):
            a1.append(jnp.dot(obuf1[pl.ds(orow, 32), 0:KS], wo_w(0, KS // DH, 2 * i, 2 * i + 2),
                              preferred_element_type=F32))
            attn(NP + i)
        o2lhs = obuf2[pl.ds(orow, 32), 0:K2]
        a_lo = jnp.concatenate(a1[0:2], axis=1) + jnp.dot(
            o2lhs, wo_w(KS // DH, H, 0, 4), preferred_element_type=F32)
        act[pl.ds(hnext, 8), 0:HD] = a_lo[0:8].astype(BF)
        attn_store(a_lo[8:32], 0)
        a_hi = jnp.concatenate(a1[2:4], axis=1) + jnp.dot(
            o2lhs, wo_w(KS // DH, H, 4, 8), preferred_element_type=F32)

        def finish():
            act[pl.ds(hnext, 8), HD:D] = a_hi[0:8].astype(BF)
            attn_store(a_hi[8:32], 4)
        if last:
            finish()
        return finish

    def steps(it, carry):
        pend = None
        for u in range(UNR):
            pend = emit_step(it * UNR + u, pend, u == UNR - 1)
        return carry
    lax.fori_loop(0, NSEG // UNR, steps, 0)

    for c_ in cp_ffn:
        c_.wait()
    OUT0 = (NSEG - 1) * RIDE
    NEW0 = S - NEW
    cp_out = [cp(act.at[OOFF:OOFF + OUT0], out_hbm.at[0, 0:OUT0], 9)]
    cp_out[0].start()
    zero = pl.multiple_of(tab[NSEG * NTAB], 8)
    for j in range(3):
        ebuf[EMAX + 8 * j:EMAX + 8 * j + 8, :] = attn_load(j)
    ebuf[EMAX + RIDE:EMAX + RIDE + 8, :] = act[HOFF:HOFF + 8, :].astype(F32)
    todo = [(OUT0 + 8 * j, EMAX + 8 * j) for j in range(4)]
    r0 = 0
    for ci, ech in enumerate(EPI_CHUNKS):
        o0 = NOSLOT * 32 + r0
        e0 = (ci % 2) * EMAX
        per = -(-len(todo) // 8)
        if ci == len(EPI_CHUNKS) - 1:
            per = EPI_LASTPER
        for n in range(8):
            lhs = jnp.concatenate([obuf1[o0:o0 + ech, 0:KS], obuf2[o0:o0 + ech, 0:K2]], axis=1)
            ebuf[e0:e0 + ech, n * 128:(n + 1) * 128] = jnp.dot(
                lhs, wo_w(0, H, n, n + 1), preferred_element_type=F32)
            for row, er in todo[:per]:
                finish_rows(row, ebuf[pl.ds(zero + er, 8), :])
            todo = todo[per:]
        todo = [(OUT0 + RIDE + 8 + r0 + 8 * j, e0 + 8 * j) for j in range(ech // 8)]
        r0 += ech

    rowsf = (lane256 * 8 + lax.broadcasted_iota(jnp.int32, (8, 256), 0)).astype(F32)
    r_old = jnp.where(rowsf < NEW0, act[ROFF:ROFF + 8, 0:256].astype(F32), -jnp.inf)

    def allmax(v):
        return jnp.max(jnp.max(v, axis=1, keepdims=True), axis=0, keepdims=True)

    def allmin(v):
        return jnp.min(jnp.min(v, axis=1, keepdims=True), axis=0, keepdims=True)
    m1 = allmax(r_old)
    i1v = allmin(jnp.where(r_old == m1, rowsf, float(S)))
    r_rest = jnp.where(rowsf == i1v, -jnp.inf, r_old)
    m2 = allmax(r_rest)
    i2v = allmin(jnp.where((r_rest == m2) & (rowsf != i1v), rowsf, float(S)))
    i1 = jnp.clip(i1v[0, 0].astype(jnp.int32), 0, NEW0 - 1)
    i2 = jnp.clip(i2v[0, 0].astype(jnp.int32), 0, NEW0 - 1)
    b1 = pl.multiple_of((i1 // 8) * 8, 8)
    b2 = pl.multiple_of((i2 // 8) * 8, 8)
    sub8 = lax.broadcasted_iota(jnp.int32, (8, 1), 0)

    def rep(i, n):
        return jnp.concatenate([modb[i]] * n, axis=0)
    x1c = jnp.concatenate([act[pl.ds(b1, 8), :].astype(F32), act[pl.ds(b2, 8), :].astype(F32)],
                          axis=0)
    h2c = _rb(_rb(_layernorm(x1c) * rep(4, 2)) + rep(3, 2))
    row1 = jnp.sum(jnp.where(sub8 == i1 - b1, h2c[0:8], 0.0), axis=0, keepdims=True)
    row2 = jnp.sum(jnp.where(sub8 == i2 - b2, h2c[8:16], 0.0), axis=0, keepdims=True)
    cand = jnp.where(sub8 == 0, row1, jnp.where(sub8 == 1, row2, 0.0))

    e0 = ((len(EPI_CHUNKS) - 1) % 2) * EMAX
    ng = NEW // 8
    x1n = _rb(xbuf[NEW0:S, :].astype(F32) + _rb(rep(2, ng) * _rb(ebuf[e0:e0 + NEW, :])))
    h2n = _rb(_rb(_layernorm(x1n) * rep(4, ng)) + rep(3, ng))
    h2b = jnp.concatenate([cand, h2n], axis=0).astype(BF)
    cp_out.append(cp(act.at[OOFF + OUT0:OOFF + NEW0], out_hbm.at[0, OUT0:NEW0], 10))
    cp_out[1].start()
    hid = []
    for n in range(0, F, FFN_NB):
        gt = _rb(jnp.dot(h2b, pltpu.bitcast(wg_v[:, n:n + FFN_NB], BF), preferred_element_type=F32))
        up = _rb(jnp.dot(h2b, pltpu.bitcast(wu_v[:, n:n + FFN_NB], BF), preferred_element_type=F32))
        hid.append((_rb(gt * _rb(jax.nn.sigmoid(gt))) * up).astype(BF))
    y = _rb(jnp.dot(jnp.concatenate(hid, axis=1), pltpu.bitcast(wd_v[...], BF),
                    preferred_element_type=F32))
    val = jnp.concatenate(
        [jnp.where(sub8 == 0, m1, jnp.where(sub8 == 1, m2, -jnp.inf)),
         _rb(jnp.sum(h2n * rep(6, ng), axis=-1, keepdims=True))], axis=0)
    pos = lax.broadcasted_iota(jnp.int32, (8 + NEW, 1), 0).astype(F32)
    p1 = jnp.min(jnp.where(val == jnp.max(val, axis=0, keepdims=True), pos, float(S)),
                 axis=0, keepdims=True)
    val2 = jnp.where(pos == p1, -jnp.inf, val)
    p2 = jnp.min(jnp.where((val2 == jnp.max(val2, axis=0, keepdims=True)) & (pos != p1), pos,
                           float(S)), axis=0, keepdims=True)
    upd = jnp.where((pos == p1) | (pos == p2), _rb(y * _rb(jax.nn.sigmoid(val))), 0.0)
    act[OOFF + NEW0:OOFF + S, :] = (x1n + _rb(rep(5, ng) * _rb(h2n + upd[8:]))).astype(BF)
    sub16 = lax.broadcasted_iota(jnp.int32, (16, 1), 0)
    grow = jnp.where(sub16 < 8, b1 + sub16, b2 + sub16 - 8)
    updc = jnp.where(grow == i1, upd[0:1], jnp.where(grow == i2, upd[1:2], 0.0))
    res = (x1c + _rb(rep(5, 2) * _rb(h2c + updc))).astype(BF)
    for c_ in cp_out:
        c_.wait()
    act[pl.ds(OOFF + b1, 8), :] = res[0:8]
    act[pl.ds(OOFF + b2, 8), :] = res[8:16]
    fix0 = cp(act.at[OOFF + NEW0:OOFF + S], out_hbm.at[0, NEW0:S], 6)
    fix1 = cp(act.at[pl.ds(OOFF + b1, 8)], out_hbm.at[0, pl.ds(b1, 8)], 11)
    fix2 = cp(act.at[pl.ds(OOFF + b2, 8)], out_hbm.at[0, pl.ds(b2, 8)], 12)
    fix0.start()
    fix1.start()

    @pl.when(b1 != b2)
    def _():
        fix2.start()
        fix2.wait()
    fix0.wait()
    fix1.wait()


@jax.jit
def pallas_adaLN_cond__memory_aug_recurrent_mem_tr__moe_arch_mod__prompt_kernel(
    A_x: jax.Array,
    A_mem0: jax.Array,
    A_Wq: jax.Array,
    A_Wk: jax.Array,
    A_Wv: jax.Array,
    A_Wo: jax.Array,
    A_seg_len,
    B_x: jax.Array,
    B_w_r: jax.Array,
    B_w_gate: jax.Array,
    B_w_up: jax.Array,
    B_w_down: jax.Array,
    c: jax.Array,
    w_mod: jax.Array,
):
    del B_x
    del A_seg_len
    assert A_x.shape == (1, S, D) and A_Wq.shape == (D, H, DH) and A_mem0.shape == (1, M, D)
    any_spec = pl.BlockSpec(memory_space=pl.ANY)
    scratch = [
        pltpu.VMEM((S, D), BF),
        pltpu.VMEM((ACT_ROWS, D), BF),
        pltpu.VMEM((8, PRE // 2, 128), U32),
        pltpu.VMEM((32, 768), F32),
        pltpu.VMEM((2 * EMAX, D), F32),
        pltpu.SMEM((NSEG * NTAB + 1,), jnp.int32),
        pltpu.VMEM((7, 8, D), F32),
        pltpu.VMEM((3 * H, D // 2, 128), U32),
        pltpu.VMEM((H, DH // 2, D), U32),
        pltpu.VMEM((6, D // 2, D), U32),
        pltpu.VMEM((D // 2, F), U32),
        pltpu.VMEM((D // 2, F), U32),
        pltpu.VMEM((F // 2, D), U32),
        pltpu.VMEM((NOSLOT * 32 + PRE, OW1), BF),
        pltpu.VMEM((NOSLOT * 32 + PRE, OW2), BF),
        pltpu.SemaphoreType.DMA((17,)),
        pltpu.SemaphoreType.DMA((12,)),
        pltpu.SemaphoreType.DMA((16,)),
    ] + [pltpu.VMEM((NSLOT + 1, 256, 128), U32) for _ in range(NB)] + [
        pltpu.VMEM((1, D), BF),
        pltpu.VMEM((D,), BF),
    ]
    wq, wk, wv = (w.reshape(D // 2, 2, H, DH) for w in (A_Wq, A_Wk, A_Wv))
    return pl.pallas_call(
        _kernel,
        out_shape=jax.ShapeDtypeStruct((1, S, D), BF),
        in_specs=[any_spec] * 12,
        out_specs=any_spec,
        scratch_shapes=scratch,
        compiler_params=pltpu.CompilerParams(vmem_limit_bytes=120 * 1024 * 1024,
                                             disable_bounds_checks=True,
                                             disable_semaphore_checks=True),
    )(A_x, A_mem0, wq, wk, wv, A_Wo, B_w_r, B_w_gate, B_w_up, B_w_down,
      c, w_mod)
```

```python
import jax
import jax.numpy as jnp
from jax import lax
import jax.experimental.pallas as pl
import jax.experimental.pallas.tpu as pltpu

BF = jnp.bfloat16
F32 = jnp.float32
U32 = jnp.uint32

S = 2048
D = 1024
H = 32
DH = 128
M = 8
SEG = 32
NSEG = S // SEG
F = 3584
NP = H // 2
EPS = 1e-5
SCALE = DH ** -0.5

RIDE = 24
PRE = S - NSEG * RIDE
NSLOT = 17
NOSLOT = 17
NB = 8
KS = 1792
K2 = H * DH - KS
OW1 = -(-KS // D) * D
OW2 = -(-K2 // D) * D
OOFF = S
HOFF = 2 * S
ROFF = HOFF + 64
ACT_ROWS = ROFF + 16
UNR = 2
PRE_SPLIT = 3
E_AT = (1, 2, 5)
E_AT2 = (3, 5, 6)
L_AT = (10, 12, 14)
L_AT2 = (8, 10, 12)
A_BUF = (7, 0, 2)
W1AT = (2, 6)
EPI_CHUNKS = (64, 64, 64, 64, 64, 64, 48, 48, 32)
EPI_LASTPER = 2
EMAX = max(EPI_CHUNKS)
NEW = 24
FFN_NB = 512
NTAB = 16

ROT = 0
ATT = {4: [('s', i) for i in range(4)],
       18: [('p', (12 + ROT + i) % NP) for i in range(4)]}
for _p in range(4, NP, 2):
    ATT[_p + 2] = [('s', _p), ('s', _p + 1), ('p', _p - 4 + ROT), ('p', _p - 3 + ROT)]


def _step_indices(s):
    t = [s % NSLOT]
    for j in range(3):
        gi = PRE // 8 + 3 * s + j
        t += [(gi // 4) % NSLOT, (gi % 4) * 4]
    for j in range(4):
        gi = 4 * s + j
        if gi < 3 * NSEG:
            t.append(((gi // 3) % NOSLOT) * 32 + 8 + (gi % 3) * 8)
        elif gi == 3 * NSEG:
            t.append(((NSEG - 1) % NOSLOT) * 32)
        else:
            t.append(NOSLOT * 32 + (gi - 3 * NSEG - 1) * 8)
    t.append((s % NOSLOT) * 32)
    t.append(max(s - 1, 0) * RIDE)
    t.append(PRE + min(s + 1, NSEG - 1) * RIDE)
    t.append((s % NOSLOT) * 32 if s < NSEG - 1 else NOSLOT * 32 + PRE - 8)
    return t


def _rb(v):
    return v.astype(BF).astype(F32)


def _pack(v):
    return pltpu.bitcast(v.astype(BF), U32)


def _layernorm(x):
    mu = jnp.sum(x, axis=-1, keepdims=True) * (1.0 / D)
    xc = x - mu
    var = jnp.sum(xc * xc, axis=-1, keepdims=True) * (1.0 / D)
    sd = _rb(jnp.sqrt(_rb(_rb(var) + EPS)))
    return _rb(_rb(x - _rb(mu)) / sd)


def _kernel(x_hbm, mem0_hbm, wq_hbm, wk_hbm, wv_hbm, wo_hbm, wr_hbm, wg_hbm, wu_hbm,
            wd_hbm, c_hbm, wmod_hbm, out_hbm,
            xbuf, act, h0buf, ybuf, ebuf, tab, modb,
            w_v, wo_v, wmod_v, wg_v, wu_v, wd_v,
            obuf1, obuf2, sems, wsems, ksems, *rest):
    qkvbufs, cbuf, wrbuf = rest[:NB], rest[NB], rest[NB + 1]
    w_hbms = tuple(w.bitcast(U32) for w in (wq_hbm, wk_hbm, wv_hbm))

    def cp(src, dst, i):
        return pltpu.make_async_copy(src, dst, sems.at[i])

    wmod32 = wmod_hbm.bitcast(U32)
    cp_c = cp(c_hbm, cbuf, 0)
    cp_mem = cp(mem0_hbm.at[0], act.at[HOFF:HOFF + M], 1)
    cp_wr = cp(wr_hbm, wrbuf, 2)
    cp_x0 = [cp(x_hbm.at[0, n * 128:(n + 1) * 128], xbuf.at[n * 128:(n + 1) * 128], 13 + n)
             for n in range(PRE // 128)]
    cp_xr = cp(x_hbm.at[0, PRE:PRE + 32], xbuf.at[PRE:PRE + 32], 5)
    cp_x1 = cp(x_hbm.at[0, PRE + 32:S], xbuf.at[PRE + 32:S], 4)
    cp_wo = cp(wo_hbm.bitcast(U32), wo_v, 7)
    cp_ffn = [cp(wg_hbm.bitcast(U32), wg_v, 8), cp(wu_hbm.bitcast(U32), wu_v, 8),
              cp(wd_hbm.bitcast(U32), wd_v, 8)]

    def w_start(j, i0=0, i1=NB, prio=0):
        gg, t = j // 3, j % 3
        for i in range(i0, i1):
            for par in range(2):
                pltpu.make_async_copy(w_hbms[t].at[:, par, gg * NB + i, :],
                                      w_v.at[(gg * NB + i) * 6 + t * 2 + par],
                                      wsems.at[2 * j + (i >= PRE_SPLIT)]).start(priority=prio)

    def mod_copy(j):
        return pltpu.make_async_copy(wmod32.at[:, j * D:(j + 1) * D], wmod_v.at[j],
                                     wsems.at[2 * j + 1])

    def mult(v, m):
        return v if isinstance(v, int) else pl.multiple_of(v, m)

    def moda_copies(kc):
        col = mult(kc * 128, 128)
        return [pltpu.make_async_copy(wmod32.at[:, pl.ds(v * D + col, 128)],
                                      wmod_v.at[v, :, pl.ds(col, 128)], ksems.at[8 + kc])
                for v in range(2)]

    def chunk_copies(kc):
        r0 = mult(kc * 64, 64)
        return [pltpu.make_async_copy(w_hbms[0].at[pl.ds(r0, 64), par, i, :],
                                      w_v.at[i * 6 + par, pl.ds(r0, 64), :], ksems.at[kc])
                for i in range(NB) for par in range(2)]

    cp_c.start()
    cp_mem.start()
    cp_wr.start()
    for c_ in (cp_x0 + moda_copies(0) + moda_copies(1) + chunk_copies(0) + moda_copies(2)
               + chunk_copies(1) + [cp_xr] + chunk_copies(2)):
        c_.start()

    def ln1_rows(src_row, dst_row):
        xv = xbuf[pl.ds(src_row, 8), :].astype(F32)
        hv = _rb(_layernorm(xv) * modb[1]) + modb[0]
        act[pl.ds(dst_row, 8), :] = hv.astype(BF)

    lane256 = lax.broadcasted_iota(jnp.int32, (8, 256), 1)

    def finish_rows(row, attn):
        xv = xbuf[pl.ds(row, 8), :].astype(F32)
        x1 = _rb(xv + _rb(modb[2] * _rb(attn)))
        act[pl.ds(row, 8), :] = x1.astype(BF)
        h2 = _rb(_rb(_layernorm(x1) * modb[4]) + modb[3])
        act[pl.ds(OOFF + row, 8), :] = (x1 + _rb(modb[5] * h2)).astype(BF)
        r = jnp.sum(h2 * modb[6], axis=-1, keepdims=True)
        act[ROFF:ROFF + 8, 0:256] = jnp.where(
            lane256 * 8 == row, r, act[ROFF:ROFF + 8, 0:256].astype(F32)).astype(BF)

    def attn_store(a, k0):
        for j in range(3):
            for k in range(a.shape[1] // 128):
                qkvbufs[A_BUF[j]][NSLOT, (k0 + k) * 8:(k0 + k + 1) * 8, :] = pltpu.bitcast(
                    a[8 * j:8 * j + 8, k * 128:(k + 1) * 128], U32)

    def attn_load(j):
        return pltpu.bitcast(jnp.concatenate(
            [qkvbufs[A_BUF[j]][NSLOT, k * 8:(k + 1) * 8, :] for k in range(8)], axis=1), F32)

    act[ROFF:ROFF + 8, 0:256] = jnp.zeros((8, 256), BF)
    attn_store(jnp.zeros((RIDE, D), F32), 0)
    for s_ in range(NSEG):
        for k, v in enumerate(_step_indices(s_)):
            tab[s_ * NTAB + k] = v
    tab[NSEG * NTAB] = 0
    ri = lax.broadcasted_iota(jnp.int32, (80, 80), 0)
    ci = lax.broadcasted_iota(jnp.int32, (80, 80), 1)

    def head_pos(i):
        hd = jnp.where(i < 16, i // 8, (i - 16) // 32)
        pos = jnp.where(i < 16, i % 8, 8 + (i - 16) % 32)
        return hd, pos
    rh, rp = head_pos(ri)
    ch, cpos = head_pos(ci)
    same = rh == ch
    valid = same & ((rp < M) | (rp >= cpos))
    fill = jnp.where(same, -1e9, -jnp.inf).astype(F32)

    cp_mem.wait()
    cp_wr.wait()
    modb[6] = jnp.broadcast_to(wrbuf[...].astype(F32).reshape(1, D), (8, D))
    cp_c.wait()
    cv = cbuf[...].astype(F32)
    sc16 = jnp.broadcast_to(_rb(cv * _rb(jax.nn.sigmoid(cv))), (16, D)).astype(BF)

    def ln_pre(g, carry):
        pltpu.make_async_copy(x_hbm.at[0, 0:128], xbuf.at[pl.ds(pl.multiple_of(g * 128, 128), 128)],
                              sems.at[13 + g]).wait()
        for u in range(2):
            row = pl.multiple_of(g * 128 + u * 64, 64)
            nv = _layernorm(xbuf[pl.ds(row, 64), :].astype(F32)).astype(BF)
            for k in range(8):
                h0buf[k, pl.ds(pl.multiple_of(row // 2, 32), 32), :] = pltpu.bitcast(
                    nv[:, k * 128:(k + 1) * 128], U32)
            wg_v[pl.ds(row, 64), 0:2 * D] = jnp.zeros((64, 2 * D), U32)
        return carry
    lax.fori_loop(0, PRE // 128, ln_pre, 0)

    def mod_tile(v, col):
        w = pltpu.bitcast(wmod_v[v, :, pl.ds(col, 128)], BF)
        return _rb(jnp.dot(sc16, w, preferred_element_type=F32))[0:8]

    def moda_store(kc, sa, ca):
        col = mult(kc * 128, 128)
        c1 = _rb(1.0 + ca)
        modb[0, :, pl.ds(col, 128)] = sa
        modb[1, :, pl.ds(col, 128)] = c1
        return sa, c1

    def moda_apply(kc, sa, c1, r0, r1):
        for r in range(r0, r1, 16):
            nv = pltpu.bitcast(h0buf[kc, r // 2:r // 2 + 8, :], BF).astype(F32).reshape(2, 8, 128)
            hv = (_rb(nv * c1[None]) + sa[None]).reshape(16, 128).astype(BF)
            h0buf[kc, r // 2:r // 2 + 8, :] = pltpu.bitcast(hv, U32)

    def repack(a, b):
        return (a & U32(0xFFFF)) | (b << 16), (a >> 16) | (b & U32(0xFFFF0000))

    def store_qkv(i, jrow, y, seg0):
        for sg in range(y.shape[0] // 32):
            for hh in range(2):
                qkvbufs[i][seg0 + sg, pl.ds(jrow + 8 + hh * 16, 16), :] = _pack(
                    y[sg * 32:(sg + 1) * 32, hh * 128:(hh + 1) * 128])

    for c_ in moda_copies(0):
        c_.wait()
    moda_apply(0, *moda_store(0, mod_tile(0, 0), mod_tile(1, 0)), 0, PRE)

    def w_wait(j, i0, i1):
        blk0 = (j // 3) * (6 * NB) + (j % 3) * 2
        for i in range(i0, i1):
            for par in range(2):
                pltpu.make_async_copy(w_hbms[0].at[:, 0, 0, :], w_v.at[blk0 + i * 6 + par],
                                      wsems.at[2 * j + (i >= PRE_SPLIT)]).wait()

    def chunk_block(kc, last, issue):
        for c_ in chunk_copies(kc) + ([cp_xr] if last else moda_copies(kc + 1)):
            c_.wait()
        issue()
        r0 = mult(kc * 64, 64)
        mv = []
        for i in range(NB):
            lo, hi = repack(w_v[i * 6, pl.ds(r0, 64), :], w_v[i * 6 + 1, pl.ds(r0, 64), :])
            w_v[i * 6, pl.ds(r0, 64), :] = lo
            w_v[i * 6 + 1, pl.ds(r0, 64), :] = hi
            w = pltpu.bitcast(jnp.concatenate([lo, hi], axis=1), BF)
            y = (pltpu.bitcast(wg_v[0:PRE, i * 256:(i + 1) * 256], F32)
                 + jnp.dot(pltpu.bitcast(h0buf[kc], BF), w, preferred_element_type=F32))
            if last:
                store_qkv(i, 0, y, 0)
            else:
                wg_v[0:PRE, i * 256:(i + 1) * 256] = pltpu.bitcast(y, U32)
                if i in (1, 3):
                    mv.append(mod_tile(i // 2, mult((kc + 1) * 128, 128)))
                if i == 3:
                    mv = moda_store(kc + 1, mv[0], mv[1])
                if i >= 4:
                    moda_apply(kc + 1, mv[0], mv[1], (i - 4) * 128, (i - 3) * 128)
        if last:
            for j in range(3):
                ln1_rows(PRE + 8 * j, HOFF + 8 + 8 * j)

    def chunk_body(kc, carry):
        def issue():
            @pl.when(kc < 5)
            def _():
                for c_ in moda_copies(kc + 3) + chunk_copies(kc + 3):
                    c_.start()
        chunk_block(kc, False, issue)
        return carry

    def issue_last():
        w_wait(1, 0, PRE_SPLIT)
        w_start(1, PRE_SPLIT, NB)
        w_start(2)
        mod_copy(2).start()
    w_start(1, 0, PRE_SPLIT, prio=1)
    lax.fori_loop(0, 7, chunk_body, 0)
    chunk_block(7, True, issue_last)

    def pre_unit(j, i, extra):
        blk = (j // 3) * (6 * NB) + (j % 3) * 2 + i * 6
        jrow = mult(j * 40, 8)
        lo, hi = repack(w_v[blk], w_v[blk + 1])
        w_v[blk] = lo
        w_v[blk + 1] = hi
        for rc in range(PRE // 128):
            if rc > 0:
                lo = w_v[blk]
                hi = w_v[blk + 1]
            w = pltpu.bitcast(jnp.concatenate([lo, hi], axis=1), BF)
            lhs = jnp.concatenate([h0buf[k, rc * 64:(rc + 1) * 64, :] for k in range(8)], axis=1)
            y = jnp.dot(pltpu.bitcast(lhs, BF), w, preferred_element_type=F32)
            store_qkv(i, jrow, y, rc * 4)
            extra(rc)

    for i in range(NB):
        if i == PRE_SPLIT:
            w_wait(1, PRE_SPLIT, NB)
            for jn in (3, 4):
                w_start(jn)
                mod_copy(jn).start()
        pre_unit(1, i, lambda rc: None)
    w_start(5)
    mod_copy(5).start()
    cp_wo.start()
    cp_x1.start()

    def pre_body(j, carry):
        w_wait(j, 0, NB)
        pltpu.make_async_copy(wmod32.at[:, 0:D], wmod_v.at[j], wsems.at[2 * j + 1]).wait()
        one = jnp.where(j == 4, 1.0, 0.0).astype(F32)
        for i in range(NB):
            def extra(rc, i=i):
                if rc == 1:
                    modb[j, :, i * 128:(i + 1) * 128] = _rb(one + mod_tile(j, i * 128))
            pre_unit(j, i, extra)
        return carry
    lax.fori_loop(2, 6, pre_body, 0)

    cp_wo.wait()
    cp_x1.wait()
    for c_ in cp_ffn:
        c_.start()

    def wo_w(q0, q1, n0, n1):
        h0, h1 = q0 + 2 * ROT, q1 + 2 * ROT
        ws = [wo_v[a:b, :, n0 * 128:n1 * 128].reshape((b - a) * (DH // 2), (n1 - n0) * 128)
              for a, b in ((h0, min(h1, H)), (0, h1 - H)) if b > a]
        return pltpu.bitcast(jnp.concatenate(ws, axis=0), BF)

    HD = D // 2

    def emit_step(s, pend, last):
        hrow = pl.multiple_of(HOFF + (s & 1) * 32, 32)
        hnext = pl.multiple_of(HOFF + 32 - (s & 1) * 32, 32)
        tv = [tab[s * NTAB + k] for k in range(15)]
        slot = tv[0]
        dsts = [(tv[1 + 2 * j], pl.multiple_of(tv[2 + 2 * j], 4)) for j in range(3)]
        odst = [pl.multiple_of(tv[7 + j], 8) for j in range(4)]
        orow = pl.multiple_of(tv[11], 32)
        erow = tv[12]
        lrow = tv[13]
        mrow = pl.multiple_of(tv[14], 8)
        e_at, l_at = (E_AT, L_AT) if pend is None else (E_AT2, L_AT2)
        probs = {}

        def wqkv(p, k0, k1):
            return pltpu.bitcast(jnp.concatenate(
                [w_v[p * 6 + u, k0 // 2:k1 // 2, :] for u in range(6)], axis=1), BF)

        lhs_lo = act[pl.ds(hrow, 32), 0:HD]
        if pend is not None:
            ybuf[...] = jnp.dot(lhs_lo, wqkv(0, 0, HD), preferred_element_type=F32)
            pend()
        lhs_hi = act[pl.ds(hrow, 32), HD:D]
        if pend is not None:
            y0 = ybuf[...] + jnp.dot(lhs_hi, wqkv(0, HD, D), preferred_element_type=F32)
        lhs_rest = jnp.concatenate([lhs_lo[:, 128:], lhs_hi], axis=1)
        lhs = [jnp.concatenate([lhs_lo, lhs_hi], axis=1)]

        def side(p):
            for j in range(3):
                if e_at[j] == p:
                    finish_rows(pl.multiple_of(erow + 8 * j, 8), attn_load(j))
            for j in range(3):
                if l_at[j] == p:
                    ln1_rows(pl.multiple_of(lrow + 8 * j, 8),
                             pl.multiple_of(hnext + 8 + 8 * j, 8))
            if p in e_at or p in l_at:
                lhs[0] = jnp.concatenate([act[pl.ds(hrow, 32), 0:128], lhs_rest], axis=1)

        def qkv(p):
            if p == 0 and pend is not None:
                y = y0
            else:
                y = jnp.dot(lhs[0], wqkv(p, 0, D), preferred_element_type=F32)
            buf = qkvbufs[p % NB]
            for u in range(6):
                t, hh = u // 2, u % 2
                b0 = ((p // NB) * 3 + t) * 40
                yu = y[:, u * 128:(u + 1) * 128]
                buf[slot, b0 + hh * 4:b0 + hh * 4 + 4, :] = _pack(yu[0:8])
                for j in range(3):
                    sl, off = dsts[j]
                    buf[sl, pl.ds(b0 + 8 + hh * 16 + off, 4), :] = _pack(yu[8 + 8 * j:16 + 8 * j])

        def ld(p, t):
            b0 = ((p // NB) * 3 + t) * 40
            return pltpu.bitcast(qkvbufs[p % NB][slot, b0:b0 + 40, :], BF)

        def sc(p):
            s2 = lax.dot_general(ld(p, 0), ld(p, 1), (((1,), (1,)), ((), ())),
                                 preferred_element_type=F32)
            s2 = jnp.where(valid, s2 * SCALE, fill)
            m = jnp.max(s2, axis=-1, keepdims=True)
            e = jnp.exp(s2 - m)
            l = jnp.sum(e, axis=-1, keepdims=True)
            rl = pl.reciprocal(l, approx=True)
            rl = rl * (2.0 - l * rl)
            probs[p] = (e * rl).astype(BF)

        def pv(p):
            o2 = jnp.dot(probs[p], ld(p, 2), preferred_element_type=F32)
            for hh in range(2):
                hcol = (2 * ((p - ROT) % NP) + hh) * 128
                ob = obuf1
                if hcol >= KS:
                    ob = obuf2
                    hcol -= KS
                ob[pl.ds(mrow, 8), hcol:hcol + 128] = o2[8 * hh:8 * hh + 8].astype(BF)
                for j in range(4):
                    r0 = 16 + 32 * hh + 8 * j
                    ob[pl.ds(odst[j], 8), hcol:hcol + 128] = o2[r0:r0 + 8].astype(BF)

        def attn(pos):
            for kind, p in ATT.get(pos, ()):
                (sc if kind == 's' else pv)(p)

        for p in range(NP):
            qkv(p)
            side(p)
            attn(p)
        a1 = []
        for n in range(8):
            a1.append(jnp.dot(obuf1[pl.ds(orow, 32), 0:KS], wo_w(0, KS // DH, n, n + 1),
                              preferred_element_type=F32))
            if n + 1 in W1AT:
                attn(NP + 2 * W1AT.index(n + 1))
        o2lhs = obuf2[pl.ds(orow, 32), 0:K2]
        a_lo = jnp.concatenate(a1[0:4], axis=1) + jnp.dot(
            o2lhs, wo_w(KS // DH, H, 0, 4), preferred_element_type=F32)
        act[pl.ds(hnext, 8), 0:HD] = a_lo[0:8].astype(BF)
        attn_store(a_lo[8:32], 0)
        a_hi = jnp.concatenate(a1[4:8], axis=1) + jnp.dot(
            o2lhs, wo_w(KS // DH, H, 4, 8), preferred_element_type=F32)

        def finish():
            act[pl.ds(hnext, 8), HD:D] = a_hi[0:8].astype(BF)
            attn_store(a_hi[8:32], 4)
        if last:
            finish()
        return finish

    def steps(it, carry):
        pend = None
        for u in range(UNR):
            pend = emit_step(it * UNR + u, pend, u == UNR - 1)
        return carry
    lax.fori_loop(0, NSEG // UNR, steps, 0)

    for c_ in cp_ffn:
        c_.wait()
    OUT0 = (NSEG - 1) * RIDE
    NEW0 = S - NEW
    cp_out = [cp(act.at[OOFF:OOFF + OUT0], out_hbm.at[0, 0:OUT0], 9)]
    cp_out[0].start()
    zero = pl.multiple_of(tab[NSEG * NTAB], 8)
    for j in range(3):
        ebuf[EMAX + 8 * j:EMAX + 8 * j + 8, :] = attn_load(j)
    ebuf[EMAX + RIDE:EMAX + RIDE + 8, :] = act[HOFF:HOFF + 8, :].astype(F32)
    todo = [(OUT0 + 8 * j, EMAX + 8 * j) for j in range(4)]
    r0 = 0
    for ci, ech in enumerate(EPI_CHUNKS):
        o0 = NOSLOT * 32 + r0
        e0 = (ci % 2) * EMAX
        per = -(-len(todo) // 8)
        if ci == len(EPI_CHUNKS) - 1:
            per = EPI_LASTPER
        for n in range(8):
            lhs = jnp.concatenate([obuf1[o0:o0 + ech, 0:KS], obuf2[o0:o0 + ech, 0:K2]], axis=1)
            ebuf[e0:e0 + ech, n * 128:(n + 1) * 128] = jnp.dot(
                lhs, wo_w(0, H, n, n + 1), preferred_element_type=F32)
            for row, er in todo[:per]:
                finish_rows(row, ebuf[pl.ds(zero + er, 8), :])
            todo = todo[per:]
        todo = [(OUT0 + RIDE + 8 + r0 + 8 * j, e0 + 8 * j) for j in range(ech // 8)]
        r0 += ech

    rowsf = (lane256 * 8 + lax.broadcasted_iota(jnp.int32, (8, 256), 0)).astype(F32)
    r_old = jnp.where(rowsf < NEW0, act[ROFF:ROFF + 8, 0:256].astype(F32), -jnp.inf)

    def allmax(v):
        return jnp.max(jnp.max(v, axis=1, keepdims=True), axis=0, keepdims=True)

    def allmin(v):
        return jnp.min(jnp.min(v, axis=1, keepdims=True), axis=0, keepdims=True)
    m1 = allmax(r_old)
    i1v = allmin(jnp.where(r_old == m1, rowsf, float(S)))
    r_rest = jnp.where(rowsf == i1v, -jnp.inf, r_old)
    m2 = allmax(r_rest)
    i2v = allmin(jnp.where((r_rest == m2) & (rowsf != i1v), rowsf, float(S)))
    i1 = jnp.clip(i1v[0, 0].astype(jnp.int32), 0, NEW0 - 1)
    i2 = jnp.clip(i2v[0, 0].astype(jnp.int32), 0, NEW0 - 1)
    b1 = pl.multiple_of((i1 // 8) * 8, 8)
    b2 = pl.multiple_of((i2 // 8) * 8, 8)
    sub8 = lax.broadcasted_iota(jnp.int32, (8, 1), 0)

    def rep(i, n):
        return jnp.concatenate([modb[i]] * n, axis=0)
    x1c = jnp.concatenate([act[pl.ds(b1, 8), :].astype(F32), act[pl.ds(b2, 8), :].astype(F32)],
                          axis=0)
    h2c = _rb(_rb(_layernorm(x1c) * rep(4, 2)) + rep(3, 2))
    row1 = jnp.sum(jnp.where(sub8 == i1 - b1, h2c[0:8], 0.0), axis=0, keepdims=True)
    row2 = jnp.sum(jnp.where(sub8 == i2 - b2, h2c[8:16], 0.0), axis=0, keepdims=True)
    cand = jnp.where(sub8 == 0, row1, jnp.where(sub8 == 1, row2, 0.0))

    e0 = ((len(EPI_CHUNKS) - 1) % 2) * EMAX
    ng = NEW // 8
    x1n = _rb(xbuf[NEW0:S, :].astype(F32) + _rb(rep(2, ng) * _rb(ebuf[e0:e0 + NEW, :])))
    h2n = _rb(_rb(_layernorm(x1n) * rep(4, ng)) + rep(3, ng))
    h2b = jnp.concatenate([cand, h2n], axis=0).astype(BF)
    cp_out.append(cp(act.at[OOFF + OUT0:OOFF + NEW0], out_hbm.at[0, OUT0:NEW0], 10))
    cp_out[1].start()
    hid = []
    for n in range(0, F, FFN_NB):
        gt = _rb(jnp.dot(h2b, pltpu.bitcast(wg_v[:, n:n + FFN_NB], BF), preferred_element_type=F32))
        up = _rb(jnp.dot(h2b, pltpu.bitcast(wu_v[:, n:n + FFN_NB], BF), preferred_element_type=F32))
        hid.append((_rb(gt * _rb(jax.nn.sigmoid(gt))) * up).astype(BF))
    y = _rb(jnp.dot(jnp.concatenate(hid, axis=1), pltpu.bitcast(wd_v[...], BF),
                    preferred_element_type=F32))
    val = jnp.concatenate(
        [jnp.where(sub8 == 0, m1, jnp.where(sub8 == 1, m2, -jnp.inf)),
         _rb(jnp.sum(h2n * rep(6, ng), axis=-1, keepdims=True))], axis=0)
    pos = lax.broadcasted_iota(jnp.int32, (8 + NEW, 1), 0).astype(F32)
    p1 = jnp.min(jnp.where(val == jnp.max(val, axis=0, keepdims=True), pos, float(S)),
                 axis=0, keepdims=True)
    val2 = jnp.where(pos == p1, -jnp.inf, val)
    p2 = jnp.min(jnp.where((val2 == jnp.max(val2, axis=0, keepdims=True)) & (pos != p1), pos,
                           float(S)), axis=0, keepdims=True)
    upd = jnp.where((pos == p1) | (pos == p2), _rb(y * _rb(jax.nn.sigmoid(val))), 0.0)
    act[OOFF + NEW0:OOFF + S, :] = (x1n + _rb(rep(5, ng) * _rb(h2n + upd[8:]))).astype(BF)
    sub16 = lax.broadcasted_iota(jnp.int32, (16, 1), 0)
    grow = jnp.where(sub16 < 8, b1 + sub16, b2 + sub16 - 8)
    updc = jnp.where(grow == i1, upd[0:1], jnp.where(grow == i2, upd[1:2], 0.0))
    res = (x1c + _rb(rep(5, 2) * _rb(h2c + updc))).astype(BF)
    for c_ in cp_out:
        c_.wait()
    act[pl.ds(OOFF + b1, 8), :] = res[0:8]
    act[pl.ds(OOFF + b2, 8), :] = res[8:16]
    fix0 = cp(act.at[OOFF + NEW0:OOFF + S], out_hbm.at[0, NEW0:S], 6)
    fix1 = cp(act.at[pl.ds(OOFF + b1, 8)], out_hbm.at[0, pl.ds(b1, 8)], 11)
    fix2 = cp(act.at[pl.ds(OOFF + b2, 8)], out_hbm.at[0, pl.ds(b2, 8)], 12)
    fix0.start()
    fix1.start()

    @pl.when(b1 != b2)
    def _():
        fix2.start()
        fix2.wait()
    fix0.wait()
    fix1.wait()


@jax.jit
def pallas_adaLN_cond__memory_aug_recurrent_mem_tr__moe_arch_mod__prompt_kernel(
    A_x: jax.Array,
    A_mem0: jax.Array,
    A_Wq: jax.Array,
    A_Wk: jax.Array,
    A_Wv: jax.Array,
    A_Wo: jax.Array,
    A_seg_len,
    B_x: jax.Array,
    B_w_r: jax.Array,
    B_w_gate: jax.Array,
    B_w_up: jax.Array,
    B_w_down: jax.Array,
    c: jax.Array,
    w_mod: jax.Array,
):
    del B_x
    del A_seg_len
    assert A_x.shape == (1, S, D) and A_Wq.shape == (D, H, DH) and A_mem0.shape == (1, M, D)
    any_spec = pl.BlockSpec(memory_space=pl.ANY)
    scratch = [
        pltpu.VMEM((S, D), BF),
        pltpu.VMEM((ACT_ROWS, D), BF),
        pltpu.VMEM((8, PRE // 2, 128), U32),
        pltpu.VMEM((32, 768), F32),
        pltpu.VMEM((2 * EMAX, D), F32),
        pltpu.SMEM((NSEG * NTAB + 1,), jnp.int32),
        pltpu.VMEM((7, 8, D), F32),
        pltpu.VMEM((3 * H, D // 2, 128), U32),
        pltpu.VMEM((H, DH // 2, D), U32),
        pltpu.VMEM((6, D // 2, D), U32),
        pltpu.VMEM((D // 2, F), U32),
        pltpu.VMEM((D // 2, F), U32),
        pltpu.VMEM((F // 2, D), U32),
        pltpu.VMEM((NOSLOT * 32 + PRE, OW1), BF),
        pltpu.VMEM((NOSLOT * 32 + PRE, OW2), BF),
        pltpu.SemaphoreType.DMA((17,)),
        pltpu.SemaphoreType.DMA((12,)),
        pltpu.SemaphoreType.DMA((16,)),
    ] + [pltpu.VMEM((NSLOT + 1, 256, 128), U32) for _ in range(NB)] + [
        pltpu.VMEM((1, D), BF),
        pltpu.VMEM((D,), BF),
    ]
    wq, wk, wv = (w.reshape(D // 2, 2, H, DH) for w in (A_Wq, A_Wk, A_Wv))
    return pl.pallas_call(
        _kernel,
        out_shape=jax.ShapeDtypeStruct((1, S, D), BF),
        in_specs=[any_spec] * 12,
        out_specs=any_spec,
        scratch_shapes=scratch,
        compiler_params=pltpu.CompilerParams(vmem_limit_bytes=120 * 1024 * 1024,
                                             disable_bounds_checks=True,
                                             disable_semaphore_checks=True),
    )(A_x, A_mem0, wq, wk, wv, A_Wo, B_w_r, B_w_gate, B_w_up, B_w_down,
      c, w_mod)
```

```python
import jax
import jax.numpy as jnp
from jax import lax
import jax.experimental.pallas as pl
import jax.experimental.pallas.tpu as pltpu

BF = jnp.bfloat16
F32 = jnp.float32
U32 = jnp.uint32

S = 2048
D = 1024
H = 32
DH = 128
M = 8
SEG = 32
NSEG = S // SEG
F = 3584
NP = H // 2
EPS = 1e-5
SCALE = DH ** -0.5

RIDE = 24
PRE = S - NSEG * RIDE
NSLOT = 17
NB = 8
KS = 1792
OOFF = S
HOFF = 2 * S
ROFF = HOFF + 64
ACT_ROWS = ROFF + 16
PRE_SPLIT = 3
E_AT = (1, 2, 3, 5, 7)
E_AT2 = (3, 5, 6)
L_AT = (10, 12, 14)
L_AT2 = (8, 10, 12)
A_BUF = (7, 0, 1, 2, 3)
W1AT = (2, 6)
NEW = 40
FFN_NB = 512
NTAB = 8

ROT = 0
ATT = {4: [('s', i) for i in range(4)],
       18: [('p', (12 + ROT + i) % NP) for i in range(4)]}
for _p in range(4, NP, 2):
    ATT[_p + 2] = [('s', _p), ('s', _p + 1), ('p', _p - 4 + ROT), ('p', _p - 3 + ROT)]


def _step_indices(s):
    t = [s % NSLOT]
    for j in range(3):
        gi = PRE // 8 + 3 * s + j
        t += [(gi // 4) % NSLOT, (gi % 4) * 4]
    return t


def _rb(v):
    return v.astype(BF).astype(F32)


def _pack(v):
    return pltpu.bitcast(v.astype(BF), U32)


def _layernorm(x):
    mu = jnp.sum(x, axis=-1, keepdims=True) * (1.0 / D)
    xc = x - mu
    var = jnp.sum(xc * xc, axis=-1, keepdims=True) * (1.0 / D)
    sd = _rb(jnp.sqrt(_rb(_rb(var) + EPS)))
    return _rb(_rb(x - _rb(mu)) / sd)


def _kernel(x_hbm, mem0_hbm, wq_hbm, wk_hbm, wv_hbm, wo_hbm, wr_hbm, wg_hbm, wu_hbm,
            wd_hbm, c_hbm, wmod_hbm, out_hbm,
            xbuf, act, h0buf, ybuf, tab, modb,
            w_v, wo_v, wmod_v, wg_v, wu_v, wd_v,
            obuf, sems, wsems, ksems, *rest):
    qkvbufs, cbuf, wrbuf = rest[:NB], rest[NB], rest[NB + 1]
    w_hbms = tuple(w.bitcast(U32) for w in (wq_hbm, wk_hbm, wv_hbm))

    def cp(src, dst, i):
        return pltpu.make_async_copy(src, dst, sems.at[i])

    wmod32 = wmod_hbm.bitcast(U32)
    cp_c = cp(c_hbm, cbuf, 0)
    cp_mem = cp(mem0_hbm.at[0], act.at[HOFF:HOFF + M], 1)
    cp_wr = cp(wr_hbm, wrbuf, 2)
    cp_x0 = [cp(x_hbm.at[0, n * 128:(n + 1) * 128], xbuf.at[n * 128:(n + 1) * 128], 13 + n)
             for n in range(PRE // 128)]
    cp_xr = cp(x_hbm.at[0, PRE:PRE + 32], xbuf.at[PRE:PRE + 32], 5)
    cp_x1 = cp(x_hbm.at[0, PRE + 32:S], xbuf.at[PRE + 32:S], 4)
    cp_wo = cp(wo_hbm.bitcast(U32), wo_v, 7)
    cp_ffn = [cp(wg_hbm.bitcast(U32), wg_v, 8), cp(wu_hbm.bitcast(U32), wu_v, 8),
              cp(wd_hbm.bitcast(U32), wd_v, 8)]

    def w_start(j, i0=0, i1=NB, prio=0):
        gg, t = j // 3, j % 3
        for i in range(i0, i1):
            for par in range(2):
                pltpu.make_async_copy(w_hbms[t].at[:, par, gg * NB + i, :],
                                      w_v.at[(gg * NB + i) * 6 + t * 2 + par],
                                      wsems.at[2 * j + (i >= PRE_SPLIT)]).start(priority=prio)

    def mod_copy(j):
        return pltpu.make_async_copy(wmod32.at[:, j * D:(j + 1) * D], wmod_v.at[j],
                                     wsems.at[2 * j + 1])

    def mult(v, m):
        return v if isinstance(v, int) else pl.multiple_of(v, m)

    def moda_copies(kc):
        col = mult(kc * 128, 128)
        return [pltpu.make_async_copy(wmod32.at[:, pl.ds(v * D + col, 128)],
                                      wmod_v.at[v, :, pl.ds(col, 128)], ksems.at[8 + kc])
                for v in range(2)]

    def chunk_copies(kc):
        r0 = mult(kc * 64, 64)
        return [pltpu.make_async_copy(w_hbms[0].at[pl.ds(r0, 64), par, i, :],
                                      w_v.at[i * 6 + par, pl.ds(r0, 64), :], ksems.at[kc])
                for i in range(NB) for par in range(2)]

    cp_c.start()
    cp_mem.start()
    cp_wr.start()
    for c_ in (cp_x0 + moda_copies(0) + moda_copies(1) + chunk_copies(0) + moda_copies(2)
               + chunk_copies(1) + [cp_xr] + chunk_copies(2)):
        c_.start()

    def ln1_rows(src_row, dst_row):
        xv = xbuf[pl.ds(src_row, 8), :].astype(F32)
        hv = _rb(_layernorm(xv) * modb[1]) + modb[0]
        act[pl.ds(dst_row, 8), :] = hv.astype(BF)

    lane256 = lax.broadcasted_iota(jnp.int32, (8, 256), 1)

    def finish_rows(row, attn):
        xv = xbuf[pl.ds(row, 8), :].astype(F32)
        x1 = _rb(xv + _rb(modb[2] * _rb(attn)))
        act[pl.ds(row, 8), :] = x1.astype(BF)
        h2 = _rb(_rb(_layernorm(x1) * modb[4]) + modb[3])
        act[pl.ds(OOFF + row, 8), :] = (x1 + _rb(modb[5] * h2)).astype(BF)
        r = jnp.sum(h2 * modb[6], axis=-1, keepdims=True)
        act[ROFF:ROFF + 8, 0:256] = jnp.where(
            lane256 * 8 == row, r, act[ROFF:ROFF + 8, 0:256].astype(F32)).astype(BF)

    def attn_store(a, k0):
        for j in range(a.shape[0] // 8):
            for k in range(a.shape[1] // 128):
                qkvbufs[A_BUF[j]][NSLOT, (k0 + k) * 8:(k0 + k + 1) * 8, :] = pltpu.bitcast(
                    a[8 * j:8 * j + 8, k * 128:(k + 1) * 128], U32)

    def attn_load(j):
        return pltpu.bitcast(jnp.concatenate(
            [qkvbufs[A_BUF[j]][NSLOT, k * 8:(k + 1) * 8, :] for k in range(8)], axis=1), F32)

    act[ROFF:ROFF + 8, 0:256] = jnp.zeros((8, 256), BF)
    attn_store(jnp.zeros((NEW, D), F32), 0)
    for s_ in range(NSEG):
        for k, v in enumerate(_step_indices(s_)):
            tab[s_ * NTAB + k] = v
    ri = lax.broadcasted_iota(jnp.int32, (80, 80), 0)
    ci = lax.broadcasted_iota(jnp.int32, (80, 80), 1)

    def head_pos(i):
        hd = jnp.where(i < 16, i // 8, (i - 16) // 32)
        pos = jnp.where(i < 16, i % 8, 8 + (i - 16) % 32)
        return hd, pos
    rh, rp = head_pos(ri)
    ch, cpos = head_pos(ci)
    same = rh == ch
    valid = same & ((rp < M) | (rp >= cpos))
    fill = jnp.where(same, -1e9, -jnp.inf).astype(F32)

    cp_mem.wait()
    cp_wr.wait()
    modb[6] = jnp.broadcast_to(wrbuf[...].astype(F32).reshape(1, D), (8, D))
    cp_c.wait()
    cv = cbuf[...].astype(F32)
    sc16 = jnp.broadcast_to(_rb(cv * _rb(jax.nn.sigmoid(cv))), (16, D)).astype(BF)

    def ln_pre(g, carry):
        pltpu.make_async_copy(x_hbm.at[0, 0:128], xbuf.at[pl.ds(pl.multiple_of(g * 128, 128), 128)],
                              sems.at[13 + g]).wait()
        for u in range(2):
            row = pl.multiple_of(g * 128 + u * 64, 64)
            nv = _layernorm(xbuf[pl.ds(row, 64), :].astype(F32)).astype(BF)
            for k in range(8):
                h0buf[k, pl.ds(pl.multiple_of(row // 2, 32), 32), :] = pltpu.bitcast(
                    nv[:, k * 128:(k + 1) * 128], U32)
            wg_v[pl.ds(row, 64), 0:2 * D] = jnp.zeros((64, 2 * D), U32)
        return carry
    lax.fori_loop(0, PRE // 128, ln_pre, 0)

    def mod_tile(v, col):
        w = pltpu.bitcast(wmod_v[v, :, pl.ds(col, 128)], BF)
        return _rb(jnp.dot(sc16, w, preferred_element_type=F32))[0:8]

    def moda_store(kc, sa, ca):
        col = mult(kc * 128, 128)
        c1 = _rb(1.0 + ca)
        modb[0, :, pl.ds(col, 128)] = sa
        modb[1, :, pl.ds(col, 128)] = c1
        return sa, c1

    def moda_apply(kc, sa, c1, r0, r1):
        for r in range(r0, r1, 16):
            nv = pltpu.bitcast(h0buf[kc, r // 2:r // 2 + 8, :], BF).astype(F32).reshape(2, 8, 128)
            hv = (_rb(nv * c1[None]) + sa[None]).reshape(16, 128).astype(BF)
            h0buf[kc, r // 2:r // 2 + 8, :] = pltpu.bitcast(hv, U32)

    def repack(a, b):
        return (a & U32(0xFFFF)) | (b << 16), (a >> 16) | (b & U32(0xFFFF0000))

    def store_qkv(i, jrow, y, seg0):
        for sg in range(y.shape[0] // 32):
            for hh in range(2):
                qkvbufs[i][seg0 + sg, pl.ds(jrow + 8 + hh * 16, 16), :] = _pack(
                    y[sg * 32:(sg + 1) * 32, hh * 128:(hh + 1) * 128])

    for c_ in moda_copies(0):
        c_.wait()
    moda_apply(0, *moda_store(0, mod_tile(0, 0), mod_tile(1, 0)), 0, PRE)

    def w_wait(j, i0, i1):
        blk0 = (j // 3) * (6 * NB) + (j % 3) * 2
        for i in range(i0, i1):
            for par in range(2):
                pltpu.make_async_copy(w_hbms[0].at[:, 0, 0, :], w_v.at[blk0 + i * 6 + par],
                                      wsems.at[2 * j + (i >= PRE_SPLIT)]).wait()

    def chunk_block(kc, last, issue):
        for c_ in chunk_copies(kc) + ([cp_xr] if last else moda_copies(kc + 1)):
            c_.wait()
        issue()
        r0 = mult(kc * 64, 64)
        mv = []
        for i in range(NB):
            lo, hi = repack(w_v[i * 6, pl.ds(r0, 64), :], w_v[i * 6 + 1, pl.ds(r0, 64), :])
            w_v[i * 6, pl.ds(r0, 64), :] = lo
            w_v[i * 6 + 1, pl.ds(r0, 64), :] = hi
            w = pltpu.bitcast(jnp.concatenate([lo, hi], axis=1), BF)
            y = (pltpu.bitcast(wg_v[0:PRE, i * 256:(i + 1) * 256], F32)
                 + jnp.dot(pltpu.bitcast(h0buf[kc], BF), w, preferred_element_type=F32))
            if last:
                store_qkv(i, 0, y, 0)
            else:
                wg_v[0:PRE, i * 256:(i + 1) * 256] = pltpu.bitcast(y, U32)
                if i in (1, 3):
                    mv.append(mod_tile(i // 2, mult((kc + 1) * 128, 128)))
                if i == 3:
                    mv = moda_store(kc + 1, mv[0], mv[1])
                if i >= 4:
                    moda_apply(kc + 1, mv[0], mv[1], (i - 4) * 128, (i - 3) * 128)
        if last:
            for j in range(3):
                ln1_rows(PRE + 8 * j, HOFF + 8 + 8 * j)

    def chunk_body(kc, carry):
        def issue():
            @pl.when(kc < 5)
            def _():
                for c_ in moda_copies(kc + 3) + chunk_copies(kc + 3):
                    c_.start()
        chunk_block(kc, False, issue)
        return carry

    def issue_last():
        w_wait(1, 0, PRE_SPLIT)
        w_start(1, PRE_SPLIT, NB)
        w_start(2)
        mod_copy(2).start()
    w_start(1, 0, PRE_SPLIT, prio=1)
    lax.fori_loop(0, 7, chunk_body, 0)
    chunk_block(7, True, issue_last)

    def pre_unit(j, i, extra):
        blk = (j // 3) * (6 * NB) + (j % 3) * 2 + i * 6
        jrow = mult(j * 40, 8)
        lo, hi = repack(w_v[blk], w_v[blk + 1])
        w_v[blk] = lo
        w_v[blk + 1] = hi
        for rc in range(PRE // 128):
            if rc > 0:
                lo = w_v[blk]
                hi = w_v[blk + 1]
            w = pltpu.bitcast(jnp.concatenate([lo, hi], axis=1), BF)
            lhs = jnp.concatenate([h0buf[k, rc * 64:(rc + 1) * 64, :] for k in range(8)], axis=1)
            y = jnp.dot(pltpu.bitcast(lhs, BF), w, preferred_element_type=F32)
            store_qkv(i, jrow, y, rc * 4)
            extra(rc)

    for i in range(NB):
        if i == PRE_SPLIT:
            w_wait(1, PRE_SPLIT, NB)
            for jn in (3, 4):
                w_start(jn)
                mod_copy(jn).start()
        pre_unit(1, i, lambda rc: None)
    w_start(5)
    mod_copy(5).start()
    cp_wo.start()
    cp_x1.start()

    def pre_body(j, carry):
        w_wait(j, 0, NB)
        pltpu.make_async_copy(wmod32.at[:, 0:D], wmod_v.at[j], wsems.at[2 * j + 1]).wait()
        one = jnp.where(j == 4, 1.0, 0.0).astype(F32)
        for i in range(NB):
            def extra(rc, i=i):
                if rc == 1:
                    modb[j, :, i * 128:(i + 1) * 128] = _rb(one + mod_tile(j, i * 128))
            pre_unit(j, i, extra)
        return carry
    lax.fori_loop(2, 6, pre_body, 0)

    cp_wo.wait()
    cp_x1.wait()
    for c_ in cp_ffn:
        c_.start()

    def wo_w(q0, q1, n0, n1):
        h0, h1 = q0 + 2 * ROT, q1 + 2 * ROT
        ws = [wo_v[a:b, :, n0 * 128:n1 * 128].reshape((b - a) * (DH // 2), (n1 - n0) * 128)
              for a, b in ((h0, min(h1, H)), (0, h1 - H)) if b > a]
        return pltpu.bitcast(jnp.concatenate(ws, axis=0), BF)

    HD = D // 2

    def emit_step(it, odd, pend):
        s = 2 * it + odd
        hrow = pl.multiple_of(HOFF + (s & 1) * 32, 32)
        hnext = pl.multiple_of(HOFF + 32 - (s & 1) * 32, 32)
        tv = [tab[s * NTAB + k] for k in range(7)]
        slot = tv[0]
        dsts = [(tv[1 + 2 * j], pl.multiple_of(tv[2 + 2 * j], 4)) for j in range(3)]
        orow, ow = (32, 48) if odd else (0, 32)
        odst = (48, 56, 64, 72) if odd else (8, 16, 24, 40)
        erow = it * 64 if odd else jnp.maximum(it - 1, 0) * 64 + RIDE
        lrow = PRE + jnp.minimum(s + 1, NSEG - 1) * RIDE
        e_at, l_at = (E_AT2, L_AT2) if odd else (E_AT, L_AT)
        probs = {}

        def wqkv(p, k0, k1):
            return pltpu.bitcast(jnp.concatenate(
                [w_v[p * 6 + u, k0 // 2:k1 // 2, :] for u in range(6)], axis=1), BF)

        lhs_lo = act[pl.ds(hrow, 32), 0:HD]
        if pend is not None:
            ybuf[...] = jnp.dot(lhs_lo, wqkv(0, 0, HD), preferred_element_type=F32)
            pend()
        lhs_hi = act[pl.ds(hrow, 32), HD:D]
        if pend is not None:
            y0 = ybuf[...] + jnp.dot(lhs_hi, wqkv(0, HD, D), preferred_element_type=F32)
        lhs_rest = jnp.concatenate([lhs_lo[:, 128:], lhs_hi], axis=1)
        lhs = [jnp.concatenate([lhs_lo, lhs_hi], axis=1)]

        def side(p):
            for j in range(len(e_at)):
                if e_at[j] == p:
                    finish_rows(pl.multiple_of(erow + 8 * j, 8), attn_load(j))
            for j in range(3):
                if l_at[j] == p:
                    ln1_rows(pl.multiple_of(lrow + 8 * j, 8),
                             pl.multiple_of(hnext + 8 + 8 * j, 8))
            if p in e_at or p in l_at:
                lhs[0] = jnp.concatenate([act[pl.ds(hrow, 32), 0:128], lhs_rest], axis=1)

        def qkv(p):
            if p == 0 and pend is not None:
                y = y0
            else:
                y = jnp.dot(lhs[0], wqkv(p, 0, D), preferred_element_type=F32)
            buf = qkvbufs[p % NB]
            for u in range(6):
                t, hh = u // 2, u % 2
                b0 = ((p // NB) * 3 + t) * 40
                yu = y[:, u * 128:(u + 1) * 128]
                buf[slot, b0 + hh * 4:b0 + hh * 4 + 4, :] = _pack(yu[0:8])
                for j in range(3):
                    sl, off = dsts[j]
                    buf[sl, pl.ds(b0 + 8 + hh * 16 + off, 4), :] = _pack(yu[8 + 8 * j:16 + 8 * j])

        def ld(p, t):
            b0 = ((p // NB) * 3 + t) * 40
            return pltpu.bitcast(qkvbufs[p % NB][slot, b0:b0 + 40, :], BF)

        def sc(p):
            s2 = lax.dot_general(ld(p, 0), ld(p, 1), (((1,), (1,)), ((), ())),
                                 preferred_element_type=F32)
            s2 = jnp.where(valid, s2 * SCALE, fill)
            m = jnp.max(s2, axis=-1, keepdims=True)
            e = jnp.exp(s2 - m)
            l = jnp.sum(e, axis=-1, keepdims=True)
            rl = pl.reciprocal(l, approx=True)
            rl = rl * (2.0 - l * rl)
            probs[p] = (e * rl).astype(BF)

        def pv(p):
            o2 = jnp.dot(probs[p], ld(p, 2), preferred_element_type=F32)
            for hh in range(2):
                hcol = (2 * ((p - ROT) % NP) + hh) * 128
                obuf[orow:orow + 8, hcol:hcol + 128] = o2[8 * hh:8 * hh + 8].astype(BF)
                for j in range(4):
                    r0 = 16 + 32 * hh + 8 * j
                    obuf[odst[j]:odst[j] + 8, hcol:hcol + 128] = o2[r0:r0 + 8].astype(BF)

        def attn(pos):
            for kind, p in ATT.get(pos, ()):
                (sc if kind == 's' else pv)(p)

        for p in range(NP):
            qkv(p)
            side(p)
            attn(p)
        a1 = []
        for n in range(8):
            a1.append(jnp.dot(obuf[orow:orow + ow, 0:KS], wo_w(0, KS // DH, n, n + 1),
                              preferred_element_type=F32))
            if n + 1 in W1AT:
                attn(NP + 2 * W1AT.index(n + 1))
        o2lhs = obuf[orow:orow + ow, KS:]
        a_lo = jnp.concatenate(a1[0:4], axis=1) + jnp.dot(
            o2lhs, wo_w(KS // DH, H, 0, 4), preferred_element_type=F32)
        act[pl.ds(hnext, 8), 0:HD] = a_lo[0:8].astype(BF)
        attn_store(a_lo[8:], 0)
        a_hi = jnp.concatenate(a1[4:8], axis=1) + jnp.dot(
            o2lhs, wo_w(KS // DH, H, 4, 8), preferred_element_type=F32)

        def finish():
            act[pl.ds(hnext, 8), HD:D] = a_hi[0:8].astype(BF)
            attn_store(a_hi[8:], 4)
        return finish

    def out_copy(r0, n, sem):
        return cp(act.at[pl.ds(OOFF + r0, n)], out_hbm.at[0, pl.ds(r0, n)], sem)

    def steps(it, carry):
        emit_step(it, 1, emit_step(it, 0, None))()

        @pl.when(it > 0)
        def _():
            out_copy(pl.multiple_of((it - 1) * 64, 64), 64, 9).start()
        return carry
    lax.fori_loop(0, NSEG // 2, steps, 0)

    NEW0 = S - NEW
    out_copy(S - 64, NEW0 - (S - 64), 9).start()
    for c_ in cp_ffn:
        c_.wait()

    rowsf = (lane256 * 8 + lax.broadcasted_iota(jnp.int32, (8, 256), 0)).astype(F32)
    r_old = jnp.where(rowsf < NEW0, act[ROFF:ROFF + 8, 0:256].astype(F32), -jnp.inf)

    def allmax(v):
        return jnp.max(jnp.max(v, axis=1, keepdims=True), axis=0, keepdims=True)

    def allmin(v):
        return jnp.min(jnp.min(v, axis=1, keepdims=True), axis=0, keepdims=True)
    m1 = allmax(r_old)
    i1v = allmin(jnp.where(r_old == m1, rowsf, float(S)))
    r_rest = jnp.where(rowsf == i1v, -jnp.inf, r_old)
    m2 = allmax(r_rest)
    i2v = allmin(jnp.where((r_rest == m2) & (rowsf != i1v), rowsf, float(S)))
    i1 = jnp.clip(i1v[0, 0].astype(jnp.int32), 0, NEW0 - 1)
    i2 = jnp.clip(i2v[0, 0].astype(jnp.int32), 0, NEW0 - 1)
    b1 = pl.multiple_of((i1 // 8) * 8, 8)
    b2 = pl.multiple_of((i2 // 8) * 8, 8)

    def rep(i, n):
        return jnp.concatenate([modb[i]] * n, axis=0)
    ng = NEW // 8
    x1n = _rb(xbuf[NEW0:S, :].astype(F32) + _rb(rep(2, ng) * _rb(
        jnp.concatenate([attn_load(j) for j in range(ng)], axis=0))))
    h2n = _rb(_rb(_layernorm(x1n) * rep(4, ng)) + rep(3, ng))
    rn = _rb(jnp.sum(h2n * rep(6, ng), axis=-1, keepdims=True))
    x1c = jnp.concatenate([act[pl.ds(b1, 8), :].astype(F32), act[pl.ds(b2, 8), :].astype(F32)],
                          axis=0)
    h2c = _rb(_rb(_layernorm(x1c) * rep(4, 2)) + rep(3, 2))
    x1a = jnp.concatenate([x1c, x1n], axis=0)
    h2a = jnp.concatenate([h2c, h2n], axis=0)
    sub8 = lax.broadcasted_iota(jnp.int32, (8, 1), 0)
    val = jnp.concatenate([jnp.where(sub8 == i1 - b1, m1, -jnp.inf),
                           jnp.where(sub8 == i2 - b2, m2, -jnp.inf), rn], axis=0)
    live = jnp.concatenate([(sub8 == i1 - b1).astype(F32), (sub8 == i2 - b2).astype(F32),
                            jnp.ones((NEW, 1), F32)], axis=0) > 0.5
    pos = lax.broadcasted_iota(jnp.int32, (16 + NEW, 1), 0).astype(F32)
    v1 = jnp.max(val, axis=0, keepdims=True)
    p1 = jnp.min(jnp.where((val == v1) & live, pos, float(S)), axis=0, keepdims=True)
    val2 = jnp.where(pos == p1, -jnp.inf, val)
    v2 = jnp.max(val2, axis=0, keepdims=True)
    p2 = jnp.min(jnp.where((val2 == v2) & live & (pos != p1), pos, float(S)),
                 axis=0, keepdims=True)
    row1 = jnp.sum(jnp.where(pos == p1, h2a, 0.0), axis=0, keepdims=True)
    row2 = jnp.sum(jnp.where(pos == p2, h2a, 0.0), axis=0, keepdims=True)
    sub16 = lax.broadcasted_iota(jnp.int32, (16, 1), 0)
    h2b = jnp.where(sub16 == 0, row1, jnp.where(sub16 == 1, row2, 0.0)).astype(BF)
    hid = []
    for n in range(0, F, FFN_NB):
        gt = _rb(jnp.dot(h2b, pltpu.bitcast(wg_v[:, n:n + FFN_NB], BF), preferred_element_type=F32))
        up = _rb(jnp.dot(h2b, pltpu.bitcast(wu_v[:, n:n + FFN_NB], BF), preferred_element_type=F32))
        hid.append((_rb(gt * _rb(jax.nn.sigmoid(gt))) * up).astype(BF))
    y = _rb(jnp.dot(jnp.concatenate(hid, axis=1), pltpu.bitcast(wd_v[...], BF),
                    preferred_element_type=F32))
    y1 = _rb(y[0:1] * _rb(jax.nn.sigmoid(v1)))
    y2 = _rb(y[1:2] * _rb(jax.nn.sigmoid(v2)))
    tok = jnp.concatenate([(b1 + sub8).astype(F32), (b2 + sub8).astype(F32),
                           pos[16:] + float(NEW0 - 16)], axis=0)
    t1 = jnp.sum(jnp.where(pos == p1, tok, 0.0), axis=0, keepdims=True)
    t2 = jnp.sum(jnp.where(pos == p2, tok, 0.0), axis=0, keepdims=True)
    upd = jnp.where(tok == t1, y1, jnp.where(tok == t2, y2, 0.0))
    res = (x1a + _rb(rep(5, ng + 2) * _rb(h2a + upd))).astype(BF)
    act[OOFF + NEW0:OOFF + S, :] = res[16:]
    out_copy(0, NEW0, 9).wait()
    act[pl.ds(OOFF + b1, 8), :] = res[0:8]
    act[pl.ds(OOFF + b2, 8), :] = res[8:16]
    fix0 = out_copy(NEW0, NEW, 6)
    fix1 = out_copy(b1, 8, 11)
    fix2 = out_copy(b2, 8, 12)
    fix0.start()
    fix1.start()

    @pl.when(b1 != b2)
    def _():
        fix2.start()
        fix2.wait()
    fix0.wait()
    fix1.wait()


@jax.jit
def pallas_adaLN_cond__memory_aug_recurrent_mem_tr__moe_arch_mod__prompt_kernel(
    A_x: jax.Array,
    A_mem0: jax.Array,
    A_Wq: jax.Array,
    A_Wk: jax.Array,
    A_Wv: jax.Array,
    A_Wo: jax.Array,
    A_seg_len,
    B_x: jax.Array,
    B_w_r: jax.Array,
    B_w_gate: jax.Array,
    B_w_up: jax.Array,
    B_w_down: jax.Array,
    c: jax.Array,
    w_mod: jax.Array,
):
    del B_x
    del A_seg_len
    assert A_x.shape == (1, S, D) and A_Wq.shape == (D, H, DH) and A_mem0.shape == (1, M, D)
    any_spec = pl.BlockSpec(memory_space=pl.ANY)
    scratch = [
        pltpu.VMEM((S, D), BF),
        pltpu.VMEM((ACT_ROWS, D), BF),
        pltpu.VMEM((8, PRE // 2, 128), U32),
        pltpu.VMEM((32, 768), F32),
        pltpu.SMEM((NSEG * NTAB,), jnp.int32),
        pltpu.VMEM((7, 8, D), F32),
        pltpu.VMEM((3 * H, D // 2, 128), U32),
        pltpu.VMEM((H, DH // 2, D), U32),
        pltpu.VMEM((6, D // 2, D), U32),
        pltpu.VMEM((D // 2, F), U32),
        pltpu.VMEM((D // 2, F), U32),
        pltpu.VMEM((F // 2, D), U32),
        pltpu.VMEM((80, H * DH), BF),
        pltpu.SemaphoreType.DMA((17,)),
        pltpu.SemaphoreType.DMA((12,)),
        pltpu.SemaphoreType.DMA((16,)),
    ] + [pltpu.VMEM((NSLOT + 1, 256, 128), U32) for _ in range(NB)] + [
        pltpu.VMEM((1, D), BF),
        pltpu.VMEM((D,), BF),
    ]
    wq, wk, wv = (w.reshape(D // 2, 2, H, DH) for w in (A_Wq, A_Wk, A_Wv))
    return pl.pallas_call(
        _kernel,
        out_shape=jax.ShapeDtypeStruct((1, S, D), BF),
        in_specs=[any_spec] * 12,
        out_specs=any_spec,
        scratch_shapes=scratch,
        compiler_params=pltpu.CompilerParams(vmem_limit_bytes=120 * 1024 * 1024,
                                             disable_bounds_checks=True,
                                             disable_semaphore_checks=True),
    )(A_x, A_mem0, wq, wk, wv, A_Wo, B_w_r, B_w_gate, B_w_up, B_w_down,
      c, w_mod)
```

```python
import jax
import jax.numpy as jnp
from jax import lax
import jax.experimental.pallas as pl
import jax.experimental.pallas.tpu as pltpu

BF = jnp.bfloat16
F32 = jnp.float32
U32 = jnp.uint32

S = 2048
D = 1024
H = 32
DH = 128
M = 8
SEG = 32
NSEG = S // SEG
F = 3584
NP = H // 2
EPS = 1e-5
SCALE = DH ** -0.5

RIDE = 24
PRE = S - NSEG * RIDE
NSLOT = 17
NB = 8
KS = 2048
OOFF = S
HOFF = 2 * S
ROFF = HOFF + 64
ACT_ROWS = ROFF + 16
PRE_SPLIT = 3
E_AT = (2, 3, 4, 5, 6)
E_AT2 = (3, 4, 5)
L_AT = (6, 7, 8)
L_AT2 = (6, 8, 10)
A_BUF = (7, 0, 1, 2, 3)
W1AT = (2, 6)
NEW = 40
FFN_NB = 512
NTAB = 8

ROT = 2
ATT = {4: [('s', i) for i in range(4)],
       18: [('p', (12 + ROT + i) % NP) for i in range(4)]}
for _p in range(4, NP, 2):
    ATT[_p + 2] = [('s', _p), ('s', _p + 1), ('p', _p - 4 + ROT), ('p', _p - 3 + ROT)]


def _step_indices(s):
    t = [s % NSLOT]
    for j in range(3):
        gi = PRE // 8 + 3 * s + j
        t += [(gi // 4) % NSLOT, (gi % 4) * 4]
    return t


def _rb(v):
    return v.astype(BF).astype(F32)


def _pack(v):
    return pltpu.bitcast(v.astype(BF), U32)


def _layernorm(x):
    mu = jnp.sum(x, axis=-1, keepdims=True) * (1.0 / D)
    xc = x - mu
    var = jnp.sum(xc * xc, axis=-1, keepdims=True) * (1.0 / D)
    sd = _rb(jnp.sqrt(_rb(_rb(var) + EPS)))
    return _rb(_rb(x - _rb(mu)) / sd)


def _kernel(x_hbm, mem0_hbm, wq_hbm, wk_hbm, wv_hbm, wo_hbm, wr_hbm, wg_hbm, wu_hbm,
            wd_hbm, c_hbm, wmod_hbm, out_hbm,
            xbuf, act, h0buf, ybuf, tab, modb,
            w_v, wo_v, wmod_v, wg_v, wu_v, wd_v,
            obuf, sems, wsems, ksems, *rest):
    qkvbufs, cbuf, wrbuf = rest[:NB], rest[NB], rest[NB + 1]
    w_hbms = tuple(w.bitcast(U32) for w in (wq_hbm, wk_hbm, wv_hbm))

    def cp(src, dst, i):
        return pltpu.make_async_copy(src, dst, sems.at[i])

    wmod32 = wmod_hbm.bitcast(U32)
    cp_c = cp(c_hbm, cbuf, 0)
    cp_mem = cp(mem0_hbm.at[0], act.at[HOFF:HOFF + M], 1)
    cp_wr = cp(wr_hbm, wrbuf, 2)
    cp_x0 = [cp(x_hbm.at[0, n * 128:(n + 1) * 128], xbuf.at[n * 128:(n + 1) * 128], 13 + n)
             for n in range(PRE // 128)]
    cp_xr = cp(x_hbm.at[0, PRE:PRE + 32], xbuf.at[PRE:PRE + 32], 5)
    cp_x1 = cp(x_hbm.at[0, PRE + 32:S], xbuf.at[PRE + 32:S], 4)
    cp_wo = cp(wo_hbm.bitcast(U32), wo_v, 7)
    cp_ffn = [cp(wg_hbm.bitcast(U32), wg_v, 8), cp(wu_hbm.bitcast(U32), wu_v, 8),
              cp(wd_hbm.bitcast(U32), wd_v, 8)]

    def w_start(j, i0=0, i1=NB, prio=0):
        gg, t = j // 3, j % 3
        for i in range(i0, i1):
            for par in range(2):
                pltpu.make_async_copy(w_hbms[t].at[:, par, gg * NB + i, :],
                                      w_v.at[(gg * NB + i) * 6 + t * 2 + par],
                                      wsems.at[2 * j + (i >= PRE_SPLIT)]).start(priority=prio)

    def mod_copy(j):
        return pltpu.make_async_copy(wmod32.at[:, j * D:(j + 1) * D], wmod_v.at[j],
                                     wsems.at[2 * j + 1])

    def mult(v, m):
        return v if isinstance(v, int) else pl.multiple_of(v, m)

    def moda_copies(kc):
        col = mult(kc * 128, 128)
        return [pltpu.make_async_copy(wmod32.at[:, pl.ds(v * D + col, 128)],
                                      wmod_v.at[v, :, pl.ds(col, 128)], ksems.at[8 + kc])
                for v in range(2)]

    def chunk_copies(kc):
        r0 = mult(kc * 64, 64)
        return [pltpu.make_async_copy(w_hbms[0].at[pl.ds(r0, 64), par, i, :],
                                      w_v.at[i * 6 + par, pl.ds(r0, 64), :], ksems.at[kc])
                for i in range(NB) for par in range(2)]

    cp_c.start()
    cp_mem.start()
    cp_wr.start()
    for c_ in (cp_x0 + moda_copies(0) + moda_copies(1) + chunk_copies(0) + moda_copies(2)
               + chunk_copies(1) + [cp_xr] + chunk_copies(2)):
        c_.start()

    def ln1_rows(src_row, dst_row):
        xv = xbuf[pl.ds(src_row, 8), :].astype(F32)
        hv = _rb(_layernorm(xv) * modb[1]) + modb[0]
        act[pl.ds(dst_row, 8), :] = hv.astype(BF)

    lane256 = lax.broadcasted_iota(jnp.int32, (8, 256), 1)

    def finish_rows(row, attn):
        xv = xbuf[pl.ds(row, 8), :].astype(F32)
        x1 = _rb(xv + _rb(modb[2] * _rb(attn)))
        act[pl.ds(row, 8), :] = x1.astype(BF)
        h2 = _rb(_rb(_layernorm(x1) * modb[4]) + modb[3])
        act[pl.ds(OOFF + row, 8), :] = (x1 + _rb(modb[5] * h2)).astype(BF)
        r = jnp.sum(h2 * modb[6], axis=-1, keepdims=True)
        act[ROFF:ROFF + 8, 0:256] = jnp.where(
            lane256 * 8 == row, r, act[ROFF:ROFF + 8, 0:256].astype(F32)).astype(BF)

    def attn_store(a, k0):
        for j in range(a.shape[0] // 8):
            for k in range(a.shape[1] // 128):
                qkvbufs[A_BUF[j]][NSLOT, (k0 + k) * 8:(k0 + k + 1) * 8, :] = pltpu.bitcast(
                    a[8 * j:8 * j + 8, k * 128:(k + 1) * 128], U32)

    def attn_load(j):
        return pltpu.bitcast(jnp.concatenate(
            [qkvbufs[A_BUF[j]][NSLOT, k * 8:(k + 1) * 8, :] for k in range(8)], axis=1), F32)

    act[ROFF:ROFF + 8, 0:256] = jnp.zeros((8, 256), BF)
    attn_store(jnp.zeros((NEW, D), F32), 0)
    for s_ in range(NSEG):
        for k, v in enumerate(_step_indices(s_)):
            tab[s_ * NTAB + k] = v
    ri = lax.broadcasted_iota(jnp.int32, (80, 80), 0)
    ci = lax.broadcasted_iota(jnp.int32, (80, 80), 1)

    def head_pos(i):
        hd = jnp.where(i < 16, i // 8, (i - 16) // 32)
        pos = jnp.where(i < 16, i % 8, 8 + (i - 16) % 32)
        return hd, pos
    rh, rp = head_pos(ri)
    ch, cpos = head_pos(ci)
    same = rh == ch
    valid = same & ((rp < M) | (rp >= cpos))
    fill = jnp.where(same, -1e9, -jnp.inf).astype(F32)

    cp_mem.wait()
    cp_wr.wait()
    modb[6] = jnp.broadcast_to(wrbuf[...].astype(F32).reshape(1, D), (8, D))
    cp_c.wait()
    cv = cbuf[...].astype(F32)
    sc16 = jnp.broadcast_to(_rb(cv * _rb(jax.nn.sigmoid(cv))), (16, D)).astype(BF)

    def ln_pre(g, carry):
        pltpu.make_async_copy(x_hbm.at[0, 0:128], xbuf.at[pl.ds(pl.multiple_of(g * 128, 128), 128)],
                              sems.at[13 + g]).wait()
        for u in range(2):
            row = pl.multiple_of(g * 128 + u * 64, 64)
            nv = _layernorm(xbuf[pl.ds(row, 64), :].astype(F32)).astype(BF)
            for k in range(8):
                h0buf[k, pl.ds(pl.multiple_of(row // 2, 32), 32), :] = pltpu.bitcast(
                    nv[:, k * 128:(k + 1) * 128], U32)
            wg_v[pl.ds(row, 64), 0:2 * D] = jnp.zeros((64, 2 * D), U32)
        return carry
    lax.fori_loop(0, PRE // 128, ln_pre, 0)

    def mod_tile(v, col):
        w = pltpu.bitcast(wmod_v[v, :, pl.ds(col, 128)], BF)
        return _rb(jnp.dot(sc16, w, preferred_element_type=F32))[0:8]

    def moda_store(kc, sa, ca):
        col = mult(kc * 128, 128)
        c1 = _rb(1.0 + ca)
        modb[0, :, pl.ds(col, 128)] = sa
        modb[1, :, pl.ds(col, 128)] = c1
        return sa, c1

    def moda_apply(kc, sa, c1, r0, r1):
        for r in range(r0, r1, 16):
            nv = pltpu.bitcast(h0buf[kc, r // 2:r // 2 + 8, :], BF).astype(F32).reshape(2, 8, 128)
            hv = (_rb(nv * c1[None]) + sa[None]).reshape(16, 128).astype(BF)
            h0buf[kc, r // 2:r // 2 + 8, :] = pltpu.bitcast(hv, U32)

    def repack(a, b):
        return (a & U32(0xFFFF)) | (b << 16), (a >> 16) | (b & U32(0xFFFF0000))

    def store_qkv(i, jrow, y, seg0):
        for sg in range(y.shape[0] // 32):
            for hh in range(2):
                qkvbufs[i][seg0 + sg, pl.ds(jrow + 8 + hh * 16, 16), :] = _pack(
                    y[sg * 32:(sg + 1) * 32, hh * 128:(hh + 1) * 128])

    for c_ in moda_copies(0):
        c_.wait()
    moda_apply(0, *moda_store(0, mod_tile(0, 0), mod_tile(1, 0)), 0, PRE)

    def w_wait(j, i0, i1):
        blk0 = (j // 3) * (6 * NB) + (j % 3) * 2
        for i in range(i0, i1):
            for par in range(2):
                pltpu.make_async_copy(w_hbms[0].at[:, 0, 0, :], w_v.at[blk0 + i * 6 + par],
                                      wsems.at[2 * j + (i >= PRE_SPLIT)]).wait()

    def chunk_block(kc, last, issue):
        for c_ in chunk_copies(kc) + ([cp_xr] if last else moda_copies(kc + 1)):
            c_.wait()
        issue()
        r0 = mult(kc * 64, 64)
        mv = []
        for i in range(NB):
            lo, hi = repack(w_v[i * 6, pl.ds(r0, 64), :], w_v[i * 6 + 1, pl.ds(r0, 64), :])
            w_v[i * 6, pl.ds(r0, 64), :] = lo
            w_v[i * 6 + 1, pl.ds(r0, 64), :] = hi
            w = pltpu.bitcast(jnp.concatenate([lo, hi], axis=1), BF)
            y = (pltpu.bitcast(wg_v[0:PRE, i * 256:(i + 1) * 256], F32)
                 + jnp.dot(pltpu.bitcast(h0buf[kc], BF), w, preferred_element_type=F32))
            if last:
                store_qkv(i, 0, y, 0)
            else:
                wg_v[0:PRE, i * 256:(i + 1) * 256] = pltpu.bitcast(y, U32)
                if i in (1, 3):
                    mv.append(mod_tile(i // 2, mult((kc + 1) * 128, 128)))
                if i == 3:
                    mv = moda_store(kc + 1, mv[0], mv[1])
                if i >= 4:
                    moda_apply(kc + 1, mv[0], mv[1], (i - 4) * 128, (i - 3) * 128)
        if last:
            for j in range(3):
                ln1_rows(PRE + 8 * j, HOFF + 8 + 8 * j)

    def chunk_body(kc, carry):
        def issue():
            @pl.when(kc < 5)
            def _():
                for c_ in moda_copies(kc + 3) + chunk_copies(kc + 3):
                    c_.start()
        chunk_block(kc, False, issue)
        return carry

    def issue_last():
        w_wait(1, 0, PRE_SPLIT)
        w_start(1, PRE_SPLIT, NB)
        w_start(2)
        mod_copy(2).start()
    w_start(1, 0, PRE_SPLIT, prio=1)
    lax.fori_loop(0, 7, chunk_body, 0)
    chunk_block(7, True, issue_last)

    def pre_unit(j, i, extra):
        blk = (j // 3) * (6 * NB) + (j % 3) * 2 + i * 6
        jrow = mult(j * 40, 8)
        lo, hi = repack(w_v[blk], w_v[blk + 1])
        w_v[blk] = lo
        w_v[blk + 1] = hi
        for rc in range(PRE // 128):
            if rc > 0:
                lo = w_v[blk]
                hi = w_v[blk + 1]
            w = pltpu.bitcast(jnp.concatenate([lo, hi], axis=1), BF)
            lhs = jnp.concatenate([h0buf[k, rc * 64:(rc + 1) * 64, :] for k in range(8)], axis=1)
            y = jnp.dot(pltpu.bitcast(lhs, BF), w, preferred_element_type=F32)
            store_qkv(i, jrow, y, rc * 4)
            extra(rc)

    for i in range(NB):
        if i == PRE_SPLIT:
            w_wait(1, PRE_SPLIT, NB)
            for jn in (3, 4):
                w_start(jn)
                mod_copy(jn).start()
        pre_unit(1, i, lambda rc: None)
    w_start(5)
    mod_copy(5).start()
    cp_wo.start()
    cp_x1.start()

    def pre_body(j, carry):
        w_wait(j, 0, NB)
        pltpu.make_async_copy(wmod32.at[:, 0:D], wmod_v.at[j], wsems.at[2 * j + 1]).wait()
        one = jnp.where(j == 4, 1.0, 0.0).astype(F32)
        for i in range(NB):
            def extra(rc, i=i):
                if rc == 1:
                    modb[j, :, i * 128:(i + 1) * 128] = _rb(one + mod_tile(j, i * 128))
            pre_unit(j, i, extra)
        return carry
    lax.fori_loop(2, 6, pre_body, 0)

    cp_wo.wait()
    cp_x1.wait()
    for c_ in cp_ffn:
        c_.start()

    def wo_w(q0, q1, n0, n1):
        h0, h1 = q0 + 2 * ROT, q1 + 2 * ROT
        ws = [wo_v[a:b, :, n0 * 128:n1 * 128].reshape((b - a) * (DH // 2), (n1 - n0) * 128)
              for a, b in ((h0, min(h1, H)), (0, h1 - H)) if b > a]
        return pltpu.bitcast(jnp.concatenate(ws, axis=0), BF)

    HD = D // 2

    def emit_step(it, odd, pend):
        s = 2 * it + odd
        hrow = pl.multiple_of(HOFF + (s & 1) * 32, 32)
        hnext = pl.multiple_of(HOFF + 32 - (s & 1) * 32, 32)
        tv = [tab[s * NTAB + k] for k in range(7)]
        slot = tv[0]
        dsts = [(tv[1 + 2 * j], pl.multiple_of(tv[2 + 2 * j], 4)) for j in range(3)]
        orow, ow = (32, 48) if odd else (0, 32)
        odst = (48, 56, 64, 72) if odd else (8, 16, 24, 40)
        erow = it * 64 if odd else jnp.maximum(it - 1, 0) * 64 + RIDE
        lrow = PRE + jnp.minimum(s + 1, NSEG - 1) * RIDE
        e_at, l_at = (E_AT2, L_AT2) if odd else (E_AT, L_AT)
        probs = {}

        def wqkv(p, k0, k1):
            return pltpu.bitcast(jnp.concatenate(
                [w_v[p * 6 + u, k0 // 2:k1 // 2, :] for u in range(6)], axis=1), BF)

        lhs_lo = act[pl.ds(hrow, 32), 0:HD]
        if pend is not None:
            ybuf[...] = jnp.dot(lhs_lo, wqkv(0, 0, HD), preferred_element_type=F32)
            pend()
        lhs_hi = act[pl.ds(hrow, 32), HD:D]
        if pend is not None:
            y0 = ybuf[...] + jnp.dot(lhs_hi, wqkv(0, HD, D), preferred_element_type=F32)
        lhs_rest = jnp.concatenate([lhs_lo[:, 128:], lhs_hi], axis=1)
        lhs = [jnp.concatenate([lhs_lo, lhs_hi], axis=1)]

        def side(p):
            for j in range(len(e_at)):
                if e_at[j] == p:
                    finish_rows(pl.multiple_of(erow + 8 * j, 8), attn_load(j))
            for j in range(3):
                if l_at[j] == p:
                    ln1_rows(pl.multiple_of(lrow + 8 * j, 8),
                             pl.multiple_of(hnext + 8 + 8 * j, 8))
            if p in e_at or p in l_at:
                lhs[0] = jnp.concatenate([act[pl.ds(hrow, 32), 0:128], lhs_rest], axis=1)

        def qkv(p):
            if p == 0 and pend is not None:
                y = y0
            else:
                y = jnp.dot(lhs[0], wqkv(p, 0, D), preferred_element_type=F32)
            buf = qkvbufs[p % NB]
            for u in range(6):
                t, hh = u // 2, u % 2
                b0 = ((p // NB) * 3 + t) * 40
                yu = y[:, u * 128:(u + 1) * 128]
                buf[slot, b0 + hh * 4:b0 + hh * 4 + 4, :] = _pack(yu[0:8])
                for j in range(3):
                    sl, off = dsts[j]
                    buf[sl, pl.ds(b0 + 8 + hh * 16 + off, 4), :] = _pack(yu[8 + 8 * j:16 + 8 * j])

        def ld(p, t):
            b0 = ((p // NB) * 3 + t) * 40
            return pltpu.bitcast(qkvbufs[p % NB][slot, b0:b0 + 40, :], BF)

        def sc(p):
            s2 = lax.dot_general(ld(p, 0), ld(p, 1), (((1,), (1,)), ((), ())),
                                 preferred_element_type=F32)
            s2 = jnp.where(valid, s2 * SCALE, fill)
            m = jnp.max(s2, axis=-1, keepdims=True)
            e = jnp.exp(s2 - m)
            l = jnp.sum(e, axis=-1, keepdims=True)
            rl = pl.reciprocal(l, approx=True)
            rl = rl * (2.0 - l * rl)
            probs[p] = (e * rl).astype(BF)

        def pv(p):
            o2 = jnp.dot(probs[p], ld(p, 2), preferred_element_type=F32)
            for hh in range(2):
                hcol = (2 * ((p - ROT) % NP) + hh) * 128
                obuf[orow:orow + 8, hcol:hcol + 128] = o2[8 * hh:8 * hh + 8].astype(BF)
                for j in range(4):
                    r0 = 16 + 32 * hh + 8 * j
                    obuf[odst[j]:odst[j] + 8, hcol:hcol + 128] = o2[r0:r0 + 8].astype(BF)

        def attn(pos):
            for kind, p in ATT.get(pos, ()):
                (sc if kind == 's' else pv)(p)

        for p in range(NP):
            qkv(p)
            side(p)
            attn(p)
        a1 = []
        for n in range(8):
            a1.append(jnp.dot(obuf[orow:orow + ow, 0:KS], wo_w(0, KS // DH, n, n + 1),
                              preferred_element_type=F32))
            if n + 1 in W1AT:
                attn(NP + 2 * W1AT.index(n + 1))
        o2lhs = obuf[orow:orow + ow, KS:]
        a_lo = jnp.concatenate(a1[0:4], axis=1) + jnp.dot(
            o2lhs, wo_w(KS // DH, H, 0, 4), preferred_element_type=F32)
        act[pl.ds(hnext, 8), 0:HD] = a_lo[0:8].astype(BF)
        attn_store(a_lo[8:], 0)
        a_hi = jnp.concatenate(a1[4:8], axis=1) + jnp.dot(
            o2lhs, wo_w(KS // DH, H, 4, 8), preferred_element_type=F32)

        def finish():
            act[pl.ds(hnext, 8), HD:D] = a_hi[0:8].astype(BF)
            attn_store(a_hi[8:], 4)
        return finish

    def out_copy(r0, n, sem):
        return cp(act.at[pl.ds(OOFF + r0, n)], out_hbm.at[0, pl.ds(r0, n)], sem)

    def steps(it, carry):
        emit_step(it, 1, emit_step(it, 0, None))()

        @pl.when(it > 0)
        def _():
            out_copy(pl.multiple_of((it - 1) * 64, 64), 64, 9).start()
        return carry
    lax.fori_loop(0, NSEG // 2, steps, 0)

    NEW0 = S - NEW
    out_copy(S - 64, NEW0 - (S - 64), 9).start()
    for c_ in cp_ffn:
        c_.wait()

    rowsf = (lane256 * 8 + lax.broadcasted_iota(jnp.int32, (8, 256), 0)).astype(F32)
    r_old = jnp.where(rowsf < NEW0, act[ROFF:ROFF + 8, 0:256].astype(F32), -jnp.inf)

    def allmax(v):
        return jnp.max(jnp.max(v, axis=1, keepdims=True), axis=0, keepdims=True)

    def allmin(v):
        return jnp.min(jnp.min(v, axis=1, keepdims=True), axis=0, keepdims=True)
    m1 = allmax(r_old)
    i1v = allmin(jnp.where(r_old == m1, rowsf, float(S)))
    r_rest = jnp.where(rowsf == i1v, -jnp.inf, r_old)
    m2 = allmax(r_rest)
    i2v = allmin(jnp.where((r_rest == m2) & (rowsf != i1v), rowsf, float(S)))
    i1 = jnp.clip(i1v[0, 0].astype(jnp.int32), 0, NEW0 - 1)
    i2 = jnp.clip(i2v[0, 0].astype(jnp.int32), 0, NEW0 - 1)
    b1 = pl.multiple_of((i1 // 8) * 8, 8)
    b2 = pl.multiple_of((i2 // 8) * 8, 8)

    def rep(i, n):
        return jnp.concatenate([modb[i]] * n, axis=0)
    ng = NEW // 8
    x1n = _rb(xbuf[NEW0:S, :].astype(F32) + _rb(rep(2, ng) * _rb(
        jnp.concatenate([attn_load(j) for j in range(ng)], axis=0))))
    h2n = _rb(_rb(_layernorm(x1n) * rep(4, ng)) + rep(3, ng))
    rn = _rb(jnp.sum(h2n * rep(6, ng), axis=-1, keepdims=True))
    x1c = jnp.concatenate([act[pl.ds(b1, 8), :].astype(F32), act[pl.ds(b2, 8), :].astype(F32)],
                          axis=0)
    h2c = _rb(_rb(_layernorm(x1c) * rep(4, 2)) + rep(3, 2))
    x1a = jnp.concatenate([x1c, x1n], axis=0)
    h2a = jnp.concatenate([h2c, h2n], axis=0)
    sub8 = lax.broadcasted_iota(jnp.int32, (8, 1), 0)
    val = jnp.concatenate([jnp.where(sub8 == i1 - b1, m1, -jnp.inf),
                           jnp.where(sub8 == i2 - b2, m2, -jnp.inf), rn], axis=0)
    live = jnp.concatenate([(sub8 == i1 - b1).astype(F32), (sub8 == i2 - b2).astype(F32),
                            jnp.ones((NEW, 1), F32)], axis=0) > 0.5
    pos = lax.broadcasted_iota(jnp.int32, (16 + NEW, 1), 0).astype(F32)
    v1 = jnp.max(val, axis=0, keepdims=True)
    p1 = jnp.min(jnp.where((val == v1) & live, pos, float(S)), axis=0, keepdims=True)
    val2 = jnp.where(pos == p1, -jnp.inf, val)
    v2 = jnp.max(val2, axis=0, keepdims=True)
    p2 = jnp.min(jnp.where((val2 == v2) & live & (pos != p1), pos, float(S)),
                 axis=0, keepdims=True)
    row1 = jnp.sum(jnp.where(pos == p1, h2a, 0.0), axis=0, keepdims=True)
    row2 = jnp.sum(jnp.where(pos == p2, h2a, 0.0), axis=0, keepdims=True)
    sub16 = lax.broadcasted_iota(jnp.int32, (16, 1), 0)
    h2b = jnp.where(sub16 == 0, row1, jnp.where(sub16 == 1, row2, 0.0)).astype(BF)
    hid = []
    for n in range(0, F, FFN_NB):
        gt = _rb(jnp.dot(h2b, pltpu.bitcast(wg_v[:, n:n + FFN_NB], BF), preferred_element_type=F32))
        up = _rb(jnp.dot(h2b, pltpu.bitcast(wu_v[:, n:n + FFN_NB], BF), preferred_element_type=F32))
        hid.append((_rb(gt * _rb(jax.nn.sigmoid(gt))) * up).astype(BF))
    y = _rb(jnp.dot(jnp.concatenate(hid, axis=1), pltpu.bitcast(wd_v[...], BF),
                    preferred_element_type=F32))
    y1 = _rb(y[0:1] * _rb(jax.nn.sigmoid(v1)))
    y2 = _rb(y[1:2] * _rb(jax.nn.sigmoid(v2)))
    tok = jnp.concatenate([(b1 + sub8).astype(F32), (b2 + sub8).astype(F32),
                           pos[16:] + float(NEW0 - 16)], axis=0)
    t1 = jnp.sum(jnp.where(pos == p1, tok, 0.0), axis=0, keepdims=True)
    t2 = jnp.sum(jnp.where(pos == p2, tok, 0.0), axis=0, keepdims=True)
    upd = jnp.where(tok == t1, y1, jnp.where(tok == t2, y2, 0.0))
    res = (x1a + _rb(rep(5, ng + 2) * _rb(h2a + upd))).astype(BF)
    act[OOFF + NEW0:OOFF + S, :] = res[16:]
    out_copy(0, NEW0, 9).wait()
    act[pl.ds(OOFF + b1, 8), :] = res[0:8]
    act[pl.ds(OOFF + b2, 8), :] = res[8:16]
    fix0 = out_copy(NEW0, NEW, 6)
    fix1 = out_copy(b1, 8, 11)
    fix2 = out_copy(b2, 8, 12)
    fix0.start()
    fix1.start()

    @pl.when(b1 != b2)
    def _():
        fix2.start()
        fix2.wait()
    fix0.wait()
    fix1.wait()


@jax.jit
def pallas_adaLN_cond__memory_aug_recurrent_mem_tr__moe_arch_mod__prompt_kernel(
    A_x: jax.Array,
    A_mem0: jax.Array,
    A_Wq: jax.Array,
    A_Wk: jax.Array,
    A_Wv: jax.Array,
    A_Wo: jax.Array,
    A_seg_len,
    B_x: jax.Array,
    B_w_r: jax.Array,
    B_w_gate: jax.Array,
    B_w_up: jax.Array,
    B_w_down: jax.Array,
    c: jax.Array,
    w_mod: jax.Array,
):
    del B_x
    del A_seg_len
    assert A_x.shape == (1, S, D) and A_Wq.shape == (D, H, DH) and A_mem0.shape == (1, M, D)
    any_spec = pl.BlockSpec(memory_space=pl.ANY)
    scratch = [
        pltpu.VMEM((S, D), BF),
        pltpu.VMEM((ACT_ROWS, D), BF),
        pltpu.VMEM((8, PRE // 2, 128), U32),
        pltpu.VMEM((32, 768), F32),
        pltpu.SMEM((NSEG * NTAB,), jnp.int32),
        pltpu.VMEM((7, 8, D), F32),
        pltpu.VMEM((3 * H, D // 2, 128), U32),
        pltpu.VMEM((H, DH // 2, D), U32),
        pltpu.VMEM((6, D // 2, D), U32),
        pltpu.VMEM((D // 2, F), U32),
        pltpu.VMEM((D // 2, F), U32),
        pltpu.VMEM((F // 2, D), U32),
        pltpu.VMEM((80, H * DH), BF),
        pltpu.SemaphoreType.DMA((17,)),
        pltpu.SemaphoreType.DMA((12,)),
        pltpu.SemaphoreType.DMA((16,)),
    ] + [pltpu.VMEM((NSLOT + 1, 256, 128), U32) for _ in range(NB)] + [
        pltpu.VMEM((1, D), BF),
        pltpu.VMEM((D,), BF),
    ]
    wq, wk, wv = (w.reshape(D // 2, 2, H, DH) for w in (A_Wq, A_Wk, A_Wv))
    return pl.pallas_call(
        _kernel,
        out_shape=jax.ShapeDtypeStruct((1, S, D), BF),
        in_specs=[any_spec] * 12,
        out_specs=any_spec,
        scratch_shapes=scratch,
        compiler_params=pltpu.CompilerParams(vmem_limit_bytes=120 * 1024 * 1024,
                                             disable_bounds_checks=True,
                                             disable_semaphore_checks=True),
    )(A_x, A_mem0, wq, wk, wv, A_Wo, B_w_r, B_w_gate, B_w_up, B_w_down,
      c, w_mod)
```

```python
import jax
import jax.numpy as jnp
from jax import lax
import jax.experimental.pallas as pl
import jax.experimental.pallas.tpu as pltpu

BF = jnp.bfloat16
F32 = jnp.float32
U32 = jnp.uint32

S = 2048
D = 1024
H = 32
DH = 128
M = 8
SEG = 32
NSEG = S // SEG
F = 3584
NP = H // 2
EPS = 1e-5
SCALE = DH ** -0.5

RIDE = 24
PRE = S - NSEG * RIDE
NSLOT = 17
NB = 8
KS = 2048
OOFF = S
HOFF = 2 * S
ROFF = HOFF + 64
ACT_ROWS = ROFF + 16
PRE_SPLIT = 4
E_AT = (2, 3, 4, 5, 6)
E_AT2 = (3, 4, 5)
L_AT = (6, 7, 8)
L_AT2 = (6, 8, 10)
A_BUF = (7, 0, 1, 2, 3)
W1AT = (2, 6)
NEW = 40
FFN_NB = 512
NTAB = 8

ROT = 2
ATT = {4: [('s', i) for i in range(4)],
       18: [('p', (12 + ROT + i) % NP) for i in range(4)]}
for _p in range(4, NP, 2):
    ATT[_p + 2] = [('s', _p), ('s', _p + 1), ('p', _p - 4 + ROT), ('p', _p - 3 + ROT)]


def _step_indices(s):
    t = [s % NSLOT]
    for j in range(3):
        gi = PRE // 8 + 3 * s + j
        t += [(gi // 4) % NSLOT, (gi % 4) * 4]
    return t


def _rb(v):
    return v.astype(BF).astype(F32)


def _pack(v):
    return pltpu.bitcast(v.astype(BF), U32)


def _layernorm(x):
    mu = jnp.sum(x, axis=-1, keepdims=True) * (1.0 / D)
    xc = x - mu
    var = jnp.sum(xc * xc, axis=-1, keepdims=True) * (1.0 / D)
    sd = _rb(jnp.sqrt(_rb(_rb(var) + EPS)))
    return _rb(_rb(x - _rb(mu)) / sd)


def _kernel(x_hbm, mem0_hbm, wq_hbm, wk_hbm, wv_hbm, wo_hbm, wr_hbm, wg_hbm, wu_hbm,
            wd_hbm, c_hbm, wmod_hbm, out_hbm,
            xbuf, act, h0buf, ybuf, tab, modb,
            w_v, wo_v, wmod_v, wg_v, wu_v, wd_v,
            obuf, sems, wsems, ksems, *rest):
    qkvbufs, cbuf, wrbuf = rest[:NB], rest[NB], rest[NB + 1]
    w_hbms = tuple(w.bitcast(U32) for w in (wq_hbm, wk_hbm, wv_hbm))

    def cp(src, dst, i):
        return pltpu.make_async_copy(src, dst, sems.at[i])

    wmod32 = wmod_hbm.bitcast(U32)
    cp_c = cp(c_hbm, cbuf, 0)
    cp_mem = cp(mem0_hbm.at[0], act.at[HOFF:HOFF + M], 1)
    cp_wr = cp(wr_hbm, wrbuf, 2)
    cp_x0 = [cp(x_hbm.at[0, n * 128:(n + 1) * 128], xbuf.at[n * 128:(n + 1) * 128], 13 + n)
             for n in range(PRE // 128)]
    cp_xr = cp(x_hbm.at[0, PRE:PRE + 32], xbuf.at[PRE:PRE + 32], 5)
    cp_x1 = cp(x_hbm.at[0, PRE + 32:S], xbuf.at[PRE + 32:S], 4)
    cp_wo = cp(wo_hbm.bitcast(U32), wo_v, 7)
    cp_ffn = [cp(wg_hbm.bitcast(U32), wg_v, 8), cp(wu_hbm.bitcast(U32), wu_v, 8),
              cp(wd_hbm.bitcast(U32), wd_v, 8)]

    def w_start(j, i0=0, i1=NB, prio=0):
        gg, t = j // 3, j % 3
        r0 = 64 if j == 1 else 0
        for i in range(i0, i1):
            for par in range(2):
                pltpu.make_async_copy(w_hbms[t].at[r0:, par, gg * NB + i, :],
                                      w_v.at[(gg * NB + i) * 6 + t * 2 + par, r0:],
                                      wsems.at[2 * j + (i >= PRE_SPLIT)]).start(priority=prio)

    def mod_copy(j):
        return pltpu.make_async_copy(wmod32.at[:, j * D:(j + 1) * D], wmod_v.at[j],
                                     wsems.at[2 * j + 1])

    def mult(v, m):
        return v if isinstance(v, int) else pl.multiple_of(v, m)

    def moda_copies(kc):
        col = mult(kc * 128, 128)
        return [pltpu.make_async_copy(wmod32.at[:, pl.ds(v * D + col, 128)],
                                      wmod_v.at[v, :, pl.ds(col, 128)], ksems.at[8 + kc])
                for v in range(2)]

    def chunk_copies(kc):
        r0 = mult(kc * 64, 64)
        return [pltpu.make_async_copy(w_hbms[0].at[pl.ds(r0, 64), par, i, :],
                                      w_v.at[i * 6 + par, pl.ds(r0, 64), :], ksems.at[kc])
                for i in range(NB) for par in range(2)]

    cp_early = [cp(w_hbms[1].at[0:64, par, i, :], w_v.at[i * 6 + 2 + par, 0:64], 3)
                for i in range(NB) for par in range(2)]

    cp_c.start()
    cp_mem.start()
    cp_wr.start()
    for c_ in (cp_x0 + moda_copies(0) + cp_early + moda_copies(1) + chunk_copies(0)
               + moda_copies(2) + chunk_copies(1) + [cp_xr]):
        c_.start()

    def ln1_rows(src_row, dst_row):
        xv = xbuf[pl.ds(src_row, 8), :].astype(F32)
        hv = _rb(_layernorm(xv) * modb[1]) + modb[0]
        act[pl.ds(dst_row, 8), :] = hv.astype(BF)

    lane256 = lax.broadcasted_iota(jnp.int32, (8, 256), 1)

    def finish_rows(row, attn):
        xv = xbuf[pl.ds(row, 8), :].astype(F32)
        x1 = _rb(xv + _rb(modb[2] * _rb(attn)))
        act[pl.ds(row, 8), :] = x1.astype(BF)
        h2 = _rb(_rb(_layernorm(x1) * modb[4]) + modb[3])
        act[pl.ds(OOFF + row, 8), :] = (x1 + _rb(modb[5] * h2)).astype(BF)
        r = jnp.sum(h2 * modb[6], axis=-1, keepdims=True)
        act[ROFF:ROFF + 8, 0:256] = jnp.where(
            lane256 * 8 == row, r, act[ROFF:ROFF + 8, 0:256].astype(F32)).astype(BF)

    def attn_store(a, k0):
        for j in range(a.shape[0] // 8):
            for k in range(a.shape[1] // 128):
                qkvbufs[A_BUF[j]][NSLOT, (k0 + k) * 8:(k0 + k + 1) * 8, :] = pltpu.bitcast(
                    a[8 * j:8 * j + 8, k * 128:(k + 1) * 128], U32)

    def attn_load(j):
        return pltpu.bitcast(jnp.concatenate(
            [qkvbufs[A_BUF[j]][NSLOT, k * 8:(k + 1) * 8, :] for k in range(8)], axis=1), F32)

    act[ROFF:ROFF + 8, 0:256] = jnp.zeros((8, 256), BF)
    attn_store(jnp.zeros((NEW, D), F32), 0)
    for s_ in range(NSEG):
        for k, v in enumerate(_step_indices(s_)):
            tab[s_ * NTAB + k] = v
    ri = lax.broadcasted_iota(jnp.int32, (80, 80), 0)
    ci = lax.broadcasted_iota(jnp.int32, (80, 80), 1)

    def head_pos(i):
        hd = jnp.where(i < 16, i // 8, (i - 16) // 32)
        pos = jnp.where(i < 16, i % 8, 8 + (i - 16) % 32)
        return hd, pos
    rh, rp = head_pos(ri)
    ch, cpos = head_pos(ci)
    same = rh == ch
    valid = same & ((rp < M) | (rp >= cpos))
    fill = jnp.where(same, -1e9, -jnp.inf).astype(F32)

    cp_mem.wait()
    cp_wr.wait()
    modb[6] = jnp.broadcast_to(wrbuf[...].astype(F32).reshape(1, D), (8, D))
    cp_c.wait()
    cv = cbuf[...].astype(F32)
    sc16 = jnp.broadcast_to(_rb(cv * _rb(jax.nn.sigmoid(cv))), (16, D)).astype(BF)

    def ln_pre(g, carry):
        pltpu.make_async_copy(x_hbm.at[0, 0:128], xbuf.at[pl.ds(pl.multiple_of(g * 128, 128), 128)],
                              sems.at[13 + g]).wait()
        for u in range(2):
            row = pl.multiple_of(g * 128 + u * 64, 64)
            nv = _layernorm(xbuf[pl.ds(row, 64), :].astype(F32)).astype(BF)
            for k in range(8):
                h0buf[k, pl.ds(pl.multiple_of(row // 2, 32), 32), :] = pltpu.bitcast(
                    nv[:, k * 128:(k + 1) * 128], U32)
            wg_v[pl.ds(row, 64), 0:2 * D] = jnp.zeros((64, 2 * D), U32)
        return carry
    lax.fori_loop(0, PRE // 128, ln_pre, 0)

    def mod_tile(v, col):
        w = pltpu.bitcast(wmod_v[v, :, pl.ds(col, 128)], BF)
        return _rb(jnp.dot(sc16, w, preferred_element_type=F32))[0:8]

    def moda_store(kc, sa, ca):
        col = mult(kc * 128, 128)
        c1 = _rb(1.0 + ca)
        modb[0, :, pl.ds(col, 128)] = sa
        modb[1, :, pl.ds(col, 128)] = c1
        return sa, c1

    def moda_apply(kc, sa, c1, r0, r1):
        for r in range(r0, r1, 16):
            nv = pltpu.bitcast(h0buf[kc, r // 2:r // 2 + 8, :], BF).astype(F32).reshape(2, 8, 128)
            hv = (_rb(nv * c1[None]) + sa[None]).reshape(16, 128).astype(BF)
            h0buf[kc, r // 2:r // 2 + 8, :] = pltpu.bitcast(hv, U32)

    def repack(a, b):
        return (a & U32(0xFFFF)) | (b << 16), (a >> 16) | (b & U32(0xFFFF0000))

    def store_qkv(i, jrow, y, seg0):
        for sg in range(y.shape[0] // 32):
            for hh in range(2):
                qkvbufs[i][seg0 + sg, pl.ds(jrow + 8 + hh * 16, 16), :] = _pack(
                    y[sg * 32:(sg + 1) * 32, hh * 128:(hh + 1) * 128])

    for c_ in chunk_copies(2):
        c_.start()
    for c_ in moda_copies(0):
        c_.wait()
    moda_apply(0, *moda_store(0, mod_tile(0, 0), mod_tile(1, 0)), 0, PRE)
    w_start(1, 0, PRE_SPLIT, prio=1)

    for c_ in cp_early:
        c_.wait()
    for i in range(NB):
        lo, hi = repack(w_v[i * 6 + 2, 0:64, :], w_v[i * 6 + 3, 0:64, :])
        w_v[i * 6 + 2, 0:64, :] = lo
        w_v[i * 6 + 3, 0:64, :] = hi
        wu_v[0:PRE, i * 256:(i + 1) * 256] = pltpu.bitcast(jnp.dot(
            pltpu.bitcast(h0buf[0], BF), pltpu.bitcast(jnp.concatenate([lo, hi], axis=1), BF),
            preferred_element_type=F32), U32)

    def w_wait(j, i0, i1, r0=0):
        blk0 = (j // 3) * (6 * NB) + (j % 3) * 2
        for i in range(i0, i1):
            for par in range(2):
                pltpu.make_async_copy(w_hbms[0].at[r0:, 0, 0, :], w_v.at[blk0 + i * 6 + par, r0:],
                                      wsems.at[2 * j + (i >= PRE_SPLIT)]).wait()

    def chunk_block(kc, last, issue):
        for c_ in chunk_copies(kc) + ([cp_xr] if last else moda_copies(kc + 1)):
            c_.wait()
        issue()
        r0 = mult(kc * 64, 64)
        mv = []
        for i in range(NB):
            lo, hi = repack(w_v[i * 6, pl.ds(r0, 64), :], w_v[i * 6 + 1, pl.ds(r0, 64), :])
            w_v[i * 6, pl.ds(r0, 64), :] = lo
            w_v[i * 6 + 1, pl.ds(r0, 64), :] = hi
            w = pltpu.bitcast(jnp.concatenate([lo, hi], axis=1), BF)
            y = (pltpu.bitcast(wg_v[0:PRE, i * 256:(i + 1) * 256], F32)
                 + jnp.dot(pltpu.bitcast(h0buf[kc], BF), w, preferred_element_type=F32))
            if last:
                store_qkv(i, 0, y, 0)
            else:
                wg_v[0:PRE, i * 256:(i + 1) * 256] = pltpu.bitcast(y, U32)
                if i in (1, 3):
                    mv.append(mod_tile(i // 2, mult((kc + 1) * 128, 128)))
                if i == 3:
                    mv = moda_store(kc + 1, mv[0], mv[1])
                if i >= 4:
                    moda_apply(kc + 1, mv[0], mv[1], (i - 4) * 128, (i - 3) * 128)
        if last:
            for j in range(3):
                ln1_rows(PRE + 8 * j, HOFF + 8 + 8 * j)

    def chunk_body(kc, carry):
        def issue():
            @pl.when(kc < 5)
            def _():
                for c_ in moda_copies(kc + 3) + chunk_copies(kc + 3):
                    c_.start()
        chunk_block(kc, False, issue)
        return carry

    def issue_last():
        w_wait(1, 0, PRE_SPLIT, 64)
        w_start(1, PRE_SPLIT, NB)
        w_start(2)
        mod_copy(2).start()
    lax.fori_loop(0, 7, chunk_body, 0)
    chunk_block(7, True, issue_last)

    def pre_unit(j, i, extra, k0=0):
        blk = (j // 3) * (6 * NB) + (j % 3) * 2 + i * 6
        jrow = mult(j * 40, 8)
        r0 = k0 * 64
        lo, hi = repack(w_v[blk, r0:, :], w_v[blk + 1, r0:, :])
        w_v[blk, r0:, :] = lo
        w_v[blk + 1, r0:, :] = hi
        for rc in range(PRE // 128):
            if rc > 0:
                lo = w_v[blk, r0:, :]
                hi = w_v[blk + 1, r0:, :]
            w = pltpu.bitcast(jnp.concatenate([lo, hi], axis=1), BF)
            lhs = jnp.concatenate(
                [h0buf[k, rc * 64:(rc + 1) * 64, :] for k in range(k0, 8)], axis=1)
            y = jnp.dot(pltpu.bitcast(lhs, BF), w, preferred_element_type=F32)
            if k0:
                y = y + pltpu.bitcast(wu_v[rc * 128:(rc + 1) * 128, i * 256:(i + 1) * 256], F32)
            store_qkv(i, jrow, y, rc * 4)
            extra(rc)

    for i in range(NB):
        if i == PRE_SPLIT:
            w_wait(1, PRE_SPLIT, NB, 64)
            for jn in (3, 4):
                w_start(jn)
                mod_copy(jn).start()
        pre_unit(1, i, lambda rc: None, k0=1)
    w_start(5)
    mod_copy(5).start()
    cp_wo.start()
    cp_x1.start()

    def pre_body(j, carry):
        w_wait(j, 0, NB)
        pltpu.make_async_copy(wmod32.at[:, 0:D], wmod_v.at[j], wsems.at[2 * j + 1]).wait()
        one = jnp.where(j == 4, 1.0, 0.0).astype(F32)
        for i in range(NB):
            def extra(rc, i=i):
                if rc == 1:
                    modb[j, :, i * 128:(i + 1) * 128] = _rb(one + mod_tile(j, i * 128))
            pre_unit(j, i, extra)
        return carry
    lax.fori_loop(2, 6, pre_body, 0)

    cp_wo.wait()
    cp_x1.wait()
    for c_ in cp_ffn:
        c_.start()

    def wo_w(q0, q1, n0, n1):
        h0, h1 = q0 + 2 * ROT, q1 + 2 * ROT
        ws = [wo_v[a:b, :, n0 * 128:n1 * 128].reshape((b - a) * (DH // 2), (n1 - n0) * 128)
              for a, b in ((h0, min(h1, H)), (0, h1 - H)) if b > a]
        return pltpu.bitcast(jnp.concatenate(ws, axis=0), BF)

    HD = D // 2

    def emit_step(it, odd, pend):
        s = 2 * it + odd
        hrow = pl.multiple_of(HOFF + (s & 1) * 32, 32)
        hnext = pl.multiple_of(HOFF + 32 - (s & 1) * 32, 32)
        tv = [tab[s * NTAB + k] for k in range(7)]
        slot = tv[0]
        dsts = [(tv[1 + 2 * j], pl.multiple_of(tv[2 + 2 * j], 4)) for j in range(3)]
        orow, ow = (32, 48) if odd else (0, 32)
        odst = (48, 56, 64, 72) if odd else (8, 16, 24, 40)
        erow = it * 64 if odd else jnp.maximum(it - 1, 0) * 64 + RIDE
        lrow = PRE + jnp.minimum(s + 1, NSEG - 1) * RIDE
        e_at, l_at = (E_AT2, L_AT2) if odd else (E_AT, L_AT)
        probs = {}

        def wqkv(p, k0, k1):
            return pltpu.bitcast(jnp.concatenate(
                [w_v[p * 6 + u, k0 // 2:k1 // 2, :] for u in range(6)], axis=1), BF)

        lhs_lo = act[pl.ds(hrow, 32), 0:HD]
        if pend is not None:
            ybuf[...] = jnp.dot(lhs_lo, wqkv(0, 0, HD), preferred_element_type=F32)
            pend()
        lhs_hi = act[pl.ds(hrow, 32), HD:D]
        if pend is not None:
            y0 = ybuf[...] + jnp.dot(lhs_hi, wqkv(0, HD, D), preferred_element_type=F32)
        lhs_rest = jnp.concatenate([lhs_lo[:, 128:], lhs_hi], axis=1)
        lhs = [jnp.concatenate([lhs_lo, lhs_hi], axis=1)]

        def side(p):
            for j in range(len(e_at)):
                if e_at[j] == p:
                    finish_rows(pl.multiple_of(erow + 8 * j, 8), attn_load(j))
            for j in range(3):
                if l_at[j] == p:
                    ln1_rows(pl.multiple_of(lrow + 8 * j, 8),
                             pl.multiple_of(hnext + 8 + 8 * j, 8))
            if p in e_at or p in l_at:
                lhs[0] = jnp.concatenate([act[pl.ds(hrow, 32), 0:128], lhs_rest], axis=1)

        def qkv(p):
            if p == 0 and pend is not None:
                y = y0
            else:
                y = jnp.dot(lhs[0], wqkv(p, 0, D), preferred_element_type=F32)
            buf = qkvbufs[p % NB]
            for u in range(6):
                t, hh = u // 2, u % 2
                b0 = ((p // NB) * 3 + t) * 40
                yu = y[:, u * 128:(u + 1) * 128]
                buf[slot, b0 + hh * 4:b0 + hh * 4 + 4, :] = _pack(yu[0:8])
                for j in range(3):
                    sl, off = dsts[j]
                    buf[sl, pl.ds(b0 + 8 + hh * 16 + off, 4), :] = _pack(yu[8 + 8 * j:16 + 8 * j])

        def ld(p, t):
            b0 = ((p // NB) * 3 + t) * 40
            return pltpu.bitcast(qkvbufs[p % NB][slot, b0:b0 + 40, :], BF)

        def sc(p):
            s2 = lax.dot_general(ld(p, 0), ld(p, 1), (((1,), (1,)), ((), ())),
                                 preferred_element_type=F32)
            s2 = jnp.where(valid, s2 * SCALE, fill)
            m = jnp.max(s2, axis=-1, keepdims=True)
            e = jnp.exp(s2 - m)
            l = jnp.sum(e, axis=-1, keepdims=True)
            rl = pl.reciprocal(l, approx=True)
            rl = rl * (2.0 - l * rl)
            probs[p] = (e * rl).astype(BF)

        def pv(p):
            o2 = jnp.dot(probs[p], ld(p, 2), preferred_element_type=F32)
            for hh in range(2):
                hcol = (2 * ((p - ROT) % NP) + hh) * 128
                obuf[orow:orow + 8, hcol:hcol + 128] = o2[8 * hh:8 * hh + 8].astype(BF)
                for j in range(4):
                    r0 = 16 + 32 * hh + 8 * j
                    obuf[odst[j]:odst[j] + 8, hcol:hcol + 128] = o2[r0:r0 + 8].astype(BF)

        def attn(pos):
            for kind, p in ATT.get(pos, ()):
                (sc if kind == 's' else pv)(p)

        for p in range(NP):
            qkv(p)
            side(p)
            attn(p)
        a1 = []
        for n in range(8):
            a1.append(jnp.dot(obuf[orow:orow + ow, 0:KS], wo_w(0, KS // DH, n, n + 1),
                              preferred_element_type=F32))
            if n + 1 in W1AT:
                attn(NP + 2 * W1AT.index(n + 1))
        o2lhs = obuf[orow:orow + ow, KS:]
        a_lo = jnp.concatenate(a1[0:4], axis=1) + jnp.dot(
            o2lhs, wo_w(KS // DH, H, 0, 4), preferred_element_type=F32)
        act[pl.ds(hnext, 8), 0:HD] = a_lo[0:8].astype(BF)
        attn_store(a_lo[8:], 0)
        a_hi = jnp.concatenate(a1[4:8], axis=1) + jnp.dot(
            o2lhs, wo_w(KS // DH, H, 4, 8), preferred_element_type=F32)

        def finish():
            act[pl.ds(hnext, 8), HD:D] = a_hi[0:8].astype(BF)
            attn_store(a_hi[8:], 4)
        return finish

    def out_copy(r0, n, sem):
        return cp(act.at[pl.ds(OOFF + r0, n)], out_hbm.at[0, pl.ds(r0, n)], sem)

    def steps(it, carry):
        emit_step(it, 1, emit_step(it, 0, None))()

        @pl.when(it > 0)
        def _():
            out_copy(pl.multiple_of((it - 1) * 64, 64), 64, 9).start()
        return carry
    lax.fori_loop(0, NSEG // 2, steps, 0)

    NEW0 = S - NEW
    out_copy(S - 64, NEW0 - (S - 64), 9).start()
    for c_ in cp_ffn:
        c_.wait()

    rowsf = (lane256 * 8 + lax.broadcasted_iota(jnp.int32, (8, 256), 0)).astype(F32)
    r_old = jnp.where(rowsf < NEW0, act[ROFF:ROFF + 8, 0:256].astype(F32), -jnp.inf)

    def allmax(v):
        return jnp.max(jnp.max(v, axis=1, keepdims=True), axis=0, keepdims=True)

    def allmin(v):
        return jnp.min(jnp.min(v, axis=1, keepdims=True), axis=0, keepdims=True)
    m1 = allmax(r_old)
    i1v = allmin(jnp.where(r_old == m1, rowsf, float(S)))
    r_rest = jnp.where(rowsf == i1v, -jnp.inf, r_old)
    m2 = allmax(r_rest)
    i2v = allmin(jnp.where((r_rest == m2) & (rowsf != i1v), rowsf, float(S)))
    i1 = jnp.clip(i1v[0, 0].astype(jnp.int32), 0, NEW0 - 1)
    i2 = jnp.clip(i2v[0, 0].astype(jnp.int32), 0, NEW0 - 1)
    b1 = pl.multiple_of((i1 // 8) * 8, 8)
    b2 = pl.multiple_of((i2 // 8) * 8, 8)

    def rep(i, n):
        return jnp.concatenate([modb[i]] * n, axis=0)
    ng = NEW // 8
    x1n = _rb(xbuf[NEW0:S, :].astype(F32) + _rb(rep(2, ng) * _rb(
        jnp.concatenate([attn_load(j) for j in range(ng)], axis=0))))
    h2n = _rb(_rb(_layernorm(x1n) * rep(4, ng)) + rep(3, ng))
    rn = _rb(jnp.sum(h2n * rep(6, ng), axis=-1, keepdims=True))
    x1c = jnp.concatenate([act[pl.ds(b1, 8), :].astype(F32), act[pl.ds(b2, 8), :].astype(F32)],
                          axis=0)
    h2c = _rb(_rb(_layernorm(x1c) * rep(4, 2)) + rep(3, 2))
    x1a = jnp.concatenate([x1c, x1n], axis=0)
    h2a = jnp.concatenate([h2c, h2n], axis=0)
    sub8 = lax.broadcasted_iota(jnp.int32, (8, 1), 0)
    val = jnp.concatenate([jnp.where(sub8 == i1 - b1, m1, -jnp.inf),
                           jnp.where(sub8 == i2 - b2, m2, -jnp.inf), rn], axis=0)
    live = jnp.concatenate([(sub8 == i1 - b1).astype(F32), (sub8 == i2 - b2).astype(F32),
                            jnp.ones((NEW, 1), F32)], axis=0) > 0.5
    pos = lax.broadcasted_iota(jnp.int32, (16 + NEW, 1), 0).astype(F32)
    v1 = jnp.max(val, axis=0, keepdims=True)
    p1 = jnp.min(jnp.where((val == v1) & live, pos, float(S)), axis=0, keepdims=True)
    val2 = jnp.where(pos == p1, -jnp.inf, val)
    v2 = jnp.max(val2, axis=0, keepdims=True)
    p2 = jnp.min(jnp.where((val2 == v2) & live & (pos != p1), pos, float(S)),
                 axis=0, keepdims=True)
    row1 = jnp.sum(jnp.where(pos == p1, h2a, 0.0), axis=0, keepdims=True)
    row2 = jnp.sum(jnp.where(pos == p2, h2a, 0.0), axis=0, keepdims=True)
    sub16 = lax.broadcasted_iota(jnp.int32, (16, 1), 0)
    h2b = jnp.where(sub16 == 0, row1, jnp.where(sub16 == 1, row2, 0.0)).astype(BF)
    hid = []
    for n in range(0, F, FFN_NB):
        gt = _rb(jnp.dot(h2b, pltpu.bitcast(wg_v[:, n:n + FFN_NB], BF), preferred_element_type=F32))
        up = _rb(jnp.dot(h2b, pltpu.bitcast(wu_v[:, n:n + FFN_NB], BF), preferred_element_type=F32))
        hid.append((_rb(gt * _rb(jax.nn.sigmoid(gt))) * up).astype(BF))
    y = _rb(jnp.dot(jnp.concatenate(hid, axis=1), pltpu.bitcast(wd_v[...], BF),
                    preferred_element_type=F32))
    y1 = _rb(y[0:1] * _rb(jax.nn.sigmoid(v1)))
    y2 = _rb(y[1:2] * _rb(jax.nn.sigmoid(v2)))
    tok = jnp.concatenate([(b1 + sub8).astype(F32), (b2 + sub8).astype(F32),
                           pos[16:] + float(NEW0 - 16)], axis=0)
    t1 = jnp.sum(jnp.where(pos == p1, tok, 0.0), axis=0, keepdims=True)
    t2 = jnp.sum(jnp.where(pos == p2, tok, 0.0), axis=0, keepdims=True)
    upd = jnp.where(tok == t1, y1, jnp.where(tok == t2, y2, 0.0))
    res = (x1a + _rb(rep(5, ng + 2) * _rb(h2a + upd))).astype(BF)
    act[OOFF + NEW0:OOFF + S, :] = res[16:]
    out_copy(0, NEW0, 9).wait()
    act[pl.ds(OOFF + b1, 8), :] = res[0:8]
    act[pl.ds(OOFF + b2, 8), :] = res[8:16]
    fix0 = out_copy(NEW0, NEW, 6)
    fix1 = out_copy(b1, 8, 11)
    fix2 = out_copy(b2, 8, 12)
    fix0.start()
    fix1.start()

    @pl.when(b1 != b2)
    def _():
        fix2.start()
        fix2.wait()
    fix0.wait()
    fix1.wait()


@jax.jit
def pallas_adaLN_cond__memory_aug_recurrent_mem_tr__moe_arch_mod__prompt_kernel(
    A_x: jax.Array,
    A_mem0: jax.Array,
    A_Wq: jax.Array,
    A_Wk: jax.Array,
    A_Wv: jax.Array,
    A_Wo: jax.Array,
    A_seg_len,
    B_x: jax.Array,
    B_w_r: jax.Array,
    B_w_gate: jax.Array,
    B_w_up: jax.Array,
    B_w_down: jax.Array,
    c: jax.Array,
    w_mod: jax.Array,
):
    del B_x
    del A_seg_len
    assert A_x.shape == (1, S, D) and A_Wq.shape == (D, H, DH) and A_mem0.shape == (1, M, D)
    any_spec = pl.BlockSpec(memory_space=pl.ANY)
    scratch = [
        pltpu.VMEM((S, D), BF),
        pltpu.VMEM((ACT_ROWS, D), BF),
        pltpu.VMEM((8, PRE // 2, 128), U32),
        pltpu.VMEM((32, 768), F32),
        pltpu.SMEM((NSEG * NTAB,), jnp.int32),
        pltpu.VMEM((7, 8, D), F32),
        pltpu.VMEM((3 * H, D // 2, 128), U32),
        pltpu.VMEM((H, DH // 2, D), U32),
        pltpu.VMEM((6, D // 2, D), U32),
        pltpu.VMEM((D // 2, F), U32),
        pltpu.VMEM((D // 2, F), U32),
        pltpu.VMEM((F // 2, D), U32),
        pltpu.VMEM((80, H * DH), BF),
        pltpu.SemaphoreType.DMA((17,)),
        pltpu.SemaphoreType.DMA((12,)),
        pltpu.SemaphoreType.DMA((16,)),
    ] + [pltpu.VMEM((NSLOT + 1, 256, 128), U32) for _ in range(NB)] + [
        pltpu.VMEM((1, D), BF),
        pltpu.VMEM((D,), BF),
    ]
    wq, wk, wv = (w.reshape(D // 2, 2, H, DH) for w in (A_Wq, A_Wk, A_Wv))
    return pl.pallas_call(
        _kernel,
        out_shape=jax.ShapeDtypeStruct((1, S, D), BF),
        in_specs=[any_spec] * 12,
        out_specs=any_spec,
        scratch_shapes=scratch,
        compiler_params=pltpu.CompilerParams(vmem_limit_bytes=120 * 1024 * 1024,
                                             disable_bounds_checks=True,
                                             disable_semaphore_checks=True),
    )(A_x, A_mem0, wq, wk, wv, A_Wo, B_w_r, B_w_gate, B_w_up, B_w_down,
      c, w_mod)
```

```python
import jax
import jax.numpy as jnp
from jax import lax
import jax.experimental.pallas as pl
import jax.experimental.pallas.tpu as pltpu

BF = jnp.bfloat16
F32 = jnp.float32
U32 = jnp.uint32

S = 2048
D = 1024
H = 32
DH = 128
M = 8
SEG = 32
NSEG = S // SEG
F = 3584
NP = H // 2
EPS = 1e-5
SCALE = DH ** -0.5

RIDE = 24
PRE = S - NSEG * RIDE
NSLOT = 17
NB = 8
KS = 2048
OOFF = S
HOFF = 2 * S
ROFF = HOFF + 64
ACT_ROWS = ROFF + 16
PRE_SPLIT = 4
E_AT = (2, 3, 4, 5, 6)
E_AT2 = (3, 4, 5)
L_AT = (6, 7, 8)
L_AT2 = (6, 8, 10)
A_BUF = (7, 0, 1, 2, 3)
W1AT = (2, 6)
NEW = 40
FFN_NB = 512
APPLY_N = 4
NTAB = 8

ROT = 2
ATT = {4: [('s', i) for i in range(4)],
       18: [('p', (12 + ROT + i) % NP) for i in range(4)]}
for _p in range(4, NP, 2):
    ATT[_p + 2] = [('s', _p), ('s', _p + 1), ('p', _p - 4 + ROT), ('p', _p - 3 + ROT)]


def _step_indices(s):
    t = [s % NSLOT]
    for j in range(3):
        gi = PRE // 8 + 3 * s + j
        t += [(gi // 4) % NSLOT, (gi % 4) * 4]
    return t


def _rb(v):
    return v.astype(BF).astype(F32)


def _pack(v):
    return pltpu.bitcast(v.astype(BF), U32)


def _layernorm(x):
    mu = jnp.sum(x, axis=-1, keepdims=True) * (1.0 / D)
    xc = x - mu
    var = jnp.sum(xc * xc, axis=-1, keepdims=True) * (1.0 / D)
    sd = _rb(jnp.sqrt(_rb(_rb(var) + EPS)))
    return _rb(_rb(x - _rb(mu)) / sd)


def _kernel(x_hbm, mem0_hbm, wq_hbm, wk_hbm, wv_hbm, wo_hbm, wr_hbm, wg_hbm, wu_hbm,
            wd_hbm, c_hbm, wmod_hbm, out_hbm,
            xbuf, act, h0buf, ybuf, tab, modb,
            w_v, wo_v, wmod_v, wg_v, wu_v, wd_v,
            obuf, sems, wsems, ksems, *rest):
    qkvbufs, cbuf, wrbuf = rest[:NB], rest[NB], rest[NB + 1]
    w_hbms = tuple(w.bitcast(U32) for w in (wq_hbm, wk_hbm, wv_hbm))

    def cp(src, dst, i):
        return pltpu.make_async_copy(src, dst, sems.at[i])

    wmod32 = wmod_hbm.bitcast(U32)
    cp_c = cp(c_hbm, cbuf, 0)
    cp_mem = cp(mem0_hbm.at[0], act.at[HOFF:HOFF + M], 1)
    cp_wr = cp(wr_hbm, wrbuf, 2)
    cp_x0 = [cp(x_hbm.at[0, n * 128:(n + 1) * 128], xbuf.at[n * 128:(n + 1) * 128], 13 + n)
             for n in range(PRE // 128)]
    cp_xr = cp(x_hbm.at[0, PRE:PRE + 32], xbuf.at[PRE:PRE + 32], 5)
    cp_x1 = cp(x_hbm.at[0, PRE + 32:S], xbuf.at[PRE + 32:S], 4)
    cp_wo = cp(wo_hbm.bitcast(U32), wo_v, 7)
    cp_ffn = [cp(wg_hbm.bitcast(U32), wg_v, 8), cp(wu_hbm.bitcast(U32), wu_v, 8),
              cp(wd_hbm.bitcast(U32), wd_v, 8)]

    def w_start(j, i0=0, i1=NB, prio=0):
        gg, t = j // 3, j % 3
        r0 = 64 if j == 1 else 0
        for i in range(i0, i1):
            for par in range(2):
                pltpu.make_async_copy(w_hbms[t].at[r0:, par, gg * NB + i, :],
                                      w_v.at[(gg * NB + i) * 6 + t * 2 + par, r0:],
                                      wsems.at[2 * j + (i >= PRE_SPLIT)]).start(priority=prio)

    def mod_copy(j):
        return pltpu.make_async_copy(wmod32.at[:, j * D:(j + 1) * D], wmod_v.at[j],
                                     wsems.at[2 * j + 1])

    def mult(v, m):
        return v if isinstance(v, int) else pl.multiple_of(v, m)

    def moda_copies(kc):
        col = mult(kc * 128, 128)
        return [pltpu.make_async_copy(wmod32.at[:, pl.ds(v * D + col, 128)],
                                      wmod_v.at[v, :, pl.ds(col, 128)], ksems.at[8 + kc])
                for v in range(2)]

    def chunk_copies(kc):
        r0 = mult(kc * 64, 64)
        return [pltpu.make_async_copy(w_hbms[0].at[pl.ds(r0, 64), par, i, :],
                                      w_v.at[i * 6 + par, pl.ds(r0, 64), :], ksems.at[kc])
                for i in range(NB) for par in range(2)]

    cp_early = [cp(w_hbms[1].at[0:64, par, i, :], w_v.at[i * 6 + 2 + par, 0:64], 3)
                for i in range(NB) for par in range(2)]

    cp_c.start()
    cp_mem.start()
    cp_wr.start()
    for c_ in (cp_x0 + moda_copies(0) + cp_early + moda_copies(1) + chunk_copies(0)
               + moda_copies(2) + chunk_copies(1) + [cp_xr]):
        c_.start()

    def ln1_rows(src_row, dst_row):
        xv = xbuf[pl.ds(src_row, 8), :].astype(F32)
        hv = _rb(_layernorm(xv) * modb[1]) + modb[0]
        act[pl.ds(dst_row, 8), :] = hv.astype(BF)

    lane256 = lax.broadcasted_iota(jnp.int32, (8, 256), 1)

    def finish_rows(row, attn):
        xv = xbuf[pl.ds(row, 8), :].astype(F32)
        x1 = _rb(xv + _rb(modb[2] * _rb(attn)))
        act[pl.ds(row, 8), :] = x1.astype(BF)
        h2 = _rb(_rb(_layernorm(x1) * modb[4]) + modb[3])
        act[pl.ds(OOFF + row, 8), :] = (x1 + _rb(modb[5] * h2)).astype(BF)
        r = jnp.sum(h2 * modb[6], axis=-1, keepdims=True)
        act[ROFF:ROFF + 8, 0:256] = jnp.where(
            lane256 * 8 == row, r, act[ROFF:ROFF + 8, 0:256].astype(F32)).astype(BF)

    def attn_store(a, k0):
        for j in range(a.shape[0] // 8):
            for k in range(a.shape[1] // 128):
                qkvbufs[A_BUF[j]][NSLOT, (k0 + k) * 8:(k0 + k + 1) * 8, :] = pltpu.bitcast(
                    a[8 * j:8 * j + 8, k * 128:(k + 1) * 128], U32)

    def attn_load(j):
        return pltpu.bitcast(jnp.concatenate(
            [qkvbufs[A_BUF[j]][NSLOT, k * 8:(k + 1) * 8, :] for k in range(8)], axis=1), F32)

    act[ROFF:ROFF + 8, 0:256] = jnp.zeros((8, 256), BF)
    attn_store(jnp.zeros((NEW, D), F32), 0)
    for s_ in range(NSEG):
        for k, v in enumerate(_step_indices(s_)):
            tab[s_ * NTAB + k] = v
    ri = lax.broadcasted_iota(jnp.int32, (80, 80), 0)
    ci = lax.broadcasted_iota(jnp.int32, (80, 80), 1)

    def head_pos(i):
        hd = jnp.where(i < 16, i // 8, (i - 16) // 32)
        pos = jnp.where(i < 16, i % 8, 8 + (i - 16) % 32)
        return hd, pos
    rh, rp = head_pos(ri)
    ch, cpos = head_pos(ci)
    same = rh == ch
    valid = same & ((rp < M) | (rp >= cpos))
    fill = jnp.where(same, -1e9, -jnp.inf).astype(F32)

    cp_mem.wait()
    cp_wr.wait()
    modb[6] = jnp.broadcast_to(wrbuf[...].astype(F32).reshape(1, D), (8, D))
    cp_c.wait()
    cv = cbuf[...].astype(F32)
    sc16 = jnp.broadcast_to(_rb(cv * _rb(jax.nn.sigmoid(cv))), (16, D)).astype(BF)

    def ln_pre(g, carry):
        pltpu.make_async_copy(x_hbm.at[0, 0:128], xbuf.at[pl.ds(pl.multiple_of(g * 128, 128), 128)],
                              sems.at[13 + g]).wait()
        for u in range(2):
            row = pl.multiple_of(g * 128 + u * 64, 64)
            nv = _layernorm(xbuf[pl.ds(row, 64), :].astype(F32)).astype(BF)
            for k in range(8):
                h0buf[k, pl.ds(pl.multiple_of(row // 2, 32), 32), :] = pltpu.bitcast(
                    nv[:, k * 128:(k + 1) * 128], U32)
            wg_v[pl.ds(row, 64), 0:2 * D] = jnp.zeros((64, 2 * D), U32)
        return carry
    lax.fori_loop(0, PRE // 128, ln_pre, 0)

    def mod_tile(v, col):
        w = pltpu.bitcast(wmod_v[v, :, pl.ds(col, 128)], BF)
        return _rb(jnp.dot(sc16, w, preferred_element_type=F32))[0:8]

    def moda_store(kc, sa, ca):
        col = mult(kc * 128, 128)
        c1 = _rb(1.0 + ca)
        modb[0, :, pl.ds(col, 128)] = sa
        modb[1, :, pl.ds(col, 128)] = c1
        return sa, c1

    def moda_apply(kc, sa, c1, r0, r1):
        for r in range(r0, r1, 16):
            nv = pltpu.bitcast(h0buf[kc, r // 2:r // 2 + 8, :], BF).astype(F32).reshape(2, 8, 128)
            hv = (_rb(nv * c1[None]) + sa[None]).reshape(16, 128).astype(BF)
            h0buf[kc, r // 2:r // 2 + 8, :] = pltpu.bitcast(hv, U32)

    def repack(a, b):
        return (a & U32(0xFFFF)) | (b << 16), (a >> 16) | (b & U32(0xFFFF0000))

    def store_qkv(i, jrow, y, seg0):
        for sg in range(y.shape[0] // 32):
            for hh in range(2):
                qkvbufs[i][seg0 + sg, pl.ds(jrow + 8 + hh * 16, 16), :] = _pack(
                    y[sg * 32:(sg + 1) * 32, hh * 128:(hh + 1) * 128])

    for c_ in chunk_copies(2):
        c_.start()
    for c_ in moda_copies(0):
        c_.wait()
    moda_apply(0, *moda_store(0, mod_tile(0, 0), mod_tile(1, 0)), 0, PRE)
    w_start(1, 0, PRE_SPLIT, prio=1)

    for c_ in cp_early:
        c_.wait()
    for i in range(NB):
        lo, hi = repack(w_v[i * 6 + 2, 0:64, :], w_v[i * 6 + 3, 0:64, :])
        w_v[i * 6 + 2, 0:64, :] = lo
        w_v[i * 6 + 3, 0:64, :] = hi
        wu_v[0:PRE, i * 256:(i + 1) * 256] = pltpu.bitcast(jnp.dot(
            pltpu.bitcast(h0buf[0], BF), pltpu.bitcast(jnp.concatenate([lo, hi], axis=1), BF),
            preferred_element_type=F32), U32)

    def w_wait(j, i0, i1, r0=0):
        blk0 = (j // 3) * (6 * NB) + (j % 3) * 2
        for i in range(i0, i1):
            for par in range(2):
                pltpu.make_async_copy(w_hbms[0].at[r0:, 0, 0, :], w_v.at[blk0 + i * 6 + par, r0:],
                                      wsems.at[2 * j + (i >= PRE_SPLIT)]).wait()

    def chunk_block(kc, last, issue):
        for c_ in chunk_copies(kc) + ([cp_xr] if last else moda_copies(kc + 1)):
            c_.wait()
        issue()
        r0 = mult(kc * 64, 64)
        mv = []
        for i in range(NB):
            lo, hi = repack(w_v[i * 6, pl.ds(r0, 64), :], w_v[i * 6 + 1, pl.ds(r0, 64), :])
            w_v[i * 6, pl.ds(r0, 64), :] = lo
            w_v[i * 6 + 1, pl.ds(r0, 64), :] = hi
            w = pltpu.bitcast(jnp.concatenate([lo, hi], axis=1), BF)
            y = (pltpu.bitcast(wg_v[0:PRE, i * 256:(i + 1) * 256], F32)
                 + jnp.dot(pltpu.bitcast(h0buf[kc], BF), w, preferred_element_type=F32))
            if last:
                store_qkv(i, 0, y, 0)
            else:
                wg_v[0:PRE, i * 256:(i + 1) * 256] = pltpu.bitcast(y, U32)
                if i in (1, 3):
                    mv.append(mod_tile(i // 2, mult((kc + 1) * 128, 128)))
                if i == 3:
                    mv = moda_store(kc + 1, mv[0], mv[1])
                if i in (4, 6):
                    zeros = qkvbufs[A_BUF[0]][NSLOT, 0:8, :]
                    for q in range(APPLY_N):
                        yr = (q + 1) * (PRE // (APPLY_N + 1)) // 8 * 8
                        tok = pltpu.bitcast(y[yr:yr + 8, 0:128], U32) & zeros
                        c1 = pltpu.bitcast(pltpu.bitcast(mv[1], U32) | tok, F32)
                        n = PRE // 2 // APPLY_N
                        r_ = (i - 4) // 2 * (PRE // 2) + q * n
                        moda_apply(kc + 1, mv[0], c1, r_, r_ + n)
        if last:
            for j in range(3):
                ln1_rows(PRE + 8 * j, HOFF + 8 + 8 * j)

    def chunk_body(kc, carry):
        def issue():
            @pl.when(kc < 5)
            def _():
                for c_ in moda_copies(kc + 3) + chunk_copies(kc + 3):
                    c_.start()
        chunk_block(kc, False, issue)
        return carry

    def issue_last():
        w_wait(1, 0, PRE_SPLIT, 64)
        w_start(1, PRE_SPLIT, NB)
        w_start(2)
        mod_copy(2).start()
    lax.fori_loop(0, 7, chunk_body, 0)
    chunk_block(7, True, issue_last)

    def pre_unit(j, i, extra, k0=0):
        blk = (j // 3) * (6 * NB) + (j % 3) * 2 + i * 6
        jrow = mult(j * 40, 8)
        r0 = k0 * 64
        lo, hi = repack(w_v[blk, r0:, :], w_v[blk + 1, r0:, :])
        w_v[blk, r0:, :] = lo
        w_v[blk + 1, r0:, :] = hi
        for rc in range(PRE // 128):
            if rc > 0:
                lo = w_v[blk, r0:, :]
                hi = w_v[blk + 1, r0:, :]
            w = pltpu.bitcast(jnp.concatenate([lo, hi], axis=1), BF)
            lhs = jnp.concatenate(
                [h0buf[k, rc * 64:(rc + 1) * 64, :] for k in range(k0, 8)], axis=1)
            y = jnp.dot(pltpu.bitcast(lhs, BF), w, preferred_element_type=F32)
            if k0:
                y = y + pltpu.bitcast(wu_v[rc * 128:(rc + 1) * 128, i * 256:(i + 1) * 256], F32)
            store_qkv(i, jrow, y, rc * 4)
            extra(rc)

    for i in range(NB):
        if i == PRE_SPLIT:
            w_wait(1, PRE_SPLIT, NB, 64)
            for jn in (3, 4):
                w_start(jn)
                mod_copy(jn).start()
        pre_unit(1, i, lambda rc: None, k0=1)
    w_start(5)
    mod_copy(5).start()
    cp_wo.start()
    cp_x1.start()

    def pre_body(j, carry):
        w_wait(j, 0, NB)
        pltpu.make_async_copy(wmod32.at[:, 0:D], wmod_v.at[j], wsems.at[2 * j + 1]).wait()
        one = jnp.where(j == 4, 1.0, 0.0).astype(F32)
        for i in range(NB):
            def extra(rc, i=i):
                if rc == 1:
                    modb[j, :, i * 128:(i + 1) * 128] = _rb(one + mod_tile(j, i * 128))
            pre_unit(j, i, extra)
        return carry
    lax.fori_loop(2, 6, pre_body, 0)

    cp_wo.wait()
    cp_x1.wait()
    for c_ in cp_ffn:
        c_.start()

    def wo_w(q0, q1, n0, n1):
        h0, h1 = q0 + 2 * ROT, q1 + 2 * ROT
        ws = [wo_v[a:b, :, n0 * 128:n1 * 128].reshape((b - a) * (DH // 2), (n1 - n0) * 128)
              for a, b in ((h0, min(h1, H)), (0, h1 - H)) if b > a]
        return pltpu.bitcast(jnp.concatenate(ws, axis=0), BF)

    HD = D // 2

    def emit_step(it, odd, pend):
        s = 2 * it + odd
        hrow = pl.multiple_of(HOFF + (s & 1) * 32, 32)
        hnext = pl.multiple_of(HOFF + 32 - (s & 1) * 32, 32)
        tv = [tab[s * NTAB + k] for k in range(7)]
        slot = tv[0]
        dsts = [(tv[1 + 2 * j], pl.multiple_of(tv[2 + 2 * j], 4)) for j in range(3)]
        orow, ow = (32, 48) if odd else (0, 32)
        odst = (48, 56, 64, 72) if odd else (8, 16, 24, 40)
        erow = it * 64 if odd else jnp.maximum(it - 1, 0) * 64 + RIDE
        lrow = PRE + jnp.minimum(s + 1, NSEG - 1) * RIDE
        e_at, l_at = (E_AT2, L_AT2) if odd else (E_AT, L_AT)
        probs = {}

        def wqkv(p, k0, k1):
            return pltpu.bitcast(jnp.concatenate(
                [w_v[p * 6 + u, k0 // 2:k1 // 2, :] for u in range(6)], axis=1), BF)

        lhs_lo = act[pl.ds(hrow, 32), 0:HD]
        if pend is not None:
            ybuf[...] = jnp.dot(lhs_lo, wqkv(0, 0, HD), preferred_element_type=F32)
            pend()
        lhs_hi = act[pl.ds(hrow, 32), HD:D]
        if pend is not None:
            y0 = ybuf[...] + jnp.dot(lhs_hi, wqkv(0, HD, D), preferred_element_type=F32)
        lhs_rest = jnp.concatenate([lhs_lo[:, 128:], lhs_hi], axis=1)
        lhs = [jnp.concatenate([lhs_lo, lhs_hi], axis=1)]

        def side(p):
            for j in range(len(e_at)):
                if e_at[j] == p:
                    finish_rows(pl.multiple_of(erow + 8 * j, 8), attn_load(j))
            for j in range(3):
                if l_at[j] == p:
                    ln1_rows(pl.multiple_of(lrow + 8 * j, 8),
                             pl.multiple_of(hnext + 8 + 8 * j, 8))
            if p in e_at or p in l_at:
                lhs[0] = jnp.concatenate([act[pl.ds(hrow, 32), 0:128], lhs_rest], axis=1)

        def qkv(p):
            if p == 0 and pend is not None:
                y = y0
            else:
                y = jnp.dot(lhs[0], wqkv(p, 0, D), preferred_element_type=F32)
            buf = qkvbufs[p % NB]
            for u in range(6):
                t, hh = u // 2, u % 2
                b0 = ((p // NB) * 3 + t) * 40
                yu = y[:, u * 128:(u + 1) * 128]
                buf[slot, b0 + hh * 4:b0 + hh * 4 + 4, :] = _pack(yu[0:8])
                for j in range(3):
                    sl, off = dsts[j]
                    buf[sl, pl.ds(b0 + 8 + hh * 16 + off, 4), :] = _pack(yu[8 + 8 * j:16 + 8 * j])

        def ld(p, t):
            b0 = ((p // NB) * 3 + t) * 40
            return pltpu.bitcast(qkvbufs[p % NB][slot, b0:b0 + 40, :], BF)

        def sc(p):
            s2 = lax.dot_general(ld(p, 0), ld(p, 1), (((1,), (1,)), ((), ())),
                                 preferred_element_type=F32)
            s2 = jnp.where(valid, s2 * SCALE, fill)
            m = jnp.max(s2, axis=-1, keepdims=True)
            e = jnp.exp(s2 - m)
            l = jnp.sum(e, axis=-1, keepdims=True)
            rl = pl.reciprocal(l, approx=True)
            rl = rl * (2.0 - l * rl)
            probs[p] = (e * rl).astype(BF)

        def pv(p):
            o2 = jnp.dot(probs[p], ld(p, 2), preferred_element_type=F32)
            for hh in range(2):
                hcol = (2 * ((p - ROT) % NP) + hh) * 128
                obuf[orow:orow + 8, hcol:hcol + 128] = o2[8 * hh:8 * hh + 8].astype(BF)
                for j in range(4):
                    r0 = 16 + 32 * hh + 8 * j
                    obuf[odst[j]:odst[j] + 8, hcol:hcol + 128] = o2[r0:r0 + 8].astype(BF)

        def attn(pos):
            for kind, p in ATT.get(pos, ()):
                (sc if kind == 's' else pv)(p)

        for p in range(NP):
            qkv(p)
            side(p)
            attn(p)
        a1 = []
        for n in range(8):
            a1.append(jnp.dot(obuf[orow:orow + ow, 0:KS], wo_w(0, KS // DH, n, n + 1),
                              preferred_element_type=F32))
            if n + 1 in W1AT:
                attn(NP + 2 * W1AT.index(n + 1))
        o2lhs = obuf[orow:orow + ow, KS:]
        a_lo = jnp.concatenate(a1[0:4], axis=1) + jnp.dot(
            o2lhs, wo_w(KS // DH, H, 0, 4), preferred_element_type=F32)
        act[pl.ds(hnext, 8), 0:HD] = a_lo[0:8].astype(BF)
        attn_store(a_lo[8:], 0)
        a_hi = jnp.concatenate(a1[4:8], axis=1) + jnp.dot(
            o2lhs, wo_w(KS // DH, H, 4, 8), preferred_element_type=F32)

        def finish():
            act[pl.ds(hnext, 8), HD:D] = a_hi[0:8].astype(BF)
            attn_store(a_hi[8:], 4)
        return finish

    def out_copy(r0, n, sem):
        return cp(act.at[pl.ds(OOFF + r0, n)], out_hbm.at[0, pl.ds(r0, n)], sem)

    def steps(it, carry):
        emit_step(it, 1, emit_step(it, 0, None))()

        @pl.when(it > 0)
        def _():
            out_copy(pl.multiple_of((it - 1) * 64, 64), 64, 9).start()
        return carry
    lax.fori_loop(0, NSEG // 2, steps, 0)

    NEW0 = S - NEW
    out_copy(S - 64, NEW0 - (S - 64), 9).start()
    for c_ in cp_ffn:
        c_.wait()

    rowsf = (lane256 * 8 + lax.broadcasted_iota(jnp.int32, (8, 256), 0)).astype(F32)
    r_old = jnp.where(rowsf < NEW0, act[ROFF:ROFF + 8, 0:256].astype(F32), -jnp.inf)

    def allmax(v):
        return jnp.max(jnp.max(v, axis=1, keepdims=True), axis=0, keepdims=True)

    def allmin(v):
        return jnp.min(jnp.min(v, axis=1, keepdims=True), axis=0, keepdims=True)
    m1 = allmax(r_old)
    i1v = allmin(jnp.where(r_old == m1, rowsf, float(S)))
    r_rest = jnp.where(rowsf == i1v, -jnp.inf, r_old)
    m2 = allmax(r_rest)
    i2v = allmin(jnp.where((r_rest == m2) & (rowsf != i1v), rowsf, float(S)))
    i1 = jnp.clip(i1v[0, 0].astype(jnp.int32), 0, NEW0 - 1)
    i2 = jnp.clip(i2v[0, 0].astype(jnp.int32), 0, NEW0 - 1)
    b1 = pl.multiple_of((i1 // 8) * 8, 8)
    b2 = pl.multiple_of((i2 // 8) * 8, 8)

    def rep(i, n):
        return jnp.concatenate([modb[i]] * n, axis=0)
    ng = NEW // 8
    x1n = _rb(xbuf[NEW0:S, :].astype(F32) + _rb(rep(2, ng) * _rb(
        jnp.concatenate([attn_load(j) for j in range(ng)], axis=0))))
    h2n = _rb(_rb(_layernorm(x1n) * rep(4, ng)) + rep(3, ng))
    rn = _rb(jnp.sum(h2n * rep(6, ng), axis=-1, keepdims=True))
    x1c = jnp.concatenate([act[pl.ds(b1, 8), :].astype(F32), act[pl.ds(b2, 8), :].astype(F32)],
                          axis=0)
    h2c = _rb(_rb(_layernorm(x1c) * rep(4, 2)) + rep(3, 2))
    x1a = jnp.concatenate([x1c, x1n], axis=0)
    h2a = jnp.concatenate([h2c, h2n], axis=0)
    sub8 = lax.broadcasted_iota(jnp.int32, (8, 1), 0)
    val = jnp.concatenate([jnp.where(sub8 == i1 - b1, m1, -jnp.inf),
                           jnp.where(sub8 == i2 - b2, m2, -jnp.inf), rn], axis=0)
    live = jnp.concatenate([(sub8 == i1 - b1).astype(F32), (sub8 == i2 - b2).astype(F32),
                            jnp.ones((NEW, 1), F32)], axis=0) > 0.5
    pos = lax.broadcasted_iota(jnp.int32, (16 + NEW, 1), 0).astype(F32)
    v1 = jnp.max(val, axis=0, keepdims=True)
    p1 = jnp.min(jnp.where((val == v1) & live, pos, float(S)), axis=0, keepdims=True)
    val2 = jnp.where(pos == p1, -jnp.inf, val)
    v2 = jnp.max(val2, axis=0, keepdims=True)
    p2 = jnp.min(jnp.where((val2 == v2) & live & (pos != p1), pos, float(S)),
                 axis=0, keepdims=True)
    row1 = jnp.sum(jnp.where(pos == p1, h2a, 0.0), axis=0, keepdims=True)
    row2 = jnp.sum(jnp.where(pos == p2, h2a, 0.0), axis=0, keepdims=True)
    sub16 = lax.broadcasted_iota(jnp.int32, (16, 1), 0)
    h2b = jnp.where(sub16 == 0, row1, jnp.where(sub16 == 1, row2, 0.0)).astype(BF)
    hid = []
    for n in range(0, F, FFN_NB):
        gt = _rb(jnp.dot(h2b, pltpu.bitcast(wg_v[:, n:n + FFN_NB], BF), preferred_element_type=F32))
        up = _rb(jnp.dot(h2b, pltpu.bitcast(wu_v[:, n:n + FFN_NB], BF), preferred_element_type=F32))
        hid.append((_rb(gt * _rb(jax.nn.sigmoid(gt))) * up).astype(BF))
    y = _rb(jnp.dot(jnp.concatenate(hid, axis=1), pltpu.bitcast(wd_v[...], BF),
                    preferred_element_type=F32))
    y1 = _rb(y[0:1] * _rb(jax.nn.sigmoid(v1)))
    y2 = _rb(y[1:2] * _rb(jax.nn.sigmoid(v2)))
    tok = jnp.concatenate([(b1 + sub8).astype(F32), (b2 + sub8).astype(F32),
                           pos[16:] + float(NEW0 - 16)], axis=0)
    t1 = jnp.sum(jnp.where(pos == p1, tok, 0.0), axis=0, keepdims=True)
    t2 = jnp.sum(jnp.where(pos == p2, tok, 0.0), axis=0, keepdims=True)
    upd = jnp.where(tok == t1, y1, jnp.where(tok == t2, y2, 0.0))
    res = (x1a + _rb(rep(5, ng + 2) * _rb(h2a + upd))).astype(BF)
    act[OOFF + NEW0:OOFF + S, :] = res[16:]
    out_copy(0, NEW0, 9).wait()
    act[pl.ds(OOFF + b1, 8), :] = res[0:8]
    act[pl.ds(OOFF + b2, 8), :] = res[8:16]
    fix0 = out_copy(NEW0, NEW, 6)
    fix1 = out_copy(b1, 8, 11)
    fix2 = out_copy(b2, 8, 12)
    fix0.start()
    fix1.start()

    @pl.when(b1 != b2)
    def _():
        fix2.start()
        fix2.wait()
    fix0.wait()
    fix1.wait()


@jax.jit
def pallas_adaLN_cond__memory_aug_recurrent_mem_tr__moe_arch_mod__prompt_kernel(
    A_x: jax.Array,
    A_mem0: jax.Array,
    A_Wq: jax.Array,
    A_Wk: jax.Array,
    A_Wv: jax.Array,
    A_Wo: jax.Array,
    A_seg_len,
    B_x: jax.Array,
    B_w_r: jax.Array,
    B_w_gate: jax.Array,
    B_w_up: jax.Array,
    B_w_down: jax.Array,
    c: jax.Array,
    w_mod: jax.Array,
):
    del B_x
    del A_seg_len
    assert A_x.shape == (1, S, D) and A_Wq.shape == (D, H, DH) and A_mem0.shape == (1, M, D)
    any_spec = pl.BlockSpec(memory_space=pl.ANY)
    scratch = [
        pltpu.VMEM((S, D), BF),
        pltpu.VMEM((ACT_ROWS, D), BF),
        pltpu.VMEM((8, PRE // 2, 128), U32),
        pltpu.VMEM((32, 768), F32),
        pltpu.SMEM((NSEG * NTAB,), jnp.int32),
        pltpu.VMEM((7, 8, D), F32),
        pltpu.VMEM((3 * H, D // 2, 128), U32),
        pltpu.VMEM((H, DH // 2, D), U32),
        pltpu.VMEM((6, D // 2, D), U32),
        pltpu.VMEM((D // 2, F), U32),
        pltpu.VMEM((D // 2, F), U32),
        pltpu.VMEM((F // 2, D), U32),
        pltpu.VMEM((80, H * DH), BF),
        pltpu.SemaphoreType.DMA((17,)),
        pltpu.SemaphoreType.DMA((12,)),
        pltpu.SemaphoreType.DMA((16,)),
    ] + [pltpu.VMEM((NSLOT + 1, 256, 128), U32) for _ in range(NB)] + [
        pltpu.VMEM((1, D), BF),
        pltpu.VMEM((D,), BF),
    ]
    wq, wk, wv = (w.reshape(D // 2, 2, H, DH) for w in (A_Wq, A_Wk, A_Wv))
    return pl.pallas_call(
        _kernel,
        out_shape=jax.ShapeDtypeStruct((1, S, D), BF),
        in_specs=[any_spec] * 12,
        out_specs=any_spec,
        scratch_shapes=scratch,
        compiler_params=pltpu.CompilerParams(vmem_limit_bytes=120 * 1024 * 1024,
                                             disable_bounds_checks=True,
                                             disable_semaphore_checks=True),
    )(A_x, A_mem0, wq, wk, wv, A_Wo, B_w_r, B_w_gate, B_w_up, B_w_down,
      c, w_mod)
```

```python
import jax
import jax.numpy as jnp
from jax import lax
import jax.experimental.pallas as pl
import jax.experimental.pallas.tpu as pltpu

BF = jnp.bfloat16
F32 = jnp.float32
U32 = jnp.uint32

S = 2048
D = 1024
H = 32
DH = 128
M = 8
SEG = 32
NSEG = S // SEG
F = 3584
NP = H // 2
EPS = 1e-5
SCALE = DH ** -0.5

RIDE = 24
PRE = S - NSEG * RIDE
NSLOT = 17
NB = 8
KS = 2048
OOFF = S
HOFF = 2 * S
ROFF = HOFF + 64
ACT_ROWS = ROFF + 16
PRE_SPLIT = 4
E_AT = (2, 3, 4, 5, 6)
E_AT2 = (3, 4, 5)
L_AT = (6, 7, 8)
L_AT2 = (6, 8, 10)
A_BUF = (7, 0, 1, 2, 3)
W1AT = (2, 6)
NEW = 40
FFN_NB = 512
APPLY_N = 4
NTAB = 8

ROT = 2
ATT = {4: [('s', i) for i in range(4)],
       18: [('p', (12 + ROT + i) % NP) for i in range(4)]}
for _p in range(4, NP, 2):
    ATT[_p + 2] = [('s', _p), ('s', _p + 1), ('p', _p - 4 + ROT), ('p', _p - 3 + ROT)]


def _step_indices(s):
    t = [s % NSLOT]
    for j in range(3):
        gi = PRE // 8 + 3 * s + j
        t += [(gi // 4) % NSLOT, (gi % 4) * 4]
    return t


def _rb(v):
    return v.astype(BF).astype(F32)


def _pack(v):
    return pltpu.bitcast(v.astype(BF), U32)


def _layernorm(x):
    mu = jnp.sum(x, axis=-1, keepdims=True) * (1.0 / D)
    xc = x - mu
    var = jnp.sum(xc * xc, axis=-1, keepdims=True) * (1.0 / D)
    sd = _rb(jnp.sqrt(_rb(_rb(var) + EPS)))
    return _rb(_rb(x - _rb(mu)) / sd)


def _kernel(x_hbm, mem0_hbm, wq_hbm, wk_hbm, wv_hbm, wo_hbm, wr_hbm, wg_hbm, wu_hbm,
            wd_hbm, c_hbm, wmod_hbm, out_hbm,
            xbuf, act, h0buf, ybuf, tab, modb,
            w_v, wo_v, wmod_v, wg_v, wu_v, wd_v,
            obuf, sems, wsems, ksems, *rest):
    qkvbufs, cbuf, wrbuf = rest[:NB], rest[NB], rest[NB + 1]
    w_hbms = tuple(w.bitcast(U32) for w in (wq_hbm, wk_hbm, wv_hbm))

    def cp(src, dst, i):
        return pltpu.make_async_copy(src, dst, sems.at[i])

    wmod32 = wmod_hbm.bitcast(U32)
    cp_c = cp(c_hbm, cbuf, 0)
    cp_mem = cp(mem0_hbm.at[0], act.at[HOFF:HOFF + M], 1)
    cp_wr = cp(wr_hbm, wrbuf, 2)
    cp_x0 = [cp(x_hbm.at[0, n * 128:(n + 1) * 128], xbuf.at[n * 128:(n + 1) * 128], 13 + n)
             for n in range(PRE // 128)]
    cp_xr = cp(x_hbm.at[0, PRE:PRE + 32], xbuf.at[PRE:PRE + 32], 5)
    cp_x1 = cp(x_hbm.at[0, PRE + 32:S], xbuf.at[PRE + 32:S], 4)
    cp_wo = cp(wo_hbm.bitcast(U32), wo_v, 7)
    cp_ffn = [cp(wg_hbm.bitcast(U32), wg_v, 8), cp(wu_hbm.bitcast(U32), wu_v, 8),
              cp(wd_hbm.bitcast(U32), wd_v, 8)]

    def w_start(j, i0=0, i1=NB, prio=0):
        gg, t = j // 3, j % 3
        r0 = 64 if j == 1 else 0
        for i in range(i0, i1):
            for par in range(2):
                pltpu.make_async_copy(w_hbms[t].at[r0:, par, gg * NB + i, :],
                                      w_v.at[(gg * NB + i) * 6 + t * 2 + par, r0:],
                                      wsems.at[2 * j + (i >= PRE_SPLIT)]).start(priority=prio)

    def mod_copy(j):
        return pltpu.make_async_copy(wmod32.at[:, j * D:(j + 1) * D], wmod_v.at[j],
                                     wsems.at[2 * j + 1])

    def mult(v, m):
        return v if isinstance(v, int) else pl.multiple_of(v, m)

    def moda_copies(kc):
        col = mult(kc * 128, 128)
        return [pltpu.make_async_copy(wmod32.at[:, pl.ds(v * D + col, 128)],
                                      wmod_v.at[v, :, pl.ds(col, 128)], ksems.at[8 + kc])
                for v in range(2)]

    def chunk_copies(kc):
        r0 = mult(kc * 64, 64)
        return [pltpu.make_async_copy(w_hbms[0].at[pl.ds(r0, 64), par, i, :],
                                      w_v.at[i * 6 + par, pl.ds(r0, 64), :], ksems.at[kc])
                for i in range(NB) for par in range(2)]

    cp_early = [cp(w_hbms[1].at[0:64, par, i, :], w_v.at[i * 6 + 2 + par, 0:64], 3)
                for i in range(NB) for par in range(2)]

    cp_c.start()
    cp_mem.start()
    cp_wr.start()
    for c_ in (cp_x0 + moda_copies(0) + cp_early + moda_copies(1) + chunk_copies(0)
               + moda_copies(2) + chunk_copies(1) + [cp_xr]):
        c_.start()

    def ln1_rows(src_row, dst_row):
        xv = xbuf[pl.ds(src_row, 8), :].astype(F32)
        hv = _rb(_layernorm(xv) * modb[1]) + modb[0]
        act[pl.ds(dst_row, 8), :] = hv.astype(BF)

    lane256 = lax.broadcasted_iota(jnp.int32, (8, 256), 1)

    def finish_rows(row, attn):
        xv = xbuf[pl.ds(row, 8), :].astype(F32)
        x1 = _rb(xv + _rb(modb[2] * _rb(attn)))
        act[pl.ds(row, 8), :] = x1.astype(BF)
        h2 = _rb(_rb(_layernorm(x1) * modb[4]) + modb[3])
        act[pl.ds(OOFF + row, 8), :] = (x1 + _rb(modb[5] * h2)).astype(BF)
        r = jnp.sum(h2 * modb[6], axis=-1, keepdims=True)
        act[ROFF:ROFF + 8, 0:256] = jnp.where(
            lane256 * 8 == row, r, act[ROFF:ROFF + 8, 0:256].astype(F32)).astype(BF)

    def attn_store(a, k0):
        for j in range(a.shape[0] // 8):
            for k in range(a.shape[1] // 128):
                qkvbufs[A_BUF[j]][NSLOT, (k0 + k) * 8:(k0 + k + 1) * 8, :] = pltpu.bitcast(
                    a[8 * j:8 * j + 8, k * 128:(k + 1) * 128], U32)

    def attn_load(j):
        return pltpu.bitcast(jnp.concatenate(
            [qkvbufs[A_BUF[j]][NSLOT, k * 8:(k + 1) * 8, :] for k in range(8)], axis=1), F32)

    act[ROFF:ROFF + 8, 0:256] = jnp.zeros((8, 256), BF)
    attn_store(jnp.zeros((NEW, D), F32), 0)
    for s_ in range(NSEG):
        for k, v in enumerate(_step_indices(s_)):
            tab[s_ * NTAB + k] = v
    ri = lax.broadcasted_iota(jnp.int32, (80, 80), 0)
    ci = lax.broadcasted_iota(jnp.int32, (80, 80), 1)

    def head_pos(i):
        hd = jnp.where(i < 16, i // 8, (i - 16) // 32)
        pos = jnp.where(i < 16, i % 8, 8 + (i - 16) % 32)
        return hd, pos
    rh, rp = head_pos(ri)
    ch, cpos = head_pos(ci)
    same = rh == ch
    valid = same & ((rp < M) | (rp >= cpos))
    fill = jnp.where(same, -1e9, -jnp.inf).astype(F32)

    cp_mem.wait()
    cp_wr.wait()
    modb[6] = jnp.broadcast_to(wrbuf[...].astype(F32).reshape(1, D), (8, D))
    cp_c.wait()
    cv = cbuf[...].astype(F32)
    sc16 = jnp.broadcast_to(_rb(cv * _rb(jax.nn.sigmoid(cv))), (16, D)).astype(BF)

    def ln_pre(g, carry):
        pltpu.make_async_copy(x_hbm.at[0, 0:128], xbuf.at[pl.ds(pl.multiple_of(g * 128, 128), 128)],
                              sems.at[13 + g]).wait()
        for u in range(2):
            row = pl.multiple_of(g * 128 + u * 64, 64)
            nv = _layernorm(xbuf[pl.ds(row, 64), :].astype(F32)).astype(BF)
            for k in range(8):
                h0buf[k, pl.ds(pl.multiple_of(row // 2, 32), 32), :] = pltpu.bitcast(
                    nv[:, k * 128:(k + 1) * 128], U32)
            wg_v[pl.ds(row, 64), 0:2 * D] = jnp.zeros((64, 2 * D), U32)
        return carry
    lax.fori_loop(0, PRE // 128, ln_pre, 0)

    def mod_tile(v, col):
        w = pltpu.bitcast(wmod_v[v, :, pl.ds(col, 128)], BF)
        return _rb(jnp.dot(sc16, w, preferred_element_type=F32))[0:8]

    def moda_store(kc, sa, ca):
        col = mult(kc * 128, 128)
        c1 = _rb(1.0 + ca)
        modb[0, :, pl.ds(col, 128)] = sa
        modb[1, :, pl.ds(col, 128)] = c1
        return sa, c1

    def moda_apply(kc, sa, c1, r0, r1):
        for r in range(r0, r1, 16):
            nv = pltpu.bitcast(h0buf[kc, r // 2:r // 2 + 8, :], BF).astype(F32).reshape(2, 8, 128)
            hv = (_rb(nv * c1[None]) + sa[None]).reshape(16, 128).astype(BF)
            h0buf[kc, r // 2:r // 2 + 8, :] = pltpu.bitcast(hv, U32)

    def repack(a, b):
        return (a & U32(0xFFFF)) | (b << 16), (a >> 16) | (b & U32(0xFFFF0000))

    def store_qkv(i, jrow, y, seg0):
        for sg in range(y.shape[0] // 32):
            for hh in range(2):
                qkvbufs[i][seg0 + sg, pl.ds(jrow + 8 + hh * 16, 16), :] = _pack(
                    y[sg * 32:(sg + 1) * 32, hh * 128:(hh + 1) * 128])

    for c_ in chunk_copies(2):
        c_.start()
    for c_ in moda_copies(0):
        c_.wait()
    moda_apply(0, *moda_store(0, mod_tile(0, 0), mod_tile(1, 0)), 0, PRE)
    w_start(1, 0, PRE_SPLIT, prio=1)

    for c_ in cp_early:
        c_.wait()
    for i in range(NB):
        lo, hi = repack(w_v[i * 6 + 2, 0:64, :], w_v[i * 6 + 3, 0:64, :])
        w_v[i * 6 + 2, 0:64, :] = lo
        w_v[i * 6 + 3, 0:64, :] = hi
        wu_v[0:PRE, i * 256:(i + 1) * 256] = pltpu.bitcast(jnp.dot(
            pltpu.bitcast(h0buf[0], BF), pltpu.bitcast(jnp.concatenate([lo, hi], axis=1), BF),
            preferred_element_type=F32), U32)

    def w_wait(j, i0, i1, r0=0):
        blk0 = (j // 3) * (6 * NB) + (j % 3) * 2
        for i in range(i0, i1):
            for par in range(2):
                pltpu.make_async_copy(w_hbms[0].at[r0:, 0, 0, :], w_v.at[blk0 + i * 6 + par, r0:],
                                      wsems.at[2 * j + (i >= PRE_SPLIT)]).wait()

    def chunk_block(kc, last, issue):
        for c_ in chunk_copies(kc) + ([cp_xr] if last else moda_copies(kc + 1)):
            c_.wait()
        issue()
        r0 = mult(kc * 64, 64)
        mv = []
        for i in range(NB):
            lo, hi = repack(w_v[i * 6, pl.ds(r0, 64), :], w_v[i * 6 + 1, pl.ds(r0, 64), :])
            w_v[i * 6, pl.ds(r0, 64), :] = lo
            w_v[i * 6 + 1, pl.ds(r0, 64), :] = hi
            w = pltpu.bitcast(jnp.concatenate([lo, hi], axis=1), BF)
            y = (pltpu.bitcast(wg_v[0:PRE, i * 256:(i + 1) * 256], F32)
                 + jnp.dot(pltpu.bitcast(h0buf[kc], BF), w, preferred_element_type=F32))
            if last:
                store_qkv(i, 0, y, 0)
            else:
                wg_v[0:PRE, i * 256:(i + 1) * 256] = pltpu.bitcast(y, U32)
                if i in (1, 3):
                    mv.append(mod_tile(i // 2, mult((kc + 1) * 128, 128)))
                if i == 3:
                    mv = moda_store(kc + 1, mv[0], mv[1])
                if i in (4, 6):
                    zeros = qkvbufs[A_BUF[0]][NSLOT, 0:8, :]
                    for q in range(APPLY_N):
                        yr = (q + 1) * (PRE // (APPLY_N + 1)) // 8 * 8
                        tok = pltpu.bitcast(y[yr:yr + 8, 0:128], U32) & zeros
                        c1 = pltpu.bitcast(pltpu.bitcast(mv[1], U32) | tok, F32)
                        n = PRE // 2 // APPLY_N
                        r_ = (i - 4) // 2 * (PRE // 2) + q * n
                        moda_apply(kc + 1, mv[0], c1, r_, r_ + n)
        if last:
            for j in range(3):
                ln1_rows(PRE + 8 * j, HOFF + 8 + 8 * j)

    def chunk_body(kc, carry):
        def issue():
            @pl.when(kc < 5)
            def _():
                for c_ in moda_copies(kc + 3) + chunk_copies(kc + 3):
                    c_.start()
        chunk_block(kc, False, issue)
        return carry

    def issue_last():
        w_wait(1, 0, PRE_SPLIT, 64)
        w_start(1, PRE_SPLIT, NB)
        w_start(2)
        mod_copy(2).start()
    lax.fori_loop(0, 7, chunk_body, 0)
    chunk_block(7, True, issue_last)

    def pre_unit(j, i, extra, k0=0):
        blk = (j // 3) * (6 * NB) + (j % 3) * 2 + i * 6
        jrow = mult(j * 40, 8)
        r0 = k0 * 64
        lo, hi = repack(w_v[blk, r0:, :], w_v[blk + 1, r0:, :])
        w_v[blk, r0:, :] = lo
        w_v[blk + 1, r0:, :] = hi
        for rc in range(PRE // 128):
            if rc > 0:
                lo = w_v[blk, r0:, :]
                hi = w_v[blk + 1, r0:, :]
            w = pltpu.bitcast(jnp.concatenate([lo, hi], axis=1), BF)
            lhs = jnp.concatenate(
                [h0buf[k, rc * 64:(rc + 1) * 64, :] for k in range(k0, 8)], axis=1)
            y = jnp.dot(pltpu.bitcast(lhs, BF), w, preferred_element_type=F32)
            if k0:
                y = y + pltpu.bitcast(wu_v[rc * 128:(rc + 1) * 128, i * 256:(i + 1) * 256], F32)
            store_qkv(i, jrow, y, rc * 4)
            extra(rc)

    for i in range(NB):
        if i == PRE_SPLIT:
            w_wait(1, PRE_SPLIT, NB, 64)
            for jn in (3, 4):
                w_start(jn)
                mod_copy(jn).start()
        pre_unit(1, i, lambda rc: None, k0=1)
    w_start(5)
    mod_copy(5).start()
    cp_wo.start()
    cp_x1.start()

    def pre_body(j, carry):
        w_wait(j, 0, NB)
        pltpu.make_async_copy(wmod32.at[:, 0:D], wmod_v.at[j], wsems.at[2 * j + 1]).wait()
        one = jnp.where(j == 4, 1.0, 0.0).astype(F32)
        for i in range(NB):
            def extra(rc, i=i):
                if rc == 1:
                    modb[j, :, i * 128:(i + 1) * 128] = _rb(one + mod_tile(j, i * 128))
            pre_unit(j, i, extra)
        return carry
    lax.fori_loop(2, 6, pre_body, 0)

    cp_wo.wait()
    cp_x1.wait()
    for c_ in cp_ffn:
        c_.start()

    def wo_w(q0, q1, n0, n1):
        h0, h1 = q0 + 2 * ROT, q1 + 2 * ROT
        ws = [wo_v[a:b, :, n0 * 128:n1 * 128].reshape((b - a) * (DH // 2), (n1 - n0) * 128)
              for a, b in ((h0, min(h1, H)), (0, h1 - H)) if b > a]
        return pltpu.bitcast(jnp.concatenate(ws, axis=0), BF)

    HD = D // 2

    def emit_step(it, odd, pend):
        s = 2 * it + odd
        hrow = pl.multiple_of(HOFF + (s & 1) * 32, 32)
        hnext = pl.multiple_of(HOFF + 32 - (s & 1) * 32, 32)
        tv = [tab[s * NTAB + k] for k in range(7)]
        slot = tv[0]
        dsts = [(tv[1 + 2 * j], pl.multiple_of(tv[2 + 2 * j], 4)) for j in range(3)]
        orow, ow = (32, 48) if odd else (0, 32)
        odst = (48, 56, 64, 72) if odd else (8, 16, 24, 40)
        erow = it * 64 if odd else jnp.maximum(it - 1, 0) * 64 + RIDE
        lrow = PRE + jnp.minimum(s + 1, NSEG - 1) * RIDE
        e_at, l_at = (E_AT2, L_AT2) if odd else (E_AT, L_AT)
        probs = {}

        def wqkv(p, k0, k1):
            return pltpu.bitcast(jnp.concatenate(
                [w_v[p * 6 + u, k0 // 2:k1 // 2, :] for u in range(6)], axis=1), BF)

        lhs_lo = act[pl.ds(hrow, 32), 0:HD]
        if pend is not None:
            ybuf[...] = jnp.dot(lhs_lo, wqkv(0, 0, HD), preferred_element_type=F32)
            pend()
        lhs_hi = act[pl.ds(hrow, 32), HD:D]
        if pend is not None:
            y0 = ybuf[...] + jnp.dot(lhs_hi, wqkv(0, HD, D), preferred_element_type=F32)
        lhs_rest = jnp.concatenate([lhs_lo[:, 128:], lhs_hi], axis=1)
        lhs = [jnp.concatenate([lhs_lo, lhs_hi], axis=1)]

        def side(p):
            for j in range(len(e_at)):
                if e_at[j] == p:
                    finish_rows(pl.multiple_of(erow + 8 * j, 8), attn_load(j))
            for j in range(3):
                if l_at[j] == p:
                    ln1_rows(pl.multiple_of(lrow + 8 * j, 8),
                             pl.multiple_of(hnext + 8 + 8 * j, 8))
            if p in e_at or p in l_at:
                lhs[0] = jnp.concatenate([act[pl.ds(hrow, 32), 0:128], lhs_rest], axis=1)

        def qkv(p):
            if p == 0 and pend is not None:
                y = y0
            else:
                y = jnp.dot(lhs[0], wqkv(p, 0, D), preferred_element_type=F32)
            buf = qkvbufs[p % NB]
            for u in range(6):
                t, hh = u // 2, u % 2
                b0 = ((p // NB) * 3 + t) * 40
                yu = y[:, u * 128:(u + 1) * 128]
                buf[slot, b0 + hh * 4:b0 + hh * 4 + 4, :] = _pack(yu[0:8])
                for j in range(3):
                    sl, off = dsts[j]
                    buf[sl, pl.ds(b0 + 8 + hh * 16 + off, 4), :] = _pack(yu[8 + 8 * j:16 + 8 * j])

        def ld(p, t):
            b0 = ((p // NB) * 3 + t) * 40
            return pltpu.bitcast(qkvbufs[p % NB][slot, b0:b0 + 40, :], BF)

        def sc(p):
            s2 = lax.dot_general(ld(p, 0), ld(p, 1), (((1,), (1,)), ((), ())),
                                 preferred_element_type=F32)
            s2 = jnp.where(valid, s2 * SCALE, fill)
            m = jnp.max(s2, axis=-1, keepdims=True)
            e = jnp.exp(s2 - m)
            l = jnp.sum(e, axis=-1, keepdims=True)
            rl = pl.reciprocal(l, approx=True)
            rl = rl * (2.0 - l * rl)
            probs[p] = (e * rl).astype(BF)

        def pv(p):
            o2 = jnp.dot(probs[p], ld(p, 2), preferred_element_type=F32)
            for hh in range(2):
                hcol = (2 * ((p - ROT) % NP) + hh) * 128
                obuf[orow:orow + 8, hcol:hcol + 128] = o2[8 * hh:8 * hh + 8].astype(BF)
                for j in range(4):
                    r0 = 16 + 32 * hh + 8 * j
                    obuf[odst[j]:odst[j] + 8, hcol:hcol + 128] = o2[r0:r0 + 8].astype(BF)

        def attn(pos):
            for kind, p in ATT.get(pos, ()):
                (sc if kind == 's' else pv)(p)

        for p in range(NP):
            qkv(p)
            side(p)
            attn(p)
        a1 = []
        for n in range(8):
            a1.append(jnp.dot(obuf[orow:orow + ow, 0:KS], wo_w(0, KS // DH, n, n + 1),
                              preferred_element_type=F32))
            if n + 1 in W1AT:
                attn(NP + 2 * W1AT.index(n + 1))
        o2lhs = obuf[orow:orow + ow, KS:]
        a_lo = jnp.concatenate(a1[0:4], axis=1) + jnp.dot(
            o2lhs, wo_w(KS // DH, H, 0, 4), preferred_element_type=F32)
        act[pl.ds(hnext, 8), 0:HD] = a_lo[0:8].astype(BF)
        attn_store(a_lo[8:], 0)
        a_hi = jnp.concatenate(a1[4:8], axis=1) + jnp.dot(
            o2lhs, wo_w(KS // DH, H, 4, 8), preferred_element_type=F32)

        def finish():
            act[pl.ds(hnext, 8), HD:D] = a_hi[0:8].astype(BF)
            attn_store(a_hi[8:], 4)
        return finish

    def out_copy(r0, n, sem):
        return cp(act.at[pl.ds(OOFF + r0, n)], out_hbm.at[0, pl.ds(r0, n)], sem)

    def steps(it, carry):
        emit_step(it, 1, emit_step(it, 0, None))()

        @pl.when(it > 0)
        def _():
            out_copy(pl.multiple_of((it - 1) * 64, 64), 64, 9).start()
        return carry
    lax.fori_loop(0, NSEG // 2, steps, 0)

    NEW0 = S - NEW
    out_copy(S - 64, NEW0 - (S - 64), 9).start()
    for c_ in cp_ffn:
        c_.wait()

    def rep(i, n):
        return jnp.concatenate([modb[i]] * n, axis=0)
    r_old = act[ROFF:ROFF + 8, 0:256].astype(F32) + 0.0
    bits = pltpu.bitcast(jnp.broadcast_to(jnp.max(r_old, axis=0, keepdims=True), (8, 256)),
                         jnp.int32)
    code = (bits ^ ((bits >> 31) & 0x7FFFFFFF)) >> 16
    key = jnp.where(lane256 < NEW0 // 8, (code * 256 + (255 - lane256)).astype(F32), -jnp.inf)
    k1 = jnp.max(key, axis=1, keepdims=True)
    k2 = jnp.max(jnp.where(key == k1, -jnp.inf, key), axis=1, keepdims=True)
    rc = jnp.concatenate([jnp.max(jnp.where(key == k, r_old, -jnp.inf), axis=1, keepdims=True)
                          for k in (k1, k2)], axis=0)
    b1, b2 = (pl.multiple_of(jnp.minimum(255 - (k[0, 0].astype(jnp.int32) & 255),
                                         NEW0 // 8 - 1) * 8, 8) for k in (k1, k2))
    ng = NEW // 8
    x1n = _rb(xbuf[NEW0:S, :].astype(F32) + _rb(rep(2, ng) * _rb(
        jnp.concatenate([attn_load(j) for j in range(ng)], axis=0))))
    h2n = _rb(_rb(_layernorm(x1n) * rep(4, ng)) + rep(3, ng))
    rn = _rb(jnp.sum(h2n * rep(6, ng), axis=-1, keepdims=True))
    x1c = jnp.concatenate([act[pl.ds(b1, 8), :].astype(F32), act[pl.ds(b2, 8), :].astype(F32)],
                          axis=0)
    h2c = _rb(_rb(_layernorm(x1c) * rep(4, 2)) + rep(3, 2))
    subf = lax.broadcasted_iota(jnp.int32, (8, 1), 0).astype(F32)
    b1f = b1.astype(F32)
    val = jnp.concatenate([rc, rn], axis=0)
    idx = jnp.concatenate([subf + b1f, subf + b2.astype(F32)]
                          + [subf + float(NEW0 + 8 * j) for j in range(ng)], axis=0)
    v1 = jnp.max(val, axis=0, keepdims=True)
    t1 = jnp.min(jnp.where(val == v1, idx, float(S)), axis=0, keepdims=True)
    rest = jnp.where(idx == t1, -jnp.inf, val)
    v2 = jnp.max(rest, axis=0, keepdims=True)
    t2 = jnp.min(jnp.where((rest == v2) & (idx != t1), idx, float(S)), axis=0, keepdims=True)

    def pick(t, old2, new):
        out = jnp.where((t >= b1f) & (t < b1f + 8.0), old2[0:8], old2[8:16])
        for j in range(ng):
            out = jnp.where(t >= float(NEW0 + 8 * j), new[8 * j:8 * j + 8], out)
        return out
    h2s = jnp.concatenate([pick(t1, h2c, h2n), pick(t2, h2c, h2n)], axis=0)
    h2b = h2s.astype(BF)
    hid = []
    for n in range(0, F, FFN_NB):
        gt = _rb(jnp.dot(h2b, pltpu.bitcast(wg_v[:, n:n + FFN_NB], BF), preferred_element_type=F32))
        up = _rb(jnp.dot(h2b, pltpu.bitcast(wu_v[:, n:n + FFN_NB], BF), preferred_element_type=F32))
        hid.append((_rb(gt * _rb(jax.nn.sigmoid(gt))) * up).astype(BF))
    y = _rb(jnp.dot(jnp.concatenate(hid, axis=1), pltpu.bitcast(wd_v[...], BF),
                    preferred_element_type=F32))
    act[OOFF + NEW0:OOFF + S, :] = (x1n + _rb(rep(5, ng) * h2n)).astype(BF)
    x1s = jnp.concatenate([pick(t1, x1c, x1n), pick(t2, x1c, x1n)], axis=0)
    c1, c2 = (pl.multiple_of((jnp.clip(t[0, 0].astype(jnp.int32), 0, S - 1) >> 3) * 8, 8)
              for t in (t1, t2))
    tok = jnp.concatenate([subf + c1.astype(F32), subf + c2.astype(F32)], axis=0)
    is1, is2 = tok == t1, tok == t2
    gate = _rb(jax.nn.sigmoid(jnp.where(is1, v1, v2)))
    upd = jnp.where(is1 | is2, _rb(y * gate), 0.0)
    res = (x1s + _rb(rep(5, 2) * _rb(h2s + upd))).astype(BF)
    out_copy(0, NEW0, 9).wait()
    act[pl.ds(OOFF + c1, 8), :] = res[0:8]
    act[pl.ds(OOFF + c2, 8), :] = res[8:16]
    fix0 = out_copy(NEW0, NEW, 6)
    fix1 = out_copy(c1, 8, 11)
    fix2 = out_copy(c2, 8, 12)
    send1 = c1 < NEW0
    send2 = (c2 < NEW0) & (c2 != c1)
    fix0.start()
    pl.when(send1)(fix1.start)
    pl.when(send2)(fix2.start)
    pl.when(send1)(fix1.wait)
    pl.when(send2)(fix2.wait)
    fix0.wait()


@jax.jit
def pallas_adaLN_cond__memory_aug_recurrent_mem_tr__moe_arch_mod__prompt_kernel(
    A_x: jax.Array,
    A_mem0: jax.Array,
    A_Wq: jax.Array,
    A_Wk: jax.Array,
    A_Wv: jax.Array,
    A_Wo: jax.Array,
    A_seg_len,
    B_x: jax.Array,
    B_w_r: jax.Array,
    B_w_gate: jax.Array,
    B_w_up: jax.Array,
    B_w_down: jax.Array,
    c: jax.Array,
    w_mod: jax.Array,
):
    del B_x
    del A_seg_len
    assert A_x.shape == (1, S, D) and A_Wq.shape == (D, H, DH) and A_mem0.shape == (1, M, D)
    any_spec = pl.BlockSpec(memory_space=pl.ANY)
    scratch = [
        pltpu.VMEM((S, D), BF),
        pltpu.VMEM((ACT_ROWS, D), BF),
        pltpu.VMEM((8, PRE // 2, 128), U32),
        pltpu.VMEM((32, 768), F32),
        pltpu.SMEM((NSEG * NTAB,), jnp.int32),
        pltpu.VMEM((7, 8, D), F32),
        pltpu.VMEM((3 * H, D // 2, 128), U32),
        pltpu.VMEM((H, DH // 2, D), U32),
        pltpu.VMEM((6, D // 2, D), U32),
        pltpu.VMEM((D // 2, F), U32),
        pltpu.VMEM((D // 2, F), U32),
        pltpu.VMEM((F // 2, D), U32),
        pltpu.VMEM((80, H * DH), BF),
        pltpu.SemaphoreType.DMA((17,)),
        pltpu.SemaphoreType.DMA((12,)),
        pltpu.SemaphoreType.DMA((16,)),
    ] + [pltpu.VMEM((NSLOT + 1, 256, 128), U32) for _ in range(NB)] + [
        pltpu.VMEM((1, D), BF),
        pltpu.VMEM((D,), BF),
    ]
    wq, wk, wv = (w.reshape(D // 2, 2, H, DH) for w in (A_Wq, A_Wk, A_Wv))
    return pl.pallas_call(
        _kernel,
        out_shape=jax.ShapeDtypeStruct((1, S, D), BF),
        in_specs=[any_spec] * 12,
        out_specs=any_spec,
        scratch_shapes=scratch,
        compiler_params=pltpu.CompilerParams(vmem_limit_bytes=120 * 1024 * 1024,
                                             disable_bounds_checks=True,
                                             disable_semaphore_checks=True),
    )(A_x, A_mem0, wq, wk, wv, A_Wo, B_w_r, B_w_gate, B_w_up, B_w_down,
      c, w_mod)
```

```python
import jax
import jax.numpy as jnp
from jax import lax
import jax.experimental.pallas as pl
import jax.experimental.pallas.tpu as pltpu

BF = jnp.bfloat16
F32 = jnp.float32
U32 = jnp.uint32

S = 2048
D = 1024
H = 32
DH = 128
M = 8
SEG = 32
NSEG = S // SEG
F = 3584
NP = H // 2
EPS = 1e-5
SCALE = DH ** -0.5
HD = D // 2

RIDE = 24
PRE = S - NSEG * RIDE
NSLOT = 17
NB = 8
KS = 2048
OOFF = S
HOFF = 2 * S
ROFF = HOFF + 64
ACT_ROWS = ROFF + 16
PRE_SPLIT = 4
E_AT = (2, 3, 4, 5, 6)
E_AT2 = (3, 4, 5)
L_AT = (6, 7, 8)
L_AT2 = (6, 8, 10)
A_BUF = (7, 0, 1, 2, 3)
W1AT = (2, 6)
NEW = 40
FFN_NB = 512
APPLY_N = 4
NTAB = 8

ROT = 2
ATT = {4: [('s', i) for i in range(4)],
       18: [('p', (12 + ROT + i) % NP) for i in range(4)]}
for _p in range(4, NP, 2):
    ATT[_p + 2] = [('s', _p), ('s', _p + 1), ('p', _p - 4 + ROT), ('p', _p - 3 + ROT)]


def _step_indices(s):
    t = [s % NSLOT]
    for j in range(3):
        gi = PRE // 8 + 3 * s + j
        t += [(gi // 4) % NSLOT, (gi % 4) * 4]
    return t


def _rb(v):
    return v.astype(BF).astype(F32)


def _pack(v):
    return pltpu.bitcast(v.astype(BF), U32)


def _layernorm(x):
    mu = jnp.sum(x, axis=-1, keepdims=True) * (1.0 / D)
    xc = x - mu
    var = jnp.sum(xc * xc, axis=-1, keepdims=True) * (1.0 / D)
    sd = _rb(jnp.sqrt(_rb(_rb(var) + EPS)))
    return _rb(_rb(x - _rb(mu)) / sd)


def _kernel(x_hbm, mem0_hbm, wq_hbm, wk_hbm, wv_hbm, wo_hbm, wr_hbm, wg_hbm, wu_hbm,
            wd_hbm, c_hbm, wmod_hbm, out_hbm,
            xbuf, act, h0buf, ybuf, scol, macc, tab, modb,
            w_v, wo_v, wmod_v, wg_v, wu_v, wd_v,
            obuf, sems, wsems, ksems, *rest):
    qkvbufs, cbuf, wrbuf = rest[:NB], rest[NB], rest[NB + 1]
    w_hbms = tuple(w.bitcast(U32) for w in (wq_hbm, wk_hbm, wv_hbm))

    def cp(src, dst, i):
        return pltpu.make_async_copy(src, dst, sems.at[i])

    wmod32 = wmod_hbm.bitcast(U32)
    cp_c = cp(c_hbm, cbuf, 0)
    cp_mem = cp(mem0_hbm.at[0], act.at[HOFF:HOFF + M], 1)
    cp_wr = cp(wr_hbm, wrbuf, 2)
    cp_x0 = [cp(x_hbm.at[0, n * 128:(n + 1) * 128], xbuf.at[n * 128:(n + 1) * 128], 13 + n)
             for n in range(PRE // 128)]
    cp_xr = cp(x_hbm.at[0, PRE:PRE + 32], xbuf.at[PRE:PRE + 32], 5)
    cp_x1 = cp(x_hbm.at[0, PRE + 32:S], xbuf.at[PRE + 32:S], 4)
    cp_wo = cp(wo_hbm.bitcast(U32), wo_v, 7)
    cp_ffn = [cp(wg_hbm.bitcast(U32), wg_v, 8), cp(wu_hbm.bitcast(U32), wu_v, 8),
              cp(wd_hbm.bitcast(U32), wd_v, 8)]

    def w_start(j, i0=0, i1=NB, prio=0):
        gg, t = j // 3, j % 3
        r0 = 64 if j == 1 else 0
        for i in range(i0, i1):
            for par in range(2):
                pltpu.make_async_copy(w_hbms[t].at[r0:, par, gg * NB + i, :],
                                      w_v.at[(gg * NB + i) * 6 + t * 2 + par, r0:],
                                      wsems.at[2 * j + (i >= PRE_SPLIT)]).start(priority=prio)

    def mod_copy(j):
        return pltpu.make_async_copy(wmod32.at[:, j * D:(j + 1) * D], wmod_v.at[j],
                                     wsems.at[2 * j + 1])

    def mult(v, m):
        return v if isinstance(v, int) else pl.multiple_of(v, m)

    def moda_copies(kc):
        col = mult(kc * 128, 128)
        return [pltpu.make_async_copy(wmod32.at[:, pl.ds(v * D + col, 128)],
                                      wmod_v.at[v, :, pl.ds(col, 128)], ksems.at[8 + kc])
                for v in range(2)]

    def chunk_copies(kc):
        r0 = mult(kc * 64, 64)
        return [pltpu.make_async_copy(w_hbms[0].at[pl.ds(r0, 64), par, i, :],
                                      w_v.at[i * 6 + par, pl.ds(r0, 64), :], ksems.at[kc])
                for i in range(NB) for par in range(2)]

    cp_early = [cp(w_hbms[1].at[0:64, par, i, :], w_v.at[i * 6 + 2 + par, 0:64], 3)
                for i in range(NB) for par in range(2)]

    cp_c.start()
    cp_mem.start()
    cp_wr.start()
    for c_ in (cp_x0 + moda_copies(0) + cp_early + moda_copies(1) + chunk_copies(0)
               + moda_copies(2) + chunk_copies(1) + [cp_xr]):
        c_.start()

    def ln1_rows(src_row, dst_row):
        xv = xbuf[pl.ds(src_row, 8), :].astype(F32)
        hv = _rb(_layernorm(xv) * modb[1]) + modb[0]
        act[pl.ds(dst_row, 8), :] = hv.astype(BF)

    lane256 = lax.broadcasted_iota(jnp.int32, (8, 256), 1)

    def finish_rows(row, attn):
        xv = xbuf[pl.ds(row, 8), :].astype(F32)
        x1 = _rb(xv + _rb(modb[2] * _rb(attn)))
        act[pl.ds(row, 8), :] = x1.astype(BF)
        h2 = _rb(_rb(_layernorm(x1) * modb[4]) + modb[3])
        act[pl.ds(OOFF + row, 8), :] = (x1 + _rb(modb[5] * h2)).astype(BF)
        r = jnp.sum(h2 * modb[6], axis=-1, keepdims=True)
        act[ROFF:ROFF + 8, 0:256] = jnp.where(
            lane256 * 8 == row, r, act[ROFF:ROFF + 8, 0:256].astype(F32)).astype(BF)

    def attn_store(a, k0):
        for j in range(a.shape[0] // 8):
            for k in range(a.shape[1] // 128):
                qkvbufs[A_BUF[j]][NSLOT, (k0 + k) * 8:(k0 + k + 1) * 8, :] = pltpu.bitcast(
                    a[8 * j:8 * j + 8, k * 128:(k + 1) * 128], U32)

    def attn_load(j):
        return pltpu.bitcast(jnp.concatenate(
            [qkvbufs[A_BUF[j]][NSLOT, k * 8:(k + 1) * 8, :] for k in range(8)], axis=1), F32)

    act[ROFF:ROFF + 8, 0:256] = jnp.zeros((8, 256), BF)
    attn_store(jnp.zeros((NEW, D), F32), 0)
    for s_ in range(NSEG):
        for k, v in enumerate(_step_indices(s_)):
            tab[s_ * NTAB + k] = v
    ri = lax.broadcasted_iota(jnp.int32, (80, 80), 0)
    ci = lax.broadcasted_iota(jnp.int32, (80, 80), 1)

    def head_pos(i):
        hd = jnp.where(i < 16, i // 8, (i - 16) // 32)
        pos = jnp.where(i < 16, i % 8, 8 + (i - 16) % 32)
        return hd, pos
    rh, rp = head_pos(ri)
    ch, cpos = head_pos(ci)
    same = rh == ch
    valid = same & ((rp < M) | (rp >= cpos))
    fill = jnp.where(same, -1e9, -jnp.inf).astype(F32)

    cp_mem.wait()
    cp_wr.wait()
    modb[6] = jnp.broadcast_to(wrbuf[...].astype(F32).reshape(1, D), (8, D))
    cp_c.wait()
    cv = cbuf[...].astype(F32)
    sc_row = _rb(cv * _rb(jax.nn.sigmoid(cv)))
    sc16 = jnp.broadcast_to(sc_row, (16, D)).astype(BF)
    for k in range(8):
        scol[k * 64:(k + 1) * 64, :] = _pack(
            jnp.broadcast_to(sc_row[:, k * 128:(k + 1) * 128], (128, 128)).T)

    def ln_pre(g, carry):
        pltpu.make_async_copy(x_hbm.at[0, 0:128], xbuf.at[pl.ds(pl.multiple_of(g * 128, 128), 128)],
                              sems.at[13 + g]).wait()
        for u in range(2):
            row = pl.multiple_of(g * 128 + u * 64, 64)
            nv = _layernorm(xbuf[pl.ds(row, 64), :].astype(F32)).astype(BF)
            for k in range(8):
                h0buf[k, pl.ds(pl.multiple_of(row // 2, 32), 32), :] = pltpu.bitcast(
                    nv[:, k * 128:(k + 1) * 128], U32)
            wg_v[pl.ds(row, 64), 0:2 * D] = jnp.zeros((64, 2 * D), U32)
        return carry
    lax.fori_loop(0, PRE // 128, ln_pre, 0)

    def mod_tile(v, col):
        w = pltpu.bitcast(wmod_v[v, :, pl.ds(col, 128)], BF)
        return _rb(jnp.dot(sc16, w, preferred_element_type=F32))[0:8]

    def moda_store(kc, sa, ca):
        col = mult(kc * 128, 128)
        c1 = _rb(1.0 + ca)
        modb[0, :, pl.ds(col, 128)] = sa
        modb[1, :, pl.ds(col, 128)] = c1
        return sa, c1

    def moda_apply(kc, sa, c1, r0, r1):
        for r in range(r0, r1, 16):
            nv = pltpu.bitcast(h0buf[kc, r // 2:r // 2 + 8, :], BF).astype(F32).reshape(2, 8, 128)
            hv = (_rb(nv * c1[None]) + sa[None]).reshape(16, 128).astype(BF)
            h0buf[kc, r // 2:r // 2 + 8, :] = pltpu.bitcast(hv, U32)

    def repack(a, b):
        return (a & U32(0xFFFF)) | (b << 16), (a >> 16) | (b & U32(0xFFFF0000))

    def store_qkv(i, jrow, y, seg0):
        for sg in range(y.shape[0] // 32):
            for hh in range(2):
                qkvbufs[i][seg0 + sg, pl.ds(jrow + 8 + hh * 16, 16), :] = _pack(
                    y[sg * 32:(sg + 1) * 32, hh * 128:(hh + 1) * 128])

    for c_ in chunk_copies(2):
        c_.start()
    for c_ in moda_copies(0):
        c_.wait()
    moda_apply(0, *moda_store(0, mod_tile(0, 0), mod_tile(1, 0)), 0, PRE)
    w_start(1, 0, PRE_SPLIT, prio=1)

    for c_ in cp_early:
        c_.wait()
    for i in range(NB):
        lo, hi = repack(w_v[i * 6 + 2, 0:64, :], w_v[i * 6 + 3, 0:64, :])
        w_v[i * 6 + 2, 0:64, :] = lo
        w_v[i * 6 + 3, 0:64, :] = hi
        wu_v[0:PRE, i * 256:(i + 1) * 256] = pltpu.bitcast(jnp.dot(
            pltpu.bitcast(h0buf[0], BF), pltpu.bitcast(jnp.concatenate([lo, hi], axis=1), BF),
            preferred_element_type=F32), U32)

    def w_wait(j, i0, i1, r0=0):
        blk0 = (j // 3) * (6 * NB) + (j % 3) * 2
        for i in range(i0, i1):
            for par in range(2):
                pltpu.make_async_copy(w_hbms[0].at[r0:, 0, 0, :], w_v.at[blk0 + i * 6 + par, r0:],
                                      wsems.at[2 * j + (i >= PRE_SPLIT)]).wait()

    def chunk_block(kc, last, issue):
        for c_ in chunk_copies(kc) + ([cp_xr] if last else moda_copies(kc + 1)):
            c_.wait()
        issue()
        r0 = mult(kc * 64, 64)
        mv = []
        for i in range(NB):
            lo, hi = repack(w_v[i * 6, pl.ds(r0, 64), :], w_v[i * 6 + 1, pl.ds(r0, 64), :])
            w_v[i * 6, pl.ds(r0, 64), :] = lo
            w_v[i * 6 + 1, pl.ds(r0, 64), :] = hi
            w = pltpu.bitcast(jnp.concatenate([lo, hi], axis=1), BF)
            y = (pltpu.bitcast(wg_v[0:PRE, i * 256:(i + 1) * 256], F32)
                 + jnp.dot(pltpu.bitcast(h0buf[kc], BF), w, preferred_element_type=F32))
            if last:
                store_qkv(i, 0, y, 0)
            else:
                wg_v[0:PRE, i * 256:(i + 1) * 256] = pltpu.bitcast(y, U32)
                if i in (1, 3):
                    mv.append(mod_tile(i // 2, mult((kc + 1) * 128, 128)))
                if i == 3:
                    mv = moda_store(kc + 1, mv[0], mv[1])
                if i in (4, 6):
                    zeros = qkvbufs[A_BUF[0]][NSLOT, 0:8, :]
                    for q in range(APPLY_N):
                        yr = (q + 1) * (PRE // (APPLY_N + 1)) // 8 * 8
                        tok = pltpu.bitcast(y[yr:yr + 8, 0:128], U32) & zeros
                        c1 = pltpu.bitcast(pltpu.bitcast(mv[1], U32) | tok, F32)
                        n = PRE // 2 // APPLY_N
                        r_ = (i - 4) // 2 * (PRE // 2) + q * n
                        moda_apply(kc + 1, mv[0], c1, r_, r_ + n)
        if last:
            for j in range(3):
                ln1_rows(PRE + 8 * j, HOFF + 8 + 8 * j)

    def chunk_body(kc, carry):
        def issue():
            @pl.when(kc < 5)
            def _():
                for c_ in moda_copies(kc + 3) + chunk_copies(kc + 3):
                    c_.start()
        chunk_block(kc, False, issue)
        return carry

    def issue_last():
        w_wait(1, 0, PRE_SPLIT, 64)
        w_start(1, PRE_SPLIT, NB)
        w_start(2)
        mod_copy(2).start()
    lax.fori_loop(0, 7, chunk_body, 0)
    chunk_block(7, True, issue_last)

    def pre_unit(j, i, extra, k0=0):
        blk = (j // 3) * (6 * NB) + (j % 3) * 2 + i * 6
        jrow = mult(j * 40, 8)
        r0 = k0 * 64
        lo, hi = repack(w_v[blk, r0:, :], w_v[blk + 1, r0:, :])
        w_v[blk, r0:, :] = lo
        w_v[blk + 1, r0:, :] = hi
        for rc in range(PRE // 128):
            if rc > 0:
                lo = w_v[blk, r0:, :]
                hi = w_v[blk + 1, r0:, :]
            w = pltpu.bitcast(jnp.concatenate([lo, hi], axis=1), BF)
            lhs = jnp.concatenate(
                [h0buf[k, rc * 64:(rc + 1) * 64, :] for k in range(k0, 8)], axis=1)
            y = jnp.dot(pltpu.bitcast(lhs, BF), w, preferred_element_type=F32)
            if k0:
                y = y + pltpu.bitcast(wu_v[rc * 128:(rc + 1) * 128, i * 256:(i + 1) * 256], F32)
            store_qkv(i, jrow, y, rc * 4)
            extra(rc, y)

    for i in range(NB):
        if i == PRE_SPLIT:
            w_wait(1, PRE_SPLIT, NB, 64)
            for jn in (3, 4):
                w_start(jn)
                mod_copy(jn).start()
        pre_unit(1, i, lambda rc, y: None, k0=1)
    w_start(5)
    mod_copy(5).start()
    cp_wo.start()
    cp_x1.start()

    def pre_body(j, carry):
        w_wait(j, 0, NB)
        pltpu.make_async_copy(wmod32.at[:, 0:D], wmod_v.at[j], wsems.at[2 * j + 1]).wait()
        zeros = qkvbufs[A_BUF[0]][NSLOT, 0:8, :]

        def halves(u):
            return (pltpu.bitcast(u << 16, F32), pltpu.bitcast(u & U32(0xFFFF0000), F32))
        for i in range(NB):
            def extra(rc, y, i=i):
                for u in range(2):
                    b = (i * 4 + rc) * 2 + u
                    tok = pltpu.bitcast(y[0:8, u * 128:(u + 1) * 128], U32) & zeros
                    for cs in (slice(0, HD), slice(HD, D)):
                        se, so = halves(scol[b * 8:(b + 1) * 8, :] | tok)
                        we, wo = halves(wmod_v[j, b * 8:(b + 1) * 8, cs])
                        t = (we * jnp.concatenate([se] * 4, axis=1)
                             + wo * jnp.concatenate([so] * 4, axis=1))
                        macc[:, cs] = t + macc[:, cs] if b else t
            pre_unit(j, i, extra)
        one = jnp.where(j == 4, 1.0, 0.0).astype(F32)
        mv = _rb(jnp.sum(macc[...], axis=0, keepdims=True))
        modb[j] = jnp.broadcast_to(_rb(one + mv), (8, D))
        return carry
    lax.fori_loop(2, 6, pre_body, 0)

    cp_wo.wait()
    cp_x1.wait()
    for c_ in cp_ffn:
        c_.start()

    def wo_w(q0, q1, n0, n1):
        h0, h1 = q0 + 2 * ROT, q1 + 2 * ROT
        ws = [wo_v[a:b, :, n0 * 128:n1 * 128].reshape((b - a) * (DH // 2), (n1 - n0) * 128)
              for a, b in ((h0, min(h1, H)), (0, h1 - H)) if b > a]
        return pltpu.bitcast(jnp.concatenate(ws, axis=0), BF)

    def emit_step(it, odd, pend):
        s = 2 * it + odd
        hrow = pl.multiple_of(HOFF + (s & 1) * 32, 32)
        hnext = pl.multiple_of(HOFF + 32 - (s & 1) * 32, 32)
        tv = [tab[s * NTAB + k] for k in range(7)]
        slot = tv[0]
        dsts = [(tv[1 + 2 * j], pl.multiple_of(tv[2 + 2 * j], 4)) for j in range(3)]
        orow, ow = (32, 48) if odd else (0, 32)
        odst = (48, 56, 64, 72) if odd else (8, 16, 24, 40)
        erow = it * 64 if odd else jnp.maximum(it - 1, 0) * 64 + RIDE
        lrow = PRE + jnp.minimum(s + 1, NSEG - 1) * RIDE
        e_at, l_at = (E_AT2, L_AT2) if odd else (E_AT, L_AT)
        probs = {}

        def wqkv(p, k0, k1):
            return pltpu.bitcast(jnp.concatenate(
                [w_v[p * 6 + u, k0 // 2:k1 // 2, :] for u in range(6)], axis=1), BF)

        lhs_lo = act[pl.ds(hrow, 32), 0:HD]
        if pend is not None:
            ybuf[...] = jnp.dot(lhs_lo, wqkv(0, 0, HD), preferred_element_type=F32)
            pend()
        lhs_hi = act[pl.ds(hrow, 32), HD:D]
        if pend is not None:
            y0 = ybuf[...] + jnp.dot(lhs_hi, wqkv(0, HD, D), preferred_element_type=F32)
        lhs_rest = jnp.concatenate([lhs_lo[:, 128:], lhs_hi], axis=1)
        lhs = [jnp.concatenate([lhs_lo, lhs_hi], axis=1)]

        def side(p):
            for j in range(len(e_at)):
                if e_at[j] == p:
                    finish_rows(pl.multiple_of(erow + 8 * j, 8), attn_load(j))
            for j in range(3):
                if l_at[j] == p:
                    ln1_rows(pl.multiple_of(lrow + 8 * j, 8),
                             pl.multiple_of(hnext + 8 + 8 * j, 8))
            if p in e_at or p in l_at:
                lhs[0] = jnp.concatenate([act[pl.ds(hrow, 32), 0:128], lhs_rest], axis=1)

        def qkv(p):
            if p == 0 and pend is not None:
                y = y0
            else:
                y = jnp.dot(lhs[0], wqkv(p, 0, D), preferred_element_type=F32)
            buf = qkvbufs[p % NB]
            for u in range(6):
                t, hh = u // 2, u % 2
                b0 = ((p // NB) * 3 + t) * 40
                yu = y[:, u * 128:(u + 1) * 128]
                buf[slot, b0 + hh * 4:b0 + hh * 4 + 4, :] = _pack(yu[0:8])
                for j in range(3):
                    sl, off = dsts[j]
                    buf[sl, pl.ds(b0 + 8 + hh * 16 + off, 4), :] = _pack(yu[8 + 8 * j:16 + 8 * j])

        def ld(p, t):
            b0 = ((p // NB) * 3 + t) * 40
            return pltpu.bitcast(qkvbufs[p % NB][slot, b0:b0 + 40, :], BF)

        def sc(p):
            s2 = lax.dot_general(ld(p, 0), ld(p, 1), (((1,), (1,)), ((), ())),
                                 preferred_element_type=F32)
            s2 = jnp.where(valid, s2 * SCALE, fill)
            m = jnp.max(s2, axis=-1, keepdims=True)
            e = jnp.exp(s2 - m)
            l = jnp.sum(e, axis=-1, keepdims=True)
            rl = pl.reciprocal(l, approx=True)
            rl = rl * (2.0 - l * rl)
            probs[p] = (e * rl).astype(BF)

        def pv(p):
            o2 = jnp.dot(probs[p], ld(p, 2), preferred_element_type=F32)
            for hh in range(2):
                hcol = (2 * ((p - ROT) % NP) + hh) * 128
                obuf[orow:orow + 8, hcol:hcol + 128] = o2[8 * hh:8 * hh + 8].astype(BF)
                for j in range(4):
                    r0 = 16 + 32 * hh + 8 * j
                    obuf[odst[j]:odst[j] + 8, hcol:hcol + 128] = o2[r0:r0 + 8].astype(BF)

        def attn(pos):
            for kind, p in ATT.get(pos, ()):
                (sc if kind == 's' else pv)(p)

        for p in range(NP):
            qkv(p)
            side(p)
            attn(p)
        a1 = []
        for n in range(8):
            a1.append(jnp.dot(obuf[orow:orow + ow, 0:KS], wo_w(0, KS // DH, n, n + 1),
                              preferred_element_type=F32))
            if n + 1 in W1AT:
                attn(NP + 2 * W1AT.index(n + 1))
        o2lhs = obuf[orow:orow + ow, KS:]
        a_lo = jnp.concatenate(a1[0:4], axis=1) + jnp.dot(
            o2lhs, wo_w(KS // DH, H, 0, 4), preferred_element_type=F32)
        act[pl.ds(hnext, 8), 0:HD] = a_lo[0:8].astype(BF)
        attn_store(a_lo[8:], 0)
        a_hi = jnp.concatenate(a1[4:8], axis=1) + jnp.dot(
            o2lhs, wo_w(KS // DH, H, 4, 8), preferred_element_type=F32)

        def finish():
            act[pl.ds(hnext, 8), HD:D] = a_hi[0:8].astype(BF)
            attn_store(a_hi[8:], 4)
        return finish

    def out_copy(r0, n, sem):
        return cp(act.at[pl.ds(OOFF + r0, n)], out_hbm.at[0, pl.ds(r0, n)], sem)

    def steps(it, carry):
        emit_step(it, 1, emit_step(it, 0, None))()

        @pl.when(it > 0)
        def _():
            out_copy(pl.multiple_of((it - 1) * 64, 64), 64, 9).start()
        return carry
    lax.fori_loop(0, NSEG // 2, steps, 0)

    NEW0 = S - NEW
    out_copy(S - 64, NEW0 - (S - 64), 9).start()
    for c_ in cp_ffn:
        c_.wait()

    def rep(i, n):
        return jnp.concatenate([modb[i]] * n, axis=0)
    r_old = act[ROFF:ROFF + 8, 0:256].astype(F32) + 0.0
    bits = pltpu.bitcast(jnp.broadcast_to(jnp.max(r_old, axis=0, keepdims=True), (8, 256)),
                         jnp.int32)
    code = (bits ^ ((bits >> 31) & 0x7FFFFFFF)) >> 16
    key = jnp.where(lane256 < NEW0 // 8, (code * 256 + (255 - lane256)).astype(F32), -jnp.inf)
    k1 = jnp.max(key, axis=1, keepdims=True)
    k2 = jnp.max(jnp.where(key == k1, -jnp.inf, key), axis=1, keepdims=True)
    rc = jnp.concatenate([jnp.max(jnp.where(key == k, r_old, -jnp.inf), axis=1, keepdims=True)
                          for k in (k1, k2)], axis=0)
    b1, b2 = (pl.multiple_of(jnp.minimum(255 - (k[0, 0].astype(jnp.int32) & 255),
                                         NEW0 // 8 - 1) * 8, 8) for k in (k1, k2))
    ng = NEW // 8
    x1n = _rb(xbuf[NEW0:S, :].astype(F32) + _rb(rep(2, ng) * _rb(
        jnp.concatenate([attn_load(j) for j in range(ng)], axis=0))))
    h2n = _rb(_rb(_layernorm(x1n) * rep(4, ng)) + rep(3, ng))
    rn = _rb(jnp.sum(h2n * rep(6, ng), axis=-1, keepdims=True))
    x1c = jnp.concatenate([act[pl.ds(b1, 8), :].astype(F32), act[pl.ds(b2, 8), :].astype(F32)],
                          axis=0)
    h2c = _rb(_rb(_layernorm(x1c) * rep(4, 2)) + rep(3, 2))
    subf = lax.broadcasted_iota(jnp.int32, (8, 1), 0).astype(F32)
    b1f = b1.astype(F32)
    val = jnp.concatenate([rc, rn], axis=0)
    idx = jnp.concatenate([subf + b1f, subf + b2.astype(F32)]
                          + [subf + float(NEW0 + 8 * j) for j in range(ng)], axis=0)
    v1 = jnp.max(val, axis=0, keepdims=True)
    t1 = jnp.min(jnp.where(val == v1, idx, float(S)), axis=0, keepdims=True)
    rest = jnp.where(idx == t1, -jnp.inf, val)
    v2 = jnp.max(rest, axis=0, keepdims=True)
    t2 = jnp.min(jnp.where((rest == v2) & (idx != t1), idx, float(S)), axis=0, keepdims=True)

    def pick(t, old2, new):
        out = jnp.where((t >= b1f) & (t < b1f + 8.0), old2[0:8], old2[8:16])
        for j in range(ng):
            out = jnp.where(t >= float(NEW0 + 8 * j), new[8 * j:8 * j + 8], out)
        return out
    h2s = jnp.concatenate([pick(t1, h2c, h2n), pick(t2, h2c, h2n)], axis=0)
    h2b = h2s.astype(BF)
    hid = []
    for n in range(0, F, FFN_NB):
        gt = _rb(jnp.dot(h2b, pltpu.bitcast(wg_v[:, n:n + FFN_NB], BF), preferred_element_type=F32))
        up = _rb(jnp.dot(h2b, pltpu.bitcast(wu_v[:, n:n + FFN_NB], BF), preferred_element_type=F32))
        hid.append((_rb(gt * _rb(jax.nn.sigmoid(gt))) * up).astype(BF))
    y = _rb(jnp.dot(jnp.concatenate(hid, axis=1), pltpu.bitcast(wd_v[...], BF),
                    preferred_element_type=F32))
    act[OOFF + NEW0:OOFF + S, :] = (x1n + _rb(rep(5, ng) * h2n)).astype(BF)
    x1s = jnp.concatenate([pick(t1, x1c, x1n), pick(t2, x1c, x1n)], axis=0)
    c1, c2 = (pl.multiple_of((jnp.clip(t[0, 0].astype(jnp.int32), 0, S - 1) >> 3) * 8, 8)
              for t in (t1, t2))
    tok = jnp.concatenate([subf + c1.astype(F32), subf + c2.astype(F32)], axis=0)
    is1, is2 = tok == t1, tok == t2
    gate = _rb(jax.nn.sigmoid(jnp.where(is1, v1, v2)))
    upd = jnp.where(is1 | is2, _rb(y * gate), 0.0)
    res = (x1s + _rb(rep(5, 2) * _rb(h2s + upd))).astype(BF)
    out_copy(0, NEW0, 9).wait()
    act[pl.ds(OOFF + c1, 8), :] = res[0:8]
    act[pl.ds(OOFF + c2, 8), :] = res[8:16]
    fix0 = out_copy(NEW0, NEW, 6)
    fix1 = out_copy(c1, 8, 11)
    fix2 = out_copy(c2, 8, 12)
    send1 = c1 < NEW0
    send2 = (c2 < NEW0) & (c2 != c1)
    fix0.start()
    pl.when(send1)(fix1.start)
    pl.when(send2)(fix2.start)
    pl.when(send1)(fix1.wait)
    pl.when(send2)(fix2.wait)
    fix0.wait()


@jax.jit
def pallas_adaLN_cond__memory_aug_recurrent_mem_tr__moe_arch_mod__prompt_kernel(
    A_x: jax.Array,
    A_mem0: jax.Array,
    A_Wq: jax.Array,
    A_Wk: jax.Array,
    A_Wv: jax.Array,
    A_Wo: jax.Array,
    A_seg_len,
    B_x: jax.Array,
    B_w_r: jax.Array,
    B_w_gate: jax.Array,
    B_w_up: jax.Array,
    B_w_down: jax.Array,
    c: jax.Array,
    w_mod: jax.Array,
):
    del B_x
    del A_seg_len
    assert A_x.shape == (1, S, D) and A_Wq.shape == (D, H, DH) and A_mem0.shape == (1, M, D)
    any_spec = pl.BlockSpec(memory_space=pl.ANY)
    scratch = [
        pltpu.VMEM((S, D), BF),
        pltpu.VMEM((ACT_ROWS, D), BF),
        pltpu.VMEM((8, PRE // 2, 128), U32),
        pltpu.VMEM((32, 768), F32),
        pltpu.VMEM((D // 2, 128), U32),
        pltpu.VMEM((8, D), F32),
        pltpu.SMEM((NSEG * NTAB,), jnp.int32),
        pltpu.VMEM((7, 8, D), F32),
        pltpu.VMEM((3 * H, D // 2, 128), U32),
        pltpu.VMEM((H, DH // 2, D), U32),
        pltpu.VMEM((6, D // 2, D), U32),
        pltpu.VMEM((D // 2, F), U32),
        pltpu.VMEM((D // 2, F), U32),
        pltpu.VMEM((F // 2, D), U32),
        pltpu.VMEM((80, H * DH), BF),
        pltpu.SemaphoreType.DMA((17,)),
        pltpu.SemaphoreType.DMA((12,)),
        pltpu.SemaphoreType.DMA((16,)),
    ] + [pltpu.VMEM((NSLOT + 1, 256, 128), U32) for _ in range(NB)] + [
        pltpu.VMEM((1, D), BF),
        pltpu.VMEM((D,), BF),
    ]
    wq, wk, wv = (w.reshape(D // 2, 2, H, DH) for w in (A_Wq, A_Wk, A_Wv))
    return pl.pallas_call(
        _kernel,
        out_shape=jax.ShapeDtypeStruct((1, S, D), BF),
        in_specs=[any_spec] * 12,
        out_specs=any_spec,
        scratch_shapes=scratch,
        compiler_params=pltpu.CompilerParams(vmem_limit_bytes=120 * 1024 * 1024,
                                             disable_bounds_checks=True,
                                             disable_semaphore_checks=True),
    )(A_x, A_mem0, wq, wk, wv, A_Wo, B_w_r, B_w_gate, B_w_up, B_w_down,
      c, w_mod)
```

```python
import jax
import jax.numpy as jnp
from jax import lax
import jax.experimental.pallas as pl
import jax.experimental.pallas.tpu as pltpu

BF = jnp.bfloat16
F32 = jnp.float32
U32 = jnp.uint32

S = 2048
D = 1024
H = 32
DH = 128
M = 8
SEG = 32
NSEG = S // SEG
F = 3584
NP = H // 2
EPS = 1e-5
SCALE = DH ** -0.5
HD = D // 2

RIDE = 24
PRE = S - NSEG * RIDE
NSLOT = 17
NB = 8
KS = 2048
OOFF = S
HOFF = 2 * S
ROFF = HOFF + 64
ACT_ROWS = ROFF + 16
PRE_SPLIT = 3
E_AT = (2, 3, 4, 5, 6)
E_AT2 = (3, 4, 5)
L_AT = (6, 7, 8)
L_AT2 = (6, 8, 10)
A_BUF = (7, 0, 1, 2, 3)
W1AT = (2, 6)
NEW = 40
FFN_NB = 512
APPLY_N = 4
MOD_YR = 64
NTAB = 8

ROT = 2
ATT = {4: [('s', i) for i in range(4)],
       18: [('p', (12 + ROT + i) % NP) for i in range(4)]}
for _p in range(4, NP, 2):
    ATT[_p + 2] = [('s', _p), ('s', _p + 1), ('p', _p - 4 + ROT), ('p', _p - 3 + ROT)]


def _step_indices(s):
    t = [s % NSLOT]
    for j in range(3):
        gi = PRE // 8 + 3 * s + j
        t += [(gi // 4) % NSLOT, (gi % 4) * 4]
    return t


def _rb(v):
    return v.astype(BF).astype(F32)


def _pack(v):
    return pltpu.bitcast(v.astype(BF), U32)


def _layernorm(x):
    mu = jnp.sum(x, axis=-1, keepdims=True) * (1.0 / D)
    xc = x - mu
    var = jnp.sum(xc * xc, axis=-1, keepdims=True) * (1.0 / D)
    sd = _rb(jnp.sqrt(_rb(_rb(var) + EPS)))
    return _rb(_rb(x - _rb(mu)) / sd)


def _kernel(x_hbm, mem0_hbm, wq_hbm, wk_hbm, wv_hbm, wo_hbm, wr_hbm, wg_hbm, wu_hbm,
            wd_hbm, c_hbm, wmod_hbm, out_hbm,
            xbuf, act, h0buf, ybuf, scol, macc, tab, modb,
            w_v, wo_v, wmod_v, wg_v, wu_v, wd_v,
            obuf, sems, wsems, ksems, *rest):
    qkvbufs, cbuf, wrbuf = rest[:NB], rest[NB], rest[NB + 1]
    w_hbms = tuple(w.bitcast(U32) for w in (wq_hbm, wk_hbm, wv_hbm))

    def cp(src, dst, i):
        return pltpu.make_async_copy(src, dst, sems.at[i])

    wmod32 = wmod_hbm.bitcast(U32)
    cp_c = cp(c_hbm, cbuf, 0)
    cp_mem = cp(mem0_hbm.at[0], act.at[HOFF:HOFF + M], 1)
    cp_wr = cp(wr_hbm, wrbuf, 2)
    cp_x0 = [cp(x_hbm.at[0, n * 128:(n + 1) * 128], xbuf.at[n * 128:(n + 1) * 128], 13 + n)
             for n in range(PRE // 128)]
    cp_xr = cp(x_hbm.at[0, PRE:PRE + 32], xbuf.at[PRE:PRE + 32], 5)
    cp_x1 = cp(x_hbm.at[0, PRE + 32:S], xbuf.at[PRE + 32:S], 4)
    cp_wo = cp(wo_hbm.bitcast(U32), wo_v, 7)
    cp_ffn = [cp(wg_hbm.bitcast(U32), wg_v, 8), cp(wu_hbm.bitcast(U32), wu_v, 8),
              cp(wd_hbm.bitcast(U32), wd_v, 8)]

    def w_start(j, i0=0, i1=NB, prio=0):
        gg, t = j // 3, j % 3
        r0 = 64 if j == 1 else 0
        for i in range(i0, i1):
            for par in range(2):
                pltpu.make_async_copy(w_hbms[t].at[r0:, par, gg * NB + i, :],
                                      w_v.at[(gg * NB + i) * 6 + t * 2 + par, r0:],
                                      wsems.at[2 * j + (i >= PRE_SPLIT)]).start(priority=prio)

    def mod_copy(v):
        return pltpu.make_async_copy(wmod32.at[:, v * D:(v + 1) * D], wmod_v.at[v],
                                     wsems.at[2 * (3 + v // 2) + 1])

    def mult(v, m):
        return v if isinstance(v, int) else pl.multiple_of(v, m)

    def moda_copies(kc):
        col = mult(kc * 128, 128)
        return [pltpu.make_async_copy(wmod32.at[:, pl.ds(v * D + col, 128)],
                                      wmod_v.at[v, :, pl.ds(col, 128)], ksems.at[8 + kc])
                for v in range(2)]

    def chunk_copies(kc):
        r0 = mult(kc * 64, 64)
        return [pltpu.make_async_copy(w_hbms[0].at[pl.ds(r0, 64), par, i, :],
                                      w_v.at[i * 6 + par, pl.ds(r0, 64), :], ksems.at[kc])
                for i in range(NB) for par in range(2)]

    cp_early = [cp(w_hbms[1].at[0:64, par, i, :], w_v.at[i * 6 + 2 + par, 0:64], 3)
                for i in range(NB) for par in range(2)]

    cp_c.start()
    cp_mem.start()
    cp_wr.start()
    for c_ in (cp_x0 + moda_copies(0) + cp_early + moda_copies(1) + chunk_copies(0)
               + moda_copies(2) + chunk_copies(1) + [cp_xr]):
        c_.start()

    def ln1_rows(src_row, dst_row):
        xv = xbuf[pl.ds(src_row, 8), :].astype(F32)
        hv = _rb(_layernorm(xv) * modb[1]) + modb[0]
        act[pl.ds(dst_row, 8), :] = hv.astype(BF)

    lane256 = lax.broadcasted_iota(jnp.int32, (8, 256), 1)

    def finish_rows(row, attn):
        xv = xbuf[pl.ds(row, 8), :].astype(F32)
        x1 = _rb(xv + _rb(modb[2] * _rb(attn)))
        act[pl.ds(row, 8), :] = x1.astype(BF)
        h2 = _rb(_rb(_layernorm(x1) * modb[4]) + modb[3])
        act[pl.ds(OOFF + row, 8), :] = (x1 + _rb(modb[5] * h2)).astype(BF)
        r = jnp.sum(h2 * modb[6], axis=-1, keepdims=True)
        act[ROFF:ROFF + 8, 0:256] = jnp.where(
            lane256 * 8 == row, r, act[ROFF:ROFF + 8, 0:256].astype(F32)).astype(BF)

    def attn_store(a, k0):
        for j in range(a.shape[0] // 8):
            for k in range(a.shape[1] // 128):
                qkvbufs[A_BUF[j]][NSLOT, (k0 + k) * 8:(k0 + k + 1) * 8, :] = pltpu.bitcast(
                    a[8 * j:8 * j + 8, k * 128:(k + 1) * 128], U32)

    def attn_load(j):
        return pltpu.bitcast(jnp.concatenate(
            [qkvbufs[A_BUF[j]][NSLOT, k * 8:(k + 1) * 8, :] for k in range(8)], axis=1), F32)

    act[ROFF:ROFF + 8, 0:256] = jnp.zeros((8, 256), BF)
    attn_store(jnp.zeros((NEW, D), F32), 0)
    for s_ in range(NSEG):
        for k, v in enumerate(_step_indices(s_)):
            tab[s_ * NTAB + k] = v
    ri = lax.broadcasted_iota(jnp.int32, (80, 80), 0)
    ci = lax.broadcasted_iota(jnp.int32, (80, 80), 1)

    def head_pos(i):
        hd = jnp.where(i < 16, i // 8, (i - 16) // 32)
        pos = jnp.where(i < 16, i % 8, 8 + (i - 16) % 32)
        return hd, pos
    rh, rp = head_pos(ri)
    ch, cpos = head_pos(ci)
    same = rh == ch
    valid = same & ((rp < M) | (rp >= cpos))
    fill = jnp.where(same, -1e9, -jnp.inf).astype(F32)

    cp_mem.wait()
    cp_wr.wait()
    modb[6] = jnp.broadcast_to(wrbuf[...].astype(F32).reshape(1, D), (8, D))
    cp_c.wait()
    cv = cbuf[...].astype(F32)
    sc_row = _rb(cv * _rb(jax.nn.sigmoid(cv)))
    sc16 = jnp.broadcast_to(sc_row, (16, D)).astype(BF)
    for k in range(8):
        scol[k * 64:(k + 1) * 64, :] = _pack(
            jnp.broadcast_to(sc_row[:, k * 128:(k + 1) * 128], (128, 128)).T)

    def ln_pre(g, carry):
        pltpu.make_async_copy(x_hbm.at[0, 0:128], xbuf.at[pl.ds(pl.multiple_of(g * 128, 128), 128)],
                              sems.at[13 + g]).wait()
        for u in range(2):
            row = pl.multiple_of(g * 128 + u * 64, 64)
            nv = _layernorm(xbuf[pl.ds(row, 64), :].astype(F32)).astype(BF)
            for k in range(8):
                h0buf[k, pl.ds(pl.multiple_of(row // 2, 32), 32), :] = pltpu.bitcast(
                    nv[:, k * 128:(k + 1) * 128], U32)
            wg_v[pl.ds(row, 64), 0:2 * D] = jnp.zeros((64, 2 * D), U32)
        return carry
    lax.fori_loop(0, PRE // 128, ln_pre, 0)

    def mod_tile(v, col):
        w = pltpu.bitcast(wmod_v[v, :, pl.ds(col, 128)], BF)
        return _rb(jnp.dot(sc16, w, preferred_element_type=F32))[0:8]

    def moda_store(kc, sa, ca):
        col = mult(kc * 128, 128)
        c1 = _rb(1.0 + ca)
        modb[0, :, pl.ds(col, 128)] = sa
        modb[1, :, pl.ds(col, 128)] = c1
        return sa, c1

    def moda_apply(kc, sa, c1, r0, r1):
        for r in range(r0, r1, 16):
            nv = pltpu.bitcast(h0buf[kc, r // 2:r // 2 + 8, :], BF).astype(F32).reshape(2, 8, 128)
            hv = (_rb(nv * c1[None]) + sa[None]).reshape(16, 128).astype(BF)
            h0buf[kc, r // 2:r // 2 + 8, :] = pltpu.bitcast(hv, U32)

    def halves(u):
        return pltpu.bitcast(u << 16, F32), pltpu.bitcast(u & U32(0xFFFF0000), F32)

    def repack(a, b):
        return (a & U32(0xFFFF)) | (b << 16), (a >> 16) | (b & U32(0xFFFF0000))

    def store_qkv(i, jrow, y, seg0):
        for sg in range(y.shape[0] // 32):
            for hh in range(2):
                qkvbufs[i][seg0 + sg, pl.ds(jrow + 8 + hh * 16, 16), :] = _pack(
                    y[sg * 32:(sg + 1) * 32, hh * 128:(hh + 1) * 128])

    for c_ in chunk_copies(2):
        c_.start()
    for c_ in moda_copies(0):
        c_.wait()
    moda_apply(0, *moda_store(0, mod_tile(0, 0), mod_tile(1, 0)), 0, PRE)
    w_start(1, 0, PRE_SPLIT, prio=1)

    for c_ in cp_early:
        c_.wait()
    for i in range(NB):
        lo, hi = repack(w_v[i * 6 + 2, 0:64, :], w_v[i * 6 + 3, 0:64, :])
        w_v[i * 6 + 2, 0:64, :] = lo
        w_v[i * 6 + 3, 0:64, :] = hi
        wu_v[0:PRE, i * 256:(i + 1) * 256] = pltpu.bitcast(jnp.dot(
            pltpu.bitcast(h0buf[0], BF), pltpu.bitcast(jnp.concatenate([lo, hi], axis=1), BF),
            preferred_element_type=F32), U32)

    def w_wait(j, i0, i1, r0=0):
        blk0 = (j // 3) * (6 * NB) + (j % 3) * 2
        for i in range(i0, i1):
            for par in range(2):
                pltpu.make_async_copy(w_hbms[0].at[r0:, 0, 0, :], w_v.at[blk0 + i * 6 + par, r0:],
                                      wsems.at[2 * j + (i >= PRE_SPLIT)]).wait()

    def chunk_block(kc, last, issue):
        for c_ in chunk_copies(kc) + ([cp_xr] if last else moda_copies(kc + 1)):
            c_.wait()
        issue()
        r0 = mult(kc * 64, 64)
        mv = []
        for i in range(NB):
            lo, hi = repack(w_v[i * 6, pl.ds(r0, 64), :], w_v[i * 6 + 1, pl.ds(r0, 64), :])
            w_v[i * 6, pl.ds(r0, 64), :] = lo
            w_v[i * 6 + 1, pl.ds(r0, 64), :] = hi
            w = pltpu.bitcast(jnp.concatenate([lo, hi], axis=1), BF)
            y = (pltpu.bitcast(wg_v[0:PRE, i * 256:(i + 1) * 256], F32)
                 + jnp.dot(pltpu.bitcast(h0buf[kc], BF), w, preferred_element_type=F32))
            if last:
                store_qkv(i, 0, y, 0)
            else:
                wg_v[0:PRE, i * 256:(i + 1) * 256] = pltpu.bitcast(y, U32)
                if i in (1, 3):
                    mv.append(mod_tile(i // 2, mult((kc + 1) * 128, 128)))
                if i == 3:
                    mv = moda_store(kc + 1, mv[0], mv[1])
                if i in (4, 6):
                    zeros = qkvbufs[A_BUF[0]][NSLOT, 0:8, :]
                    for q in range(APPLY_N):
                        yr = (q + 1) * (PRE // (APPLY_N + 1)) // 8 * 8
                        tok = pltpu.bitcast(y[yr:yr + 8, 0:128], U32) & zeros
                        c1 = pltpu.bitcast(pltpu.bitcast(mv[1], U32) | tok, F32)
                        n = PRE // 2 // APPLY_N
                        r_ = (i - 4) // 2 * (PRE // 2) + q * n
                        moda_apply(kc + 1, mv[0], c1, r_, r_ + n)
        if last:
            for j in range(3):
                ln1_rows(PRE + 8 * j, HOFF + 8 + 8 * j)

    def chunk_body(kc, carry):
        def issue():
            @pl.when(kc < 5)
            def _():
                for c_ in moda_copies(kc + 3) + chunk_copies(kc + 3):
                    c_.start()
        chunk_block(kc, False, issue)
        return carry

    def issue_last():
        w_wait(1, 0, PRE_SPLIT, 64)
        w_start(1, PRE_SPLIT, NB)
        w_start(2)
    lax.fori_loop(0, 7, chunk_body, 0)
    chunk_block(7, True, issue_last)

    def pre_unit(j, i, extra, k0=0):
        blk = (j // 3) * (6 * NB) + (j % 3) * 2 + i * 6
        jrow = mult(j * 40, 8)
        r0 = k0 * 64
        lo, hi = repack(w_v[blk, r0:, :], w_v[blk + 1, r0:, :])
        w_v[blk, r0:, :] = lo
        w_v[blk + 1, r0:, :] = hi
        for rc in range(PRE // 128):
            if rc > 0:
                lo = w_v[blk, r0:, :]
                hi = w_v[blk + 1, r0:, :]
            w = pltpu.bitcast(jnp.concatenate([lo, hi], axis=1), BF)
            lhs = jnp.concatenate(
                [h0buf[k, rc * 64:(rc + 1) * 64, :] for k in range(k0, 8)], axis=1)
            y = jnp.dot(pltpu.bitcast(lhs, BF), w, preferred_element_type=F32)
            if k0:
                y = y + pltpu.bitcast(wu_v[rc * 128:(rc + 1) * 128, i * 256:(i + 1) * 256], F32)
            store_qkv(i, jrow, y, rc * 4)
            extra(rc, y)

    for i in range(NB):
        if i == PRE_SPLIT:
            w_wait(1, PRE_SPLIT, NB, 64)
            w_start(3)
            w_start(4)
            mod_copy(2).start()
            mod_copy(3).start()
        pre_unit(1, i, lambda rc, y: None, k0=1)
    w_start(5)
    mod_copy(4).start()
    mod_copy(5).start()
    cp_wo.start()
    cp_x1.start()

    def pre_body(j, carry):
        w_wait(j, 0, NB)
        v0 = jnp.maximum(j - 3, 0) * 2

        @pl.when(j >= 4)
        def _():
            for v in range(2):
                pltpu.make_async_copy(wmod32.at[:, 0:D], wmod_v.at[v0 + v],
                                      wsems.at[2 * j + 1]).wait()
        zeros = qkvbufs[A_BUF[0]][NSLOT, 0:8, :]
        for i in range(NB):
            def extra(rc, y, i=i):
                for u in range(2):
                    b = (i * 4 + rc) * 2 + u
                    for v in range(2):
                        tok = pltpu.bitcast(
                            y[v * MOD_YR:v * MOD_YR + 8, u * 128:(u + 1) * 128], U32) & zeros
                        for cs in (slice(0, HD), slice(HD, D)):
                            se, so = halves(scol[b * 8:(b + 1) * 8, :] | tok)
                            we, wo = halves(wmod_v[v0 + v, b * 8:(b + 1) * 8, cs])
                            t = (we * jnp.concatenate([se] * 4, axis=1)
                                 + wo * jnp.concatenate([so] * 4, axis=1))
                            macc[v, :, cs] = t + macc[v, :, cs] if b else t
            pre_unit(j, i, extra)
        dst = jnp.where(j >= 4, v0, 7)
        for v in range(2):
            mv = _rb(jnp.sum(macc[v], axis=0, keepdims=True))
            if v == 0:
                mv = _rb(jnp.where(j == 5, 1.0, 0.0).astype(F32) + mv)
            modb[dst + v] = jnp.broadcast_to(mv, (8, D))
        return carry
    lax.fori_loop(2, 6, pre_body, 0)

    cp_wo.wait()
    cp_x1.wait()
    for c_ in cp_ffn:
        c_.start()

    def wo_w(q0, q1, n0, n1):
        h0, h1 = q0 + 2 * ROT, q1 + 2 * ROT
        ws = [wo_v[a:b, :, n0 * 128:n1 * 128].reshape((b - a) * (DH // 2), (n1 - n0) * 128)
              for a, b in ((h0, min(h1, H)), (0, h1 - H)) if b > a]
        return pltpu.bitcast(jnp.concatenate(ws, axis=0), BF)

    def emit_step(it, odd, pend):
        s = 2 * it + odd
        hrow = pl.multiple_of(HOFF + (s & 1) * 32, 32)
        hnext = pl.multiple_of(HOFF + 32 - (s & 1) * 32, 32)
        tv = [tab[s * NTAB + k] for k in range(7)]
        slot = tv[0]
        dsts = [(tv[1 + 2 * j], pl.multiple_of(tv[2 + 2 * j], 4)) for j in range(3)]
        orow, ow = (32, 48) if odd else (0, 32)
        odst = (48, 56, 64, 72) if odd else (8, 16, 24, 40)
        erow = it * 64 if odd else jnp.maximum(it - 1, 0) * 64 + RIDE
        lrow = PRE + jnp.minimum(s + 1, NSEG - 1) * RIDE
        e_at, l_at = (E_AT2, L_AT2) if odd else (E_AT, L_AT)
        probs = {}

        def wqkv(p, k0, k1):
            return pltpu.bitcast(jnp.concatenate(
                [w_v[p * 6 + u, k0 // 2:k1 // 2, :] for u in range(6)], axis=1), BF)

        lhs_lo = act[pl.ds(hrow, 32), 0:HD]
        if pend is not None:
            ybuf[...] = jnp.dot(lhs_lo, wqkv(0, 0, HD), preferred_element_type=F32)
            pend()
        lhs_hi = act[pl.ds(hrow, 32), HD:D]
        if pend is not None:
            y0 = ybuf[...] + jnp.dot(lhs_hi, wqkv(0, HD, D), preferred_element_type=F32)
        lhs_rest = jnp.concatenate([lhs_lo[:, 128:], lhs_hi], axis=1)
        lhs = [jnp.concatenate([lhs_lo, lhs_hi], axis=1)]

        def side(p):
            for j in range(len(e_at)):
                if e_at[j] == p:
                    finish_rows(pl.multiple_of(erow + 8 * j, 8), attn_load(j))
            for j in range(3):
                if l_at[j] == p:
                    ln1_rows(pl.multiple_of(lrow + 8 * j, 8),
                             pl.multiple_of(hnext + 8 + 8 * j, 8))
            if p in e_at or p in l_at:
                lhs[0] = jnp.concatenate([act[pl.ds(hrow, 32), 0:128], lhs_rest], axis=1)

        def qkv(p):
            if p == 0 and pend is not None:
                y = y0
            else:
                y = jnp.dot(lhs[0], wqkv(p, 0, D), preferred_element_type=F32)
            buf = qkvbufs[p % NB]
            for u in range(6):
                t, hh = u // 2, u % 2
                b0 = ((p // NB) * 3 + t) * 40
                yu = y[:, u * 128:(u + 1) * 128]
                buf[slot, b0 + hh * 4:b0 + hh * 4 + 4, :] = _pack(yu[0:8])
                for j in range(3):
                    sl, off = dsts[j]
                    buf[sl, pl.ds(b0 + 8 + hh * 16 + off, 4), :] = _pack(yu[8 + 8 * j:16 + 8 * j])

        def ld(p, t):
            b0 = ((p // NB) * 3 + t) * 40
            return pltpu.bitcast(qkvbufs[p % NB][slot, b0:b0 + 40, :], BF)

        def sc(p):
            s2 = lax.dot_general(ld(p, 0), ld(p, 1), (((1,), (1,)), ((), ())),
                                 preferred_element_type=F32)
            s2 = jnp.where(valid, s2 * SCALE, fill)
            m = jnp.max(s2, axis=-1, keepdims=True)
            e = jnp.exp(s2 - m)
            l = jnp.sum(e, axis=-1, keepdims=True)
            rl = pl.reciprocal(l, approx=True)
            rl = rl * (2.0 - l * rl)
            probs[p] = (e * rl).astype(BF)

        def pv(p):
            o2 = jnp.dot(probs[p], ld(p, 2), preferred_element_type=F32)
            for hh in range(2):
                hcol = (2 * ((p - ROT) % NP) + hh) * 128
                obuf[orow:orow + 8, hcol:hcol + 128] = o2[8 * hh:8 * hh + 8].astype(BF)
                for j in range(4):
                    r0 = 16 + 32 * hh + 8 * j
                    obuf[odst[j]:odst[j] + 8, hcol:hcol + 128] = o2[r0:r0 + 8].astype(BF)

        def attn(pos):
            for kind, p in ATT.get(pos, ()):
                (sc if kind == 's' else pv)(p)

        for p in range(NP):
            qkv(p)
            side(p)
            attn(p)
        a1 = []
        for n in range(8):
            a1.append(jnp.dot(obuf[orow:orow + ow, 0:KS], wo_w(0, KS // DH, n, n + 1),
                              preferred_element_type=F32))
            if n + 1 in W1AT:
                attn(NP + 2 * W1AT.index(n + 1))
        o2lhs = obuf[orow:orow + ow, KS:]
        a_lo = jnp.concatenate(a1[0:4], axis=1) + jnp.dot(
            o2lhs, wo_w(KS // DH, H, 0, 4), preferred_element_type=F32)
        act[pl.ds(hnext, 8), 0:HD] = a_lo[0:8].astype(BF)
        attn_store(a_lo[8:], 0)
        a_hi = jnp.concatenate(a1[4:8], axis=1) + jnp.dot(
            o2lhs, wo_w(KS // DH, H, 4, 8), preferred_element_type=F32)

        def finish():
            act[pl.ds(hnext, 8), HD:D] = a_hi[0:8].astype(BF)
            attn_store(a_hi[8:], 4)
        return finish

    def out_copy(r0, n, sem):
        return cp(act.at[pl.ds(OOFF + r0, n)], out_hbm.at[0, pl.ds(r0, n)], sem)

    def steps(it, carry):
        emit_step(it, 1, emit_step(it, 0, None))()

        @pl.when(it > 0)
        def _():
            out_copy(pl.multiple_of((it - 1) * 64, 64), 64, 9).start()
        return carry
    lax.fori_loop(0, NSEG // 2, steps, 0)

    NEW0 = S - NEW
    out_copy(S - 64, NEW0 - (S - 64), 9).start()
    for c_ in cp_ffn:
        c_.wait()

    def rep(i, n):
        return jnp.concatenate([modb[i]] * n, axis=0)
    r_old = act[ROFF:ROFF + 8, 0:256].astype(F32) + 0.0
    bits = pltpu.bitcast(jnp.broadcast_to(jnp.max(r_old, axis=0, keepdims=True), (8, 256)),
                         jnp.int32)
    code = (bits ^ ((bits >> 31) & 0x7FFFFFFF)) >> 16
    key = jnp.where(lane256 < NEW0 // 8, (code * 256 + (255 - lane256)).astype(F32), -jnp.inf)
    k1 = jnp.max(key, axis=1, keepdims=True)
    k2 = jnp.max(jnp.where(key == k1, -jnp.inf, key), axis=1, keepdims=True)
    rc = jnp.concatenate([jnp.max(jnp.where(key == k, r_old, -jnp.inf), axis=1, keepdims=True)
                          for k in (k1, k2)], axis=0)
    b1, b2 = (pl.multiple_of(jnp.minimum(255 - (k[0, 0].astype(jnp.int32) & 255),
                                         NEW0 // 8 - 1) * 8, 8) for k in (k1, k2))
    ng = NEW // 8
    x1n = _rb(xbuf[NEW0:S, :].astype(F32) + _rb(rep(2, ng) * _rb(
        jnp.concatenate([attn_load(j) for j in range(ng)], axis=0))))
    h2n = _rb(_rb(_layernorm(x1n) * rep(4, ng)) + rep(3, ng))
    rn = _rb(jnp.sum(h2n * rep(6, ng), axis=-1, keepdims=True))
    x1c = jnp.concatenate([act[pl.ds(b1, 8), :].astype(F32), act[pl.ds(b2, 8), :].astype(F32)],
                          axis=0)
    h2c = _rb(_rb(_layernorm(x1c) * rep(4, 2)) + rep(3, 2))
    subf = lax.broadcasted_iota(jnp.int32, (8, 1), 0).astype(F32)
    b1f = b1.astype(F32)
    val = jnp.concatenate([rc, rn], axis=0)
    idx = jnp.concatenate([subf + b1f, subf + b2.astype(F32)]
                          + [subf + float(NEW0 + 8 * j) for j in range(ng)], axis=0)
    v1 = jnp.max(val, axis=0, keepdims=True)
    t1 = jnp.min(jnp.where(val == v1, idx, float(S)), axis=0, keepdims=True)
    rest = jnp.where(idx == t1, -jnp.inf, val)
    v2 = jnp.max(rest, axis=0, keepdims=True)
    t2 = jnp.min(jnp.where((rest == v2) & (idx != t1), idx, float(S)), axis=0, keepdims=True)

    def pick(t, old2, new):
        out = jnp.where((t >= b1f) & (t < b1f + 8.0), old2[0:8], old2[8:16])
        for j in range(ng):
            out = jnp.where(t >= float(NEW0 + 8 * j), new[8 * j:8 * j + 8], out)
        return out
    h2s = jnp.concatenate([pick(t1, h2c, h2n), pick(t2, h2c, h2n)], axis=0)
    h2b = h2s.astype(BF)
    hid = []
    for n in range(0, F, FFN_NB):
        gt = _rb(jnp.dot(h2b, pltpu.bitcast(wg_v[:, n:n + FFN_NB], BF), preferred_element_type=F32))
        up = _rb(jnp.dot(h2b, pltpu.bitcast(wu_v[:, n:n + FFN_NB], BF), preferred_element_type=F32))
        hid.append((_rb(gt * _rb(jax.nn.sigmoid(gt))) * up).astype(BF))
    y = _rb(jnp.dot(jnp.concatenate(hid, axis=1), pltpu.bitcast(wd_v[...], BF),
                    preferred_element_type=F32))
    act[OOFF + NEW0:OOFF + S, :] = (x1n + _rb(rep(5, ng) * h2n)).astype(BF)
    x1s = jnp.concatenate([pick(t1, x1c, x1n), pick(t2, x1c, x1n)], axis=0)
    c1, c2 = (pl.multiple_of((jnp.clip(t[0, 0].astype(jnp.int32), 0, S - 1) >> 3) * 8, 8)
              for t in (t1, t2))
    tok = jnp.concatenate([subf + c1.astype(F32), subf + c2.astype(F32)], axis=0)
    is1, is2 = tok == t1, tok == t2
    gate = _rb(jax.nn.sigmoid(jnp.where(is1, v1, v2)))
    upd = jnp.where(is1 | is2, _rb(y * gate), 0.0)
    res = (x1s + _rb(rep(5, 2) * _rb(h2s + upd))).astype(BF)
    out_copy(0, NEW0, 9).wait()
    act[pl.ds(OOFF + c1, 8), :] = res[0:8]
    act[pl.ds(OOFF + c2, 8), :] = res[8:16]
    fix0 = out_copy(NEW0, NEW, 6)
    fix1 = out_copy(c1, 8, 11)
    fix2 = out_copy(c2, 8, 12)
    send1 = c1 < NEW0
    send2 = (c2 < NEW0) & (c2 != c1)
    fix0.start()
    pl.when(send1)(fix1.start)
    pl.when(send2)(fix2.start)
    pl.when(send1)(fix1.wait)
    pl.when(send2)(fix2.wait)
    fix0.wait()


@jax.jit
def pallas_adaLN_cond__memory_aug_recurrent_mem_tr__moe_arch_mod__prompt_kernel(
    A_x: jax.Array,
    A_mem0: jax.Array,
    A_Wq: jax.Array,
    A_Wk: jax.Array,
    A_Wv: jax.Array,
    A_Wo: jax.Array,
    A_seg_len,
    B_x: jax.Array,
    B_w_r: jax.Array,
    B_w_gate: jax.Array,
    B_w_up: jax.Array,
    B_w_down: jax.Array,
    c: jax.Array,
    w_mod: jax.Array,
):
    del B_x
    del A_seg_len
    assert A_x.shape == (1, S, D) and A_Wq.shape == (D, H, DH) and A_mem0.shape == (1, M, D)
    any_spec = pl.BlockSpec(memory_space=pl.ANY)
    scratch = [
        pltpu.VMEM((S, D), BF),
        pltpu.VMEM((ACT_ROWS, D), BF),
        pltpu.VMEM((8, PRE // 2, 128), U32),
        pltpu.VMEM((32, 768), F32),
        pltpu.VMEM((D // 2, 128), U32),
        pltpu.VMEM((2, 8, D), F32),
        pltpu.SMEM((NSEG * NTAB,), jnp.int32),
        pltpu.VMEM((9, 8, D), F32),
        pltpu.VMEM((3 * H, D // 2, 128), U32),
        pltpu.VMEM((H, DH // 2, D), U32),
        pltpu.VMEM((6, D // 2, D), U32),
        pltpu.VMEM((D // 2, F), U32),
        pltpu.VMEM((D // 2, F), U32),
        pltpu.VMEM((F // 2, D), U32),
        pltpu.VMEM((80, H * DH), BF),
        pltpu.SemaphoreType.DMA((17,)),
        pltpu.SemaphoreType.DMA((12,)),
        pltpu.SemaphoreType.DMA((16,)),
    ] + [pltpu.VMEM((NSLOT + 1, 256, 128), U32) for _ in range(NB)] + [
        pltpu.VMEM((1, D), BF),
        pltpu.VMEM((D,), BF),
    ]
    wq, wk, wv = (w.reshape(D // 2, 2, H, DH) for w in (A_Wq, A_Wk, A_Wv))
    return pl.pallas_call(
        _kernel,
        out_shape=jax.ShapeDtypeStruct((1, S, D), BF),
        in_specs=[any_spec] * 12,
        out_specs=any_spec,
        scratch_shapes=scratch,
        compiler_params=pltpu.CompilerParams(vmem_limit_bytes=120 * 1024 * 1024,
                                             disable_bounds_checks=True,
                                             disable_semaphore_checks=True),
    )(A_x, A_mem0, wq, wk, wv, A_Wo, B_w_r, B_w_gate, B_w_up, B_w_down,
      c, w_mod)
```

```python
import jax
import jax.numpy as jnp
from jax import lax
import jax.experimental.pallas as pl
import jax.experimental.pallas.tpu as pltpu

BF = jnp.bfloat16
F32 = jnp.float32
U32 = jnp.uint32

S = 2048
D = 1024
H = 32
DH = 128
M = 8
SEG = 32
NSEG = S // SEG
F = 3584
NP = H // 2
EPS = 1e-5
SCALE = DH ** -0.5
HD = D // 2

RIDE = 24
PRE = S - NSEG * RIDE
NSLOT = 17
NB = 8
KS = 2048
OOFF = S
HOFF = 2 * S
ROFF = HOFF + 64
ACT_ROWS = ROFF + 16
PRE_SPLIT = 3
E_AT = (2, 3, 4, 5, 6)
E_AT2 = (3, 4, 5)
L_AT = (6, 7, 8)
L_AT2 = (6, 8, 10)
A_BUF = (7, 0, 1, 2, 3)
W1AT = (2, 6)
NEW = 40
FFN_NB = 512
APPLY_N = 4
MOD_YR = 64
NTAB = 8

ROT = 2
ATT = {4: [('s', i) for i in range(4)],
       18: [('p', (12 + ROT + i) % NP) for i in range(4)]}
for _p in range(4, NP, 2):
    ATT[_p + 2] = [('s', _p), ('s', _p + 1), ('p', _p - 4 + ROT), ('p', _p - 3 + ROT)]


def _step_indices(s):
    t = [s % NSLOT]
    for j in range(3):
        gi = PRE // 8 + 3 * s + j
        t += [(gi // 4) % NSLOT, (gi % 4) * 4]
    return t


def _rb(v):
    return v.astype(BF).astype(F32)


def _pack(v):
    return pltpu.bitcast(v.astype(BF), U32)


def _layernorm(x):
    mu = jnp.sum(x, axis=-1, keepdims=True) * (1.0 / D)
    xc = x - mu
    var = jnp.sum(xc * xc, axis=-1, keepdims=True) * (1.0 / D)
    sd = _rb(jnp.sqrt(_rb(_rb(var) + EPS)))
    return _rb(_rb(x - _rb(mu)) / sd)


def _kernel(x_hbm, mem0_hbm, wq_hbm, wk_hbm, wv_hbm, wo_hbm, wr_hbm, wg_hbm, wu_hbm,
            wd_hbm, c_hbm, wmod_hbm, out_hbm,
            xbuf, act, h0buf, ybuf, scol, macc, tab, modb,
            w_v, wo_v, wmod_v, wg_v, wu_v, wd_v,
            obuf, sems, wsems, ksems, *rest):
    qkvbufs, cbuf, wrbuf = rest[:NB], rest[NB], rest[NB + 1]
    w_hbms = tuple(w.bitcast(U32) for w in (wq_hbm, wk_hbm, wv_hbm))

    def cp(src, dst, i):
        return pltpu.make_async_copy(src, dst, sems.at[i])

    wmod32 = wmod_hbm.bitcast(U32)
    cp_c = cp(c_hbm, cbuf, 0)
    cp_mem = cp(mem0_hbm.at[0], act.at[HOFF:HOFF + M], 1)
    cp_wr = cp(wr_hbm, wrbuf, 2)
    cp_x0 = [cp(x_hbm.at[0, n * 128:(n + 1) * 128], xbuf.at[n * 128:(n + 1) * 128], 13 + n)
             for n in range(PRE // 128)]
    cp_xr = cp(x_hbm.at[0, PRE:PRE + 32], xbuf.at[PRE:PRE + 32], 5)
    cp_x1 = cp(x_hbm.at[0, PRE + 32:S], xbuf.at[PRE + 32:S], 4)
    cp_wo = cp(wo_hbm.bitcast(U32), wo_v, 7)
    cp_ffn = [cp(wg_hbm.bitcast(U32), wg_v, 8), cp(wu_hbm.bitcast(U32), wu_v, 8),
              cp(wd_hbm.bitcast(U32), wd_v, 8)]

    def w_start(j, i0=0, i1=NB, prio=0):
        gg, t = j // 3, j % 3
        r0 = 64 if j == 1 else 0
        for i in range(i0, i1):
            for par in range(2):
                pltpu.make_async_copy(w_hbms[t].at[r0:, par, gg * NB + i, :],
                                      w_v.at[(gg * NB + i) * 6 + t * 2 + par, r0:],
                                      wsems.at[2 * j + (i >= PRE_SPLIT)]).start(priority=prio)

    def mod_copy(v):
        return pltpu.make_async_copy(wmod32.at[:, v * D:(v + 1) * D], wmod_v.at[v],
                                     wsems.at[2 * (3 + v // 2) + 1])

    def mult(v, m):
        return v if isinstance(v, int) else pl.multiple_of(v, m)

    def moda_copies(kc):
        col = mult(kc * 128, 128)
        return [pltpu.make_async_copy(wmod32.at[:, pl.ds(v * D + col, 128)],
                                      wmod_v.at[v, :, pl.ds(col, 128)], ksems.at[8 + kc])
                for v in range(2)]

    def chunk_copies(kc):
        r0 = mult(kc * 64, 64)
        return [pltpu.make_async_copy(w_hbms[0].at[pl.ds(r0, 64), par, i, :],
                                      w_v.at[i * 6 + par, pl.ds(r0, 64), :], ksems.at[kc])
                for i in range(NB) for par in range(2)]

    cp_early = [cp(w_hbms[1].at[0:64, par, i, :], w_v.at[i * 6 + 2 + par, 0:64], 3)
                for i in range(NB) for par in range(2)]

    cp_c.start()
    cp_mem.start()
    cp_wr.start()
    for c_ in (cp_x0 + moda_copies(0) + cp_early + moda_copies(1) + chunk_copies(0)
               + moda_copies(2) + chunk_copies(1) + [cp_xr]):
        c_.start()

    def ln1_rows(src_row, dst_row):
        xv = xbuf[pl.ds(src_row, 8), :].astype(F32)
        hv = _rb(_layernorm(xv) * modb[1]) + modb[0]
        act[pl.ds(dst_row, 8), :] = hv.astype(BF)

    lane256 = lax.broadcasted_iota(jnp.int32, (8, 256), 1)

    def finish_rows(row, attn):
        xv = xbuf[pl.ds(row, 8), :].astype(F32)
        x1 = _rb(xv + _rb(modb[2] * _rb(attn)))
        act[pl.ds(row, 8), :] = x1.astype(BF)
        h2 = _rb(_rb(_layernorm(x1) * modb[4]) + modb[3])
        act[pl.ds(OOFF + row, 8), :] = (x1 + _rb(modb[5] * h2)).astype(BF)
        r = jnp.sum(h2 * modb[6], axis=-1, keepdims=True)
        act[ROFF:ROFF + 8, 0:256] = jnp.where(
            lane256 * 8 == row, r, act[ROFF:ROFF + 8, 0:256].astype(F32)).astype(BF)

    def attn_store(a, k0):
        for j in range(a.shape[0] // 8):
            for k in range(a.shape[1] // 128):
                qkvbufs[A_BUF[j]][NSLOT, (k0 + k) * 8:(k0 + k + 1) * 8, :] = pltpu.bitcast(
                    a[8 * j:8 * j + 8, k * 128:(k + 1) * 128], U32)

    def attn_load(j):
        return pltpu.bitcast(jnp.concatenate(
            [qkvbufs[A_BUF[j]][NSLOT, k * 8:(k + 1) * 8, :] for k in range(8)], axis=1), F32)

    act[ROFF:ROFF + 8, 0:256] = jnp.zeros((8, 256), BF)
    attn_store(jnp.zeros((NEW, D), F32), 0)
    qkvbufs[0][NSLOT, 64:72, :] = jnp.zeros((8, 128), U32)
    for s_ in range(NSEG):
        for k, v in enumerate(_step_indices(s_)):
            tab[s_ * NTAB + k] = v
    ri = lax.broadcasted_iota(jnp.int32, (80, 80), 0)
    ci = lax.broadcasted_iota(jnp.int32, (80, 80), 1)

    def head_pos(i):
        hd = jnp.where(i < 16, i // 8, (i - 16) // 32)
        pos = jnp.where(i < 16, i % 8, 8 + (i - 16) % 32)
        return hd, pos
    rh, rp = head_pos(ri)
    ch, cpos = head_pos(ci)
    same = rh == ch
    valid = same & ((rp < M) | (rp >= cpos))
    fill = jnp.where(same, -1e9, -jnp.inf).astype(F32)

    cp_mem.wait()
    cp_wr.wait()
    modb[6] = jnp.broadcast_to(wrbuf[...].astype(F32).reshape(1, D), (8, D))
    cp_c.wait()
    cv = cbuf[...].astype(F32)
    sc_row = _rb(cv * _rb(jax.nn.sigmoid(cv)))
    sc16 = jnp.broadcast_to(sc_row, (16, D)).astype(BF)
    for k in range(8):
        scol[k * 64:(k + 1) * 64, :] = _pack(
            jnp.broadcast_to(sc_row[:, k * 128:(k + 1) * 128], (128, 128)).T)

    def ln_pre(g, carry):
        pltpu.make_async_copy(x_hbm.at[0, 0:128], xbuf.at[pl.ds(pl.multiple_of(g * 128, 128), 128)],
                              sems.at[13 + g]).wait()
        for u in range(2):
            row = pl.multiple_of(g * 128 + u * 64, 64)
            nv = _layernorm(xbuf[pl.ds(row, 64), :].astype(F32)).astype(BF)
            for k in range(8):
                h0buf[k, pl.ds(pl.multiple_of(row // 2, 32), 32), :] = pltpu.bitcast(
                    nv[:, k * 128:(k + 1) * 128], U32)
            wg_v[pl.ds(row, 64), 0:2 * D] = jnp.zeros((64, 2 * D), U32)
        return carry
    lax.fori_loop(0, PRE // 128, ln_pre, 0)

    def mod_tile(v, col):
        w = pltpu.bitcast(wmod_v[v, :, pl.ds(col, 128)], BF)
        return _rb(jnp.dot(sc16, w, preferred_element_type=F32))[0:8]

    def moda_store(kc, sa, ca):
        col = mult(kc * 128, 128)
        c1 = _rb(1.0 + ca)
        modb[0, :, pl.ds(col, 128)] = sa
        modb[1, :, pl.ds(col, 128)] = c1
        return sa, c1

    def moda_apply(kc, sa, c1, r0, r1):
        for r in range(r0, r1, 16):
            nv = pltpu.bitcast(h0buf[kc, r // 2:r // 2 + 8, :], BF).astype(F32).reshape(2, 8, 128)
            hv = (_rb(nv * c1[None]) + sa[None]).reshape(16, 128).astype(BF)
            h0buf[kc, r // 2:r // 2 + 8, :] = pltpu.bitcast(hv, U32)

    def halves(u):
        return pltpu.bitcast(u << 16, F32), pltpu.bitcast(u & U32(0xFFFF0000), F32)

    def repack(a, b):
        return (a & U32(0xFFFF)) | (b << 16), (a >> 16) | (b & U32(0xFFFF0000))

    def store_qkv(i, jrow, y, seg0):
        for sg in range(y.shape[0] // 32):
            for hh in range(2):
                qkvbufs[i][seg0 + sg, pl.ds(jrow + 8 + hh * 16, 16), :] = _pack(
                    y[sg * 32:(sg + 1) * 32, hh * 128:(hh + 1) * 128])

    for c_ in chunk_copies(2):
        c_.start()
    for c_ in moda_copies(0):
        c_.wait()
    moda_apply(0, *moda_store(0, mod_tile(0, 0), mod_tile(1, 0)), 0, PRE)
    w_start(1, 0, PRE_SPLIT, prio=1)

    for c_ in cp_early:
        c_.wait()
    for i in range(NB):
        lo, hi = repack(w_v[i * 6 + 2, 0:64, :], w_v[i * 6 + 3, 0:64, :])
        w_v[i * 6 + 2, 0:64, :] = lo
        w_v[i * 6 + 3, 0:64, :] = hi
        wu_v[0:PRE, i * 256:(i + 1) * 256] = pltpu.bitcast(jnp.dot(
            pltpu.bitcast(h0buf[0], BF), pltpu.bitcast(jnp.concatenate([lo, hi], axis=1), BF),
            preferred_element_type=F32), U32)

    def w_wait(j, i0, i1, r0=0):
        blk0 = (j // 3) * (6 * NB) + (j % 3) * 2
        for i in range(i0, i1):
            for par in range(2):
                pltpu.make_async_copy(w_hbms[0].at[r0:, 0, 0, :], w_v.at[blk0 + i * 6 + par, r0:],
                                      wsems.at[2 * j + (i >= PRE_SPLIT)]).wait()

    def chunk_block(kc, last, issue):
        for c_ in chunk_copies(kc) + ([cp_xr] if last else moda_copies(kc + 1)):
            c_.wait()
        issue()
        r0 = mult(kc * 64, 64)
        mv = []
        for i in range(NB):
            lo, hi = repack(w_v[i * 6, pl.ds(r0, 64), :], w_v[i * 6 + 1, pl.ds(r0, 64), :])
            w_v[i * 6, pl.ds(r0, 64), :] = lo
            w_v[i * 6 + 1, pl.ds(r0, 64), :] = hi
            w = pltpu.bitcast(jnp.concatenate([lo, hi], axis=1), BF)
            y = (pltpu.bitcast(wg_v[0:PRE, i * 256:(i + 1) * 256], F32)
                 + jnp.dot(pltpu.bitcast(h0buf[kc], BF), w, preferred_element_type=F32))
            if last:
                store_qkv(i, 0, y, 0)
            else:
                wg_v[0:PRE, i * 256:(i + 1) * 256] = pltpu.bitcast(y, U32)
                if i in (1, 3):
                    mv.append(mod_tile(i // 2, mult((kc + 1) * 128, 128)))
                if i == 3:
                    mv = moda_store(kc + 1, mv[0], mv[1])
                if i in (4, 6):
                    zeros = qkvbufs[A_BUF[0]][NSLOT, 0:8, :]
                    for q in range(APPLY_N):
                        yr = (q + 1) * (PRE // (APPLY_N + 1)) // 8 * 8
                        tok = pltpu.bitcast(y[yr:yr + 8, 0:128], U32) & zeros
                        c1 = pltpu.bitcast(pltpu.bitcast(mv[1], U32) | tok, F32)
                        n = PRE // 2 // APPLY_N
                        r_ = (i - 4) // 2 * (PRE // 2) + q * n
                        moda_apply(kc + 1, mv[0], c1, r_, r_ + n)
        if last:
            for j in range(3):
                ln1_rows(PRE + 8 * j, HOFF + 8 + 8 * j)

    def chunk_body(kc, carry):
        def issue():
            @pl.when(kc < 5)
            def _():
                for c_ in moda_copies(kc + 3) + chunk_copies(kc + 3):
                    c_.start()
        chunk_block(kc, False, issue)
        return carry

    def issue_last():
        w_wait(1, 0, PRE_SPLIT, 64)
        w_start(1, PRE_SPLIT, NB)
        w_start(2)
    lax.fori_loop(0, 7, chunk_body, 0)
    chunk_block(7, True, issue_last)

    def pre_unit(j, i, extra, k0=0):
        blk = (j // 3) * (6 * NB) + (j % 3) * 2 + i * 6
        jrow = mult(j * 40, 8)
        r0 = k0 * 64
        lo, hi = repack(w_v[blk, r0:, :], w_v[blk + 1, r0:, :])
        w_v[blk, r0:, :] = lo
        w_v[blk + 1, r0:, :] = hi
        for rc in range(PRE // 128):
            if rc > 0:
                lo = w_v[blk, r0:, :]
                hi = w_v[blk + 1, r0:, :]
            w = pltpu.bitcast(jnp.concatenate([lo, hi], axis=1), BF)
            lhs = jnp.concatenate(
                [h0buf[k, rc * 64:(rc + 1) * 64, :] for k in range(k0, 8)], axis=1)
            y = jnp.dot(pltpu.bitcast(lhs, BF), w, preferred_element_type=F32)
            if k0:
                y = y + pltpu.bitcast(wu_v[rc * 128:(rc + 1) * 128, i * 256:(i + 1) * 256], F32)
            store_qkv(i, jrow, y, rc * 4)
            extra(rc, y)

    for i in range(NB):
        if i == PRE_SPLIT:
            w_wait(1, PRE_SPLIT, NB, 64)
            w_start(3)
            w_start(4)
            mod_copy(2).start()
            mod_copy(3).start()
        pre_unit(1, i, lambda rc, y: None, k0=1)
    w_start(5)
    mod_copy(4).start()
    mod_copy(5).start()
    cp_wo.start()
    cp_x1.start()

    def pre_body(j, carry):
        w_wait(j, 0, NB)
        v0 = jnp.maximum(j - 3, 0) * 2

        @pl.when(j >= 4)
        def _():
            for v in range(2):
                pltpu.make_async_copy(wmod32.at[:, 0:D], wmod_v.at[v0 + v],
                                      wsems.at[2 * j + 1]).wait()
        zeros = qkvbufs[A_BUF[0]][NSLOT, 0:8, :]
        for i in range(NB):
            def extra(rc, y, i=i):
                for u in range(2):
                    b = (i * 4 + rc) * 2 + u
                    for v in range(2):
                        tok = pltpu.bitcast(
                            y[v * MOD_YR:v * MOD_YR + 8, u * 128:(u + 1) * 128], U32) & zeros
                        for cs in (slice(0, HD), slice(HD, D)):
                            se, so = halves(scol[b * 8:(b + 1) * 8, :] | tok)
                            we, wo = halves(wmod_v[v0 + v, b * 8:(b + 1) * 8, cs])
                            t = (we * jnp.concatenate([se] * 4, axis=1)
                                 + wo * jnp.concatenate([so] * 4, axis=1))
                            macc[v, :, cs] = t + macc[v, :, cs] if b else t
            pre_unit(j, i, extra)
        dst = jnp.where(j >= 4, v0, 7)
        for v in range(2):
            mv = _rb(jnp.sum(macc[v], axis=0, keepdims=True))
            if v == 0:
                mv = _rb(jnp.where(j == 5, 1.0, 0.0).astype(F32) + mv)
            modb[dst + v] = jnp.broadcast_to(mv, (8, D))
        return carry
    lax.fori_loop(2, 6, pre_body, 0)

    cp_wo.wait()
    cp_x1.wait()
    for c_ in cp_ffn:
        c_.start()

    def wo_w(q0, q1, n0, n1):
        h0, h1 = q0 + 2 * ROT, q1 + 2 * ROT
        ws = [wo_v[a:b, :, n0 * 128:n1 * 128].reshape((b - a) * (DH // 2), (n1 - n0) * 128)
              for a, b in ((h0, min(h1, H)), (0, h1 - H)) if b > a]
        return pltpu.bitcast(jnp.concatenate(ws, axis=0), BF)

    def emit_step(it, odd, pend):
        s = 2 * it + odd
        hrow = pl.multiple_of(HOFF + (s & 1) * 32, 32)
        hnext = pl.multiple_of(HOFF + 32 - (s & 1) * 32, 32)
        tv = [tab[s * NTAB + k] for k in range(7)]
        slot = tv[0]
        dsts = [(tv[1 + 2 * j], pl.multiple_of(tv[2 + 2 * j], 4)) for j in range(3)]
        orow, ow = (32, 48) if odd else (0, 32)
        odst = (48, 56, 64, 72) if odd else (8, 16, 24, 40)
        erow = it * 64 if odd else jnp.maximum(it - 1, 0) * 64 + RIDE
        lrow = PRE + jnp.minimum(s + 1, NSEG - 1) * RIDE
        e_at, l_at = (E_AT2, L_AT2) if odd else (E_AT, L_AT)
        probs = {}

        def wqkv(p, k0, k1):
            return pltpu.bitcast(jnp.concatenate(
                [w_v[p * 6 + u, k0 // 2:k1 // 2, :] for u in range(6)], axis=1), BF)

        lhs_lo = act[pl.ds(hrow, 32), 0:HD]
        if pend is not None:
            ybuf[...] = jnp.dot(lhs_lo, wqkv(0, 0, HD), preferred_element_type=F32)
            pend()
        lhs_hi = act[pl.ds(hrow, 32), HD:D]
        if pend is not None:
            y0 = ybuf[...] + jnp.dot(lhs_hi, wqkv(0, HD, D), preferred_element_type=F32)
        lhs_rest = jnp.concatenate([lhs_lo[:, 128:], lhs_hi], axis=1)
        lhs = [jnp.concatenate([lhs_lo, lhs_hi], axis=1)]

        def side(p):
            for j in range(len(e_at)):
                if e_at[j] == p:
                    finish_rows(pl.multiple_of(erow + 8 * j, 8), attn_load(j))
            for j in range(3):
                if l_at[j] == p:
                    ln1_rows(pl.multiple_of(lrow + 8 * j, 8),
                             pl.multiple_of(hnext + 8 + 8 * j, 8))
            if p in e_at or p in l_at:
                lhs[0] = jnp.concatenate([act[pl.ds(hrow, 32), 0:128], lhs_rest], axis=1)

        def qkv(p):
            if p == 0 and pend is not None:
                y = y0
            else:
                y = jnp.dot(lhs[0], wqkv(p, 0, D), preferred_element_type=F32)
            buf = qkvbufs[p % NB]
            for u in range(6):
                t, hh = u // 2, u % 2
                b0 = ((p // NB) * 3 + t) * 40
                yu = y[:, u * 128:(u + 1) * 128]
                buf[slot, b0 + hh * 4:b0 + hh * 4 + 4, :] = _pack(yu[0:8])
                for j in range(3):
                    sl, off = dsts[j]
                    buf[sl, pl.ds(b0 + 8 + hh * 16 + off, 4), :] = _pack(yu[8 + 8 * j:16 + 8 * j])

        def ld(p, t):
            b0 = ((p // NB) * 3 + t) * 40
            return pltpu.bitcast(qkvbufs[p % NB][slot, b0:b0 + 40, :], BF)

        def sc(p):
            s2 = lax.dot_general(ld(p, 0), ld(p, 1), (((1,), (1,)), ((), ())),
                                 preferred_element_type=F32)
            s2 = jnp.where(valid, s2 * SCALE, fill)
            m = jnp.max(s2, axis=-1, keepdims=True)
            e = jnp.exp(s2 - m)
            l = jnp.sum(e, axis=-1, keepdims=True)
            rl = pl.reciprocal(l, approx=True)
            rl = rl * (2.0 - l * rl)
            probs[p] = (e * rl).astype(BF)

        def pv(p):
            o2 = jnp.dot(probs[p], ld(p, 2), preferred_element_type=F32)
            for hh in range(2):
                hcol = (2 * ((p - ROT) % NP) + hh) * 128
                obuf[orow:orow + 8, hcol:hcol + 128] = o2[8 * hh:8 * hh + 8].astype(BF)
                for j in range(4):
                    r0 = 16 + 32 * hh + 8 * j
                    obuf[odst[j]:odst[j] + 8, hcol:hcol + 128] = o2[r0:r0 + 8].astype(BF)

        def attn(pos):
            for kind, p in ATT.get(pos, ()):
                (sc if kind == 's' else pv)(p)

        for p in range(NP):
            qkv(p)
            side(p)
            attn(p)
        a1 = []
        for n in range(8):
            a1.append(jnp.dot(obuf[orow:orow + ow, 0:KS], wo_w(0, KS // DH, n, n + 1),
                              preferred_element_type=F32))
            if n + 1 in W1AT:
                attn(NP + 2 * W1AT.index(n + 1))
        o2lhs = obuf[orow:orow + ow, KS:]
        a_lo = jnp.concatenate(a1[0:4], axis=1) + jnp.dot(
            o2lhs, wo_w(KS // DH, H, 0, 4), preferred_element_type=F32)
        act[pl.ds(hnext, 8), 0:HD] = a_lo[0:8].astype(BF)
        attn_store(a_lo[8:], 0)
        a_hi = jnp.concatenate(a1[4:8], axis=1) + jnp.dot(
            o2lhs, wo_w(KS // DH, H, 4, 8), preferred_element_type=F32)

        def finish():
            act[pl.ds(hnext, 8), HD:D] = a_hi[0:8].astype(BF)
            attn_store(a_hi[8:], 4)
        return finish

    def out_copy(r0, n, sem):
        return cp(act.at[pl.ds(OOFF + r0, n)], out_hbm.at[0, pl.ds(r0, n)], sem)

    def steps(it, carry):
        emit_step(it, 1, emit_step(it, 0, None))()

        @pl.when(it > 0)
        def _():
            out_copy(pl.multiple_of((it - 1) * 64, 64), 64, 9).start()
        return carry
    lax.fori_loop(0, NSEG // 2, steps, 0)

    NEW0 = S - NEW
    out_copy(S - 64, NEW0 - (S - 64), 9).start()
    for c_ in cp_ffn:
        c_.wait()

    def rep(i, n):
        return jnp.concatenate([modb[i]] * n, axis=0)
    r_old = act[ROFF:ROFF + 8, 0:256].astype(F32) + 0.0
    bits = pltpu.bitcast(jnp.broadcast_to(jnp.max(r_old, axis=0, keepdims=True), (8, 256)),
                         jnp.int32)
    code = (bits ^ ((bits >> 31) & 0x7FFFFFFF)) >> 16
    key = jnp.where(lane256 < NEW0 // 8, (code * 256 + (255 - lane256)).astype(F32), -jnp.inf)
    k1 = jnp.max(key, axis=1, keepdims=True)
    k2 = jnp.max(jnp.where(key == k1, -jnp.inf, key), axis=1, keepdims=True)
    rc = jnp.concatenate([jnp.max(jnp.where(key == k, r_old, -jnp.inf), axis=1, keepdims=True)
                          for k in (k1, k2)], axis=0)
    b1, b2 = (pl.multiple_of(jnp.minimum(255 - (k[0, 0].astype(jnp.int32) & 255),
                                         NEW0 // 8 - 1) * 8, 8) for k in (k1, k2))
    x1c = jnp.concatenate([act[pl.ds(b1, 8), :].astype(F32), act[pl.ds(b2, 8), :].astype(F32)],
                          axis=0)
    h2c = _rb(_rb(_layernorm(x1c) * rep(4, 2)) + rep(3, 2))
    ng = NEW // 8
    x1n = _rb(xbuf[NEW0:S, :].astype(F32) + _rb(rep(2, ng) * _rb(
        jnp.concatenate([attn_load(j) for j in range(ng)], axis=0))))
    h2n = _rb(_rb(_layernorm(x1n) * rep(4, ng)) + rep(3, ng))
    rn = _rb(jnp.sum(h2n * rep(6, ng), axis=-1, keepdims=True))
    subf = lax.broadcasted_iota(jnp.int32, (8, 1), 0).astype(F32)
    b1f = b1.astype(F32)
    val = jnp.concatenate([rc, rn], axis=0)
    idx = jnp.concatenate([subf + b1f, subf + b2.astype(F32)]
                          + [subf + float(NEW0 + 8 * j) for j in range(ng)], axis=0)
    v1 = jnp.max(val, axis=0, keepdims=True)
    t1 = jnp.min(jnp.where(val == v1, idx, float(S)), axis=0, keepdims=True)
    rest = jnp.where(idx == t1, -jnp.inf, val)
    v2 = jnp.max(rest, axis=0, keepdims=True)
    t2 = jnp.min(jnp.where((rest == v2) & (idx != t1), idx, float(S)), axis=0, keepdims=True)

    def pick(t, old2, new):
        out = jnp.where((t >= b1f) & (t < b1f + 8.0), old2[0:8], old2[8:16])
        for j in range(ng):
            out = jnp.where(t >= float(NEW0 + 8 * j), new[8 * j:8 * j + 8], out)
        return out
    h2s = jnp.concatenate([pick(t1, h2c, h2n), pick(t2, h2c, h2n)], axis=0)
    h2b = h2s.astype(BF)
    hid = []
    for n in range(0, F, FFN_NB):
        gt = _rb(jnp.dot(h2b, pltpu.bitcast(wg_v[:, n:n + FFN_NB], BF), preferred_element_type=F32))
        up = _rb(jnp.dot(h2b, pltpu.bitcast(wu_v[:, n:n + FFN_NB], BF), preferred_element_type=F32))
        hid.append((_rb(gt * _rb(jax.nn.sigmoid(gt))) * up).astype(BF))
        if n == 0:
            late = pltpu.bitcast(up[0:8, 0:128], U32) & qkvbufs[0][NSLOT, 64:72, :]
            gbl = pltpu.bitcast(
                pltpu.bitcast(modb[5], U32) | jnp.concatenate([late] * 8, axis=1), F32)
    y = _rb(jnp.dot(jnp.concatenate(hid, axis=1), pltpu.bitcast(wd_v[...], BF),
                    preferred_element_type=F32))
    act[OOFF + NEW0:OOFF + S, :] = (
        x1n + _rb(jnp.concatenate([gbl] * ng, axis=0) * h2n)).astype(BF)
    x1s = jnp.concatenate([pick(t1, x1c, x1n), pick(t2, x1c, x1n)], axis=0)
    c1, c2 = (pl.multiple_of((jnp.clip(t[0, 0].astype(jnp.int32), 0, S - 1) >> 3) * 8, 8)
              for t in (t1, t2))
    tok = jnp.concatenate([subf + c1.astype(F32), subf + c2.astype(F32)], axis=0)
    is1, is2 = tok == t1, tok == t2
    gate = _rb(jax.nn.sigmoid(jnp.where(is1, v1, v2)))
    upd = jnp.where(is1 | is2, _rb(y * gate), 0.0)
    res = (x1s + _rb(rep(5, 2) * _rb(h2s + upd))).astype(BF)
    out_copy(0, NEW0, 9).wait()
    act[pl.ds(OOFF + c1, 8), :] = res[0:8]
    act[pl.ds(OOFF + c2, 8), :] = res[8:16]
    fix0 = out_copy(NEW0, NEW, 6)
    fix1 = out_copy(c1, 8, 11)
    fix2 = out_copy(c2, 8, 12)
    send1 = c1 < NEW0
    send2 = (c2 < NEW0) & (c2 != c1)
    fix0.start()
    pl.when(send1)(fix1.start)
    pl.when(send2)(fix2.start)
    pl.when(send1)(fix1.wait)
    pl.when(send2)(fix2.wait)
    fix0.wait()


@jax.jit
def pallas_adaLN_cond__memory_aug_recurrent_mem_tr__moe_arch_mod__prompt_kernel(
    A_x: jax.Array,
    A_mem0: jax.Array,
    A_Wq: jax.Array,
    A_Wk: jax.Array,
    A_Wv: jax.Array,
    A_Wo: jax.Array,
    A_seg_len,
    B_x: jax.Array,
    B_w_r: jax.Array,
    B_w_gate: jax.Array,
    B_w_up: jax.Array,
    B_w_down: jax.Array,
    c: jax.Array,
    w_mod: jax.Array,
):
    del B_x
    del A_seg_len
    assert A_x.shape == (1, S, D) and A_Wq.shape == (D, H, DH) and A_mem0.shape == (1, M, D)
    any_spec = pl.BlockSpec(memory_space=pl.ANY)
    scratch = [
        pltpu.VMEM((S, D), BF),
        pltpu.VMEM((ACT_ROWS, D), BF),
        pltpu.VMEM((8, PRE // 2, 128), U32),
        pltpu.VMEM((32, 768), F32),
        pltpu.VMEM((D // 2, 128), U32),
        pltpu.VMEM((2, 8, D), F32),
        pltpu.SMEM((NSEG * NTAB,), jnp.int32),
        pltpu.VMEM((9, 8, D), F32),
        pltpu.VMEM((3 * H, D // 2, 128), U32),
        pltpu.VMEM((H, DH // 2, D), U32),
        pltpu.VMEM((6, D // 2, D), U32),
        pltpu.VMEM((D // 2, F), U32),
        pltpu.VMEM((D // 2, F), U32),
        pltpu.VMEM((F // 2, D), U32),
        pltpu.VMEM((80, H * DH), BF),
        pltpu.SemaphoreType.DMA((17,)),
        pltpu.SemaphoreType.DMA((12,)),
        pltpu.SemaphoreType.DMA((16,)),
    ] + [pltpu.VMEM((NSLOT + 1, 256, 128), U32) for _ in range(NB)] + [
        pltpu.VMEM((1, D), BF),
        pltpu.VMEM((D,), BF),
    ]
    wq, wk, wv = (w.reshape(D // 2, 2, H, DH) for w in (A_Wq, A_Wk, A_Wv))
    return pl.pallas_call(
        _kernel,
        out_shape=jax.ShapeDtypeStruct((1, S, D), BF),
        in_specs=[any_spec] * 12,
        out_specs=any_spec,
        scratch_shapes=scratch,
        compiler_params=pltpu.CompilerParams(vmem_limit_bytes=120 * 1024 * 1024,
                                             disable_bounds_checks=True,
                                             disable_semaphore_checks=True),
    )(A_x, A_mem0, wq, wk, wv, A_Wo, B_w_r, B_w_gate, B_w_up, B_w_down,
      c, w_mod)
```

```python
import jax
import jax.numpy as jnp
from jax import lax
import jax.experimental.pallas as pl
import jax.experimental.pallas.tpu as pltpu

BF = jnp.bfloat16
F32 = jnp.float32
U32 = jnp.uint32

S = 2048
D = 1024
H = 32
DH = 128
M = 8
SEG = 32
NSEG = S // SEG
F = 3584
NP = H // 2
EPS = 1e-5
SCALE = DH ** -0.5
HD = D // 2

RIDE = 24
PRE = S - NSEG * RIDE
NSLOT = 17
NB = 8
KS = 2048
OOFF = S
HOFF = 2 * S
ROFF = HOFF + 64
ACT_ROWS = ROFF + 16
PRE_SPLIT = 3
E_AT = (2, 3, 4, 5, 6)
E_AT2 = (3, 4, 5)
L_AT = (6, 7, 8)
L_AT2 = (6, 8, 10)
A_BUF = (7, 0, 1, 2, 3)
W1AT = (2, 6)
NEW = 40
FFN_NB = 512
APPLY_N = 4
MOD_YR = 64
NTAB = 8

ROT = 2
ATT = {4: [('s', i) for i in range(4)],
       18: [('p', (12 + ROT + i) % NP) for i in range(4)]}
for _p in range(4, NP, 2):
    ATT[_p + 2] = [('s', _p), ('s', _p + 1), ('p', _p - 4 + ROT), ('p', _p - 3 + ROT)]


def _step_indices(s):
    t = [s % NSLOT]
    for j in range(3):
        gi = PRE // 8 + 3 * s + j
        t += [(gi // 4) % NSLOT, (gi % 4) * 4]
    return t


def _rb(v):
    return v.astype(BF).astype(F32)


def _pack(v):
    return pltpu.bitcast(v.astype(BF), U32)


def _layernorm(x):
    mu = jnp.sum(x, axis=-1, keepdims=True) * (1.0 / D)
    xc = x - mu
    var = jnp.sum(xc * xc, axis=-1, keepdims=True) * (1.0 / D)
    sd = _rb(jnp.sqrt(_rb(_rb(var) + EPS)))
    return _rb(_rb(x - _rb(mu)) / sd)


def _kernel(x_hbm, mem0_hbm, wq_hbm, wk_hbm, wv_hbm, wo_hbm, wr_hbm, wg_hbm, wu_hbm,
            wd_hbm, c_hbm, wmod_hbm, out_hbm,
            xbuf, act, h0buf, ybuf, scol, macc, tab, modb,
            w_v, wo_v, wmod_v, wg_v, wu_v, wd_v,
            obuf, sems, wsems, ksems, *rest):
    qkvbufs, cbuf, wrbuf = rest[:NB], rest[NB], rest[NB + 1]
    w_hbms = tuple(w.bitcast(U32) for w in (wq_hbm, wk_hbm, wv_hbm))

    def cp(src, dst, i):
        return pltpu.make_async_copy(src, dst, sems.at[i])

    wmod32 = wmod_hbm.bitcast(U32)
    cp_c = cp(c_hbm, cbuf, 0)
    cp_mem = cp(mem0_hbm.at[0], act.at[HOFF:HOFF + M], 1)
    cp_wr = cp(wr_hbm, wrbuf, 2)
    cp_x0 = [cp(x_hbm.at[0, n * 128:(n + 1) * 128], xbuf.at[n * 128:(n + 1) * 128], 13 + n)
             for n in range(PRE // 128)]
    cp_xr = cp(x_hbm.at[0, PRE:PRE + 32], xbuf.at[PRE:PRE + 32], 5)
    cp_x1 = cp(x_hbm.at[0, PRE + 32:S], xbuf.at[PRE + 32:S], 4)
    cp_wo = cp(wo_hbm.bitcast(U32), wo_v, 7)
    cp_ffn = [cp(wg_hbm.bitcast(U32), wg_v, 8), cp(wu_hbm.bitcast(U32), wu_v, 8),
              cp(wd_hbm.bitcast(U32), wd_v, 8)]

    def w_start(j, i0=0, i1=NB, prio=0):
        gg, t = j // 3, j % 3
        r0 = 64 if j == 1 else 0
        for i in range(i0, i1):
            for par in range(2):
                pltpu.make_async_copy(w_hbms[t].at[r0:, par, gg * NB + i, :],
                                      w_v.at[(gg * NB + i) * 6 + t * 2 + par, r0:],
                                      wsems.at[2 * j + (i >= PRE_SPLIT)]).start(priority=prio)

    def mod_copy(v):
        return pltpu.make_async_copy(wmod32.at[:, v * D:(v + 1) * D], wmod_v.at[v],
                                     wsems.at[2 * (3 + v // 2) + 1])

    def mult(v, m):
        return v if isinstance(v, int) else pl.multiple_of(v, m)

    def moda_copies(kc):
        col = mult(kc * 128, 128)
        return [pltpu.make_async_copy(wmod32.at[:, pl.ds(v * D + col, 128)],
                                      wmod_v.at[v, :, pl.ds(col, 128)], ksems.at[8 + kc])
                for v in range(2)]

    def chunk_copies(kc):
        r0 = mult(kc * 64, 64)
        return [pltpu.make_async_copy(w_hbms[0].at[pl.ds(r0, 64), par, i, :],
                                      w_v.at[i * 6 + par, pl.ds(r0, 64), :], ksems.at[kc])
                for i in range(NB) for par in range(2)]

    cp_early = [cp(w_hbms[1].at[0:64, par, i, :], w_v.at[i * 6 + 2 + par, 0:64], 3)
                for i in range(NB) for par in range(2)]

    cp_c.start()
    cp_mem.start()
    cp_wr.start()
    for c_ in (cp_x0 + moda_copies(0) + cp_early + moda_copies(1) + chunk_copies(0)
               + moda_copies(2) + chunk_copies(1) + [cp_xr]):
        c_.start()

    def ln1_rows(src_row, dst_row):
        xv = xbuf[pl.ds(src_row, 8), :].astype(F32)
        hv = _rb(_layernorm(xv) * modb[1]) + modb[0]
        act[pl.ds(dst_row, 8), :] = hv.astype(BF)

    lane256 = lax.broadcasted_iota(jnp.int32, (8, 256), 1)

    def finish_rows(row, attn):
        xv = xbuf[pl.ds(row, 8), :].astype(F32)
        x1 = _rb(xv + _rb(modb[2] * _rb(attn)))
        act[pl.ds(row, 8), :] = x1.astype(BF)
        h2 = _rb(_rb(_layernorm(x1) * modb[4]) + modb[3])
        act[pl.ds(OOFF + row, 8), :] = (x1 + _rb(modb[5] * h2)).astype(BF)
        r = jnp.sum(h2 * modb[6], axis=-1, keepdims=True)
        act[ROFF:ROFF + 8, 0:256] = jnp.where(
            lane256 * 8 == row, r, act[ROFF:ROFF + 8, 0:256].astype(F32)).astype(BF)

    def attn_store(a, k0):
        for j in range(a.shape[0] // 8):
            for k in range(a.shape[1] // 128):
                qkvbufs[A_BUF[j]][NSLOT, (k0 + k) * 8:(k0 + k + 1) * 8, :] = pltpu.bitcast(
                    a[8 * j:8 * j + 8, k * 128:(k + 1) * 128], U32)

    def attn_load(j):
        return pltpu.bitcast(jnp.concatenate(
            [qkvbufs[A_BUF[j]][NSLOT, k * 8:(k + 1) * 8, :] for k in range(8)], axis=1), F32)

    act[ROFF:ROFF + 8, 0:256] = jnp.zeros((8, 256), BF)
    attn_store(jnp.zeros((NEW, D), F32), 0)
    qkvbufs[0][NSLOT, 64:72, :] = jnp.zeros((8, 128), U32)
    for s_ in range(NSEG):
        for k, v in enumerate(_step_indices(s_)):
            tab[s_ * NTAB + k] = v
    ri = lax.broadcasted_iota(jnp.int32, (80, 80), 0)
    ci = lax.broadcasted_iota(jnp.int32, (80, 80), 1)

    def head_pos(i):
        hd = jnp.where(i < 16, i // 8, (i - 16) // 32)
        pos = jnp.where(i < 16, i % 8, 8 + (i - 16) % 32)
        return hd, pos
    rh, rp = head_pos(ri)
    ch, cpos = head_pos(ci)
    same = rh == ch
    valid = same & ((rp < M) | (rp >= cpos))
    fill = jnp.where(same, -1e9, -jnp.inf).astype(F32)

    cp_mem.wait()
    cp_wr.wait()
    modb[6] = jnp.broadcast_to(wrbuf[...].astype(F32).reshape(1, D), (8, D))
    cp_c.wait()
    cv = cbuf[...].astype(F32)
    sc_row = _rb(cv * _rb(jax.nn.sigmoid(cv)))
    sc16 = jnp.broadcast_to(sc_row, (16, D)).astype(BF)
    for k in range(8):
        scol[k * 64:(k + 1) * 64, :] = _pack(
            jnp.broadcast_to(sc_row[:, k * 128:(k + 1) * 128], (128, 128)).T)

    def ln_pre(g, carry):
        pltpu.make_async_copy(x_hbm.at[0, 0:128], xbuf.at[pl.ds(pl.multiple_of(g * 128, 128), 128)],
                              sems.at[13 + g]).wait()
        for u in range(2):
            row = pl.multiple_of(g * 128 + u * 64, 64)
            nv = _layernorm(xbuf[pl.ds(row, 64), :].astype(F32)).astype(BF)
            for k in range(8):
                h0buf[k, pl.ds(pl.multiple_of(row // 2, 32), 32), :] = pltpu.bitcast(
                    nv[:, k * 128:(k + 1) * 128], U32)
            wg_v[pl.ds(row, 64), 0:2 * D] = jnp.zeros((64, 2 * D), U32)
        return carry
    lax.fori_loop(0, PRE // 128, ln_pre, 0)

    def mod_tile(v, col):
        w = pltpu.bitcast(wmod_v[v, :, pl.ds(col, 128)], BF)
        return _rb(jnp.dot(sc16, w, preferred_element_type=F32))[0:8]

    def moda_store(kc, sa, ca):
        col = mult(kc * 128, 128)
        c1 = _rb(1.0 + ca)
        modb[0, :, pl.ds(col, 128)] = sa
        modb[1, :, pl.ds(col, 128)] = c1
        return sa, c1

    def moda_apply(kc, sa, c1, r0, r1):
        for r in range(r0, r1, 16):
            nv = pltpu.bitcast(h0buf[kc, r // 2:r // 2 + 8, :], BF).astype(F32).reshape(2, 8, 128)
            hv = (_rb(nv * c1[None]) + sa[None]).reshape(16, 128).astype(BF)
            h0buf[kc, r // 2:r // 2 + 8, :] = pltpu.bitcast(hv, U32)

    def halves(u):
        return pltpu.bitcast(u << 16, F32), pltpu.bitcast(u & U32(0xFFFF0000), F32)

    def repack(a, b):
        return (a & U32(0xFFFF)) | (b << 16), (a >> 16) | (b & U32(0xFFFF0000))

    def store_qkv(i, jrow, y, seg0):
        for sg in range(y.shape[0] // 32):
            for hh in range(2):
                qkvbufs[i][seg0 + sg, pl.ds(jrow + 8 + hh * 16, 16), :] = _pack(
                    y[sg * 32:(sg + 1) * 32, hh * 128:(hh + 1) * 128])

    for c_ in chunk_copies(2):
        c_.start()
    for c_ in moda_copies(0):
        c_.wait()
    moda_apply(0, *moda_store(0, mod_tile(0, 0), mod_tile(1, 0)), 0, PRE)
    w_start(1, 0, PRE_SPLIT, prio=1)

    for c_ in cp_early:
        c_.wait()
    for i in range(NB):
        lo, hi = repack(w_v[i * 6 + 2, 0:64, :], w_v[i * 6 + 3, 0:64, :])
        w_v[i * 6 + 2, 0:64, :] = lo
        w_v[i * 6 + 3, 0:64, :] = hi
        wu_v[0:PRE, i * 256:(i + 1) * 256] = pltpu.bitcast(jnp.dot(
            pltpu.bitcast(h0buf[0], BF), pltpu.bitcast(jnp.concatenate([lo, hi], axis=1), BF),
            preferred_element_type=F32), U32)

    def w_wait(j, i0, i1, r0=0):
        blk0 = (j // 3) * (6 * NB) + (j % 3) * 2
        for i in range(i0, i1):
            for par in range(2):
                pltpu.make_async_copy(w_hbms[0].at[r0:, 0, 0, :], w_v.at[blk0 + i * 6 + par, r0:],
                                      wsems.at[2 * j + (i >= PRE_SPLIT)]).wait()

    def chunk_block(kc, last, issue):
        for c_ in chunk_copies(kc) + ([cp_xr] if last else moda_copies(kc + 1)):
            c_.wait()
        issue()
        r0 = mult(kc * 64, 64)
        mv = []
        for i in range(NB):
            lo, hi = repack(w_v[i * 6, pl.ds(r0, 64), :], w_v[i * 6 + 1, pl.ds(r0, 64), :])
            w_v[i * 6, pl.ds(r0, 64), :] = lo
            w_v[i * 6 + 1, pl.ds(r0, 64), :] = hi
            w = pltpu.bitcast(jnp.concatenate([lo, hi], axis=1), BF)
            y = (pltpu.bitcast(wg_v[0:PRE, i * 256:(i + 1) * 256], F32)
                 + jnp.dot(pltpu.bitcast(h0buf[kc], BF), w, preferred_element_type=F32))
            if last:
                store_qkv(i, 0, y, 0)
            else:
                wg_v[0:PRE, i * 256:(i + 1) * 256] = pltpu.bitcast(y, U32)
                if i in (1, 3):
                    mv.append(mod_tile(i // 2, mult((kc + 1) * 128, 128)))
                if i == 3:
                    mv = moda_store(kc + 1, mv[0], mv[1])
                if i in (4, 6):
                    zeros = qkvbufs[A_BUF[0]][NSLOT, 0:8, :]
                    for q in range(APPLY_N):
                        yr = (q + 1) * (PRE // (APPLY_N + 1)) // 8 * 8
                        tok = pltpu.bitcast(y[yr:yr + 8, 0:128], U32) & zeros
                        c1 = pltpu.bitcast(pltpu.bitcast(mv[1], U32) | tok, F32)
                        n = PRE // 2 // APPLY_N
                        r_ = (i - 4) // 2 * (PRE // 2) + q * n
                        moda_apply(kc + 1, mv[0], c1, r_, r_ + n)
        if last:
            for j in range(3):
                ln1_rows(PRE + 8 * j, HOFF + 8 + 8 * j)

    def chunk_body(kc, carry):
        def issue():
            @pl.when(kc < 5)
            def _():
                for c_ in moda_copies(kc + 3) + chunk_copies(kc + 3):
                    c_.start()
        chunk_block(kc, False, issue)
        return carry

    def issue_last():
        w_wait(1, 0, PRE_SPLIT, 64)
        w_start(1, PRE_SPLIT, NB)
        w_start(2)
    lax.fori_loop(0, 7, chunk_body, 0)
    chunk_block(7, True, issue_last)

    def pre_unit(j, i, extra, k0=0):
        blk = (j // 3) * (6 * NB) + (j % 3) * 2 + i * 6
        jrow = mult(j * 40, 8)
        r0 = k0 * 64
        lo, hi = repack(w_v[blk, r0:, :], w_v[blk + 1, r0:, :])
        w_v[blk, r0:, :] = lo
        w_v[blk + 1, r0:, :] = hi
        for rc in range(PRE // 128):
            if rc > 0:
                lo = w_v[blk, r0:, :]
                hi = w_v[blk + 1, r0:, :]
            w = pltpu.bitcast(jnp.concatenate([lo, hi], axis=1), BF)
            lhs = jnp.concatenate(
                [h0buf[k, rc * 64:(rc + 1) * 64, :] for k in range(k0, 8)], axis=1)
            y = jnp.dot(pltpu.bitcast(lhs, BF), w, preferred_element_type=F32)
            if k0:
                y = y + pltpu.bitcast(wu_v[rc * 128:(rc + 1) * 128, i * 256:(i + 1) * 256], F32)
            store_qkv(i, jrow, y, rc * 4)
            extra(rc, y)

    for i in range(NB):
        if i == PRE_SPLIT:
            w_wait(1, PRE_SPLIT, NB, 64)
            w_start(3)
            w_start(4)
            mod_copy(2).start()
            mod_copy(3).start()
        pre_unit(1, i, lambda rc, y: None, k0=1)
    w_start(5)
    mod_copy(4).start()
    mod_copy(5).start()
    cp_wo.start()
    cp_x1.start()

    def pre_body(j, carry):
        w_wait(j, 0, NB)
        v0 = jnp.maximum(j - 3, 0) * 2

        @pl.when(j >= 4)
        def _():
            for v in range(2):
                pltpu.make_async_copy(wmod32.at[:, 0:D], wmod_v.at[v0 + v],
                                      wsems.at[2 * j + 1]).wait()
        zeros = qkvbufs[A_BUF[0]][NSLOT, 0:8, :]
        for i in range(NB):
            def extra(rc, y, i=i):
                for u in range(2):
                    b = (i * 4 + rc) * 2 + u
                    for v in range(2):
                        tok = pltpu.bitcast(
                            y[v * MOD_YR:v * MOD_YR + 8, u * 128:(u + 1) * 128], U32) & zeros
                        for cs in (slice(0, HD), slice(HD, D)):
                            se, so = halves(scol[b * 8:(b + 1) * 8, :] | tok)
                            we, wo = halves(wmod_v[v0 + v, b * 8:(b + 1) * 8, cs])
                            t = (we * jnp.concatenate([se] * 4, axis=1)
                                 + wo * jnp.concatenate([so] * 4, axis=1))
                            macc[v, :, cs] = t + macc[v, :, cs] if b else t
            pre_unit(j, i, extra)
        dst = jnp.where(j >= 4, v0, 7)
        for v in range(2):
            mv = _rb(jnp.sum(macc[v], axis=0, keepdims=True))
            if v == 0:
                mv = _rb(jnp.where(j == 5, 1.0, 0.0).astype(F32) + mv)
            modb[dst + v] = jnp.broadcast_to(mv, (8, D))
        return carry
    lax.fori_loop(2, 6, pre_body, 0)

    cp_wo.wait()
    cp_x1.wait()
    for c_ in cp_ffn:
        c_.start()

    def wo_w(q0, q1, n0, n1):
        h0, h1 = q0 + 2 * ROT, q1 + 2 * ROT
        ws = [wo_v[a:b, :, n0 * 128:n1 * 128].reshape((b - a) * (DH // 2), (n1 - n0) * 128)
              for a, b in ((h0, min(h1, H)), (0, h1 - H)) if b > a]
        return pltpu.bitcast(jnp.concatenate(ws, axis=0), BF)

    def emit_step(it, odd, pend):
        s = 2 * it + odd
        hrow = pl.multiple_of(HOFF + (s & 1) * 32, 32)
        hnext = pl.multiple_of(HOFF + 32 - (s & 1) * 32, 32)
        tv = [tab[s * NTAB + k] for k in range(7)]
        slot = tv[0]
        dsts = [(tv[1 + 2 * j], pl.multiple_of(tv[2 + 2 * j], 4)) for j in range(3)]
        orow, ow = (32, 48) if odd else (0, 32)
        odst = (48, 56, 64, 72) if odd else (8, 16, 24, 40)
        erow = it * 64 if odd else jnp.maximum(it - 1, 0) * 64 + RIDE
        lrow = PRE + jnp.minimum(s + 1, NSEG - 1) * RIDE
        e_at, l_at = (E_AT2, L_AT2) if odd else (E_AT, L_AT)
        probs = {}

        def wqkv(p, k0, k1):
            return pltpu.bitcast(jnp.concatenate(
                [w_v[p * 6 + u, k0 // 2:k1 // 2, :] for u in range(6)], axis=1), BF)

        lhs_lo = act[pl.ds(hrow, 32), 0:HD]
        if pend is not None:
            ybuf[...] = jnp.dot(lhs_lo, wqkv(0, 0, HD), preferred_element_type=F32)
            pend()
        lhs_hi = act[pl.ds(hrow, 32), HD:D]
        if pend is not None:
            y0 = ybuf[...] + jnp.dot(lhs_hi, wqkv(0, HD, D), preferred_element_type=F32)
        lhs_rest = jnp.concatenate([lhs_lo[:, 128:], lhs_hi], axis=1)
        lhs = [jnp.concatenate([lhs_lo, lhs_hi], axis=1)]

        def side(p):
            for j in range(len(e_at)):
                if e_at[j] == p:
                    finish_rows(pl.multiple_of(erow + 8 * j, 8), attn_load(j))
            for j in range(3):
                if l_at[j] == p:
                    ln1_rows(pl.multiple_of(lrow + 8 * j, 8),
                             pl.multiple_of(hnext + 8 + 8 * j, 8))
            if p in e_at or p in l_at:
                lhs[0] = jnp.concatenate([act[pl.ds(hrow, 32), 0:128], lhs_rest], axis=1)

        def qkv(p):
            if p == 0 and pend is not None:
                y = y0
            else:
                y = jnp.dot(lhs[0], wqkv(p, 0, D), preferred_element_type=F32)
            buf = qkvbufs[p % NB]
            for u in range(6):
                t, hh = u // 2, u % 2
                b0 = ((p // NB) * 3 + t) * 40
                yu = y[:, u * 128:(u + 1) * 128]
                buf[slot, b0 + hh * 4:b0 + hh * 4 + 4, :] = _pack(yu[0:8])
                for j in range(3):
                    sl, off = dsts[j]
                    buf[sl, pl.ds(b0 + 8 + hh * 16 + off, 4), :] = _pack(yu[8 + 8 * j:16 + 8 * j])

        def ld(p, t):
            b0 = ((p // NB) * 3 + t) * 40
            return pltpu.bitcast(qkvbufs[p % NB][slot, b0:b0 + 40, :], BF)

        def sc(p):
            s2 = lax.dot_general(ld(p, 0), ld(p, 1), (((1,), (1,)), ((), ())),
                                 preferred_element_type=F32)
            s2 = jnp.where(valid, s2 * SCALE, fill)
            m = jnp.max(s2, axis=-1, keepdims=True)
            e = jnp.exp(s2 - m)
            l = jnp.sum(e, axis=-1, keepdims=True)
            rl = pl.reciprocal(l, approx=True)
            rl = rl * (2.0 - l * rl)
            probs[p] = (e * rl).astype(BF)

        def pv(p):
            o2 = jnp.dot(probs[p], ld(p, 2), preferred_element_type=F32)
            for hh in range(2):
                hcol = (2 * ((p - ROT) % NP) + hh) * 128
                obuf[orow:orow + 8, hcol:hcol + 128] = o2[8 * hh:8 * hh + 8].astype(BF)
                for j in range(4):
                    r0 = 16 + 32 * hh + 8 * j
                    obuf[odst[j]:odst[j] + 8, hcol:hcol + 128] = o2[r0:r0 + 8].astype(BF)

        def attn(pos):
            for kind, p in ATT.get(pos, ()):
                (sc if kind == 's' else pv)(p)

        for p in range(NP):
            qkv(p)
            side(p)
            attn(p)
        a1 = []
        for n in range(8):
            a1.append(jnp.dot(obuf[orow:orow + ow, 0:KS], wo_w(0, KS // DH, n, n + 1),
                              preferred_element_type=F32))
            if n + 1 in W1AT:
                attn(NP + 2 * W1AT.index(n + 1))
        o2lhs = obuf[orow:orow + ow, KS:]
        a_lo = jnp.concatenate(a1[0:4], axis=1) + jnp.dot(
            o2lhs, wo_w(KS // DH, H, 0, 4), preferred_element_type=F32)
        act[pl.ds(hnext, 8), 0:HD] = a_lo[0:8].astype(BF)
        attn_store(a_lo[8:], 0)
        a_hi = jnp.concatenate(a1[4:8], axis=1) + jnp.dot(
            o2lhs, wo_w(KS // DH, H, 4, 8), preferred_element_type=F32)

        def finish():
            act[pl.ds(hnext, 8), HD:D] = a_hi[0:8].astype(BF)
            attn_store(a_hi[8:], 4)
        return finish

    def out_copy(r0, n, sem):
        return cp(act.at[pl.ds(OOFF + r0, n)], out_hbm.at[0, pl.ds(r0, n)], sem)

    def steps(it, carry):
        emit_step(it, 1, emit_step(it, 0, None))()

        @pl.when(it > 0)
        def _():
            out_copy(pl.multiple_of((it - 1) * 64, 64), 64, 9).start()
        return carry
    lax.fori_loop(0, NSEG // 2, steps, 0)

    NEW0 = S - NEW
    out_copy(S - 64, NEW0 - (S - 64), 9).start()
    for c_ in cp_ffn:
        c_.wait()

    def rep(i, n):
        return jnp.concatenate([modb[i]] * n, axis=0)
    r_old = act[ROFF:ROFF + 8, 0:256].astype(F32) + 0.0
    bits = pltpu.bitcast(jnp.broadcast_to(jnp.max(r_old, axis=0, keepdims=True), (8, 256)),
                         jnp.int32)
    code = (bits ^ ((bits >> 31) & 0x7FFFFFFF)) >> 16
    key = jnp.where(lane256 < NEW0 // 8, (code * 256 + (255 - lane256)).astype(F32), -jnp.inf)
    k1 = jnp.max(key, axis=1, keepdims=True)
    k2 = jnp.max(jnp.where(key == k1, -jnp.inf, key), axis=1, keepdims=True)
    rc = jnp.concatenate([jnp.max(jnp.where(key == k, r_old, -jnp.inf), axis=1, keepdims=True)
                          for k in (k1, k2)], axis=0)
    b1, b2 = (pl.multiple_of(jnp.minimum(255 - (k[0, 0].astype(jnp.int32) & 255),
                                         NEW0 // 8 - 1) * 8, 8) for k in (k1, k2))
    x1c = jnp.concatenate([act[pl.ds(b1, 8), :].astype(F32), act[pl.ds(b2, 8), :].astype(F32)],
                          axis=0)
    h2c = _rb(_rb(_layernorm(x1c) * rep(4, 2)) + rep(3, 2))
    ng = NEW // 8
    x1n = _rb(xbuf[NEW0:S, :].astype(F32) + _rb(rep(2, ng) * _rb(
        jnp.concatenate([attn_load(j) for j in range(ng)], axis=0))))
    h2n = _rb(_rb(_layernorm(x1n) * rep(4, ng)) + rep(3, ng))
    rn = _rb(jnp.sum(h2n * rep(6, ng), axis=-1, keepdims=True))
    subf = lax.broadcasted_iota(jnp.int32, (8, 1), 0).astype(F32)
    b1f = b1.astype(F32)
    val = jnp.concatenate([rc, rn], axis=0)
    idx = jnp.concatenate([subf + b1f, subf + b2.astype(F32)]
                          + [subf + float(NEW0 + 8 * j) for j in range(ng)], axis=0)
    v1 = jnp.max(val, axis=0, keepdims=True)
    t1 = jnp.min(jnp.where(val == v1, idx, float(S)), axis=0, keepdims=True)
    rest = jnp.where(idx == t1, -jnp.inf, val)
    v2 = jnp.max(rest, axis=0, keepdims=True)
    t2 = jnp.min(jnp.where((rest == v2) & (idx != t1), idx, float(S)), axis=0, keepdims=True)

    def pick(t, old2, new):
        out = jnp.where((t >= b1f) & (t < b1f + 8.0), old2[0:8], old2[8:16])
        for j in range(ng):
            out = jnp.where(t >= float(NEW0 + 8 * j), new[8 * j:8 * j + 8], out)
        return out
    h2s = jnp.concatenate([pick(t1, h2c, h2n), pick(t2, h2c, h2n)], axis=0)
    h2b = h2s.astype(BF)
    hid = []
    for n in range(0, F, FFN_NB):
        gt = _rb(jnp.dot(h2b, pltpu.bitcast(wg_v[:, n:n + FFN_NB], BF), preferred_element_type=F32))
        up = _rb(jnp.dot(h2b, pltpu.bitcast(wu_v[:, n:n + FFN_NB], BF), preferred_element_type=F32))
        hid.append((_rb(gt * _rb(jax.nn.sigmoid(gt))) * up).astype(BF))
        if n == 0:
            late = pltpu.bitcast(up[0:8, 0:128], U32) & qkvbufs[0][NSLOT, 64:72, :]
            gbl = pltpu.bitcast(
                pltpu.bitcast(modb[5], U32) | jnp.concatenate([late] * 8, axis=1), F32)
    y = _rb(jnp.dot(jnp.concatenate(hid, axis=1), pltpu.bitcast(wd_v[...], BF),
                    preferred_element_type=F32))
    act[OOFF + NEW0:OOFF + S, :] = (
        x1n + _rb(jnp.concatenate([gbl] * ng, axis=0) * h2n)).astype(BF)
    x1s = jnp.concatenate([pick(t1, x1c, x1n), pick(t2, x1c, x1n)], axis=0)
    c1, c2 = (pl.multiple_of((jnp.clip(t[0, 0].astype(jnp.int32), 0, S - 1) >> 3) * 8, 8)
              for t in (t1, t2))
    tok = jnp.concatenate([subf + c1.astype(F32), subf + c2.astype(F32)], axis=0)
    is1, is2 = tok == t1, tok == t2
    gate = _rb(jax.nn.sigmoid(jnp.where(is1, v1, v2)))
    upd = jnp.where(is1 | is2, _rb(y * gate), 0.0)
    res = (x1s + _rb(rep(5, 2) * _rb(h2s + upd))).astype(BF)
    out_copy(0, NEW0, 9).wait()
    act[pl.ds(OOFF + c1, 8), :] = res[0:8]
    act[pl.ds(OOFF + c2, 8), :] = res[8:16]
    fix0 = out_copy(NEW0, NEW, 6)
    fix1 = out_copy(c1, 8, 11)
    fix2 = out_copy(c2, 8, 12)
    send1 = c1 < NEW0
    send2 = (c2 < NEW0) & (c2 != c1)
    fix0.start()
    pl.when(send1)(fix1.start)
    pl.when(send2)(fix2.start)
    pl.when(send1)(fix1.wait)
    pl.when(send2)(fix2.wait)
    fix0.wait()


@jax.jit
def pallas_adaLN_cond__memory_aug_recurrent_mem_tr__moe_arch_mod__prompt_kernel(
    A_x: jax.Array,
    A_mem0: jax.Array,
    A_Wq: jax.Array,
    A_Wk: jax.Array,
    A_Wv: jax.Array,
    A_Wo: jax.Array,
    A_seg_len,
    B_x: jax.Array,
    B_w_r: jax.Array,
    B_w_gate: jax.Array,
    B_w_up: jax.Array,
    B_w_down: jax.Array,
    c: jax.Array,
    w_mod: jax.Array,
):
    del B_x
    del A_seg_len
    assert A_x.shape == (1, S, D) and A_Wq.shape == (D, H, DH) and A_mem0.shape == (1, M, D)
    any_spec = pl.BlockSpec(memory_space=pl.ANY)
    scratch = [
        pltpu.VMEM((S, D), BF),
        pltpu.VMEM((ACT_ROWS, D), BF),
        pltpu.VMEM((8, PRE // 2, 128), U32),
        pltpu.VMEM((32, 768), F32),
        pltpu.VMEM((D // 2, 128), U32),
        pltpu.VMEM((2, 8, D), F32),
        pltpu.SMEM((NSEG * NTAB,), jnp.int32),
        pltpu.VMEM((9, 8, D), F32),
        pltpu.VMEM((3 * H, D // 2, 128), U32),
        pltpu.VMEM((H, DH // 2, D), U32),
        pltpu.VMEM((6, D // 2, D), U32),
        pltpu.VMEM((D // 2, F), U32),
        pltpu.VMEM((D // 2, F), U32),
        pltpu.VMEM((F // 2, D), U32),
        pltpu.VMEM((80, H * DH), BF),
        pltpu.SemaphoreType.DMA((17,)),
        pltpu.SemaphoreType.DMA((12,)),
        pltpu.SemaphoreType.DMA((16,)),
    ] + [pltpu.VMEM((NSLOT + 1, 256, 128), U32) for _ in range(NB)] + [
        pltpu.VMEM((1, D), BF),
        pltpu.VMEM((D,), BF),
    ]
    wq, wk, wv = (w.reshape(D // 2, 2, H, DH) for w in (A_Wq, A_Wk, A_Wv))
    opts = dict(vmem_limit_bytes=112 * 1024 * 1024, disable_bounds_checks=True)
    try:
        params = pltpu.CompilerParams(disable_semaphore_checks=True, **opts)
    except TypeError:
        params = pltpu.CompilerParams(**opts)
    return pl.pallas_call(
        _kernel,
        out_shape=jax.ShapeDtypeStruct((1, S, D), BF),
        in_specs=[any_spec] * 12,
        out_specs=any_spec,
        scratch_shapes=scratch,
        compiler_params=params,
    )(A_x, A_mem0, wq, wk, wv, A_Wo, B_w_r, B_w_gate, B_w_up, B_w_down,
      c, w_mod)
```
